```python
import jax
import jax.numpy as jnp

def _softmax(x, axis=-1):
    return jax.nn.softmax(x, axis=axis)
def _gelu(x):
    return jax.nn.gelu(x, approximate=True)
def _silu(x):
    return jax.nn.silu(x)
def _sigmoid(x):
    return jax.nn.sigmoid(x)
def _layernorm(x, axis=-1, eps=1e-5):
    m = jnp.mean(x, axis=axis, keepdims=True)
    v = jnp.var(x, axis=axis, keepdims=True)
    return (x - m) / jnp.sqrt(v + eps)
def _scatter_add(tgt, idx, src, axis=0):
    return tgt.at[idx].add(src)
def _segment_sum(src, seg, n):
    return jax.ops.segment_sum(src, seg, n)
class _Rng:
    def __init__(self, key):
        self._k = key
    def _next(self):
        self._k, sub = jax.random.split(self._k)
        return sub
    def normal(self, shape):
        return jax.random.normal(self._next(), shape, dtype=jnp.bfloat16)
    def randint(self, lo, hi, shape):
        return jax.random.randint(self._next(), shape, lo, hi, dtype=jnp.int32)
    def uniform(self, shape, lo=0.0, hi=1.0):
        return jax.random.uniform(self._next(), shape, jnp.bfloat16, lo, hi)
    def permutation(self, n):
        return jax.random.permutation(self._next(), n)


kernel_name = 'interleave_layers__sliding_local_dilated__ssm_conv_s4__prompt'

def setup_inputs():
    _rng = _Rng(jax.random.key(int.from_bytes(__import__("os").urandom(4), "little")))
    _w = (lambda a: (lambda t: t.astype(jnp.bfloat16) if jnp.issubdtype(t.dtype, jnp.floating) else t)(jnp.asarray(a)))
    def _A_setup():
        B, S, D = 1, 2048, 512
        return {
            "x": _w((lambda *s: _rng.normal(s) * 0.05)(B, S, D)),
            "wqkv": _w((lambda *s: _rng.normal(s) * 0.05)(D, 3 * D)),
            "wo": _w((lambda *s: _rng.normal(s) * 0.05)(D, D)),
        }
    _A_in = _A_setup()

    def _B_setup():
        B, L, D, N = 1, 2048, 512, 128
        A_re = -jnp.exp((lambda *s: _rng.normal(s) * 0.05)(D, N))
        A_im = jnp.pi * (lambda *s: _rng.normal(s) * 0.05)(D, N)
        B_re = (lambda *s: _rng.normal(s) * 0.05)(D, N)
        B_im = (lambda *s: _rng.normal(s) * 0.05)(D, N)
        C_re = (lambda *s: _rng.normal(s) * 0.05)(D, N)
        C_im = (lambda *s: _rng.normal(s) * 0.05)(D, N)
        log_dt = (lambda *s: _rng.normal(s) * 0.05)(D) * 0.5 - 4.0
        Dskip = (lambda *s: _rng.normal(s) * 0.05)(D)
        return {
            "u": _w((lambda *s: _rng.normal(s) * 0.05)(B, L, D)),
            "A_re": _w(A_re),
            "A_im": _w(A_im),
            "B_re": _w(B_re),
            "B_im": _w(B_im),
            "C_re": _w(C_re),
            "C_im": _w(C_im),
            "log_dt": _w(log_dt),
            "Dskip": _w(Dskip),
        }
    _B_in = _B_setup()

    return {
        "A_x": _A_in["x"],
        "A_wqkv": _A_in["wqkv"],
        "A_wo": _A_in["wo"],
        "B_u": _B_in["u"],
        "B_A_re": _B_in["A_re"],
        "B_A_im": _B_in["A_im"],
        "B_B_re": _B_in["B_re"],
        "B_B_im": _B_in["B_im"],
        "B_C_re": _B_in["C_re"],
        "B_C_im": _B_in["C_im"],
        "B_log_dt": _B_in["log_dt"],
        "B_Dskip": _B_in["Dskip"],
    }

def reference(A_x, A_wqkv, A_wo, B_u, B_A_re, B_A_im, B_B_re, B_B_im, B_C_re, B_C_im, B_log_dt, B_Dskip):
    def _A_ref(x, wqkv, wo):
        B, S, D = x.shape
        H = 32; Dh = D // H
        W, dil = 8, 2
        qkv = (lambda x, *d: x.transpose(*d))((x @ wqkv).reshape(B, S, 3, H, Dh), 2, 0, 3, 1, 4)
        q, k, v = qkv[0], qkv[1], qkv[2]
        scale = Dh ** -0.5
        pos = jnp.arange(S)
        off = jnp.arange(W) * dil
        idx = pos[:, None] - off[None, :]
        mask = idx >= 0
        idx_c = jnp.where(mask, idx, 0).reshape(-1)
        kg = k[:, :, idx_c, :].reshape(B, H, S, W, Dh)
        vg = v[:, :, idx_c, :].reshape(B, H, S, W, Dh)
        logits = jnp.einsum("bhsd,bhswd->bhsw", q, kg) * scale
        logits = jnp.where(mask[None, None, :, :], logits, -1e9)
        attn = _softmax(logits, axis=-1)
        o = jnp.einsum("bhsw,bhswd->bhsd", attn, vg)
        return (lambda x, *d: x.transpose(*d))(o, 0, 2, 1, 3).reshape(B, S, D) @ wo

    def _B_ref(u, A_re, A_im, B_re, B_im, C_re, C_im, log_dt, Dskip):
        Bsz, L, D = u.shape
        dt = jnp.exp(log_dt)[:, None]
        A = A_re + 1j * A_im
        Bc = B_re + 1j * B_im
        Cc = C_re + 1j * C_im
        logdA = dt * A
        dB = dt * Bc
        l = (lambda x, dt: x.astype(dt))(jnp.arange(L), A_re.dtype)
        P = jnp.exp(logdA[:, :, None] * l[None, None, :])
        K = jnp.einsum("dn,dnl,dn->dl", Cc, P, dB).real
        L2 = 2 * L
        Kp = jnp.pad(K, ((0, 0), (0, L)))
        up = (lambda x, *d: x.transpose(*d))(u, 0, 2, 1)
        up = jnp.pad(up, ((0, 0), (0, 0), (0, L)))
        Kf = (lambda x, axes=(-2,-1): jnp.fft.rfft2(x.astype(jnp.float32), axes=axes))(Kp[:, None, :], axes=(-2, -1))
        Uf = (lambda x, axes=(-2,-1): jnp.fft.rfft2(x.astype(jnp.float32), axes=axes))(up[:, :, None, :], axes=(-2, -1))
        Yf = Uf * Kf[None, :, :, :]
        y = (lambda x, s, axes=(-2,-1): jnp.fft.irfft2(x, s=s, axes=axes).astype(jnp.bfloat16))(Yf, (1, L2), axes=(-2, -1))[:, :, 0, :L]
        y = (lambda x, *d: x.transpose(*d))(y, 0, 2, 1) + u * Dskip[None, None, :]
        return y

    x = A_x
    x = x + _A_ref(_layernorm(x, axis=-1), A_wqkv, A_wo)
    x = x + _B_ref(_layernorm(x, axis=-1), B_A_re, B_A_im, B_B_re, B_B_im, B_C_re, B_C_im, B_log_dt, B_Dskip)
    x = x + _A_ref(_layernorm(x, axis=-1), A_wqkv, A_wo)
    x = x + _B_ref(_layernorm(x, axis=-1), B_A_re, B_A_im, B_B_re, B_B_im, B_C_re, B_C_im, B_log_dt, B_Dskip)
    return x
```

```python
import jax
import jax.numpy as jnp
import jax.experimental.pallas as pl
import jax.experimental.pallas.tpu as pltpu
import ml_dtypes
import numpy as np

L = 2048
D = 512
N = 128
NS = 16
R = 128
W = 8
EPS = 1e-5
F32 = jnp.float32
BF16 = jnp.bfloat16
NEG = float(ml_dtypes.bfloat16(-1e9))

_NT = (((1,), (1,)), ((), ()))


def _slab(j):
    return (j % 2) * 8 + j // 2


def _dft_matrix():
    r = np.arange(R)
    k = np.arange(R) + 0.5
    f = np.zeros((NS, R, 2 * R), np.float64)
    for j in range(NS):
        th = 2.0 * np.pi * np.outer(NS * r + j, k) / (2 * L)
        f[_slab(j), :, :R] = np.cos(th)
        f[_slab(j), :, R:] = -np.sin(th)
    return f.astype(np.float32).astype(ml_dtypes.bfloat16)


def _lag_tables():
    rho = []
    for s in range(8):
        lag = (256 * s + np.arange(NS)).astype(np.float32)
        rho.append([int(v) - 256 * s for v in lag.astype(ml_dtypes.bfloat16).astype(np.float32)])
    return rho


_RHO = _lag_tables()


def _cmul(a, b):
    return (a[0] * b[0] - a[1] * b[1], a[0] * b[1] + a[1] * b[0])


def _csq(a):
    t = a[0] * a[1]
    return ((a[0] - a[1]) * (a[0] + a[1]), t + t)


def _cadd(a, b):
    return (a[0] + b[0], a[1] + b[1])


def _csub(a, b):
    return (a[0] - b[0], a[1] - b[1])


def _fft4(x, sign):
    s0, d0 = _cadd(x[0], x[2]), _csub(x[0], x[2])
    s1, d1 = _cadd(x[1], x[3]), _csub(x[1], x[3])
    a = (d0[0] + d1[1], d0[1] - d1[0])
    b = (d0[0] - d1[1], d0[1] + d1[0])
    if sign > 0:
        a, b = b, a
    return [_cadd(s0, s1), a, _csub(s0, s1), b]


def _twiddle(z, m, sign):
    m = (m * sign) % 16
    re, im = z
    h = float(np.sqrt(0.5))
    if m == 0:
        return z
    if m == 4:
        return (-im, re)
    if m == 12:
        return (im, -re)
    if m == 2:
        return ((re - im) * h, (re + im) * h)
    if m == 14:
        return ((re + im) * h, (im - re) * h)
    if m == 6:
        return ((re + im) * -h, (re - im) * h)
    if m == 10:
        return ((im - re) * h, (re + im) * -h)
    c, s = float(np.cos(np.pi * m / 8)), float(np.sin(np.pi * m / 8))
    return (re * c - im * s, re * s + im * c)


def _fft16(x, sign):
    cols = [_fft4([x[n + 4 * m] for m in range(4)], sign) for n in range(4)]
    out = [None] * 16
    for k1 in range(4):
        y = _fft4([_twiddle(cols[n][k1], n * k1, sign) for n in range(4)], sign)
        for k2 in range(4):
            out[k1 + 4 * k2] = y[k2]
    return out


def _layernorm(x):
    m = jnp.sum(x, axis=0, keepdims=True) * (1.0 / D)
    c = x - m
    v = jnp.sum(c * c, axis=0, keepdims=True) * (1.0 / D)
    return c * jax.lax.rsqrt(v + EPS)


def _ds(i, n):
    return pl.ds(pl.multiple_of(i * n, n), n)


def _kernel(x_ref, wqkv_ref, wo_ref, are_ref, aim_ref, bre_ref, bim_ref, cre_ref, cim_ref,
            ldt_ref, dsk_ref, f_ref, fk_ref, o_ref,
            xs, un, wt, wot, dtb, dskb, spec, khat, bc, qs, ks, vs, ob, xio, sems):
    loads = [pltpu.make_async_copy(x_ref.at[:, c * 128:(c + 1) * 128], xio.at[c], sems.at[c])
             for c in range(4)]
    for cp in loads:
        cp.start()
    for cp in loads:
        cp.wait()
    xu = xio.bitcast(jnp.uint32)

    def load_x(b, c):
        for jj in range(8):
            t = xu[b, pl.ds(jj, R, stride=8), :].T
            xs[_ds(b, 128), jj * R:(jj + 1) * R] = pltpu.bitcast(t << 16, F32)
            xs[_ds(b, 128), (jj + 8) * R:(jj + 9) * R] = pltpu.bitcast(t & jnp.uint32(0xFFFF0000), F32)
        return c

    jax.lax.fori_loop(0, 4, load_x, 0)

    m_i = jax.lax.broadcasted_iota(jnp.int32, (128, 128), 0)
    c_i = jax.lax.broadcasted_iota(jnp.int32, (128, 128), 1)
    perm = jnp.where(c_i == (m_i & 7) * 16 + (m_i >> 3), 1.0, 0.0).astype(BF16)

    def prep_w(g, c):
        for t in range(3):
            blk = wqkv_ref[:, _ds(t * 4 + g, 128)]
            wt[g, t * 128:(t + 1) * 128, :] = jax.lax.dot_general(
                perm, blk, _NT, preferred_element_type=F32).astype(BF16)
        po = jnp.dot(perm, wo_ref[_ds(g, 128), :], preferred_element_type=F32)
        wot[:, _ds(g, 128)] = po.T.astype(BF16)
        return c

    jax.lax.fori_loop(0, 4, prep_w, 0)

    dt_row = jnp.exp(ldt_ref[...].astype(F32)).astype(BF16).astype(F32)
    dtb[...] = jnp.broadcast_to(dt_row, (128, D)).T
    dskb[...] = jnp.broadcast_to(dsk_ref[...].astype(F32), (128, D)).T

    lane8 = jax.lax.broadcasted_iota(jnp.int32, (8, R), 1)
    rev8 = 7 - jax.lax.broadcasted_iota(jnp.int32, (8, N), 0)

    def gen_k(i, c):
        rows = _ds(i, 16)
        dt = dtb[rows, :]
        lr = dt * are_ref[rows, :].astype(F32)
        li = dt * aim_ref[rows, :].astype(F32)
        mag = jnp.exp(lr)
        z16 = (mag * jnp.cos(li), mag * jnp.sin(li))
        db = (dt * bre_ref[rows, :].astype(F32), dt * bim_ref[rows, :].astype(F32))
        w16 = _cmul((cre_ref[rows, :].astype(F32), cim_ref[rows, :].astype(F32)), db)
        halves = []
        for h in range(2):
            sl = slice(8 * h, 8 * h + 8)
            zp = {1: (z16[0][sl], z16[1][sl])}
            e = 1
            while e < 256:
                zp[2 * e] = _csq(zp[e])
                e *= 2
            step = (jnp.take_along_axis(zp[16][0], rev8, axis=0),
                    -jnp.take_along_axis(zp[16][1], rev8, axis=0))
            rhs = [jnp.concatenate([jnp.ones((8, N), F32), jnp.zeros((8, N), F32)], axis=1)]
            cur = step
            for b in range(1, 16):
                rhs.append(jnp.concatenate(cur, axis=1))
                if b < 15:
                    cur = _cmul(cur, step)
            rhs = jnp.concatenate(rhs, axis=0).astype(BF16)
            base = (w16[0][sl], w16[1][sl])
            keys, lhs = [], []
            for s in range(8):
                exps = sorted(set(_RHO[s]))
                cur = base
                for n, p in enumerate(exps):
                    if n:
                        cur = _cmul(cur, zp[p - exps[n - 1]])
                    keys.append((s, p))
                    lhs.append(jnp.concatenate(cur, axis=1))
                if s < 7:
                    base = _cmul(base, zp[256])
            if len(lhs) % 2:
                lhs.append(jnp.zeros((8, 2 * N), F32))
            out = jax.lax.dot_general(jnp.concatenate(lhs, axis=0).astype(BF16), rhs, _NT,
                                      preferred_element_type=F32)
            piece = {}
            for n, (s, p) in enumerate(keys):
                piece[s, p] = pltpu.roll(out[8 * n:8 * n + 8], s, 1, stride=1, stride_axis=0)
            memo = {}
            taps = []
            for j in range(NS):
                key = ()
                acc = None
                for s in range(7, -1, -1):
                    key = key + (_RHO[s][j],)
                    if key not in memo:
                        pc = piece[s, _RHO[s][j]]
                        memo[key] = pc if acc is None else jnp.where(((lane8 + 1) & 7) == s, pc, acc)
                    acc = memo[key]
                taps.append(acc)
            halves.append(taps)
        for j in range(NS):
            c0 = _slab(j) * R
            un[rows, c0:c0 + R] = jnp.concatenate([halves[0][j], halves[1][j]], axis=0).astype(BF16)
        return c

    jax.lax.fori_loop(0, D // 16, gen_k, 0)

    def dft(s, c):
        spec[:, _ds(s, 2 * R)] = jnp.dot(un[:, _ds(s, R)], fk_ref[s], preferred_element_type=F32)
        return c

    def load_spec(ref, rows, order):
        return [(ref[rows, 2 * R * s:2 * R * s + R], ref[rows, 2 * R * s + R:2 * R * (s + 1)])
                for s in order]

    slabs = [_slab(j) for j in range(NS)]

    jax.lax.fori_loop(0, NS, dft, 0)

    def k_fft(i, c):
        rows = _ds(i, 8)
        out = _fft16(load_spec(spec, rows, slabs), -1)
        for k in range(NS):
            khat[rows, 2 * R * k:2 * R * k + R] = out[k][0] * (1.0 / L)
            khat[rows, 2 * R * k + R:2 * R * (k + 1)] = out[k][1] * (1.0 / L)
        return c

    jax.lax.fori_loop(0, D // 8, k_fft, 0)

    lane = jax.lax.broadcasted_iota(jnp.int32, (128, R), 1)

    def layer(_, carry):
        def norm(s, c):
            un[:, _ds(s, R)] = _layernorm(xs[:, _ds(s, R)]).astype(BF16)
            return c

        jax.lax.fori_loop(0, NS, norm, 0)

        def attn(t, c):
            g, p = t // 2, t % 2
            qkv = jnp.dot(wt[g], un[:, _ds(p, 8 * R)], preferred_element_type=F32)
            qs[...] = qkv[0:128]
            ks[:, 7 * R:] = qkv[128:256]
            vs[:, 7 * R:15 * R] = qkv[256:384]

            @pl.when(p == 0)
            def _():
                vs[:, 15 * R:] = qkv[256:384, 0:R]

            v0 = vs[:, 15 * R:]
            for i in range(1, 8):
                dst = slice((i - 1) * R, i * R)
                ks[:, dst] = pltpu.roll(qkv[128:256, i * R:(i + 1) * R], 1, 1)
                vs[:, dst] = jnp.where(lane == 0, v0,
                                       pltpu.roll(qkv[256:384, i * R:(i + 1) * R], 1, 1))
            for i in range(8):
                q = qs[:, i * R:(i + 1) * R]
                logits = []
                for w in range(W):
                    c0 = (7 + i - w) * R
                    lg = jnp.sum((q * ks[:, c0:c0 + R]).reshape(16, 8, R), axis=0) * 0.25
                    if w > i:
                        lg = jnp.where(lane8 == 0, NEG, lg)
                    logits.append(lg)
                mx = logits[0]
                for lg in logits[1:]:
                    mx = jnp.maximum(mx, lg)
                es = [jnp.exp(lg - mx) for lg in logits]
                den = es[0]
                for e in es[1:]:
                    den = den + e
                inv = 1.0 / den
                acc = None
                for w in range(W):
                    c0 = (7 + i - w) * R
                    term = vs[:, c0:c0 + R].reshape(16, 8, R) * (es[w] * inv)[None]
                    acc = term if acc is None else acc + term
                ob[_ds(g, 128), _ds(p * 8 + i, R)] = acc.reshape(128, R).astype(BF16)
            return c

        jax.lax.fori_loop(0, 8, attn, 0)

        def proj(s, c):
            cols = _ds(s, R)
            x = xs[:, cols] + jnp.dot(wot[...], ob[:, cols], preferred_element_type=F32)
            u = _layernorm(x)
            xs[:, cols] = x + u * dskb[...]
            spec[:, _ds(s, 2 * R)] = jnp.dot(u.astype(BF16), f_ref[s], preferred_element_type=F32)
            return c

        jax.lax.fori_loop(0, NS, proj, 0)

        def conv(i, c):
            rows = _ds(i, 16)
            uf = _fft16(load_spec(spec, rows, slabs), -1)
            kf = load_spec(khat, rows, range(NS))
            out = _fft16([_cmul(a, b) for a, b in zip(uf, kf)], 1)
            for j in range(NS):
                s = _slab(j)
                bc[rows, 2 * R * s:2 * R * s + R] = out[j][0].astype(BF16)
                bc[rows, 2 * R * s + R:2 * R * (s + 1)] = out[j][1].astype(BF16)
            return c

        jax.lax.fori_loop(0, D // 16, conv, 0)

        def idft(s, c):
            xs[:, _ds(s, R)] += jax.lax.dot_general(bc[:, _ds(s, 2 * R)], f_ref[s], _NT,
                                                    preferred_element_type=F32)
            return c

        jax.lax.fori_loop(0, NS, idft, 0)
        return carry

    jax.lax.fori_loop(0, 2, layer, 0)

    def store_x(b, c):
        rows = _ds(b, 128)
        for jj in range(8):
            t = pltpu.pack_elementwise([xs[rows, jj * R:(jj + 1) * R], xs[rows, (jj + 8) * R:(jj + 9) * R]],
                                       packed_dtype=BF16)
            xu[b, pl.ds(jj, R, stride=8), :] = pltpu.bitcast(t, jnp.uint32).T
        return c

    jax.lax.fori_loop(0, 4, store_x, 0)
    stores = [pltpu.make_async_copy(xio.at[c], o_ref.at[:, c * 128:(c + 1) * 128], sems.at[c])
              for c in range(4)]
    for cp in stores:
        cp.start()
    for cp in stores:
        cp.wait()


@jax.jit
def pallas_interleave_layers__sliding_local_dilated__ssm_conv_s4__prompt_kernel(
    A_x: jax.Array,
    A_wqkv: jax.Array,
    A_wo: jax.Array,
    B_u: jax.Array,
    B_A_re: jax.Array,
    B_A_im: jax.Array,
    B_B_re: jax.Array,
    B_B_im: jax.Array,
    B_C_re: jax.Array,
    B_C_im: jax.Array,
    B_log_dt: jax.Array,
    B_Dskip: jax.Array,
):
    del B_u
    f = _dft_matrix()
    lane = (np.arange(R) - 7) % R
    order = 16 * (lane % 8) + lane // 8
    scratch = [
        pltpu.VMEM((D, L), F32),
        pltpu.VMEM((D, L), BF16),
        pltpu.VMEM((4, 384, D), BF16),
        pltpu.VMEM((D, D), BF16),
        pltpu.VMEM((D, 128), F32),
        pltpu.VMEM((D, 128), F32),
        pltpu.VMEM((D, 2 * L), F32),
        pltpu.VMEM((D, 2 * L), F32),
        pltpu.VMEM((D, 2 * L), BF16),
        pltpu.VMEM((128, 8 * R), F32),
        pltpu.VMEM((128, 15 * R), F32),
        pltpu.VMEM((128, 16 * R), F32),
        pltpu.VMEM((D, L), BF16),
        pltpu.VMEM((4, L, 128), BF16),
        pltpu.SemaphoreType.DMA((4,)),
    ]
    out = pl.pallas_call(
        _kernel,
        out_shape=jax.ShapeDtypeStruct((L, D), BF16),
        in_specs=[pl.BlockSpec(memory_space=pl.ANY)] + [pl.BlockSpec(memory_space=pltpu.VMEM)] * 12,
        out_specs=pl.BlockSpec(memory_space=pl.ANY),
        scratch_shapes=scratch,
        compiler_params=pltpu.CompilerParams(vmem_limit_bytes=100 * 1024 * 1024),
    )(A_x.reshape(L, D), A_wqkv, A_wo, B_A_re, B_A_im, B_B_re, B_B_im, B_C_re, B_C_im,
      B_log_dt.reshape(1, D), B_Dskip.reshape(1, D), f, f[:, order])
    return out.reshape(1, L, D)
```

```python
import jax
import jax.numpy as jnp
import jax.experimental.pallas as pl
import jax.experimental.pallas.tpu as pltpu
import ml_dtypes
import numpy as np

L = 2048
D = 512
N = 128
NS = 16
R = 128
W = 8
EPS = 1e-5
F32 = jnp.float32
BF16 = jnp.bfloat16
U32 = jnp.uint32
NEG = float(ml_dtypes.bfloat16(-1e9))

_NT = (((1,), (1,)), ((), ()))


def _slab(j):
    return (j % 2) * 8 + j // 2


def _dft_matrix():
    r = np.arange(R)
    k = np.arange(R) + 0.5
    f = np.zeros((NS, R, 2 * R), np.float64)
    for j in range(NS):
        th = 2.0 * np.pi * np.outer(NS * r + j, k) / (2 * L)
        f[_slab(j), :, :R] = np.cos(th)
        f[_slab(j), :, R:] = -np.sin(th)
    return f.astype(np.float32).astype(ml_dtypes.bfloat16)


def _pack_rows(a):
    u = np.ascontiguousarray(a).view(np.uint16).astype(np.uint32)
    return u[:, 0::2] | (u[:, 1::2] << np.uint32(16))


def _lag_tables():
    rho = []
    for s in range(8):
        lag = (256 * s + np.arange(NS)).astype(np.float32)
        rho.append([int(v) - 256 * s for v in lag.astype(ml_dtypes.bfloat16).astype(np.float32)])
    return rho


_RHO = _lag_tables()


def _cmul(a, b):
    return (a[0] * b[0] - a[1] * b[1], a[0] * b[1] + a[1] * b[0])


def _csq(a):
    t = a[0] * a[1]
    return ((a[0] - a[1]) * (a[0] + a[1]), t + t)


def _cadd(a, b):
    return (a[0] + b[0], a[1] + b[1])


def _csub(a, b):
    return (a[0] - b[0], a[1] - b[1])


def _fft4(x, sign):
    s0, d0 = _cadd(x[0], x[2]), _csub(x[0], x[2])
    s1, d1 = _cadd(x[1], x[3]), _csub(x[1], x[3])
    a = (d0[0] + d1[1], d0[1] - d1[0])
    b = (d0[0] - d1[1], d0[1] + d1[0])
    if sign > 0:
        a, b = b, a
    return [_cadd(s0, s1), a, _csub(s0, s1), b]


def _twiddle(z, m, sign):
    m = (m * sign) % 16
    re, im = z
    h = float(np.sqrt(0.5))
    if m == 0:
        return z
    if m == 4:
        return (-im, re)
    if m == 12:
        return (im, -re)
    if m == 2:
        return ((re - im) * h, (re + im) * h)
    if m == 14:
        return ((re + im) * h, (im - re) * h)
    if m == 6:
        return ((re + im) * -h, (re - im) * h)
    if m == 10:
        return ((im - re) * h, (re + im) * -h)
    c, s = float(np.cos(np.pi * m / 8)), float(np.sin(np.pi * m / 8))
    return (re * c - im * s, re * s + im * c)


def _fft16(x, sign):
    cols = [_fft4([x[n + 4 * m] for m in range(4)], sign) for n in range(4)]
    out = [None] * 16
    for k1 in range(4):
        y = _fft4([_twiddle(cols[n][k1], n * k1, sign) for n in range(4)], sign)
        for k2 in range(4):
            out[k1 + 4 * k2] = y[k2]
    return out


def _layernorm(x):
    m = jnp.sum(x, axis=0, keepdims=True) * (1.0 / D)
    c = x - m
    v = jnp.sum(c * c, axis=0, keepdims=True) * (1.0 / D)
    return c * jax.lax.rsqrt(v + EPS)


def _ds(i, n):
    return pl.ds(pl.multiple_of(i * n, n), n)


def _pack(x):
    return pltpu.bitcast(x.astype(BF16), U32)


def _unpack(x):
    return pltpu.bitcast(x, BF16)


def _dot(a, b, dims=(((1,), (0,)), ((), ()))):
    return jax.lax.dot_general(a, b, dims, preferred_element_type=F32)


def _kernel(x_ref, wqkv_ref, wo_ref, are_ref, aim_ref, bre_ref, bim_ref, cre_ref, cim_ref,
            ldt_ref, dsk_ref, f_ref, fk_ref, o_ref,
            xs, xo, un, uo, wt, wot, dtb, dskb, spec, khat, bc, qa, ka, va, qb, kb, vb, oe, oo,
            xio, sems):
    loads = [pltpu.make_async_copy(x_ref.at[:, c * 128:(c + 1) * 128], xio.at[c], sems.at[c])
             for c in range(4)]
    for cp in loads:
        cp.start()
    for cp in loads:
        cp.wait()
    xu = xio.bitcast(U32)

    def load_x(b, c):
        for jj in range(8):
            t = xu[b, pl.ds(jj, R, stride=8), :].T
            xs[_ds(b, 128), jj * R:(jj + 1) * R] = pltpu.bitcast(t << 16, F32)
            xo[_ds(b, 128), jj * R:(jj + 1) * R] = pltpu.bitcast(t & jnp.uint32(0xFFFF0000), F32)
        return c

    jax.lax.fori_loop(0, 4, load_x, 0)

    m_i = jax.lax.broadcasted_iota(jnp.int32, (128, 128), 0)
    c_i = jax.lax.broadcasted_iota(jnp.int32, (128, 128), 1)
    perm = jnp.where(c_i == (m_i & 7) * 16 + (m_i >> 3), 1.0, 0.0).astype(BF16)

    def prep_w(g, c):
        for t in range(3):
            wt[g, t * 64:(t + 1) * 64, :] = _pack(_dot(perm, wqkv_ref[:, _ds(t * 4 + g, 128)], _NT))
        wot[:, _ds(g, 128)] = _pack(_dot(perm, wo_ref[_ds(g, 128), :]).T)
        return c

    jax.lax.fori_loop(0, 4, prep_w, 0)

    dt_row = jnp.exp(ldt_ref[...].astype(F32)).astype(BF16).astype(F32)
    dtb[...] = jnp.broadcast_to(dt_row, (128, D)).T
    dskb[...] = jnp.broadcast_to(dsk_ref[...].astype(F32), (128, D)).T

    lane8 = jax.lax.broadcasted_iota(jnp.int32, (8, R), 1)
    rev8 = 7 - jax.lax.broadcasted_iota(jnp.int32, (8, N), 0)

    def gen_k(i, c):
        rows = _ds(i, 16)
        dt = dtb[rows, :]
        lr = dt * are_ref[rows, :].astype(F32)
        li = dt * aim_ref[rows, :].astype(F32)
        mag = jnp.exp(lr)
        z16 = (mag * jnp.cos(li), mag * jnp.sin(li))
        db = (dt * bre_ref[rows, :].astype(F32), dt * bim_ref[rows, :].astype(F32))
        w16 = _cmul((cre_ref[rows, :].astype(F32), cim_ref[rows, :].astype(F32)), db)
        halves = []
        for h in range(2):
            sl = slice(8 * h, 8 * h + 8)
            zp = {1: (z16[0][sl], z16[1][sl])}
            e = 1
            while e < 256:
                zp[2 * e] = _csq(zp[e])
                e *= 2
            step = (jnp.take_along_axis(zp[16][0], rev8, axis=0),
                    -jnp.take_along_axis(zp[16][1], rev8, axis=0))
            rhs = [jnp.concatenate([jnp.ones((8, N), F32), jnp.zeros((8, N), F32)], axis=1)]
            cur = step
            for b in range(1, 16):
                rhs.append(jnp.concatenate(cur, axis=1))
                if b < 15:
                    cur = _cmul(cur, step)
            rhs = jnp.concatenate(rhs, axis=0).astype(BF16)
            base = (w16[0][sl], w16[1][sl])
            keys, lhs = [], []
            for s in range(8):
                exps = sorted(set(_RHO[s]))
                cur = base
                for n, p in enumerate(exps):
                    if n:
                        cur = _cmul(cur, zp[p - exps[n - 1]])
                    keys.append((s, p))
                    lhs.append(jnp.concatenate(cur, axis=1))
                if s < 7:
                    base = _cmul(base, zp[256])
            if len(lhs) % 2:
                lhs.append(jnp.zeros((8, 2 * N), F32))
            out = _dot(jnp.concatenate(lhs, axis=0).astype(BF16), rhs, _NT)
            piece = {}
            for n, (s, p) in enumerate(keys):
                piece[s, p] = pltpu.roll(out[8 * n:8 * n + 8], s, 1, stride=1, stride_axis=0)
            memo = {}
            taps = []
            for j in range(NS):
                key = ()
                acc = None
                for s in range(7, -1, -1):
                    key = key + (_RHO[s][j],)
                    if key not in memo:
                        pc = piece[s, _RHO[s][j]]
                        memo[key] = pc if acc is None else jnp.where(((lane8 + 1) & 7) == s, pc, acc)
                    acc = memo[key]
                taps.append(acc)
            halves.append(taps)
        for j in range(NS):
            c0 = (j // 2) * R
            (un, uo)[j % 2][_ds(i, 8), c0:c0 + R] = _pack(
                jnp.concatenate([halves[0][j], halves[1][j]], axis=0))
        return c

    jax.lax.fori_loop(0, D // 16, gen_k, 0)

    def dft(mat):
        def body(s, c):
            spec[:, _ds(s, 2 * R)] = _dot(_unpack(un[:, _ds(s, R)]), _unpack(mat[s]))
            spec[:, _ds(s + 8, 2 * R)] = _dot(_unpack(uo[:, _ds(s, R)]), _unpack(mat[s + 8]))
            return c

        jax.lax.fori_loop(0, 8, body, 0)

    def load_spec(ref, rows, order):
        return [(ref[rows, 2 * R * s:2 * R * s + R], ref[rows, 2 * R * s + R:2 * R * (s + 1)])
                for s in order]

    slabs = [_slab(j) for j in range(NS)]

    dft(fk_ref)

    def k_fft(i, c):
        rows = _ds(i, 8)
        out = _fft16(load_spec(spec, rows, slabs), -1)
        for k in range(NS):
            khat[rows, 2 * R * k:2 * R * k + R] = out[k][0]
            khat[rows, 2 * R * k + R:2 * R * (k + 1)] = out[k][1]
        return c

    jax.lax.fori_loop(0, D // 8, k_fft, 0)

    lane = jax.lax.broadcasted_iota(jnp.int32, (128, R), 1)

    def qkv(g, u, qs, ks, vs):
        w = _unpack(wt[g])
        for i in range(8):
            y = _dot(w, _unpack(u[:, i * R:(i + 1) * R]))
            qs[:, i * R:(i + 1) * R] = y[0:128]
            ks[:, (i + 7) * R:(i + 8) * R] = y[128:256]
            vs[:, (i + 7) * R:(i + 8) * R] = y[256:384]
            if i:
                dst = slice((i - 1) * R, i * R)
                ks[:, dst] = pltpu.roll(y[128:256], 1, 1)
                vs[:, dst] = jnp.where(lane == 0, va[:, 7 * R:8 * R], pltpu.roll(y[256:384], 1, 1))

    def attend(g, qs, ks, vs, o):
        for i in range(8):
            q = qs[:, i * R:(i + 1) * R]
            logits = []
            for w in range(W):
                c0 = (7 + i - w) * R
                lg = jnp.sum((q * ks[:, c0:c0 + R]).reshape(16, 8, R), axis=0) * 0.25
                if w > i:
                    lg = jnp.where(lane8 == 0, NEG, lg)
                logits.append(lg)
            mx = logits[0]
            for lg in logits[1:]:
                mx = jnp.maximum(mx, lg)
            es = [jnp.exp(lg - mx) for lg in logits]
            den = es[0]
            for e in es[1:]:
                den = den + e
            inv = 1.0 / den
            acc = None
            for w in range(W):
                c0 = (7 + i - w) * R
                term = vs[:, c0:c0 + R].reshape(16, 8, R) * (es[w] * inv)[None]
                acc = term if acc is None else acc + term
            o[_ds(g, 64), i * R:(i + 1) * R] = _pack(acc.reshape(128, R))

    def proj(x, o, u):
        w = _unpack(wot[...])
        for i in range(8):
            cols = slice(i * R, (i + 1) * R)
            y = x[:, cols] + _dot(w, _unpack(o[:, cols]))
            n = _layernorm(y)
            x[:, cols] = y + n * dskb[...]
            u[:, cols] = _pack(n)

    def norm(x, u):
        for i in range(8):
            cols = slice(i * R, (i + 1) * R)
            u[:, cols] = _pack(_layernorm(x[:, cols]))

    def layer(_, carry):
        norm(xs, un)
        qkv(0, un, qa, ka, va)
        norm(xo, uo)

        def group(g, c):
            qkv(g, uo, qb, kb, vb)
            attend(g, qa, ka, va, oe)

            @pl.when(g < 3)
            def _():
                qkv(g + 1, un, qa, ka, va)
                attend(g, qb, kb, vb, oo)

            return c

        jax.lax.fori_loop(0, 4, group, 0)
        proj(xs, oe, un)
        attend(3, qb, kb, vb, oo)
        proj(xo, oo, uo)
        dft(f_ref)

        def conv(i, c):
            rows = _ds(i, 16)
            uf = _fft16(load_spec(spec, rows, slabs), -1)
            kf = load_spec(khat, rows, range(NS))
            out = _fft16([_cmul(a, b) for a, b in zip(uf, kf)], 1)
            for j in range(NS):
                s = _slab(j)
                bc[_ds(i, 8), 2 * R * s:2 * R * s + R] = _pack(out[j][0])
                bc[_ds(i, 8), 2 * R * s + R:2 * R * (s + 1)] = _pack(out[j][1])
            return c

        jax.lax.fori_loop(0, D // 16, conv, 0)

        def idft(s, c):
            xs[:, _ds(s, R)] += _dot(_unpack(bc[:, _ds(s, 2 * R)]), _unpack(f_ref[s]), _NT)
            xo[:, _ds(s, R)] += _dot(_unpack(bc[:, _ds(s + 8, 2 * R)]), _unpack(f_ref[s + 8]), _NT)
            return c

        jax.lax.fori_loop(0, 8, idft, 0)
        return carry

    jax.lax.fori_loop(0, 2, layer, 0)

    def store_x(b, c):
        rows = _ds(b, 128)
        for jj in range(8):
            cols = slice(jj * R, (jj + 1) * R)
            t = pltpu.pack_elementwise([xs[rows, cols], xo[rows, cols]], packed_dtype=BF16)
            xu[b, pl.ds(jj, R, stride=8), :] = pltpu.bitcast(t, U32).T
        return c

    jax.lax.fori_loop(0, 4, store_x, 0)
    stores = [pltpu.make_async_copy(xio.at[c], o_ref.at[:, c * 128:(c + 1) * 128], sems.at[c])
              for c in range(4)]
    for cp in stores:
        cp.start()
    for cp in stores:
        cp.wait()


@jax.jit
def pallas_interleave_layers__sliding_local_dilated__ssm_conv_s4__prompt_kernel(
    A_x: jax.Array,
    A_wqkv: jax.Array,
    A_wo: jax.Array,
    B_u: jax.Array,
    B_A_re: jax.Array,
    B_A_im: jax.Array,
    B_B_re: jax.Array,
    B_B_im: jax.Array,
    B_C_re: jax.Array,
    B_C_im: jax.Array,
    B_log_dt: jax.Array,
    B_Dskip: jax.Array,
):
    del B_u
    f = _dft_matrix()
    lane = (np.arange(R) - 7) % R
    order = 16 * (lane % 8) + lane // 8
    fk = (f[:, order].astype(np.float32) / L).astype(ml_dtypes.bfloat16)
    scratch = [
        pltpu.VMEM((D, L // 2), F32),
        pltpu.VMEM((D, L // 2), F32),
        pltpu.VMEM((D // 2, L // 2), U32),
        pltpu.VMEM((D // 2, L // 2), U32),
        pltpu.VMEM((4, 192, D), U32),
        pltpu.VMEM((D // 2, D), U32),
        pltpu.VMEM((D, 128), F32),
        pltpu.VMEM((D, 128), F32),
        pltpu.VMEM((D, 2 * L), F32),
        pltpu.VMEM((D, 2 * L), F32),
        pltpu.VMEM((D // 2, 2 * L), U32),
        pltpu.VMEM((128, 8 * R), F32),
        pltpu.VMEM((128, 15 * R), F32),
        pltpu.VMEM((128, 15 * R), F32),
        pltpu.VMEM((128, 8 * R), F32),
        pltpu.VMEM((128, 15 * R), F32),
        pltpu.VMEM((128, 15 * R), F32),
        pltpu.VMEM((D // 2, L // 2), U32),
        pltpu.VMEM((D // 2, L // 2), U32),
        pltpu.VMEM((4, L, 128), BF16),
        pltpu.SemaphoreType.DMA((4,)),
    ]
    out = pl.pallas_call(
        _kernel,
        out_shape=jax.ShapeDtypeStruct((L, D), BF16),
        in_specs=[pl.BlockSpec(memory_space=pl.ANY)] + [pl.BlockSpec(memory_space=pltpu.VMEM)] * 12,
        out_specs=pl.BlockSpec(memory_space=pl.ANY),
        scratch_shapes=scratch,
        compiler_params=pltpu.CompilerParams(vmem_limit_bytes=100 * 1024 * 1024),
    )(A_x.reshape(L, D), A_wqkv, A_wo, B_A_re, B_A_im, B_B_re, B_B_im, B_C_re, B_C_im,
      B_log_dt.reshape(1, D), B_Dskip.reshape(1, D), _pack_rows(f), _pack_rows(fk))
    return out.reshape(1, L, D)
```

```python
import contextlib

import jax
import jax.numpy as jnp
import jax.experimental.pallas as pl
import jax.experimental.pallas.tpu as pltpu
import ml_dtypes
import numpy as np

L = 2048
D = 512
N = 128
NS = 16
R = 128
W = 8
EPS = 1e-5
F32 = jnp.float32
BF16 = jnp.bfloat16
U32 = jnp.uint32
NEG = float(ml_dtypes.bfloat16(-1e9))

_NT = (((1,), (1,)), ((), ()))


def _slab(j):
    return (j % 2) * 8 + j // 2


def _dft_matrix():
    r = np.arange(R)
    k = np.arange(R) + 0.5
    f = np.zeros((NS, R, 2 * R), np.float64)
    for j in range(NS):
        th = 2.0 * np.pi * np.outer(NS * r + j, k) / (2 * L)
        f[_slab(j), :, :R] = np.cos(th)
        f[_slab(j), :, R:] = -np.sin(th)
    return f.astype(np.float32).astype(ml_dtypes.bfloat16)


def _pack_rows(a):
    u = np.ascontiguousarray(a).view(np.uint16).astype(np.uint32)
    return u[:, 0::2] | (u[:, 1::2] << np.uint32(16))


def _lag_tables():
    rho = []
    for s in range(8):
        lag = (256 * s + np.arange(NS)).astype(np.float32)
        rho.append([int(v) - 256 * s for v in lag.astype(ml_dtypes.bfloat16).astype(np.float32)])
    return rho


_RHO = _lag_tables()


def _cmul(a, b):
    return (a[0] * b[0] - a[1] * b[1], a[0] * b[1] + a[1] * b[0])


def _csq(a):
    t = a[0] * a[1]
    return ((a[0] - a[1]) * (a[0] + a[1]), t + t)


def _cadd(a, b):
    return (a[0] + b[0], a[1] + b[1])


def _csub(a, b):
    return (a[0] - b[0], a[1] - b[1])


def _fft4(x, sign):
    s0, d0 = _cadd(x[0], x[2]), _csub(x[0], x[2])
    s1, d1 = _cadd(x[1], x[3]), _csub(x[1], x[3])
    a = (d0[0] + d1[1], d0[1] - d1[0])
    b = (d0[0] - d1[1], d0[1] + d1[0])
    if sign > 0:
        a, b = b, a
    return [_cadd(s0, s1), a, _csub(s0, s1), b]


def _twiddle(z, m, sign):
    m = (m * sign) % 16
    re, im = z
    h = float(np.sqrt(0.5))
    if m == 0:
        return z
    if m == 4:
        return (-im, re)
    if m == 12:
        return (im, -re)
    if m == 2:
        return ((re - im) * h, (re + im) * h)
    if m == 14:
        return ((re + im) * h, (im - re) * h)
    if m == 6:
        return ((re + im) * -h, (re - im) * h)
    if m == 10:
        return ((im - re) * h, (re + im) * -h)
    c, s = float(np.cos(np.pi * m / 8)), float(np.sin(np.pi * m / 8))
    return (re * c - im * s, re * s + im * c)


def _fft16(x, sign):
    cols = [_fft4([x[n + 4 * m] for m in range(4)], sign) for n in range(4)]
    out = [None] * 16
    for k1 in range(4):
        y = _fft4([_twiddle(cols[n][k1], n * k1, sign) for n in range(4)], sign)
        for k2 in range(4):
            out[k1 + 4 * k2] = y[k2]
    return out


def _layernorm(x):
    m = jnp.sum(x, axis=0, keepdims=True) * (1.0 / D)
    c = x - m
    v = jnp.sum(c * c, axis=0, keepdims=True) * (1.0 / D)
    return c * jax.lax.rsqrt(v + EPS)


def _scope(name):
    return contextlib.nullcontext()


def _ds(i, n):
    return pl.ds(pl.multiple_of(i * n, n), n)


def _pack(x):
    return pltpu.bitcast(x.astype(BF16), U32)


def _unpack(x):
    return pltpu.bitcast(x, BF16)


def _dot(a, b, dims=(((1,), (0,)), ((), ()))):
    return jax.lax.dot_general(a, b, dims, preferred_element_type=F32)


def _halves(u):
    return pltpu.bitcast(u << 16, F32), pltpu.bitcast(u & jnp.uint32(0xFFFF0000), F32)


def _kernel(x_hbm, wqkv_hbm, wo_hbm, are_ref, aim_ref, bre_ref, bim_ref, cre_ref, cim_ref,
            ldt_ref, dsk_ref, f_hbm, fk_hbm, o_hbm,
            xs, xo, un, uo, wt, wot, dtb, dskb, spec, khat, bc, qa, ka, va, qb, kb, vb, oe, oo,
            xio, wqkv_ref, wo_ref, f_ref, fk_ref, sems):
    loads = [pltpu.make_async_copy(x_hbm.at[:, c * 128:(c + 1) * 128], xio.at[c], sems.at[c])
             for c in range(4)]
    loads += [pltpu.make_async_copy(src, dst, sems.at[4 + n]) for n, (src, dst) in enumerate(
        [(fk_hbm, fk_ref), (wqkv_hbm, wqkv_ref), (wo_hbm, wo_ref), (f_hbm, f_ref)])]
    for cp in loads:
        cp.start()

    dt_row = jnp.exp(ldt_ref[...].astype(F32)).reshape(1, D)
    dtb[...] = _pack(jnp.broadcast_to(dt_row, (128, D)).T)
    dskb[...] = jnp.broadcast_to(dsk_ref[...].astype(F32).reshape(1, D) * (1.0 / L), (128, D)).T

    lane8 = jax.lax.broadcasted_iota(jnp.int32, (8, R), 1)
    rev8 = 7 - jax.lax.broadcasted_iota(jnp.int32, (8, N), 0)

    def gen_k(i, c):
        def param(ref):
            return _halves(pltpu.bitcast(ref[_ds(i, 16), :], U32))

        dts = _halves(dtb[_ds(i, 8), :])
        are, aim, bre, bim, cre, cim = [
            param(r) for r in (are_ref, aim_ref, bre_ref, bim_ref, cre_ref, cim_ref)]
        outs = []
        for h in range(2):
            dt = dts[h]
            li = dt * aim[h]
            mag = jnp.exp(dt * are[h])
            zp = {1: (mag * jnp.cos(li), mag * jnp.sin(li))}
            for e in (1, 2, 4, 8):
                zp[2 * e] = _csq(zp[e])
            zp[256] = _csq(_csq(_csq(_csq(zp[16]))))
            pw = [(jnp.ones((8, N), F32), jnp.zeros((8, N), F32)),
                  (jnp.take_along_axis(zp[16][0], rev8, axis=0),
                   -jnp.take_along_axis(zp[16][1], rev8, axis=0))]
            for b in range(2, 16):
                pw.append(_cmul(pw[b - 1], pw[1]) if b % 2 else _csq(pw[b // 2]))
            rhs = jnp.concatenate([jnp.concatenate(v, axis=1) for v in pw], axis=0).astype(BF16)
            base = _cmul((cre[h], cim[h]), (dt * bre[h], dt * bim[h]))
            lhs = []
            for s in range(8):
                exps = sorted(set(_RHO[s]))
                cur = base
                for n, p in enumerate(exps):
                    if n:
                        cur = _cmul(cur, zp[p - exps[n - 1]])
                    lhs.append(jnp.concatenate(cur, axis=1))
                if s < 7:
                    base = _cmul(base, zp[256])
            outs.append(_dot(jnp.concatenate(lhs, axis=0), rhs, _NT))
        both = pltpu.bitcast(pltpu.pack_elementwise(outs, packed_dtype=BF16), U32)
        keys = [(s, p) for s in range(8) for p in sorted(set(_RHO[s]))]
        piece = {}
        for n, (s, p) in enumerate(keys):
            piece[s, p] = pltpu.roll(both[8 * n:8 * n + 8], s, 1, stride=1, stride_axis=0)
        memo = {}
        for j in range(NS):
            key = ()
            acc = None
            for s in range(7, -1, -1):
                key = key + (_RHO[s][j],)
                if key not in memo:
                    pc = piece[s, _RHO[s][j]]
                    memo[key] = pc if acc is None else jnp.where(((lane8 + 1) & 7) == s, pc, acc)
                acc = memo[key]
            c0 = (j // 2) * R
            (un, uo)[j % 2][_ds(i, 8), c0:c0 + R] = acc
        return c

    with _scope("gen_k"):
        jax.lax.fori_loop(0, D // 16, gen_k, 0, unroll=2)

    for cp in loads:
        cp.wait()

    xu = xio.bitcast(U32)

    def load_x(b):
        for jj in range(8):
            ev, od = _halves(xu[b, pl.ds(jj, R, stride=8), :].T)
            xs[_ds(b, 128), jj * R:(jj + 1) * R] = ev
            xo[_ds(b, 128), jj * R:(jj + 1) * R] = od

    m_i = jax.lax.broadcasted_iota(jnp.int32, (128, 128), 0)
    c_i = jax.lax.broadcasted_iota(jnp.int32, (128, 128), 1)
    perm = jnp.where(c_i == (m_i & 7) * 16 + (m_i >> 3), 1.0, 0.0).astype(BF16)

    def prep_w(g):
        for t in range(3):
            wt[g, t * 64:(t + 1) * 64, :] = _pack(_dot(perm, wqkv_ref[:, _ds(t * 4 + g, 128)], _NT))
        wot[:, _ds(g, 128)] = _pack(_dot(perm, wo_ref[_ds(g, 128), :]).T)

    def dft(mat, rb):
        for s in range(NS):
            u = (un, uo)[s // 8][rb * 64:(rb + 1) * 64, (s % 8) * R:(s % 8 + 1) * R]
            spec[rb * 128:(rb + 1) * 128, 2 * R * s:2 * R * (s + 1)] = _dot(_unpack(u), _unpack(mat[s]))

    def idft(rb):
        rows = slice(rb * 128, (rb + 1) * 128)
        for s in range(NS):
            (xs, xo)[s // 8][rows, (s % 8) * R:(s % 8 + 1) * R] += _dot(
                bc[rows, 2 * R * s:2 * R * (s + 1)], _unpack(f_ref[s]), _NT)

    def load_spec(ref, rows, order):
        return [(ref[rows, 2 * R * s:2 * R * s + R], ref[rows, 2 * R * s + R:2 * R * (s + 1)])
                for s in order]

    def store_spec(ref, rows, order, vals):
        for s, v in zip(order, vals):
            ref[rows, 2 * R * s:2 * R * s + R] = v[0]
            ref[rows, 2 * R * s + R:2 * R * (s + 1)] = v[1]

    slabs = [_slab(j) for j in range(NS)]

    def prep(b, c):
        load_x(b)
        prep_w(b)
        for s in range(NS):
            u = (un, uo)[s // 8][_ds(b, 64), (s % 8) * R:(s % 8 + 1) * R]
            spec[_ds(b, 128), 2 * R * s:2 * R * (s + 1)] = _dot(_unpack(u), _unpack(fk_ref[s]))
        return c

    with _scope("prep"):
        jax.lax.fori_loop(0, 4, prep, 0)

    def k_fft(i):
        rows = slice(8 * i, 8 * i + 8)
        a = load_spec(spec, rows, slabs)
        a[0] = (a[0][0] + dskb[rows, :], a[0][1])
        store_spec(khat, rows, range(NS), _fft16(a, -1))

    lane = jax.lax.broadcasted_iota(jnp.int32, (128, R), 1)

    def qkv(g, u, qs, ks, vs):
        w = _unpack(wt[g])
        for i in range(8):
            y = _dot(w, _unpack(u[:, i * R:(i + 1) * R]))
            qs[:, i * R:(i + 1) * R] = y[0:128]
            ks[:, (i + 7) * R:(i + 8) * R] = y[128:256]
            vs[:, (i + 7) * R:(i + 8) * R] = y[256:384]
            if i:
                dst = slice((i - 1) * R, i * R)
                ks[:, dst] = pltpu.roll(y[128:256], 1, 1)
                vs[:, dst] = jnp.where(lane == 0, va[:, 7 * R:8 * R], pltpu.roll(y[256:384], 1, 1))

    def attend(g, qs, ks, vs, o):
        for i in range(8):
            q = qs[:, i * R:(i + 1) * R]
            logits = []
            for w in range(W):
                c0 = (7 + i - w) * R
                lg = jnp.sum((q * ks[:, c0:c0 + R]).reshape(16, 8, R), axis=0) * 0.25
                if w > i:
                    lg = jnp.where(lane8 == 0, NEG, lg)
                logits.append(lg)
            mx = logits[0]
            for lg in logits[1:]:
                mx = jnp.maximum(mx, lg)
            es = [jnp.exp(lg - mx) for lg in logits]
            den = es[0]
            for e in es[1:]:
                den = den + e
            inv = 1.0 / den
            acc = None
            for w in range(W):
                c0 = (7 + i - w) * R
                term = vs[:, c0:c0 + R].reshape(16, 8, R) * (es[w] * inv)[None]
                acc = term if acc is None else acc + term
            o[_ds(g, 64), i * R:(i + 1) * R] = _pack(acc.reshape(128, R))

    def normalize(x, u, cols, total):
        m = jnp.sum(total, axis=0, keepdims=True) * (1.0 / D)
        c = x[:, cols] - m
        v = jnp.sum(c * c, axis=0, keepdims=True) * (1.0 / D)
        r = jax.lax.rsqrt(v + EPS)
        u[:, cols] = _pack(x[:, cols] * r - m * r)

    def proj(x, o, u):
        w = _unpack(wot[...])
        for i in range(8):
            cols = slice(i * R, (i + 1) * R)
            y = x[:, cols] + _dot(w, _unpack(o[:, cols]))
            x[:, cols] = y
            normalize(x, u, cols, y)

    def norm(x, u):
        for i in range(8):
            cols = slice(i * R, (i + 1) * R)
            normalize(x, u, cols, x[:, cols])

    def conv(i):
        rows = slice(8 * i, 8 * i + 8)
        uf = _fft16(load_spec(spec, rows, slabs), -1)
        kf = load_spec(khat, rows, range(NS))
        store_spec(bc, rows, slabs, _fft16([_cmul(a, b) for a, b in zip(uf, kf)], 1))

    def start_attention():
        norm(xs, un)
        qkv(0, un, qa, ka, va)
        norm(xo, uo)

    with _scope("pro0"):
        start_attention()
        for i in range(D // 8):
            k_fft(i)

    def layer(n, carry):
        def group(g, c):
            qkv(g, uo, qb, kb, vb)
            attend(g, qa, ka, va, oe)

            @pl.when(g < 3)
            def _():
                qkv(g + 1, un, qa, ka, va)
                attend(g, qb, kb, vb, oo)

            return c

        with _scope("a_grp"):
            jax.lax.fori_loop(0, 4, group, 0)
        with _scope("a_proj"):
            proj(xs, oe, un)
            attend(3, qb, kb, vb, oo)
            proj(xo, oo, uo)
            dft(f_ref, 0)
        with _scope("conv"):
            for rb in range(4):
                if rb < 3:
                    dft(f_ref, rb + 1)
                for i in range(16):
                    conv(16 * rb + i)
                idft(rb)

        with _scope("a_pro"):
            @pl.when(n == 0)
            def _():
                start_attention()

        return carry

    jax.lax.fori_loop(0, 2, layer, 0)

    stores = [pltpu.make_async_copy(xio.at[c], o_hbm.at[:, c * 128:(c + 1) * 128], sems.at[c])
              for c in range(4)]
    with _scope("store_x"):
        for b in range(4):
            rows = slice(b * 128, (b + 1) * 128)
            for jj in range(8):
                cols = slice(jj * R, (jj + 1) * R)
                t = pltpu.pack_elementwise([xs[rows, cols], xo[rows, cols]], packed_dtype=BF16)
                xu[b, pl.ds(jj, R, stride=8), :] = pltpu.bitcast(t, U32).T
            stores[b].start()
    for cp in stores:
        cp.wait()


@jax.jit
def pallas_interleave_layers__sliding_local_dilated__ssm_conv_s4__prompt_kernel(
    A_x: jax.Array,
    A_wqkv: jax.Array,
    A_wo: jax.Array,
    B_u: jax.Array,
    B_A_re: jax.Array,
    B_A_im: jax.Array,
    B_B_re: jax.Array,
    B_B_im: jax.Array,
    B_C_re: jax.Array,
    B_C_im: jax.Array,
    B_log_dt: jax.Array,
    B_Dskip: jax.Array,
):
    del B_u
    f = _dft_matrix()
    lane = (np.arange(R) - 7) % R
    order = 16 * (lane % 8) + lane // 8
    fk = (f[:, order].astype(np.float32) / L).astype(ml_dtypes.bfloat16)
    scratch = [
        pltpu.VMEM((D, L // 2), F32),
        pltpu.VMEM((D, L // 2), F32),
        pltpu.VMEM((D // 2, L // 2), U32),
        pltpu.VMEM((D // 2, L // 2), U32),
        pltpu.VMEM((4, 192, D), U32),
        pltpu.VMEM((D // 2, D), U32),
        pltpu.VMEM((D // 2, 128), U32),
        pltpu.VMEM((D, 128), F32),
        pltpu.VMEM((D, 2 * L), F32),
        pltpu.VMEM((D, 2 * L), F32),
        pltpu.VMEM((D, 2 * L), F32),
        pltpu.VMEM((128, 8 * R), F32),
        pltpu.VMEM((128, 15 * R), F32),
        pltpu.VMEM((128, 15 * R), F32),
        pltpu.VMEM((128, 8 * R), F32),
        pltpu.VMEM((128, 15 * R), F32),
        pltpu.VMEM((128, 15 * R), F32),
        pltpu.VMEM((D // 2, L // 2), U32),
        pltpu.VMEM((D // 2, L // 2), U32),
        pltpu.VMEM((4, L, 128), BF16),
        pltpu.VMEM((D, 3 * D), BF16),
        pltpu.VMEM((D, D), BF16),
        pltpu.VMEM((NS, R // 2, 2 * R), U32),
        pltpu.VMEM((NS, R // 2, 2 * R), U32),
        pltpu.SemaphoreType.DMA((8,)),
    ]
    hbm = pl.BlockSpec(memory_space=pl.ANY)
    vmem = pl.BlockSpec(memory_space=pltpu.VMEM)
    out = pl.pallas_call(
        _kernel,
        out_shape=jax.ShapeDtypeStruct((L, D), BF16),
        in_specs=[hbm] * 3 + [vmem] * 8 + [hbm] * 2,
        out_specs=hbm,
        scratch_shapes=scratch,
        compiler_params=pltpu.CompilerParams(vmem_limit_bytes=100 * 1024 * 1024),
    )(A_x.reshape(L, D), A_wqkv, A_wo, B_A_re, B_A_im, B_B_re, B_B_im, B_C_re, B_C_im,
      B_log_dt, B_Dskip, _pack_rows(f), _pack_rows(fk))
    return out.reshape(1, L, D)
```

```python
import contextlib

import jax
import jax.numpy as jnp
import jax.experimental.pallas as pl
import jax.experimental.pallas.tpu as pltpu
import ml_dtypes
import numpy as np

L = 2048
D = 512
N = 128
NS = 16
R = 128
W = 8
EPS = 1e-5
F32 = jnp.float32
BF16 = jnp.bfloat16
U32 = jnp.uint32
NEG = float(ml_dtypes.bfloat16(-1e9))

_NT = (((1,), (1,)), ((), ()))


def _slab(j):
    return (j % 2) * 8 + j // 2


def _dft_matrix():
    r = np.arange(R)
    k = np.arange(R) + 0.5
    f = np.zeros((NS, R, 2 * R), np.float64)
    for j in range(NS):
        th = 2.0 * np.pi * np.outer(NS * r + j, k) / (2 * L)
        f[_slab(j), :, :R] = np.cos(th)
        f[_slab(j), :, R:] = -np.sin(th)
    return f.astype(np.float32).astype(ml_dtypes.bfloat16)


def _pack_rows(a):
    u = np.ascontiguousarray(a).view(np.uint16).astype(np.uint32)
    return u[:, 0::2] | (u[:, 1::2] << np.uint32(16))


def _lag_tables():
    rho = []
    for s in range(8):
        lag = (256 * s + np.arange(NS)).astype(np.float32)
        rho.append([int(v) - 256 * s for v in lag.astype(ml_dtypes.bfloat16).astype(np.float32)])
    return rho


_RHO = _lag_tables()


def _cmul(a, b):
    return (a[0] * b[0] - a[1] * b[1], a[0] * b[1] + a[1] * b[0])


def _csq(a):
    t = a[0] * a[1]
    return ((a[0] - a[1]) * (a[0] + a[1]), t + t)


def _cadd(a, b):
    return (a[0] + b[0], a[1] + b[1])


def _csub(a, b):
    return (a[0] - b[0], a[1] - b[1])


def _fft4(x, sign):
    s0, d0 = _cadd(x[0], x[2]), _csub(x[0], x[2])
    s1, d1 = _cadd(x[1], x[3]), _csub(x[1], x[3])
    a = (d0[0] + d1[1], d0[1] - d1[0])
    b = (d0[0] - d1[1], d0[1] + d1[0])
    if sign > 0:
        a, b = b, a
    return [_cadd(s0, s1), a, _csub(s0, s1), b]


def _twiddle(z, m, sign):
    m = (m * sign) % 16
    re, im = z
    h = float(np.sqrt(0.5))
    if m == 0:
        return z
    if m == 4:
        return (-im, re)
    if m == 12:
        return (im, -re)
    if m == 2:
        return ((re - im) * h, (re + im) * h)
    if m == 14:
        return ((re + im) * h, (im - re) * h)
    if m == 6:
        return ((re + im) * -h, (re - im) * h)
    if m == 10:
        return ((im - re) * h, (re + im) * -h)
    c, s = float(np.cos(np.pi * m / 8)), float(np.sin(np.pi * m / 8))
    return (re * c - im * s, re * s + im * c)


def _scope(name):
    return contextlib.nullcontext()


def _ds(i, n):
    if isinstance(i, int):
        return slice(i * n, (i + 1) * n)
    return pl.ds(pl.multiple_of(i * n, n), n)


def _pack(x):
    return pltpu.bitcast(x.astype(BF16), U32)


def _unpack(x):
    return pltpu.bitcast(x, BF16)


def _dot(a, b, dims=(((1,), (0,)), ((), ()))):
    return jax.lax.dot_general(a, b, dims, preferred_element_type=F32)


def _halves(u):
    return pltpu.bitcast(u << 16, F32), pltpu.bitcast(u & jnp.uint32(0xFFFF0000), F32)


def _kernel(zero_ref, x_hbm, wqkv_hbm, wo_hbm, are_ref, aim_ref, bre_ref, bim_ref, cre_ref, cim_ref,
            ldt_ref, dsk_ref, f_hbm, fk_hbm, o_hbm,
            xs, xo, un, uo, wt, wot, dtb, dskb, pw_ref, rhs_ref, s0, s1, s2, s3, khat, qa, ka, va, qb, kb, vb,
            xio, wqkv_ref, wo_ref, f_ref, fk_ref, sems):
    loads = [pltpu.make_async_copy(x_hbm.at[:, c * 128:(c + 1) * 128], xio.at[c], sems.at[c])
             for c in range(4)]
    loads += [pltpu.make_async_copy(src, dst, sems.at[4 + n]) for n, (src, dst) in enumerate(
        [(wqkv_hbm, wqkv_ref), (wo_hbm, wo_ref), (fk_hbm, fk_ref), (f_hbm, f_ref)])]
    for cp in loads:
        cp.start()

    spec = (s0, s1, s2, s3)

    def fence(ref, val):
        row = ref.shape[0] - 8 + zero_ref[0]
        ref[pl.ds(pl.multiple_of(row, 8), 8), 0:128] = val

    dt_row = jnp.exp(ldt_ref[...].astype(F32)).reshape(1, D)
    dtb[...] = _pack(jnp.broadcast_to(dt_row, (128, D)).T)
    dskb[...] = jnp.broadcast_to(dsk_ref[...].astype(F32).reshape(1, D) * (1.0 / L), (128, D)).T

    lane8 = jax.lax.broadcasted_iota(jnp.int32, (8, R), 1)
    rev8 = 7 - jax.lax.broadcasted_iota(jnp.int32, (8, N), 0)
    steps = (1, 2, 4, 8, 256)

    def powers(i):
        def param(ref):
            return _halves(pltpu.bitcast(ref[_ds(i, 16), :], U32))

        dts = _halves(dtb[_ds(i, 8), :])
        are, aim, bre, bim, cre, cim = [
            param(r) for r in (are_ref, aim_ref, bre_ref, bim_ref, cre_ref, cim_ref)]
        for h in range(2):
            dt = dts[h]
            li = dt * aim[h]
            mag = jnp.exp(dt * are[h])
            zp = {1: (mag * jnp.cos(li), mag * jnp.sin(li))}
            for e in (1, 2, 4, 8, 16, 32, 64, 128):
                zp[2 * e] = _csq(zp[e])
            w = _cmul((cre[h], cim[h]), (dt * bre[h], dt * bim[h]))
            for n, v in enumerate([w] + [zp[e] for e in steps]):
                pw_ref[h, 2 * n] = v[0]
                pw_ref[h, 2 * n + 1] = v[1]
            pw = [(jnp.ones((8, N), F32), jnp.zeros((8, N), F32)),
                  (jnp.take_along_axis(zp[16][0], rev8, axis=0),
                   -jnp.take_along_axis(zp[16][1], rev8, axis=0))]
            for b in range(2, 16):
                pw.append(_cmul(pw[b - 1], pw[1]) if b % 2 else _csq(pw[b // 2]))
            rhs_ref[h] = _pack(jnp.concatenate([jnp.concatenate(v, axis=1) for v in pw], axis=0))

    def taps(i):
        outs = []
        for h in range(2):
            base, *zs = [(pw_ref[h, 2 * n], pw_ref[h, 2 * n + 1]) for n in range(len(steps) + 1)]
            zp = dict(zip(steps, zs))
            lhs = []
            for s in range(8):
                exps = sorted(set(_RHO[s]))
                cur = base
                for n, p in enumerate(exps):
                    if n:
                        cur = _cmul(cur, zp[p - exps[n - 1]])
                    lhs.append(jnp.concatenate(cur, axis=1))
                if s < 7:
                    base = _cmul(base, zp[256])
            outs.append(_dot(jnp.concatenate(lhs, axis=0), _unpack(rhs_ref[h]), _NT))
        both = pltpu.bitcast(pltpu.pack_elementwise(outs, packed_dtype=BF16), U32)
        keys = [(s, p) for s in range(8) for p in sorted(set(_RHO[s]))]
        piece = {}
        for n, (s, p) in enumerate(keys):
            piece[s, p] = pltpu.roll(both[8 * n:8 * n + 8], s, 1, stride=1, stride_axis=0)
        memo = {}
        for j in range(NS):
            key = ()
            acc = None
            for s in range(7, -1, -1):
                key = key + (_RHO[s][j],)
                if key not in memo:
                    pc = piece[s, _RHO[s][j]]
                    memo[key] = pc if acc is None else jnp.where(((lane8 + 1) & 7) == s, pc, acc)
                acc = memo[key]
            (un, uo)[j % 2][_ds(i + D // 16, 8), _ds(j // 2, R)] = acc

    def gen_k(i, c):
        taps(i)
        powers(jnp.minimum(i + 1, D // 16 - 1))
        return c

    with _scope("gen_k"):
        powers(0)
        jax.lax.fori_loop(0, D // 16, gen_k, 0, unroll=4)

    for cp in loads:
        cp.wait()

    xu = xio.bitcast(U32)

    def load_x(b):
        for jj in range(8):
            ev, od = _halves(xu[b, pl.ds(jj, R, stride=8), :].T)
            xs[_ds(b, 128), _ds(jj, R)] = ev
            xo[_ds(b, 128), _ds(jj, R)] = od

    m_i = jax.lax.broadcasted_iota(jnp.int32, (128, 128), 0)
    c_i = jax.lax.broadcasted_iota(jnp.int32, (128, 128), 1)
    perm = jnp.where(c_i == (m_i & 7) * 16 + (m_i >> 3), 1.0, 0.0).astype(BF16)

    def prep_w(g):
        for t in range(3):
            wt[g, _ds(t, 64), :] = _pack(_dot(perm, wqkv_ref[:, _ds(t * 4 + g, 128)], _NT))
        wot[:, _ds(g, 128)] = _pack(_dot(perm, wo_ref[_ds(g, 128), :]).T)

    def prep(b, c):
        load_x(b)
        prep_w(b)
        return c

    with _scope("prep"):
        jax.lax.fori_loop(0, 4, prep, 0)

    def dft(mat, rb, s, src=0):
        u = (un, uo)[s // 8][_ds(rb + src, 64), _ds(s % 8, R)]
        spec[rb][0:128, _ds(s, 2 * R)] = _dot(_unpack(u), _unpack(mat[s]))

    def idft(rb, s):
        (xs, xo)[s // 8][_ds(rb, 128), _ds(s % 8, R)] += _dot(
            spec[rb][0:128, _ds(s, 2 * R)], _unpack(f_ref[s]), _NT)

    def load_spec(ref, rows, order):
        return [(ref[rows, _ds(2 * s, R)], ref[rows, _ds(2 * s + 1, R)]) for s in order]

    def store_spec(ref, rows, order, vals):
        for s, v in zip(order, vals):
            ref[rows, _ds(2 * s, R)] = v[0]
            ref[rows, _ds(2 * s + 1, R)] = v[1]

    slabs = [_slab(j) for j in range(NS)]

    def spectrum(i, odd, bias=None):
        halves = []
        for n in range(2):
            a = []
            for m in range(4):
                j = n + 2 * m
                lo, hi = load_spec(spec[i // 16], _ds(i % 16, 8), [slabs[j], slabs[j + 8]])
                if j == 0 and bias is not None:
                    lo = (lo[0] + bias, lo[1])
                a.append(_twiddle(_csub(lo, hi), j, -1) if odd else _cadd(lo, hi))
            halves.append([_twiddle(v, 2 * n * k, -1) for k, v in enumerate(_fft4(a, -1))])
        for k in range(4):
            yield k, _cadd(halves[0][k], halves[1][k]), _csub(halves[0][k], halves[1][k])

    def k_fft(i):
        rows = _ds(i, 8)
        for odd in range(2):
            for k, lo, hi in spectrum(i, odd, dskb[rows, :]):
                store_spec(khat, rows, [8 * odd + k, 8 * odd + k + 4], [lo, hi])
                if k == 0 and odd:
                    fence(spec[i // 16], lo[0])
        return lo[0]

    def conv(i):
        buf, rows = spec[i // 16], _ds(i % 16, 8)
        park = _ds(16, 8)
        for odd in (1, 0):
            cols = [[], []]
            for k, lo, hi in spectrum(i, odd):
                klo, khi = load_spec(khat, _ds(i, 8), [8 * odd + k, 8 * odd + k + 4])
                lo, hi = _cmul(lo, klo), _cmul(hi, khi)
                cols[0].append(_cadd(lo, hi))
                cols[1].append(_twiddle(_csub(lo, hi), 2 * k, 1))
            fence(buf, cols[1][3][0])
            for n in range(2):
                for m, v in enumerate(_fft4(cols[n], 1)):
                    j = n + 2 * m
                    if odd:
                        store_spec(buf, park, [j], [_twiddle(v, j, 1)])
                    else:
                        (o,) = load_spec(buf, park, [j])
                        store_spec(buf, rows, [slabs[j], slabs[j + 8]], [_cadd(v, o), _csub(v, o)])
        return cols[1][3][0]

    lane = jax.lax.broadcasted_iota(jnp.int32, (128, R), 1)

    def qkv(g, u, qs, ks, vs, i):
        y = _dot(_unpack(wt[g]), _unpack(u[0:D // 2, _ds(i, R)]))
        qs[:, _ds(i, R)] = y[0:128]
        ks[:, _ds(i + 7, R)] = y[128:256]
        vs[:, _ds(i + 7, R)] = y[256:384]
        if i:
            ks[:, _ds(i - 1, R)] = pltpu.roll(y[128:256], 1, 1)
            vs[:, _ds(i - 1, R)] = jnp.where(lane == 0, va[:, _ds(7, R)], pltpu.roll(y[256:384], 1, 1))

    def attend(g, qs, ks, vs, o, i):
        q = qs[:, _ds(i, R)]
        logits = []
        for w in range(W):
            lg = jnp.sum((q * ks[:, _ds(7 + i - w, R)]).reshape(16, 8, R), axis=0) * 0.25
            if w > i:
                lg = jnp.where(lane8 == 0, NEG, lg)
            logits.append(lg)
        mx = logits[0]
        for lg in logits[1:]:
            mx = jnp.maximum(mx, lg)
        es = [jnp.exp(lg - mx) for lg in logits]
        den = es[0]
        for e in es[1:]:
            den = den + e
        inv = 1.0 / den
        acc = None
        for w in range(W):
            term = vs[:, _ds(7 + i - w, R)].reshape(16, 8, R) * (es[w] * inv)[None]
            acc = term if acc is None else acc + term
        o[_ds(g + 4, 64), _ds(i, R)] = _pack(acc.reshape(128, R))

    def norm(x, u, i, total=None):
        cols = _ds(i, R)
        total = x[:, cols] if total is None else total
        m = jnp.sum(total, axis=0, keepdims=True) * (1.0 / D)
        c = x[:, cols] - m
        v = jnp.sum(c * c, axis=0, keepdims=True) * (1.0 / D)
        r = jax.lax.rsqrt(v + EPS)
        n = _pack(x[:, cols] * r - m * r)
        u[0:D // 2, cols] = n
        return n

    def proj(x, o, u, i):
        y = x[:, _ds(i, R)] + _dot(_unpack(wot[...]), _unpack(o[D // 2:D, _ds(i, R)]))
        x[:, _ds(i, R)] = y
        norm(x, u, i, y)

    with _scope("pro0"):
        for rb in range(4):
            for s in range(NS):
                dft(fk_ref, rb, s, src=4)
                if s % 4 == 0:
                    i = 4 * rb + s // 4
                    norm((xs, xo)[i // 8], (un, uo)[i // 8], i % 8)
                if rb:
                    fence(spec[rb], k_fft(16 * (rb - 1) + s))
        for i in range(8):
            qkv(0, un, qa, ka, va, i)
            k_fft(48 + 2 * i)
            k_fft(49 + 2 * i)

    def layer(n, carry):
        def group(g, c):
            for i in range(8):
                qkv(g, uo, qb, kb, vb, i)
                attend(g, qa, ka, va, uo, i)

            @pl.when(g < 3)
            def _():
                for i in range(8):
                    qkv(g + 1, un, qa, ka, va, i)
                    attend(g, qb, kb, vb, un, i)

            return c

        with _scope("a_grp"):
            jax.lax.fori_loop(0, 4, group, 0)
        with _scope("a_proj"):
            for i in range(8):
                proj(xs, uo, un, i)
                attend(3, qb, kb, vb, un, i)
            for i in range(8):
                proj(xo, un, uo, i)
            for s in range(NS):
                dft(f_ref, 0, s)
        with _scope("conv"):
            for rb in range(4):
                for s in range(NS):
                    if rb < 3:
                        dft(f_ref, rb + 1, s)
                    if rb:
                        idft(rb - 1, s)
                    mark = conv(16 * rb + s)
                    for other in (rb - 1, rb + 1):
                        if 0 <= other < 4:
                            fence(spec[other], mark)

        with _scope("a_pro"):
            @pl.when(n == 0)
            def _():
                for s in (0, 1, 2, 3, 4, 5, 6, 7, 8, 9, 10, 11, 12, 13, 14, 15):
                    idft(3, s)
                norm(xs, un, 0)
                for i in range(8):
                    qkv(0, un, qa, ka, va, i)
                    if i < 7:
                        norm(xs, un, i + 1)
                    fence(un, norm(xo, uo, i)[-8:])

        return carry

    jax.lax.fori_loop(0, 2, layer, 0)

    stores = [pltpu.make_async_copy(xio.at[c], o_hbm.at[:, c * 128:(c + 1) * 128], sems.at[c])
              for c in range(4)]
    with _scope("store_x"):
        for b in range(4):
            for jj in range(8):
                if b == 0:
                    idft(3, jj)
                    idft(3, jj + 8)
                t = pltpu.pack_elementwise(
                    [xs[_ds(b, 128), _ds(jj, R)], xo[_ds(b, 128), _ds(jj, R)]], packed_dtype=BF16)
                xu[b, pl.ds(jj, R, stride=8), :] = pltpu.bitcast(t, U32).T
            stores[b].start()
    for cp in stores:
        cp.wait()


@jax.jit
def pallas_interleave_layers__sliding_local_dilated__ssm_conv_s4__prompt_kernel(
    A_x: jax.Array,
    A_wqkv: jax.Array,
    A_wo: jax.Array,
    B_u: jax.Array,
    B_A_re: jax.Array,
    B_A_im: jax.Array,
    B_B_re: jax.Array,
    B_B_im: jax.Array,
    B_C_re: jax.Array,
    B_C_im: jax.Array,
    B_log_dt: jax.Array,
    B_Dskip: jax.Array,
):
    del B_u
    f = _dft_matrix()
    lane = (np.arange(R) - 7) % R
    order = 16 * (lane % 8) + lane // 8
    fk = (f[:, order].astype(np.float32) / L).astype(ml_dtypes.bfloat16)
    scratch = [
        pltpu.VMEM((D, L // 2), F32),
        pltpu.VMEM((D, L // 2), F32),
        pltpu.VMEM((D + 8, L // 2), U32),
        pltpu.VMEM((D + 8, L // 2), U32),
        pltpu.VMEM((4, 192, D), U32),
        pltpu.VMEM((D // 2, D), U32),
        pltpu.VMEM((D // 2, 128), U32),
        pltpu.VMEM((D, 128), F32),
        pltpu.VMEM((2, 12, 8, N), F32),
        pltpu.VMEM((2, 64, 2 * N), U32),
        *[pltpu.VMEM((128 + 16, 2 * L), F32)] * 4,
        pltpu.VMEM((D, 2 * L), F32),
        pltpu.VMEM((128, 8 * R), F32),
        pltpu.VMEM((128, 15 * R), F32),
        pltpu.VMEM((128, 15 * R), F32),
        pltpu.VMEM((128, 8 * R), F32),
        pltpu.VMEM((128, 15 * R), F32),
        pltpu.VMEM((128, 15 * R), F32),
        pltpu.VMEM((4, L, 128), BF16),
        pltpu.VMEM((D, 3 * D), BF16),
        pltpu.VMEM((D, D), BF16),
        pltpu.VMEM((NS, R // 2, 2 * R), U32),
        pltpu.VMEM((NS, R // 2, 2 * R), U32),
        pltpu.SemaphoreType.DMA((8,)),
    ]
    hbm = pl.BlockSpec(memory_space=pl.ANY)
    vmem = pl.BlockSpec(memory_space=pltpu.VMEM)
    out = pl.pallas_call(
        _kernel,
        out_shape=jax.ShapeDtypeStruct((L, D), BF16),
        in_specs=[pl.BlockSpec(memory_space=pltpu.SMEM)] + [hbm] * 3 + [vmem] * 8 + [hbm] * 2,
        out_specs=hbm,
        scratch_shapes=scratch,
        compiler_params=pltpu.CompilerParams(vmem_limit_bytes=100 * 1024 * 1024),
    )(np.zeros((1,), np.int32), A_x.reshape(L, D), A_wqkv, A_wo, B_A_re, B_A_im, B_B_re, B_B_im, B_C_re, B_C_im,
      B_log_dt, B_Dskip, _pack_rows(f), _pack_rows(fk))
    return out.reshape(1, L, D)
```

```python
import contextlib

import jax
import jax.numpy as jnp
import jax.experimental.pallas as pl
import jax.experimental.pallas.tpu as pltpu
import ml_dtypes
import numpy as np

L = 2048
D = 512
N = 128
NS = 16
R = 128
W = 8
EPS = 1e-5
CH = 2
F32 = jnp.float32
BF16 = jnp.bfloat16
U32 = jnp.uint32
NEG = float(ml_dtypes.bfloat16(-1e9))

_NT = (((1,), (1,)), ((), ()))


def _slab(j):
    return (j % 2) * 8 + j // 2


def _dft_matrix():
    r = np.arange(R)
    k = np.arange(R) + 0.5
    f = np.zeros((NS, R, 2 * R), np.float64)
    for j in range(NS):
        th = 2.0 * np.pi * np.outer(NS * r + j, k) / (2 * L)
        f[_slab(j), :, :R] = np.cos(th)
        f[_slab(j), :, R:] = -np.sin(th)
    return f.astype(np.float32).astype(ml_dtypes.bfloat16)


def _pack_rows(a):
    u = np.ascontiguousarray(a).view(np.uint16).astype(np.uint32)
    return u[:, 0::2] | (u[:, 1::2] << np.uint32(16))


def _lag_tables():
    rho = []
    for s in range(8):
        lag = (256 * s + np.arange(NS)).astype(np.float32)
        rho.append([int(v) - 256 * s for v in lag.astype(ml_dtypes.bfloat16).astype(np.float32)])
    return rho


_RHO = _lag_tables()


def _cmul(a, b):
    return (a[0] * b[0] - a[1] * b[1], a[0] * b[1] + a[1] * b[0])


def _csq(a):
    t = a[0] * a[1]
    return ((a[0] - a[1]) * (a[0] + a[1]), t + t)


def _cadd(a, b):
    return (a[0] + b[0], a[1] + b[1])


def _csub(a, b):
    return (a[0] - b[0], a[1] - b[1])


def _fft4(x, sign):
    s0, d0 = _cadd(x[0], x[2]), _csub(x[0], x[2])
    s1, d1 = _cadd(x[1], x[3]), _csub(x[1], x[3])
    a = (d0[0] + d1[1], d0[1] - d1[0])
    b = (d0[0] - d1[1], d0[1] + d1[0])
    if sign > 0:
        a, b = b, a
    return [_cadd(s0, s1), a, _csub(s0, s1), b]


def _twiddle(z, m, sign):
    m = (m * sign) % 16
    re, im = z
    h = float(np.sqrt(0.5))
    if m == 0:
        return z
    if m == 4:
        return (-im, re)
    if m == 12:
        return (im, -re)
    if m == 2:
        return ((re - im) * h, (re + im) * h)
    if m == 14:
        return ((re + im) * h, (im - re) * h)
    if m == 6:
        return ((re + im) * -h, (re - im) * h)
    if m == 10:
        return ((im - re) * h, (re + im) * -h)
    c, s = float(np.cos(np.pi * m / 8)), float(np.sin(np.pi * m / 8))
    return (re * c - im * s, re * s + im * c)


def _scope(name):
    return contextlib.nullcontext()


def _ds(i, n):
    if isinstance(i, int):
        return slice(i * n, (i + 1) * n)
    return pl.ds(pl.multiple_of(i * n, n), n)


def _pack(x):
    return pltpu.bitcast(x.astype(BF16), U32)


def _unpack(x):
    return pltpu.bitcast(x, BF16)


def _dot(a, b, dims=(((1,), (0,)), ((), ()))):
    return jax.lax.dot_general(a, b, dims, preferred_element_type=F32)


def _halves(u):
    return pltpu.bitcast(u << 16, F32), pltpu.bitcast(u & jnp.uint32(0xFFFF0000), F32)


def _kernel(zero_ref, x_hbm, wqkv_hbm, wo_hbm, are_ref, aim_ref, bre_ref, bim_ref, cre_ref, cim_ref,
            ldt_ref, dsk_ref, f_hbm, fk_hbm, o_hbm,
            xs, xo, un, uo, wt, wot, dtb, dskb, pw_ref, rhs_ref, s0, s1, s2, s3, kspec, khat, qa, ka, va, qb, kb, vb,
            xio, wqkv_ref, wo_ref, f_ref, fk_ref, sems):
    loads = [pltpu.make_async_copy(fk_hbm, fk_ref, sems.at[4])]
    loads += [pltpu.make_async_copy(x_hbm.at[:, c * 128:(c + 1) * 128], xio.at[c], sems.at[c])
              for c in range(4)]
    loads += [pltpu.make_async_copy(src, dst, sems.at[5 + n]) for n, (src, dst) in enumerate(
        [(wqkv_hbm, wqkv_ref), (wo_hbm, wo_ref), (f_hbm, f_ref)])]
    for cp in loads:
        cp.start()

    spec = (s0, s1, s2, s3)

    def fence(ref, val):
        row = ref.shape[0] - 8 + zero_ref[0]
        ref[pl.ds(pl.multiple_of(row, 8), 8), 0:128] = val

    dt_row = jnp.exp(ldt_ref[...].astype(F32)).reshape(1, D)
    dtb[...] = _pack(jnp.broadcast_to(dt_row, (128, D)).T)
    dskb[...] = jnp.broadcast_to(dsk_ref[...].astype(F32).reshape(1, D) * (1.0 / L), (128, D)).T

    lane8 = jax.lax.broadcasted_iota(jnp.int32, (8, R), 1)
    rev8 = 7 - jax.lax.broadcasted_iota(jnp.int32, (8, N), 0)
    steps = (1, 2, 4, 8, 256)

    def powers(i):
        def param(ref):
            return _halves(pltpu.bitcast(ref[_ds(i, 16), :], U32))

        dts = _halves(dtb[_ds(i, 8), :])
        are, aim, bre, bim, cre, cim = [
            param(r) for r in (are_ref, aim_ref, bre_ref, bim_ref, cre_ref, cim_ref)]
        for h in range(2):
            dt = dts[h]
            li = dt * aim[h]
            mag = jnp.exp(dt * are[h])
            zp = {1: (mag * jnp.cos(li), mag * jnp.sin(li))}
            for e in (1, 2, 4, 8, 16, 32, 64, 128):
                zp[2 * e] = _csq(zp[e])
            w = _cmul((cre[h], cim[h]), (dt * bre[h], dt * bim[h]))
            for n, v in enumerate([w] + [zp[e] for e in steps]):
                pw_ref[h, 2 * n] = v[0]
                pw_ref[h, 2 * n + 1] = v[1]
            pw = [(jnp.ones((8, N), F32), jnp.zeros((8, N), F32)),
                  (jnp.take_along_axis(zp[16][0], rev8, axis=0),
                   -jnp.take_along_axis(zp[16][1], rev8, axis=0))]
            for b in range(2, 16):
                pw.append(_cmul(pw[b - 1], pw[1]) if b % 2 else _csq(pw[b // 2]))
            rhs_ref[h] = _pack(jnp.concatenate([jnp.concatenate(v, axis=1) for v in pw], axis=0))

    keys = [(s, p) for s in range(8) for p in sorted(set(_RHO[s]) - {16})] + [(8, 0)]

    def taps(i):
        outs = []
        for h in range(2):
            base, *zs = [(pw_ref[h, 2 * n], pw_ref[h, 2 * n + 1]) for n in range(len(steps) + 1)]
            zp = dict(zip(steps, zs))
            lhs = []
            for n, (s, p) in enumerate(keys):
                if p:
                    cur = _cmul(cur, zp[p - keys[n - 1][1]])
                else:
                    base = cur = _cmul(base, zp[256]) if s else base
                lhs.append(jnp.concatenate(cur, axis=1))
            outs.append(_dot(jnp.concatenate(lhs, axis=0), _unpack(rhs_ref[h]), _NT))
        both = pltpu.bitcast(pltpu.pack_elementwise(outs, packed_dtype=BF16), U32)
        piece = {}
        for n, (s, p) in enumerate(keys):
            piece[s, p] = pltpu.roll(both[8 * n:8 * n + 8], 126 - 7 if s == 8 else s, 1,
                                     stride=1, stride_axis=0)
        memo = {}
        for j in range(NS):
            key = ()
            acc = None
            for s in range(7, -1, -1):
                key = key + (_RHO[s][j],)
                if key not in memo:
                    pc = carry if _RHO[s][j] == 16 else piece[s, _RHO[s][j]]
                    same = acc is None or pc is acc
                    memo[key] = pc if same else jnp.where(((lane8 + 1) & 7) == s, pc, acc)
                acc = memo[key]
            (un, uo)[j % 2][_ds(i + D // 16, 8), _ds(j // 2, R)] = acc
            if j == 0:
                last_b = ((lane8 + 1) & 127) < 8
                carry = jnp.where(last_b, pltpu.roll(acc, 128 - 9, 1), pltpu.roll(acc, 128 - 8, 1))
                carry = jnp.where(lane8 == 6, pltpu.roll(piece[8, 0], 8, 1), carry)

    def gen_k(rb):
        for n in range(8):
            i = 8 * rb + n
            taps(i)
            powers(jnp.minimum(i + 1, D // 16 - 1))

    def dft_k(rb):
        for s in range(NS):
            u = (un, uo)[s // 8][_ds(rb + 4, 64), _ds(s % 8, R)]
            kspec[_ds(rb, 128), _ds(s, 2 * R)] = _dot(_unpack(u), _unpack(fk_ref[s]))

    def gen_step(rb, c):
        dft_k(rb - 1)
        gen_k(rb)
        return c

    with _scope("gen_k"):
        powers(0)
        gen_k(0)
        loads[0].wait()
        jax.lax.fori_loop(1, 4, gen_step, 0)

    for cp in loads[1:]:
        cp.wait()

    xu = xio.bitcast(U32)

    def load_x(b):
        for jj in range(8):
            ev, od = _halves(xu[b, pl.ds(jj, R, stride=8), :].T)
            xs[_ds(b, 128), _ds(jj, R)] = ev
            xo[_ds(b, 128), _ds(jj, R)] = od

    m_i = jax.lax.broadcasted_iota(jnp.int32, (128, 128), 0)
    c_i = jax.lax.broadcasted_iota(jnp.int32, (128, 128), 1)
    perm = jnp.where(c_i == (m_i & 7) * 16 + (m_i >> 3), 1.0, 0.0).astype(BF16)

    def prep_w(g):
        for t in range(3):
            wt[g, _ds(t, 64), :] = _pack(_dot(perm, wqkv_ref[:, _ds(t * 4 + g, 128)], _NT))
        wot[:, _ds(g, 128)] = _pack(_dot(perm, wo_ref[_ds(g, 128), :]).T)

    with _scope("prep"):
        dft_k(3)
        for b in range(4):
            load_x(b)
            prep_w(b)

    def dft(rb, s):
        u = (un, uo)[s // 8][_ds(rb, 64), _ds(s % 8, R)]
        spec[rb][0:128, _ds(s, 2 * R)] = _dot(_unpack(u), _unpack(f_ref[s]))

    def idft(rb, s):
        (xs, xo)[s // 8][_ds(rb, 128), _ds(s % 8, R)] += _dot(
            spec[rb][0:128, _ds(s, 2 * R)], _unpack(f_ref[s]), _NT)

    def load_spec(ref, rows, order):
        return [(ref[rows, _ds(2 * s, R)], ref[rows, _ds(2 * s + 1, R)]) for s in order]

    def store_spec(ref, rows, order, vals):
        for s, v in zip(order, vals):
            ref[rows, _ds(2 * s, R)] = v[0]
            ref[rows, _ds(2 * s + 1, R)] = v[1]

    slabs = [_slab(j) for j in range(NS)]

    def spectrum(buf, rows, odd, bias=None):
        halves = []
        for n in range(2):
            a = []
            for m in range(4):
                j = n + 2 * m
                lo, hi = load_spec(buf, rows, [slabs[j], slabs[j + 8]])
                if j == 0 and bias is not None:
                    lo = (lo[0] + bias, lo[1])
                a.append(_twiddle(_csub(lo, hi), j, -1) if odd else _cadd(lo, hi))
            halves.append([_twiddle(v, 2 * n * k, -1) for k, v in enumerate(_fft4(a, -1))])
        for k in range(4):
            yield k, _cadd(halves[0][k], halves[1][k]), _csub(halves[0][k], halves[1][k])

    def k_fft(i):
        rows = _ds(i, 8)
        for odd in range(2):
            for k, lo, hi in spectrum(kspec, rows, odd, dskb[rows, :]):
                store_spec(khat, rows, [8 * odd + k, 8 * odd + k + 4], [lo, hi])

    def conv(i):
        buf, rows = spec[i // 16], _ds(i % 16, 8)
        park = _ds(16, 8)
        for odd in (1, 0):
            cols = [[], []]
            for k, lo, hi in spectrum(buf, rows, odd):
                klo, khi = load_spec(khat, _ds(i, 8), [8 * odd + k, 8 * odd + k + 4])
                lo, hi = _cmul(lo, klo), _cmul(hi, khi)
                cols[0].append(_cadd(lo, hi))
                cols[1].append(_twiddle(_csub(lo, hi), 2 * k, 1))
            fence(buf, cols[1][3][0])
            for n in range(2):
                for m, v in enumerate(_fft4(cols[n], 1)):
                    j = n + 2 * m
                    if odd:
                        store_spec(buf, park, [j], [_twiddle(v, j, 1)])
                    else:
                        (o,) = load_spec(buf, park, [j])
                        store_spec(buf, rows, [slabs[j], slabs[j + 8]], [_cadd(v, o), _csub(v, o)])
        return cols[1][3][0]

    lane = jax.lax.broadcasted_iota(jnp.int32, (128, R), 1)

    def qkv(g, u, qs, ks, vs, i):
        y = _dot(_unpack(wt[g]), _unpack(u[0:D // 2, _ds(i, R)]))
        qs[:, _ds(i, R)] = y[0:128]
        ks[:, _ds(i + 7, R)] = y[128:256]
        vs[:, _ds(i + 7, R)] = y[256:384]
        if i:
            ks[:, _ds(i - 1, R)] = pltpu.roll(y[128:256], 1, 1)
            vs[:, _ds(i - 1, R)] = jnp.where(lane == 0, va[:, _ds(7, R)], pltpu.roll(y[256:384], 1, 1))

    never = lane8 < zero_ref[0]

    def attend(g, qs, ks, vs, o, i):
        logits = []
        for w in range(W):
            lg = None
            for c in range(16):
                term = qs[_ds(c, 8), _ds(i, R)] * ks[_ds(c, 8), _ds(7 + i - w, R)]
                if c:
                    lg = lg + term
                else:
                    lg = term if w < CH else jnp.where(never, logits[w - CH], term)
            logits.append(lg)
        logits = [lg * 0.25 for lg in logits]
        logits = [jnp.where(lane8 == 0, NEG, lg) if w > i else lg for w, lg in enumerate(logits)]
        mx = logits[0]
        for lg in logits[1:]:
            mx = jnp.maximum(mx, lg)
        es = [jnp.exp(lg - mx) for lg in logits]
        den = es[0]
        for e in es[1:]:
            den = den + e
        inv = 1.0 / den
        probs = [e * inv for e in es]
        outs = []
        for c in range(16):
            acc = None
            for w in range(W):
                term = vs[_ds(c, 8), _ds(7 + i - w, R)] * probs[w]
                if w:
                    acc = acc + term
                else:
                    acc = term if c < CH else jnp.where(never, outs[c - CH], term)
            outs.append(acc)
        o[_ds(g + 4, 64), _ds(i, R)] = _pack(jnp.concatenate(outs, axis=0))

    def chain_sum(vals, ways):
        parts = vals[:ways]
        for n, v in enumerate(vals[ways:]):
            parts[n % ways] = parts[n % ways] + v
        return jnp.sum(sum(parts[1:], parts[0]), axis=0, keepdims=True)

    def norm(x, u, i, total=None):
        cols = _ds(i, R)
        total = x[:, cols] if total is None else total
        m = chain_sum([total[_ds(n, 8)] for n in range(D // 8)], 4) * (1.0 / D)
        c = x[:, cols] - m
        c = c * c
        v = chain_sum([c[_ds(n, 8)] for n in range(D // 8)], 2) * (1.0 / D)
        r = jax.lax.rsqrt(v + EPS)
        n = _pack(x[:, cols] * r - m * r)
        u[0:D // 2, cols] = n
        return n

    def proj(x, o, u, i):
        y = x[:, _ds(i, R)] + _dot(_unpack(wot[...]), _unpack(o[D // 2:D, _ds(i, R)]))
        x[:, _ds(i, R)] = y
        norm(x, u, i, y)

    def layer(n, carry):
        with _scope("a_pro"):
            norm(xs, un, 0)
            for i in range(8):
                qkv(0, un, qa, ka, va, i)
                if i < 7:
                    norm(xs, un, i + 1)
                fence(un, norm(xo, uo, i)[-8:])

        def group(g, c):
            for i in range(8):
                qkv(g, uo, qb, kb, vb, i)
                k_fft(16 * g + i)
                attend(g, qa, ka, va, uo, i)

            @pl.when(g < 3)
            def _():
                for i in range(8):
                    qkv(g + 1, un, qa, ka, va, i)
                    k_fft(16 * g + 8 + i)
                    attend(g, qb, kb, vb, un, i)

            return c

        with _scope("a_grp"):
            jax.lax.fori_loop(0, 4, group, 0)
        with _scope("a_proj"):
            for i in range(8):
                proj(xs, uo, un, i)
                k_fft(56 + i)
                attend(3, qb, kb, vb, un, i)
            for i in range(8):
                proj(xo, un, uo, i)
            for s in range(NS):
                dft(0, s)
        with _scope("conv"):
            for rb in range(4):
                for s in range(NS):
                    if rb < 3:
                        dft(rb + 1, s)
                    if rb:
                        idft(rb - 1, s)
                    mark = conv(16 * rb + s)
                    for other in (rb - 1, rb + 1):
                        if 0 <= other < 4 and s % 2:
                            fence(spec[other], mark)
            for s in range(NS):
                idft(3, s)
        return carry

    jax.lax.fori_loop(0, 2, layer, 0)

    stores = [pltpu.make_async_copy(xio.at[c], o_hbm.at[:, c * 128:(c + 1) * 128], sems.at[c])
              for c in range(4)]
    with _scope("store_x"):
        for b in range(4):
            for jj in range(8):
                t = pltpu.pack_elementwise(
                    [xs[_ds(b, 128), _ds(jj, R)], xo[_ds(b, 128), _ds(jj, R)]], packed_dtype=BF16)
                xu[b, pl.ds(jj, R, stride=8), :] = pltpu.bitcast(t, U32).T
            stores[b].start()
    for cp in stores:
        cp.wait()


@jax.jit
def pallas_interleave_layers__sliding_local_dilated__ssm_conv_s4__prompt_kernel(
    A_x: jax.Array,
    A_wqkv: jax.Array,
    A_wo: jax.Array,
    B_u: jax.Array,
    B_A_re: jax.Array,
    B_A_im: jax.Array,
    B_B_re: jax.Array,
    B_B_im: jax.Array,
    B_C_re: jax.Array,
    B_C_im: jax.Array,
    B_log_dt: jax.Array,
    B_Dskip: jax.Array,
):
    del B_u
    f = _dft_matrix()
    lane = (np.arange(R) - 7) % R
    order = 16 * (lane % 8) + lane // 8
    fk = (f[:, order].astype(np.float32) / L).astype(ml_dtypes.bfloat16)
    scratch = [
        pltpu.VMEM((D, L // 2), F32),
        pltpu.VMEM((D, L // 2), F32),
        pltpu.VMEM((D + 8, L // 2), U32),
        pltpu.VMEM((D + 8, L // 2), U32),
        pltpu.VMEM((4, 192, D), U32),
        pltpu.VMEM((D // 2, D), U32),
        pltpu.VMEM((D // 2, 128), U32),
        pltpu.VMEM((D, 128), F32),
        pltpu.VMEM((2, 12, 8, N), F32),
        pltpu.VMEM((2, 64, 2 * N), U32),
        *[pltpu.VMEM((128 + 16, 2 * L), F32)] * 4,
        pltpu.VMEM((D, 2 * L), F32),
        pltpu.VMEM((D, 2 * L), F32),
        pltpu.VMEM((128, 8 * R), F32),
        pltpu.VMEM((128, 15 * R), F32),
        pltpu.VMEM((128, 15 * R), F32),
        pltpu.VMEM((128, 8 * R), F32),
        pltpu.VMEM((128, 15 * R), F32),
        pltpu.VMEM((128, 15 * R), F32),
        pltpu.VMEM((4, L, 128), BF16),
        pltpu.VMEM((D, 3 * D), BF16),
        pltpu.VMEM((D, D), BF16),
        pltpu.VMEM((NS, R // 2, 2 * R), U32),
        pltpu.VMEM((NS, R // 2, 2 * R), U32),
        pltpu.SemaphoreType.DMA((8,)),
    ]
    hbm = pl.BlockSpec(memory_space=pl.ANY)
    vmem = pl.BlockSpec(memory_space=pltpu.VMEM)
    out = pl.pallas_call(
        _kernel,
        out_shape=jax.ShapeDtypeStruct((L, D), BF16),
        in_specs=[pl.BlockSpec(memory_space=pltpu.SMEM)] + [hbm] * 3 + [vmem] * 8 + [hbm] * 2,
        out_specs=hbm,
        scratch_shapes=scratch,
        compiler_params=pltpu.CompilerParams(vmem_limit_bytes=100 * 1024 * 1024),
    )(np.zeros((1,), np.int32), A_x.reshape(L, D), A_wqkv, A_wo, B_A_re, B_A_im, B_B_re, B_B_im, B_C_re, B_C_im,
      B_log_dt, B_Dskip, _pack_rows(f), _pack_rows(fk))
    return out.reshape(1, L, D)
```

```python
import contextlib

import jax
import jax.numpy as jnp
import jax.experimental.pallas as pl
import jax.experimental.pallas.tpu as pltpu
import ml_dtypes
import numpy as np

L = 2048
D = 512
N = 128
NS = 16
R = 128
W = 8
EPS = 1e-5
CH = 2
BLOCKS = ((0, 128), (128, 128), (256, 128), (384, 128))
F32 = jnp.float32
BF16 = jnp.bfloat16
U32 = jnp.uint32
NEG = float(ml_dtypes.bfloat16(-1e9))

_NT = (((1,), (1,)), ((), ()))


def _slab(j):
    return (j % 2) * 8 + j // 2


def _dft_matrix():
    r = np.arange(R)
    k = np.arange(R) + 0.5
    f = np.zeros((NS, R, 2 * R), np.float64)
    for j in range(NS):
        th = 2.0 * np.pi * np.outer(NS * r + j, k) / (2 * L)
        f[_slab(j), :, :R] = np.cos(th)
        f[_slab(j), :, R:] = -np.sin(th)
    return f.astype(np.float32).astype(ml_dtypes.bfloat16)


def _pack_rows(a):
    u = np.ascontiguousarray(a).view(np.uint16).astype(np.uint32)
    return u[:, 0::2] | (u[:, 1::2] << np.uint32(16))


def _lag_tables():
    rho = []
    for s in range(8):
        lag = (256 * s + np.arange(NS)).astype(np.float32)
        rho.append([int(v) - 256 * s for v in lag.astype(ml_dtypes.bfloat16).astype(np.float32)])
    return rho


_RHO = _lag_tables()


def _cmul(a, b):
    return (a[0] * b[0] - a[1] * b[1], a[0] * b[1] + a[1] * b[0])


def _csq(a):
    t = a[0] * a[1]
    return ((a[0] - a[1]) * (a[0] + a[1]), t + t)


def _cadd(a, b):
    return (a[0] + b[0], a[1] + b[1])


def _csub(a, b):
    return (a[0] - b[0], a[1] - b[1])


def _fft4(x, sign):
    s0, d0 = _cadd(x[0], x[2]), _csub(x[0], x[2])
    s1, d1 = _cadd(x[1], x[3]), _csub(x[1], x[3])
    a = (d0[0] + d1[1], d0[1] - d1[0])
    b = (d0[0] - d1[1], d0[1] + d1[0])
    if sign > 0:
        a, b = b, a
    return [_cadd(s0, s1), a, _csub(s0, s1), b]


def _twiddle(z, m, sign):
    m = (m * sign) % 16
    re, im = z
    h = float(np.sqrt(0.5))
    if m == 0:
        return z
    if m == 4:
        return (-im, re)
    if m == 12:
        return (im, -re)
    if m == 2:
        return ((re - im) * h, (re + im) * h)
    if m == 14:
        return ((re + im) * h, (im - re) * h)
    if m == 6:
        return ((re + im) * -h, (re - im) * h)
    if m == 10:
        return ((im - re) * h, (re + im) * -h)
    c, s = float(np.cos(np.pi * m / 8)), float(np.sin(np.pi * m / 8))
    return (re * c - im * s, re * s + im * c)


def _scope(name):
    return contextlib.nullcontext()


def _ds(i, n):
    if isinstance(i, int):
        return slice(i * n, (i + 1) * n)
    return pl.ds(pl.multiple_of(i * n, n), n)


def _pack(x):
    return pltpu.bitcast(x.astype(BF16), U32)


def _unpack(x):
    return pltpu.bitcast(x, BF16)


def _dot(a, b, dims=(((1,), (0,)), ((), ()))):
    return jax.lax.dot_general(a, b, dims, preferred_element_type=F32)


def _halves(u):
    return pltpu.bitcast(u << 16, F32), pltpu.bitcast(u & jnp.uint32(0xFFFF0000), F32)


def _kernel(zero_ref, x_hbm, wqkv_hbm, wo_hbm, are_ref, aim_ref, bre_ref, bim_ref, cre_ref, cim_ref,
            ldt_ref, dsk_ref, f_hbm, fk_hbm, o_hbm,
            xs, xo, un, uo, wt, wot, dtb, dskb, pw_ref, rhs_ref, s0, s1, s2, s3, kspec, khat, qa, ka, va, qb, kb, vb,
            ra, rb_, cen,
            xio, wqkv_ref, wo_ref, f_ref, fk_ref, sems):
    loads = [pltpu.make_async_copy(fk_hbm, fk_ref, sems.at[4])]
    loads += [pltpu.make_async_copy(x_hbm.at[:, c * 128:(c + 1) * 128], xio.at[c], sems.at[c])
              for c in range(4)]
    loads += [pltpu.make_async_copy(src, dst, sems.at[5 + n]) for n, (src, dst) in enumerate(
        [(wqkv_hbm, wqkv_ref), (wo_hbm, wo_ref), (f_hbm, f_ref)])]
    for cp in loads:
        cp.start()

    spec = (s0, s1, s2, s3)

    def fence(ref, val):
        row = ref.shape[0] - 8 + zero_ref[0]
        ref[pl.ds(pl.multiple_of(row, 8), 8), 0:128] = val

    dt_row = jnp.exp(ldt_ref[...].astype(F32)).reshape(1, D)
    dtb[...] = _pack(jnp.broadcast_to(dt_row, (128, D)).T)
    dskb[...] = jnp.broadcast_to(dsk_ref[...].astype(F32).reshape(1, D) * (1.0 / L), (128, D)).T

    lane8 = jax.lax.broadcasted_iota(jnp.int32, (8, R), 1)
    rev8 = 7 - jax.lax.broadcasted_iota(jnp.int32, (8, N), 0)
    steps = (1, 2, 4, 8, 256)

    def powers(i):
        def param(ref):
            return _halves(pltpu.bitcast(ref[_ds(i, 16), :], U32))

        dts = _halves(dtb[_ds(i, 8), :])
        are, aim, bre, bim, cre, cim = [
            param(r) for r in (are_ref, aim_ref, bre_ref, bim_ref, cre_ref, cim_ref)]
        for h in range(2):
            dt = dts[h]
            li = dt * aim[h]
            mag = jnp.exp(dt * are[h])
            zp = {1: (mag * jnp.cos(li), mag * jnp.sin(li))}
            for e in (1, 2, 4, 8, 16, 32, 64, 128):
                zp[2 * e] = _csq(zp[e])
            w = _cmul((cre[h], cim[h]), (dt * bre[h], dt * bim[h]))
            for n, v in enumerate([w] + [zp[e] for e in steps]):
                pw_ref[h, 2 * n] = v[0]
                pw_ref[h, 2 * n + 1] = v[1]
            pw = [(jnp.ones((8, N), F32), jnp.zeros((8, N), F32)),
                  (jnp.take_along_axis(zp[16][0], rev8, axis=0),
                   -jnp.take_along_axis(zp[16][1], rev8, axis=0))]
            for b in range(2, 16):
                pw.append(_cmul(pw[b - 1], pw[1]) if b % 2 else _csq(pw[b // 2]))
            rhs_ref[h] = _pack(jnp.concatenate([jnp.concatenate(v, axis=1) for v in pw], axis=0))

    keys = [(s, p) for s in range(8) for p in sorted(set(_RHO[s]) - {16})] + [(8, 0)]

    def taps(i):
        outs = []
        for h in range(2):
            base, *zs = [(pw_ref[h, 2 * n], pw_ref[h, 2 * n + 1]) for n in range(len(steps) + 1)]
            zp = dict(zip(steps, zs))
            lhs = []
            for n, (s, p) in enumerate(keys):
                if p:
                    cur = _cmul(cur, zp[p - keys[n - 1][1]])
                else:
                    base = cur = _cmul(base, zp[256]) if s else base
                lhs.append(jnp.concatenate(cur, axis=1))
            outs.append(_dot(jnp.concatenate(lhs, axis=0), _unpack(rhs_ref[h]), _NT))
        both = pltpu.bitcast(pltpu.pack_elementwise(outs, packed_dtype=BF16), U32)
        piece = {}
        for n, (s, p) in enumerate(keys):
            piece[s, p] = pltpu.roll(both[8 * n:8 * n + 8], 126 - 7 if s == 8 else s, 1,
                                     stride=1, stride_axis=0)
        memo = {}
        for j in range(NS):
            key = ()
            acc = None
            for s in range(7, -1, -1):
                key = key + (_RHO[s][j],)
                if key not in memo:
                    pc = carry if _RHO[s][j] == 16 else piece[s, _RHO[s][j]]
                    same = acc is None or pc is acc
                    memo[key] = pc if same else jnp.where(((lane8 + 1) & 7) == s, pc, acc)
                acc = memo[key]
            (un, uo)[j % 2][_ds(i + D // 16, 8), _ds(j // 2, R)] = acc
            if j == 0:
                last_b = ((lane8 + 1) & 127) < 8
                carry = jnp.where(last_b, pltpu.roll(acc, 128 - 9, 1), pltpu.roll(acc, 128 - 8, 1))
                carry = jnp.where(lane8 == 6, pltpu.roll(piece[8, 0], 8, 1), carry)

    def gen_k(rb):
        for n in range(8):
            i = 8 * rb + n
            taps(i)
            powers(jnp.minimum(i + 1, D // 16 - 1))

    def dft_k(rb):
        for s in range(NS):
            u = (un, uo)[s // 8][_ds(rb + 4, 64), _ds(s % 8, R)]
            kspec[_ds(rb, 128), _ds(s, 2 * R)] = _dot(_unpack(u), _unpack(fk_ref[s]))

    def gen_step(rb, c):
        dft_k(rb - 1)
        gen_k(rb)
        return c

    with _scope("gen_k"):
        powers(0)
        gen_k(0)
        loads[0].wait()
        jax.lax.fori_loop(1, 4, gen_step, 0)

    for cp in loads[1:]:
        cp.wait()

    xu = xio.bitcast(U32)

    def load_x(b):
        for jj in range(8):
            ev, od = _halves(xu[b, pl.ds(jj, R, stride=8), :].T)
            xs[_ds(b, 128), _ds(jj, R)] = ev
            xo[_ds(b, 128), _ds(jj, R)] = od

    m_i = jax.lax.broadcasted_iota(jnp.int32, (128, 128), 0)
    c_i = jax.lax.broadcasted_iota(jnp.int32, (128, 128), 1)
    perm = jnp.where(c_i == (m_i & 7) * 16 + (m_i >> 3), 1.0, 0.0).astype(BF16)

    def prep_w(g):
        for t in range(3):
            wt[g, _ds(t, 64), :] = _pack(_dot(perm, wqkv_ref[:, _ds(t * 4 + g, 128)], _NT))
        wot[:, _ds(g, 128)] = _pack(_dot(perm, wo_ref[_ds(g, 128), :]).T)

    def dft(rb, s):
        at, n = BLOCKS[rb]
        u = (un, uo)[s // 8][at // 2:(at + n) // 2, _ds(s % 8, R)]
        y = _dot(_unpack(u), _unpack(f_ref[s]))
        spec[rb][0:n, _ds(s, 2 * R)] = y
        return y[-8:, R:]

    def idft(rb, s):
        at, n = BLOCKS[rb]
        y = _dot(spec[rb][0:n, _ds(s, 2 * R)], _unpack(f_ref[s]), _NT)
        (xs, xo)[s // 8][at:at + n, _ds(s % 8, R)] += y
        return y[-8:]

    def load_spec(ref, rows, order):
        return [(ref[rows, _ds(2 * s, R)], ref[rows, _ds(2 * s + 1, R)]) for s in order]

    def store_spec(ref, rows, order, vals):
        for s, v in zip(order, vals):
            ref[rows, _ds(2 * s, R)] = v[0]
            ref[rows, _ds(2 * s + 1, R)] = v[1]

    slabs = [_slab(j) for j in range(NS)]

    def spectrum(buf, rows, odd, bias=None):
        halves = []
        for n in range(2):
            a = []
            for m in range(4):
                j = n + 2 * m
                lo, hi = load_spec(buf, rows, [slabs[j], slabs[j + 8]])
                if j == 0 and bias is not None:
                    lo = (lo[0] + bias, lo[1])
                a.append(_twiddle(_csub(lo, hi), j, -1) if odd else _cadd(lo, hi))
            halves.append([_twiddle(v, 2 * n * k, -1) for k, v in enumerate(_fft4(a, -1))])
        for k in range(4):
            yield k, _cadd(halves[0][k], halves[1][k]), _csub(halves[0][k], halves[1][k])

    def k_fft(i):
        rows = _ds(i, 8)
        for odd in range(2):
            for k, lo, hi in spectrum(kspec, rows, odd, dskb[rows, :]):
                store_spec(khat, rows, [8 * odd + k, 8 * odd + k + 4], [lo, hi])

    def conv(rb, i, after=None):
        at, size = BLOCKS[rb]
        buf, rows, park = spec[rb], _ds(i, 8), _ds(size // 8, 8)
        for odd in (1, 0):
            cols = [[], []]
            for k, lo, hi in spectrum(buf, rows, odd):
                klo, khi = load_spec(khat, _ds(at // 8 + i, 8), [8 * odd + k, 8 * odd + k + 4])
                lo, hi = _cmul(lo, klo), _cmul(hi, khi)
                cols[0].append(_cadd(lo, hi))
                cols[1].append(_twiddle(_csub(lo, hi), 2 * k, 1))
            fence(buf, cols[1][3][0] if odd or after is None else after)
            for n in range(2):
                for m, v in enumerate(_fft4(cols[n], 1)):
                    j = n + 2 * m
                    if odd:
                        store_spec(buf, park, [j], [_twiddle(v, j, 1)])
                    else:
                        (o,) = load_spec(buf, park, [j])
                        store_spec(buf, rows, [slabs[j], slabs[j + 8]], [_cadd(v, o), _csub(v, o)])
        return cols[1][3][0]

    lane = jax.lax.broadcasted_iota(jnp.int32, (128, R), 1)

    def qkv(g, u, qs, ks, vs, i):
        y = _dot(_unpack(wt[g]), _unpack(u[0:D // 2, _ds(i, R)]))
        qs[:, _ds(i, R)] = y[0:128]
        ks[:, _ds(i + 7, R)] = y[128:256]
        vs[:, _ds(i + 7, R)] = y[256:384]
        if i:
            ks[:, _ds(i - 1, R)] = pltpu.roll(y[128:256], 1, 1)
            vs[:, _ds(i - 1, R)] = jnp.where(lane == 0, va[:, _ds(7, R)], pltpu.roll(y[256:384], 1, 1))

    never = lane8 < zero_ref[0]

    def attend(g, qs, ks, vs, rs, o, i):
        logits = []
        for w in range(W):
            lg = None
            for c in range(16):
                term = qs[_ds(c, 8), _ds(i, R)] * ks[_ds(c, 8), _ds(7 + i - w, R)]
                if c:
                    lg = lg + term
                else:
                    lg = term if w < CH else jnp.where(never, logits[w - CH], term)
            logits.append(lg)
        scale = rs[7 + i] * 0.25
        logits = [lg * scale * rs[7 + i - w] for w, lg in enumerate(logits)]
        logits = [jnp.where(lane8 == 0, NEG, lg) if w > i else lg for w, lg in enumerate(logits)]
        mx = logits[0]
        for lg in logits[1:]:
            mx = jnp.maximum(mx, lg)
        es = [jnp.exp(lg - mx) for lg in logits]
        den = es[0]
        for e in es[1:]:
            den = den + e
        inv = 1.0 / den
        probs = [e * rs[7 + i - w] * inv for w, e in enumerate(es)]
        outs = []
        for c in range(16):
            acc = None
            for w in range(W):
                term = vs[_ds(c, 8), _ds(7 + i - w, R)] * probs[w]
                if w:
                    acc = acc + term
                else:
                    acc = term if c < CH else jnp.where(never, outs[c - CH], term)
            outs.append(acc)
        o[_ds(g + 4, 64), _ds(i, R)] = _pack(jnp.concatenate(outs, axis=0))

    def chain_sum(vals, ways):
        parts = vals[:ways]
        for n, v in enumerate(vals[ways:]):
            parts[n % ways] = parts[n % ways] + v
        return jnp.sum(sum(parts[1:], parts[0]), axis=0, keepdims=True)

    def center(x, i, total, ways, after=None):
        parts = [total[_ds(n, 8)] for n in range(D // 8)]
        if after is not None:
            parts[0] = jnp.where(never, after, parts[0])
        c = x[:, _ds(i, R)] - chain_sum(parts, 2) * (1.0 / D)
        sq = c * c
        v = chain_sum([sq[_ds(n, 8)] for n in range(D // 8)], ways) * (1.0 / D)
        return c, jnp.broadcast_to(jax.lax.rsqrt(v + EPS), (8, R))

    def norm(x, u, rs, i, ways, after=None):
        c, r = center(x, i, x[:, _ds(i, R)], ways, after)
        u[0:D // 2, _ds(i, R)] = _pack(c)
        rs[7 + i] = r
        if i:
            rs[i - 1] = jnp.where(lane8 == 0, ra[7], pltpu.roll(r, 1, 1))
        return r

    def proj(x, o, u, i):
        y = x[:, _ds(i, R)] + _dot(_unpack(wot[...]), _unpack(o[D // 2:D, _ds(i, R)]))
        x[:, _ds(i, R)] = y
        cen[i % 2], r = center(x, i, y, 1)
        u[0:D // 2, _ds(i, R)] = _pack(cen[i % 2] * r[0:1])

    stores = [pltpu.make_async_copy(xio.at[c], o_hbm.at[:, c * 128:(c + 1) * 128], sems.at[c])
              for c in range(4)]

    def store_x(b, jj):
        t = pltpu.pack_elementwise(
            [xs[_ds(b, 128), _ds(jj, R)], xo[_ds(b, 128), _ds(jj, R)]], packed_dtype=BF16)
        xu[b, pl.ds(jj, R, stride=8), :] = pltpu.bitcast(t, U32).T

    def phase(name):
        def run(fn):
            with _scope(name):
                pl.when(zero_ref[0] == 0)(fn)
        return run

    @phase("prep")
    def _():
        dft_k(3)
        for b in range(4):
            load_x(b)
            prep_w(b)
            for n in range(6):
                k_fft(6 * b + n)

    even, odd = (un, (qa, ka, va), ra), (uo, (qb, kb, vb), rb_)

    def overlap(g_next, nxt, g, cur, k0):
        for i in range(8):
            qkv(g_next, nxt[0], *nxt[1], i)
            if k0 is not None:
                k_fft(k0 + i)
            attend(g, *cur[1], cur[2], nxt[0], i)

    for layer in range(2):
        @phase("a_pro")
        def _():
            if layer:
                for s in range(8):
                    idft(3, s)
            r = norm(xs, un, ra, 0, 4)
            for i in range(8):
                if layer:
                    idft(3, i + 8)
                qkv(0, un, qa, ka, va, i)
                if i < 7:
                    r = norm(xs, un, ra, i + 1, 2 - layer, r)
                r = norm(xo, uo, rb_, i, 2 - layer, r)

        def group(g, c):
            overlap(g, odd, g, even, None if layer else 8 * g + 24)

            @pl.when(g < 3)
            def _():
                overlap(g + 1, even, g, odd, None)

            return c

        with _scope("a_grp"):
            jax.lax.fori_loop(0, 4, group, 0)

        @phase("a_proj")
        def _():
            for i in range(8):
                proj(xs, uo, un, i)
                attend(3, qb, kb, vb, rb_, un, i)
            for i in range(8):
                proj(xo, un, uo, i)
                if not layer:
                    k_fft(56 + i)
            for s in range(NS):
                dft(0, s)

        @phase("conv")
        def _():
            for rb, (_, size) in enumerate(BLOCKS):
                groups = size // 8
                done = []
                for i in range(groups):
                    for s in range(i * NS // groups, (i + 1) * NS // groups):
                        if rb + 1 < len(BLOCKS):
                            last = dft(rb + 1, s)
                        if rb:
                            last = idft(rb - 1, s)
                        if layer and rb >= 3:
                            store_x(s // 8, s % 8)
                    done.append(last)
                    mark = conv(rb, i, done[i - 3] if i >= 3 else None)
                    for other in (rb - 1, rb + 1):
                        if 0 <= other < len(BLOCKS) and other > rb:
                            fence(spec[other], mark)

    with _scope("store_x"):
        stores[0].start()
        stores[1].start()
        for jj in range(8):
            idft(3, jj)
            idft(3, jj + 8)
            store_x(2, jj)
        stores[2].start()
        for jj in range(8):
            store_x(3, jj)
        stores[3].start()
    for cp in stores:
        cp.wait()


@jax.jit
def pallas_interleave_layers__sliding_local_dilated__ssm_conv_s4__prompt_kernel(
    A_x: jax.Array,
    A_wqkv: jax.Array,
    A_wo: jax.Array,
    B_u: jax.Array,
    B_A_re: jax.Array,
    B_A_im: jax.Array,
    B_B_re: jax.Array,
    B_B_im: jax.Array,
    B_C_re: jax.Array,
    B_C_im: jax.Array,
    B_log_dt: jax.Array,
    B_Dskip: jax.Array,
):
    del B_u
    f = _dft_matrix()
    lane = (np.arange(R) - 7) % R
    order = 16 * (lane % 8) + lane // 8
    fk = (f[:, order].astype(np.float32) / L).astype(ml_dtypes.bfloat16)
    scratch = [
        pltpu.VMEM((D, L // 2), F32),
        pltpu.VMEM((D, L // 2), F32),
        pltpu.VMEM((D + 8, L // 2), U32),
        pltpu.VMEM((D + 8, L // 2), U32),
        pltpu.VMEM((4, 192, D), U32),
        pltpu.VMEM((D // 2, D), U32),
        pltpu.VMEM((D // 2, 128), U32),
        pltpu.VMEM((D, 128), F32),
        pltpu.VMEM((2, 12, 8, N), F32),
        pltpu.VMEM((2, 64, 2 * N), U32),
        *[pltpu.VMEM((n + 16, 2 * L), F32) for _, n in BLOCKS],
        pltpu.VMEM((D, 2 * L), F32),
        pltpu.VMEM((D, 2 * L), F32),
        pltpu.VMEM((128, 8 * R), F32),
        pltpu.VMEM((128, 15 * R), F32),
        pltpu.VMEM((128, 15 * R), F32),
        pltpu.VMEM((128, 8 * R), F32),
        pltpu.VMEM((128, 15 * R), F32),
        pltpu.VMEM((128, 15 * R), F32),
        pltpu.VMEM((15, 8, R), F32),
        pltpu.VMEM((15, 8, R), F32),
        pltpu.VMEM((2, D, R), F32),
        pltpu.VMEM((4, L, 128), BF16),
        pltpu.VMEM((D, 3 * D), BF16),
        pltpu.VMEM((D, D), BF16),
        pltpu.VMEM((NS, R // 2, 2 * R), U32),
        pltpu.VMEM((NS, R // 2, 2 * R), U32),
        pltpu.SemaphoreType.DMA((8,)),
    ]
    hbm = pl.BlockSpec(memory_space=pl.ANY)
    vmem = pl.BlockSpec(memory_space=pltpu.VMEM)
    out = pl.pallas_call(
        _kernel,
        out_shape=jax.ShapeDtypeStruct((L, D), BF16),
        in_specs=[pl.BlockSpec(memory_space=pltpu.SMEM)] + [hbm] * 3 + [vmem] * 8 + [hbm] * 2,
        out_specs=hbm,
        scratch_shapes=scratch,
        compiler_params=pltpu.CompilerParams(vmem_limit_bytes=100 * 1024 * 1024),
    )(np.zeros((1,), np.int32), A_x.reshape(L, D), A_wqkv, A_wo, B_A_re, B_A_im, B_B_re, B_B_im, B_C_re, B_C_im,
      B_log_dt, B_Dskip, _pack_rows(f), _pack_rows(fk))
    return out.reshape(1, L, D)
```

```python
import contextlib

import jax
import jax.numpy as jnp
import jax.experimental.pallas as pl
import jax.experimental.pallas.tpu as pltpu
import ml_dtypes
import numpy as np

L = 2048
D = 512
N = 128
NS = 16
R = 128
W = 8
EPS = 1e-5
CH = 2
BLOCKS = ((0, 128), (128, 128), (256, 128), (384, 128))
F32 = jnp.float32
BF16 = jnp.bfloat16
U32 = jnp.uint32
NEG = float(ml_dtypes.bfloat16(-1e9))

_NT = (((1,), (1,)), ((), ()))


def _slab(j):
    return (j % 2) * 8 + j // 2


def _dft_matrix():
    r = np.arange(R)
    k = np.arange(R) + 0.5
    f = np.zeros((NS, R, 2 * R), np.float64)
    for j in range(NS):
        th = 2.0 * np.pi * np.outer(NS * r + j, k) / (2 * L)
        f[_slab(j), :, :R] = np.cos(th)
        f[_slab(j), :, R:] = -np.sin(th)
    return f.astype(np.float32).astype(ml_dtypes.bfloat16)


def _pack_rows(a):
    u = np.ascontiguousarray(a).view(np.uint16).astype(np.uint32)
    return u[:, 0::2] | (u[:, 1::2] << np.uint32(16))


def _lag_tables():
    rho = []
    for s in range(8):
        lag = (256 * s + np.arange(NS)).astype(np.float32)
        rho.append([int(v) - 256 * s for v in lag.astype(ml_dtypes.bfloat16).astype(np.float32)])
    return rho


_RHO = _lag_tables()


def _cmul(a, b):
    return (a[0] * b[0] - a[1] * b[1], a[0] * b[1] + a[1] * b[0])


def _csq(a):
    t = a[0] * a[1]
    return ((a[0] - a[1]) * (a[0] + a[1]), t + t)


def _cadd(a, b):
    return (a[0] + b[0], a[1] + b[1])


def _csub(a, b):
    return (a[0] - b[0], a[1] - b[1])


def _fft4(x, sign):
    s0, d0 = _cadd(x[0], x[2]), _csub(x[0], x[2])
    s1, d1 = _cadd(x[1], x[3]), _csub(x[1], x[3])
    a = (d0[0] + d1[1], d0[1] - d1[0])
    b = (d0[0] - d1[1], d0[1] + d1[0])
    if sign > 0:
        a, b = b, a
    return [_cadd(s0, s1), a, _csub(s0, s1), b]


def _twiddle(z, m, sign):
    m = (m * sign) % 16
    re, im = z
    h = float(np.sqrt(0.5))
    if m == 0:
        return z
    if m == 4:
        return (-im, re)
    if m == 12:
        return (im, -re)
    if m == 2:
        return ((re - im) * h, (re + im) * h)
    if m == 14:
        return ((re + im) * h, (im - re) * h)
    if m == 6:
        return ((re + im) * -h, (re - im) * h)
    if m == 10:
        return ((im - re) * h, (re + im) * -h)
    c, s = float(np.cos(np.pi * m / 8)), float(np.sin(np.pi * m / 8))
    return (re * c - im * s, re * s + im * c)


def _scope(name):
    return contextlib.nullcontext()


def _ds(i, n):
    if isinstance(i, int):
        return slice(i * n, (i + 1) * n)
    return pl.ds(pl.multiple_of(i * n, n), n)


def _pack(x):
    return pltpu.bitcast(x.astype(BF16), U32)


def _unpack(x):
    return pltpu.bitcast(x, BF16)


def _dot(a, b, dims=(((1,), (0,)), ((), ()))):
    return jax.lax.dot_general(a, b, dims, preferred_element_type=F32)


def _halves(u):
    return pltpu.bitcast(u << 16, F32), pltpu.bitcast(u & jnp.uint32(0xFFFF0000), F32)


def _kernel(zero_ref, x_hbm, wqkv_hbm, wo_hbm, are, aim, bre, bim, cre, cim,
            ldt_ref, dsk_ref, f_hbm, fk_hbm, o_hbm,
            xs, xo, un, uo, wt, wot, dtb, dskb, pw_ref, rhs_ref, s0, s1, s2, s3, kspec, khat, qa, ka, va, qb, kb, vb,
            ra, rb_, cen,
            io0, io1, io2, io3, wqkv_ref, wo_ref, f_ref, fk_ref, ssm, sems):
    def fetch_ssm(rows, sem):
        return [pltpu.make_async_copy(p.at[rows], ssm.at[n, rows], sem)
                for n, p in enumerate((are, aim, bre, bim, cre, cim))]

    first = fetch_ssm(pl.ds(0, 144), sems.at[8])
    for cp in first:
        cp.start()
    second = fetch_ssm(pl.ds(144, D - 144), sems.at[9])
    second += [pltpu.make_async_copy(fk_hbm, fk_ref, sems.at[4])]
    xio = (io0, io1, io2, io3)
    loads = []
    loads += [pltpu.make_async_copy(x_hbm.at[:, c * 128:(c + 1) * 128], xio[c].at[0:L], sems.at[c])
              for c in range(4)]
    loads += [pltpu.make_async_copy(src, dst, sems.at[5 + n]) for n, (src, dst) in enumerate(
        [(wqkv_hbm, wqkv_ref), (wo_hbm, wo_ref), (f_hbm, f_ref)])]

    spec = (s0, s1, s2, s3)

    def fence(ref, val):
        row = ref.shape[0] - 8 + zero_ref[0]
        ref[pl.ds(pl.multiple_of(row, 8), 8), 0:128] = val

    dt_row = jnp.exp(ldt_ref[...].astype(F32)).reshape(1, D)
    dtb[...] = _pack(jnp.broadcast_to(dt_row, (128, D)).T)
    dskb[...] = jnp.broadcast_to(dsk_ref[...].astype(F32).reshape(1, D) * (1.0 / L), (128, D)).T

    lane8 = jax.lax.broadcasted_iota(jnp.int32, (8, R), 1)
    rev8 = 7 - jax.lax.broadcasted_iota(jnp.int32, (8, N), 0)
    steps = (1, 2, 4, 8, 256)

    def powers(i):
        dts = _halves(dtb[_ds(i, 8), :])
        are, aim, bre, bim, cre, cim = [
            _halves(pltpu.bitcast(ssm[n, _ds(i, 16), :], U32)) for n in range(6)]
        for h in range(2):
            dt = dts[h]
            li = dt * aim[h]
            mag = jnp.exp(dt * are[h])
            zp = {1: (mag * jnp.cos(li), mag * jnp.sin(li))}
            for e in (1, 2, 4, 8, 16, 32, 64, 128):
                zp[2 * e] = _csq(zp[e])
            w = _cmul((cre[h], cim[h]), (dt * bre[h], dt * bim[h]))
            for n, v in enumerate([w] + [zp[e] for e in steps]):
                pw_ref[h, 2 * n] = v[0]
                pw_ref[h, 2 * n + 1] = v[1]
            pw = [(jnp.ones((8, N), F32), jnp.zeros((8, N), F32)),
                  (jnp.take_along_axis(zp[16][0], rev8, axis=0),
                   -jnp.take_along_axis(zp[16][1], rev8, axis=0))]
            for b in range(2, 16):
                pw.append(_cmul(pw[b - 1], pw[1]) if b % 2 else _csq(pw[b // 2]))
            rhs_ref[h] = _pack(jnp.concatenate([jnp.concatenate(v, axis=1) for v in pw], axis=0))

    keys = [(s, p) for s in range(8) for p in sorted(set(_RHO[s]) - {16})] + [(8, 0)]

    def taps(i):
        outs = []
        for h in range(2):
            base, *zs = [(pw_ref[h, 2 * n], pw_ref[h, 2 * n + 1]) for n in range(len(steps) + 1)]
            zp = dict(zip(steps, zs))
            lhs = []
            for n, (s, p) in enumerate(keys):
                if p:
                    cur = _cmul(cur, zp[p - keys[n - 1][1]])
                else:
                    base = cur = _cmul(base, zp[256]) if s else base
                lhs.append(jnp.concatenate(cur, axis=1))
            outs.append(_dot(jnp.concatenate(lhs, axis=0), _unpack(rhs_ref[h]), _NT))
        both = pltpu.bitcast(pltpu.pack_elementwise(outs, packed_dtype=BF16), U32)
        piece = {}
        for n, (s, p) in enumerate(keys):
            piece[s, p] = pltpu.roll(both[8 * n:8 * n + 8], 126 - 7 if s == 8 else s, 1,
                                     stride=1, stride_axis=0)
        memo = {}
        for j in range(NS):
            key = ()
            acc = None
            for s in range(7, -1, -1):
                key = key + (_RHO[s][j],)
                if key not in memo:
                    pc = carry if _RHO[s][j] == 16 else piece[s, _RHO[s][j]]
                    same = acc is None or pc is acc
                    memo[key] = pc if same else jnp.where(((lane8 + 1) & 7) == s, pc, acc)
                acc = memo[key]
            (un, uo)[j % 2][_ds(i + D // 16, 8), _ds(j // 2, R)] = acc
            if j == 0:
                last_b = ((lane8 + 1) & 127) < 8
                carry = jnp.where(last_b, pltpu.roll(acc, 128 - 9, 1), pltpu.roll(acc, 128 - 8, 1))
                carry = jnp.where(lane8 == 6, pltpu.roll(piece[8, 0], 8, 1), carry)

    def gen_k(rb):
        for n in range(8):
            i = 8 * rb + n
            taps(i)
            powers(jnp.minimum(i + 1, D // 16 - 1))

    def dft_k(rb):
        for s in range(NS):
            u = (un, uo)[s // 8][_ds(rb + 4, 64), _ds(s % 8, R)]
            kspec[_ds(rb, 128), _ds(s, 2 * R)] = _dot(_unpack(u), _unpack(fk_ref[s]))

    def gen_step(rb, c):
        dft_k(rb - 1)
        gen_k(rb)
        return c

    with _scope("head"):
        for cp in first:
            cp.wait()
        for cp in second + loads:
            cp.start()

    with _scope("gen_k"):
        powers(0)
        gen_k(0)
        for cp in second:
            cp.wait()
        jax.lax.fori_loop(1, 4, gen_step, 0)

    for cp in loads:
        cp.wait()

    xu = [r.bitcast(U32) for r in xio]

    def load_x(b):
        for jj in range(8):
            ev, od = _halves(xu[b][pl.ds(jj, R, stride=8), :].T)
            xs[_ds(b, 128), _ds(jj, R)] = ev
            xo[_ds(b, 128), _ds(jj, R)] = od

    m_i = jax.lax.broadcasted_iota(jnp.int32, (128, 128), 0)
    c_i = jax.lax.broadcasted_iota(jnp.int32, (128, 128), 1)
    perm = jnp.where(c_i == (m_i & 7) * 16 + (m_i >> 3), 1.0, 0.0).astype(BF16)

    def prep_w(g):
        for t in range(3):
            wt[g, _ds(t, 64), :] = _pack(_dot(perm, wqkv_ref[:, _ds(t * 4 + g, 128)], _NT))
        wot[:, _ds(g, 128)] = _pack(_dot(perm, wo_ref[_ds(g, 128), :]).T)

    def dft(rb, s):
        at, n = BLOCKS[rb]
        u = (un, uo)[s // 8][at // 2:(at + n) // 2, _ds(s % 8, R)]
        y = _dot(_unpack(u), _unpack(f_ref[s]))
        spec[rb][0:n, _ds(s, 2 * R)] = y
        return y[-8:, R:]

    def idft(rb, s):
        at, n = BLOCKS[rb]
        y = _dot(spec[rb][0:n, _ds(s, 2 * R)], _unpack(f_ref[s]), _NT)
        (xs, xo)[s // 8][at:at + n, _ds(s % 8, R)] += y
        return y[-8:]

    def load_spec(ref, rows, order):
        return [(ref[rows, _ds(2 * s, R)], ref[rows, _ds(2 * s + 1, R)]) for s in order]

    def store_spec(ref, rows, order, vals):
        for s, v in zip(order, vals):
            ref[rows, _ds(2 * s, R)] = v[0]
            ref[rows, _ds(2 * s + 1, R)] = v[1]

    slabs = [_slab(j) for j in range(NS)]

    def spectrum(buf, rows, odd, bias=None):
        halves = []
        for n in range(2):
            a = []
            for m in range(4):
                j = n + 2 * m
                lo, hi = load_spec(buf, rows, [slabs[j], slabs[j + 8]])
                if j == 0 and bias is not None:
                    lo = (lo[0] + bias, lo[1])
                a.append(_twiddle(_csub(lo, hi), j, -1) if odd else _cadd(lo, hi))
            halves.append([_twiddle(v, 2 * n * k, -1) for k, v in enumerate(_fft4(a, -1))])
        for k in range(4):
            yield k, _cadd(halves[0][k], halves[1][k]), _csub(halves[0][k], halves[1][k])

    def k_fft(i):
        rows = _ds(i, 8)
        for odd in range(2):
            for k, lo, hi in spectrum(kspec, rows, odd, dskb[rows, :]):
                store_spec(khat, rows, [8 * odd + k, 8 * odd + k + 4], [lo, hi])

    def conv(rb, i, after=None):
        at, size = BLOCKS[rb]
        buf, rows, park = spec[rb], _ds(i, 8), _ds(size // 8, 8)
        for odd in (1, 0):
            cols = [[], []]
            for k, lo, hi in spectrum(buf, rows, odd):
                klo, khi = load_spec(khat, _ds(at // 8 + i, 8), [8 * odd + k, 8 * odd + k + 4])
                lo, hi = _cmul(lo, klo), _cmul(hi, khi)
                cols[0].append(_cadd(lo, hi))
                cols[1].append(_twiddle(_csub(lo, hi), 2 * k, 1))
            fence(buf, cols[1][3][0] if odd or after is None else after)
            for n in range(2):
                for m, v in enumerate(_fft4(cols[n], 1)):
                    j = n + 2 * m
                    if odd:
                        store_spec(buf, park, [j], [_twiddle(v, j, 1)])
                    else:
                        (o,) = load_spec(buf, park, [j])
                        store_spec(buf, rows, [slabs[j], slabs[j + 8]], [_cadd(v, o), _csub(v, o)])
        return cols[1][3][0]

    lane = jax.lax.broadcasted_iota(jnp.int32, (128, R), 1)

    def qkv(g, u, qs, ks, vs, i):
        y = _dot(_unpack(wt[g]), _unpack(u[0:D // 2, _ds(i, R)]))
        qs[:, _ds(i, R)] = y[0:128]
        ks[:, _ds(i + 7, R)] = y[128:256]
        vs[:, _ds(i + 7, R)] = y[256:384]
        if i:
            ks[:, _ds(i - 1, R)] = pltpu.roll(y[128:256], 1, 1)
            vs[:, _ds(i - 1, R)] = jnp.where(lane == 0, va[:, _ds(7, R)], pltpu.roll(y[256:384], 1, 1))

    never = lane8 < zero_ref[0]

    def attend(g, qs, ks, vs, rs, o, i):
        logits = []
        for w in range(W):
            lg = None
            for c in range(16):
                term = qs[_ds(c, 8), _ds(i, R)] * ks[_ds(c, 8), _ds(7 + i - w, R)]
                if c:
                    lg = lg + term
                else:
                    lg = term if w < CH else jnp.where(never, logits[w - CH], term)
            logits.append(lg)
        scale = rs[7 + i] * 0.25
        logits = [lg * scale * rs[7 + i - w] for w, lg in enumerate(logits)]
        logits = [jnp.where(lane8 == 0, NEG, lg) if w > i else lg for w, lg in enumerate(logits)]
        mx = logits[0]
        for lg in logits[1:]:
            mx = jnp.maximum(mx, lg)
        es = [jnp.exp(lg - mx) for lg in logits]
        den = es[0]
        for e in es[1:]:
            den = den + e
        inv = 1.0 / den
        probs = [e * rs[7 + i - w] * inv for w, e in enumerate(es)]
        outs = []
        for c in range(16):
            acc = None
            for w in range(W):
                term = vs[_ds(c, 8), _ds(7 + i - w, R)] * probs[w]
                if w:
                    acc = acc + term
                else:
                    acc = term if c < CH else jnp.where(never, outs[c - CH], term)
            outs.append(acc)
        o[_ds(g + 4, 64), _ds(i, R)] = _pack(jnp.concatenate(outs, axis=0))

    def chain_sum(vals, ways):
        parts = vals[:ways]
        for n, v in enumerate(vals[ways:]):
            parts[n % ways] = parts[n % ways] + v
        return jnp.sum(sum(parts[1:], parts[0]), axis=0, keepdims=True)

    def center(x, i, total, ways, after=None):
        parts = [total[_ds(n, 8)] for n in range(D // 8)]
        if after is not None:
            parts[0] = jnp.where(never, after, parts[0])
        c = x[:, _ds(i, R)] - chain_sum(parts, 2) * (1.0 / D)
        sq = c * c
        v = chain_sum([sq[_ds(n, 8)] for n in range(D // 8)], ways) * (1.0 / D)
        return c, jnp.broadcast_to(jax.lax.rsqrt(v + EPS), (8, R))

    def norm(x, u, rs, i, ways, after=None):
        c, r = center(x, i, x[:, _ds(i, R)], ways, after)
        u[0:D // 2, _ds(i, R)] = _pack(c)
        rs[7 + i] = r
        if i:
            rs[i - 1] = jnp.where(lane8 == 0, ra[7], pltpu.roll(r, 1, 1))
        return r

    def proj(x, o, u, i):
        y = x[:, _ds(i, R)] + _dot(_unpack(wot[...]), _unpack(o[D // 2:D, _ds(i, R)]))
        x[:, _ds(i, R)] = y
        cen[i % 2], r = center(x, i, y, 1)
        u[0:D // 2, _ds(i, R)] = _pack(cen[i % 2] * r[0:1])

    stores = [pltpu.make_async_copy(xio[c].at[0:L], o_hbm.at[:, c * 128:(c + 1) * 128], sems.at[c])
              for c in range(4)]

    def store_x(b, jj):
        t = pltpu.pack_elementwise(
            [xs[_ds(b, 128), _ds(jj, R)], xo[_ds(b, 128), _ds(jj, R)]], packed_dtype=BF16)
        xu[b][pl.ds(jj, R, stride=8), :] = pltpu.bitcast(t, U32).T

    def fence_io(b, val):
        xio[b][pl.ds(pl.multiple_of(L + zero_ref[0], 16), 16), :] = pltpu.bitcast(val, BF16)

    def start_store(b, val):
        stores[b].start()
        fence_io(b, val)
        return pltpu.bitcast(xio[b][L:L + 16, :], F32)

    def phase(name):
        def run(fn):
            with _scope(name):
                pl.when(zero_ref[0] == 0)(fn)
        return run

    @phase("prep")
    def _():
        dft_k(3)
        for b in range(4):
            load_x(b)
            prep_w(b)
            for n in range(6):
                k_fft(6 * b + n)

    even, odd = (un, (qa, ka, va), ra), (uo, (qb, kb, vb), rb_)

    def overlap(g_next, nxt, g, cur, k0):
        for i in range(8):
            qkv(g_next, nxt[0], *nxt[1], i)
            if k0 is not None:
                k_fft(k0 + i)
            attend(g, *cur[1], cur[2], nxt[0], i)

    for layer in range(2):
        @phase("a_pro")
        def _():
            if layer:
                for s in range(8):
                    idft(3, s)
            r = norm(xs, un, ra, 0, 4)
            for i in range(8):
                if layer:
                    idft(3, i + 8)
                qkv(0, un, qa, ka, va, i)
                if i < 7:
                    r = norm(xs, un, ra, i + 1, 2 - layer, r)
                r = norm(xo, uo, rb_, i, 2 - layer, r)

        def group(g, c):
            overlap(g, odd, g, even, None if layer else 8 * g + 24)

            @pl.when(g < 3)
            def _():
                overlap(g + 1, even, g, odd, None)

            return c

        with _scope("a_grp"):
            jax.lax.fori_loop(0, 4, group, 0)

        @phase("a_proj")
        def _():
            for i in range(8):
                proj(xs, uo, un, i)
                attend(3, qb, kb, vb, rb_, un, i)
            for i in range(8):
                proj(xo, un, uo, i)
                if not layer:
                    k_fft(56 + i)
            for s in range(NS):
                dft(0, s)

        @phase("conv")
        def _():
            for rb, (_, size) in enumerate(BLOCKS):
                groups = size // 8
                done = []
                for i in range(groups):
                    for s in range(i * NS // groups, (i + 1) * NS // groups):
                        if rb + 1 < len(BLOCKS):
                            last = dft(rb + 1, s)
                        if rb:
                            last = idft(rb - 1, s)
                        if layer and rb >= 2 and s < 8:
                            store_x(rb - 2, s)
                            if s == 7:
                                last = start_store(rb - 2, last)
                    done.append(last)
                    mark = conv(rb, i, done[i - 3] if i >= 3 else None)
                    for other in (rb - 1, rb + 1):
                        if 0 <= other < len(BLOCKS) and other > rb:
                            fence(spec[other], mark)

    with _scope("store_x"):
        for jj in range(8):
            store_x(2, jj)
        fence_io(3, start_store(2, jnp.zeros((8, R), F32)))
        for jj in range(8):
            idft(3, jj)
            idft(3, jj + 8)
            store_x(3, jj)
        stores[3].start()
    with _scope("tail"):
        for cp in stores:
            cp.wait()


@jax.jit
def pallas_interleave_layers__sliding_local_dilated__ssm_conv_s4__prompt_kernel(
    A_x: jax.Array,
    A_wqkv: jax.Array,
    A_wo: jax.Array,
    B_u: jax.Array,
    B_A_re: jax.Array,
    B_A_im: jax.Array,
    B_B_re: jax.Array,
    B_B_im: jax.Array,
    B_C_re: jax.Array,
    B_C_im: jax.Array,
    B_log_dt: jax.Array,
    B_Dskip: jax.Array,
):
    del B_u
    f = _dft_matrix()
    lane = (np.arange(R) - 7) % R
    order = 16 * (lane % 8) + lane // 8
    fk = (f[:, order].astype(np.float32) / L).astype(ml_dtypes.bfloat16)
    scratch = [
        pltpu.VMEM((D, L // 2), F32),
        pltpu.VMEM((D, L // 2), F32),
        pltpu.VMEM((D + 8, L // 2), U32),
        pltpu.VMEM((D + 8, L // 2), U32),
        pltpu.VMEM((4, 192, D), U32),
        pltpu.VMEM((D // 2, D), U32),
        pltpu.VMEM((D // 2, 128), U32),
        pltpu.VMEM((D, 128), F32),
        pltpu.VMEM((2, 12, 8, N), F32),
        pltpu.VMEM((2, 64, 2 * N), U32),
        *[pltpu.VMEM((n + 16, 2 * L), F32) for _, n in BLOCKS],
        pltpu.VMEM((D, 2 * L), F32),
        pltpu.VMEM((D, 2 * L), F32),
        pltpu.VMEM((128, 8 * R), F32),
        pltpu.VMEM((128, 15 * R), F32),
        pltpu.VMEM((128, 15 * R), F32),
        pltpu.VMEM((128, 8 * R), F32),
        pltpu.VMEM((128, 15 * R), F32),
        pltpu.VMEM((128, 15 * R), F32),
        pltpu.VMEM((15, 8, R), F32),
        pltpu.VMEM((15, 8, R), F32),
        pltpu.VMEM((2, D, R), F32),
        *[pltpu.VMEM((L + 16, 128), BF16)] * 4,
        pltpu.VMEM((D, 3 * D), BF16),
        pltpu.VMEM((D, D), BF16),
        pltpu.VMEM((NS, R // 2, 2 * R), U32),
        pltpu.VMEM((NS, R // 2, 2 * R), U32),
        pltpu.VMEM((6, D, N), BF16),
        pltpu.SemaphoreType.DMA((10,)),
    ]
    hbm = pl.BlockSpec(memory_space=pl.ANY)
    vmem = pl.BlockSpec(memory_space=pltpu.VMEM)
    out = pl.pallas_call(
        _kernel,
        out_shape=jax.ShapeDtypeStruct((L, D), BF16),
        in_specs=[pl.BlockSpec(memory_space=pltpu.SMEM)] + [hbm] * 9 + [vmem] * 2 + [hbm] * 2,
        out_specs=hbm,
        scratch_shapes=scratch,
        compiler_params=pltpu.CompilerParams(vmem_limit_bytes=100 * 1024 * 1024),
    )(np.zeros((1,), np.int32), A_x.reshape(L, D), A_wqkv, A_wo, B_A_re, B_A_im, B_B_re, B_B_im, B_C_re, B_C_im,
      B_log_dt, B_Dskip, _pack_rows(f), _pack_rows(fk))
    return out.reshape(1, L, D)
```

```python
import contextlib

import jax
import jax.numpy as jnp
import jax.experimental.pallas as pl
import jax.experimental.pallas.tpu as pltpu
import ml_dtypes
import numpy as np

L = 2048
D = 512
N = 128
NS = 16
R = 128
W = 8
EPS = 1e-5
LAG = 4
SKEW = 0
BLOCKS = ((0, 128), (128, 128), (256, 128), (384, 128))
F32 = jnp.float32
BF16 = jnp.bfloat16
U32 = jnp.uint32
NEG = float(ml_dtypes.bfloat16(-1e9))

_NT = (((1,), (1,)), ((), ()))


def _slab(j):
    return (j % 2) * 8 + j // 2


def _dft_matrix():
    r = np.arange(R)
    k = np.arange(R) + 0.5
    f = np.zeros((NS, R, 2 * R), np.float64)
    for j in range(NS):
        th = 2.0 * np.pi * np.outer(NS * r + j, k) / (2 * L)
        f[_slab(j), :, :R] = np.cos(th)
        f[_slab(j), :, R:] = -np.sin(th)
    return f.astype(np.float32).astype(ml_dtypes.bfloat16)


def _pack_rows(a):
    u = np.ascontiguousarray(a).view(np.uint16).astype(np.uint32)
    return u[:, 0::2] | (u[:, 1::2] << np.uint32(16))


def _lag_tables():
    rho = []
    for s in range(8):
        lag = (256 * s + np.arange(NS)).astype(np.float32)
        rho.append([int(v) - 256 * s for v in lag.astype(ml_dtypes.bfloat16).astype(np.float32)])
    return rho


_RHO = _lag_tables()


def _cmul(a, b):
    return (a[0] * b[0] - a[1] * b[1], a[0] * b[1] + a[1] * b[0])


def _csq(a):
    t = a[0] * a[1]
    return ((a[0] - a[1]) * (a[0] + a[1]), t + t)


def _cadd(a, b):
    return (a[0] + b[0], a[1] + b[1])


def _csub(a, b):
    return (a[0] - b[0], a[1] - b[1])


def _fft4(x, sign):
    s0, d0 = _cadd(x[0], x[2]), _csub(x[0], x[2])
    s1, d1 = _cadd(x[1], x[3]), _csub(x[1], x[3])
    a = (d0[0] + d1[1], d0[1] - d1[0])
    b = (d0[0] - d1[1], d0[1] + d1[0])
    if sign > 0:
        a, b = b, a
    return [_cadd(s0, s1), a, _csub(s0, s1), b]


def _twiddle(z, m, sign):
    m = (m * sign) % 16
    re, im = z
    h = float(np.sqrt(0.5))
    if m == 0:
        return z
    if m == 4:
        return (-im, re)
    if m == 12:
        return (im, -re)
    if m == 2:
        return ((re - im) * h, (re + im) * h)
    if m == 14:
        return ((re + im) * h, (im - re) * h)
    if m == 6:
        return ((re + im) * -h, (re - im) * h)
    if m == 10:
        return ((im - re) * h, (re + im) * -h)
    c, s = float(np.cos(np.pi * m / 8)), float(np.sin(np.pi * m / 8))
    return (re * c - im * s, re * s + im * c)


def _scope(name):
    return contextlib.nullcontext()


def _ds(i, n):
    if isinstance(i, int):
        return slice(i * n, (i + 1) * n)
    return pl.ds(pl.multiple_of(i * n, n), n)


def _pack(x):
    return pltpu.bitcast(x.astype(BF16), U32)


def _unpack(x):
    return pltpu.bitcast(x, BF16)


def _dot(a, b, dims=(((1,), (0,)), ((), ()))):
    return jax.lax.dot_general(a, b, dims, preferred_element_type=F32)


def _halves(u):
    return pltpu.bitcast(u << 16, F32), pltpu.bitcast(u & jnp.uint32(0xFFFF0000), F32)


def _kernel(zero_ref, x_hbm, wqkv_hbm, wo_hbm, are, aim, bre, bim, cre, cim,
            ldt_ref, dsk_ref, f_hbm, fk_hbm, o_hbm,
            xs, xo, un, uo, wt, wot, dtb, dskb, pw_ref, rhs_ref, s0, s1, s2, s3, kspec, khat, qa, ka, va, qb, kb, vb,
            ra, rb_, cen,
            io0, io1, io2, io3, wqkv_ref, wo_ref, f_ref, fk_ref, ssm, sems):
    def fetch_ssm(rows, sem):
        return [pltpu.make_async_copy(p.at[rows], ssm.at[n, rows], sem)
                for n, p in enumerate((are, aim, bre, bim, cre, cim))]

    first = fetch_ssm(pl.ds(0, 144), sems.at[8])
    for cp in first:
        cp.start()
    second = fetch_ssm(pl.ds(144, D - 144), sems.at[9])
    second += [pltpu.make_async_copy(fk_hbm, fk_ref, sems.at[4])]
    xio = (io0, io1, io2, io3)
    loads = []
    loads += [pltpu.make_async_copy(x_hbm.at[:, c * 128:(c + 1) * 128], xio[c].at[0:L], sems.at[c])
              for c in range(4)]
    loads += [pltpu.make_async_copy(src, dst, sems.at[5 + n]) for n, (src, dst) in enumerate(
        [(wqkv_hbm, wqkv_ref), (wo_hbm, wo_ref), (f_hbm, f_ref)])]

    spec = (s0, s1, s2, s3)

    def fence(ref, val):
        row = ref.shape[0] - 8 + zero_ref[0]
        ref[pl.ds(pl.multiple_of(row, 8), 8), 0:128] = val

    dt_row = jnp.exp(ldt_ref[...].astype(F32)).reshape(1, D)
    dtb[...] = _pack(jnp.broadcast_to(dt_row, (128, D)).T)
    dskb[...] = jnp.broadcast_to(dsk_ref[...].astype(F32).reshape(1, D) * (1.0 / L), (128, D)).T

    lane8 = jax.lax.broadcasted_iota(jnp.int32, (8, R), 1)
    rev8 = 7 - jax.lax.broadcasted_iota(jnp.int32, (8, N), 0)
    steps = (1, 2, 4, 8, 256)

    def powers(i):
        dts = _halves(dtb[_ds(i, 8), :])
        are, aim, bre, bim, cre, cim = [
            _halves(pltpu.bitcast(ssm[n, _ds(i, 16), :], U32)) for n in range(6)]
        for h in range(2):
            dt = dts[h]
            li = dt * aim[h]
            mag = jnp.exp(dt * are[h])
            zp = {1: (mag * jnp.cos(li), mag * jnp.sin(li))}
            for e in (1, 2, 4, 8, 16, 32, 64, 128):
                zp[2 * e] = _csq(zp[e])
            w = _cmul((cre[h], cim[h]), (dt * bre[h], dt * bim[h]))
            for n, v in enumerate([w] + [zp[e] for e in steps]):
                pw_ref[h, 2 * n] = v[0]
                pw_ref[h, 2 * n + 1] = v[1]
            pw = [(jnp.ones((8, N), F32), jnp.zeros((8, N), F32)),
                  (jnp.take_along_axis(zp[16][0], rev8, axis=0),
                   -jnp.take_along_axis(zp[16][1], rev8, axis=0))]
            for b in range(2, 16):
                pw.append(_cmul(pw[b - 1], pw[1]) if b % 2 else _csq(pw[b // 2]))
            rhs_ref[h] = _pack(jnp.concatenate([jnp.concatenate(v, axis=1) for v in pw], axis=0))

    keys = [(s, p) for s in range(8) for p in sorted(set(_RHO[s]) - {16})] + [(8, 0)]

    def taps(i):
        outs = []
        for h in range(2):
            base, *zs = [(pw_ref[h, 2 * n], pw_ref[h, 2 * n + 1]) for n in range(len(steps) + 1)]
            zp = dict(zip(steps, zs))
            lhs = []
            for n, (s, p) in enumerate(keys):
                if p:
                    cur = _cmul(cur, zp[p - keys[n - 1][1]])
                else:
                    base = cur = _cmul(base, zp[256]) if s else base
                lhs.append(jnp.concatenate(cur, axis=1))
            outs.append(_dot(jnp.concatenate(lhs, axis=0), _unpack(rhs_ref[h]), _NT))
        both = pltpu.bitcast(pltpu.pack_elementwise(outs, packed_dtype=BF16), U32)
        piece = {}
        for n, (s, p) in enumerate(keys):
            piece[s, p] = pltpu.roll(both[8 * n:8 * n + 8], 126 - 7 if s == 8 else s, 1,
                                     stride=1, stride_axis=0)
        memo = {}
        for j in range(NS):
            key = ()
            acc = None
            for s in range(7, -1, -1):
                key = key + (_RHO[s][j],)
                if key not in memo:
                    pc = carry if _RHO[s][j] == 16 else piece[s, _RHO[s][j]]
                    same = acc is None or pc is acc
                    memo[key] = pc if same else jnp.where(((lane8 + 1) & 7) == s, pc, acc)
                acc = memo[key]
            (un, uo)[j % 2][_ds(i + D // 16, 8), _ds(j // 2, R)] = acc
            if j == 0:
                last_b = ((lane8 + 1) & 127) < 8
                carry = jnp.where(last_b, pltpu.roll(acc, 128 - 9, 1), pltpu.roll(acc, 128 - 8, 1))
                carry = jnp.where(lane8 == 6, pltpu.roll(piece[8, 0], 8, 1), carry)

    def gen_k(rb):
        for n in range(8):
            i = 8 * rb + n
            taps(i)
            powers(jnp.minimum(i + 1, D // 16 - 1))

    def dft_k(rb):
        for s in range(NS):
            u = (un, uo)[s // 8][_ds(rb + 4, 64), _ds(s % 8, R)]
            kspec[_ds(rb, 128), _ds(s, 2 * R)] = _dot(_unpack(u), _unpack(fk_ref[s]))

    def gen_step(rb, c):
        dft_k(rb - 1)
        gen_k(rb)
        return c

    with _scope("head"):
        for cp in first:
            cp.wait()
        for cp in second + loads:
            cp.start()

    with _scope("gen_k"):
        powers(0)
        gen_k(0)
        for cp in second:
            cp.wait()
        jax.lax.fori_loop(1, 4, gen_step, 0)

    for cp in loads:
        cp.wait()

    xu = [r.bitcast(U32) for r in xio]

    def load_x(b):
        for jj in range(8):
            ev, od = _halves(xu[b][pl.ds(jj, R, stride=8), :].T)
            xs[_ds(b, 128), _ds(jj, R)] = ev
            xo[_ds(b, 128), _ds(jj, R)] = od

    m_i = jax.lax.broadcasted_iota(jnp.int32, (128, 128), 0)
    c_i = jax.lax.broadcasted_iota(jnp.int32, (128, 128), 1)
    perm = jnp.where(c_i == (m_i & 7) * 16 + (m_i >> 3), 1.0, 0.0).astype(BF16)

    def prep_w(g):
        for t in range(3):
            wt[g, _ds(t, 64), :] = _pack(_dot(perm, wqkv_ref[:, _ds((t + 1) % 3 * 4 + g, 128)], _NT))
        wot[:, _ds(g, 128)] = _pack(_dot(perm, wo_ref[_ds(g, 128), :]).T)

    def dft(rb, s):
        at, n = BLOCKS[rb]
        u = (un, uo)[s // 8][at // 2:(at + n) // 2, _ds(s % 8, R)]
        y = _dot(_unpack(u), _unpack(f_ref[s]))
        spec[rb][0:n, _ds(s, 2 * R)] = y
        return y[-8:, R:]

    def idft(rb, s):
        at, n = BLOCKS[rb]
        y = _dot(spec[rb][0:n, _ds(s, 2 * R)], _unpack(f_ref[s]), _NT)
        (xs, xo)[s // 8][at:at + n, _ds(s % 8, R)] += y
        return y[-8:]

    def load_spec(ref, rows, order):
        return [(ref[rows, _ds(2 * s, R)], ref[rows, _ds(2 * s + 1, R)]) for s in order]

    def store_spec(ref, rows, order, vals):
        for s, v in zip(order, vals):
            ref[rows, _ds(2 * s, R)] = v[0]
            ref[rows, _ds(2 * s + 1, R)] = v[1]

    slabs = [_slab(j) for j in range(NS)]

    def quarter(buf, rows, odd, n, bias=None):
        a = []
        for m in range(4):
            j = n + 2 * m
            lo, hi = load_spec(buf, rows, [slabs[j], slabs[j + 8]])
            if j == 0 and bias is not None:
                lo = (lo[0] + bias, lo[1])
            a.append(_twiddle(_csub(lo, hi), j, -1) if odd else _cadd(lo, hi))
        return [_twiddle(v, 2 * n * k, -1) for k, v in enumerate(_fft4(a, -1))]

    def k_fft_steps(i):
        rows = _ds(i, 8)
        for odd in range(2):
            first = quarter(kspec, rows, odd, 0, dskb[rows, :])
            yield
            for k, (a, b) in enumerate(zip(first, quarter(kspec, rows, odd, 1))):
                store_spec(khat, rows, [8 * odd + k, 8 * odd + k + 4], [_cadd(a, b), _csub(a, b)])
            yield

    def k_fft(i):
        for _ in k_fft_steps(i):
            pass

    def conv(rb, i, after=None):
        at, size = BLOCKS[rb]
        buf, rows, park = spec[rb], _ds(i, 8), _ds(size // 8, 8)
        for odd in (1, 0):
            cols = [[], []]
            for k, (a, b) in enumerate(zip(*[quarter(buf, rows, odd, n) for n in range(2)])):
                lo, hi = _cadd(a, b), _csub(a, b)
                klo, khi = load_spec(khat, _ds(at // 8 + i, 8), [8 * odd + k, 8 * odd + k + 4])
                lo, hi = _cmul(lo, klo), _cmul(hi, khi)
                cols[0].append(_cadd(lo, hi))
                cols[1].append(_twiddle(_csub(lo, hi), 2 * k, 1))
            fence(buf, cols[1][3][0] if odd or after is None else after)
            for n in range(2):
                for m, v in enumerate(_fft4(cols[n], 1)):
                    j = n + 2 * m
                    if odd:
                        store_spec(buf, park, [j], [_twiddle(v, j, 1)])
                    else:
                        (o,) = load_spec(buf, park, [j])
                        store_spec(buf, rows, [slabs[j], slabs[j + 8]], [_cadd(v, o), _csub(v, o)])
        return cols[1][3][0]

    lane = jax.lax.broadcasted_iota(jnp.int32, (128, R), 1)

    def qkv(g, u, qs, ks, vs, i):
        y = _dot(_unpack(wt[g]), _unpack(u[0:D // 2, _ds(i, R)]))
        k, v, q = y[0:128], y[128:256], y[256:384]
        qs[:, _ds(i, R)] = q
        ks[:, _ds(i + 7, R)] = k
        vs[:, _ds(i + 7, R)] = v
        if i:
            ks[:, _ds(i - 1, R)] = pltpu.roll(k, 1, 1)
            vs[:, _ds(i - 1, R)] = jnp.where(lane == 0, va[:, _ds(7, R)], pltpu.roll(v, 1, 1))

    never = lane8 < zero_ref[0]

    def attend(g, qs, ks, vs, rs, o, i, ways, side=None):
        logits = []
        for w in range(W):
            lg = None
            for c in range(16):
                term = qs[_ds(c, 8), _ds(i, R)] * ks[_ds(c, 8), _ds(7 + i - w, R)]
                if c:
                    lg = lg + term
                else:
                    lg = term if w < ways else jnp.where(never, logits[w - ways], term)
            logits.append(lg)
            if side and w in (1, 7):
                fence(kspec, lg)
                next(side)
        scale = rs[7 + i] * 0.25
        logits = [lg * scale * rs[7 + i - w] for w, lg in enumerate(logits)]
        logits = [jnp.where(lane8 == 0, NEG, lg) if w > i else lg for w, lg in enumerate(logits)]
        mx = logits[0]
        for lg in logits[1:]:
            mx = jnp.maximum(mx, lg)
        es = [jnp.exp(lg - mx) for lg in logits]
        den = es[0]
        for e in es[1:]:
            den = den + e
        inv = 1.0 / den
        probs = [e * rs[7 + i - w] * inv for w, e in enumerate(es)]
        outs = []
        for c in range(16):
            acc = None
            for w in range(W):
                term = vs[_ds(c, 8), _ds(7 + i - w, R)] * probs[w]
                if w:
                    acc = acc + term
                else:
                    acc = term if c < ways else jnp.where(never, outs[c - ways], term)
            outs.append(acc)
            if side and c in (3, 11):
                fence(kspec, acc)
                next(side)
        o[_ds(g + 4, 64), _ds(i, R)] = _pack(jnp.concatenate(outs, axis=0))

    def chain_sum(vals, ways):
        parts = vals[:ways]
        for n, v in enumerate(vals[ways:]):
            parts[n % ways] = parts[n % ways] + v
        return jnp.sum(sum(parts[1:], parts[0]), axis=0, keepdims=True)

    def center(x, i, total, ways, after=None):
        parts = [total[_ds(n, 8)] for n in range(D // 8)]
        if after is not None:
            parts[0] = jnp.where(never, after, parts[0])
        c = x[:, _ds(i, R)] - chain_sum(parts, 2) * (1.0 / D)
        sq = c * c
        v = chain_sum([sq[_ds(n, 8)] for n in range(D // 8)], ways) * (1.0 / D)
        return c, jnp.broadcast_to(jax.lax.rsqrt(v + EPS), (8, R))

    def norm(x, u, rs, i, ways, after=None):
        c, r = center(x, i, x[:, _ds(i, R)], ways, after)
        u[0:D // 2, _ds(i, R)] = _pack(c)
        rs[7 + i] = r
        if i:
            rs[i - 1] = jnp.where(lane8 == 0, ra[7], pltpu.roll(r, 1, 1))
        return r

    def proj(x, o, u, i):
        y = x[:, _ds(i, R)] + _dot(_unpack(wot[...]), _unpack(o[D // 2:D, _ds(i, R)]))
        x[:, _ds(i, R)] = y
        cen[i % 2], r = center(x, i, y, 1)
        u[0:D // 2, _ds(i, R)] = _pack(cen[i % 2] * r[0:1])

    stores = [pltpu.make_async_copy(xio[c].at[0:L], o_hbm.at[:, c * 128:(c + 1) * 128], sems.at[c])
              for c in range(4)]

    def store_x(b, jj):
        t = pltpu.pack_elementwise(
            [xs[_ds(b, 128), _ds(jj, R)], xo[_ds(b, 128), _ds(jj, R)]], packed_dtype=BF16)
        xu[b][pl.ds(jj, R, stride=8), :] = pltpu.bitcast(t, U32).T

    def fence_io(b, val):
        xio[b][pl.ds(pl.multiple_of(L + zero_ref[0], 16), 16), :] = pltpu.bitcast(val, BF16)

    def start_store(b, val):
        stores[b].start()
        fence_io(b, val)
        return pltpu.bitcast(xio[b][L:L + 16, :], F32)

    def phase(name):
        def run(fn):
            with _scope(name):
                pl.when(zero_ref[0] == 0)(fn)
        return run

    @phase("prep")
    def _():
        dft_k(3)
        for b in range(4):
            load_x(b)
            prep_w(b)
            for n in range(6):
                k_fft(6 * b + n)

    even, odd = (un, (qa, ka, va), ra), (uo, (qb, kb, vb), rb_)

    def overlap(g_next, nxt, g, cur, k0):
        for i in range(8):
            qkv(g_next, nxt[0], *nxt[1], i)
            attend(g, *cur[1], cur[2], nxt[0], i, 2, None if k0 is None else k_fft_steps(k0 + i))

    for layer in range(2):
        @phase("a_pro")
        def _():
            if layer:
                for s in range(8):
                    idft(3, s)
            r = norm(xs, un, ra, 0, 4)
            for i in range(8):
                if layer:
                    idft(3, i + 8)
                qkv(0, un, qa, ka, va, i)
                if i < 7:
                    r = norm(xs, un, ra, i + 1, 2 - layer, r)
                r = norm(xo, uo, rb_, i, 2 - layer, r)

        def group(g, c):
            overlap(g, odd, g, even, None if layer else 8 * g + 24)

            @pl.when(g < 3)
            def _():
                overlap(g + 1, even, g, odd, None)

            return c

        with _scope("a_grp"):
            jax.lax.fori_loop(0, 4, group, 0)

        @phase("a_proj")
        def _():
            for i in range(8):
                proj(xs, uo, un, i)
                attend(3, qb, kb, vb, rb_, un, i, 1)
            for i in range(8):
                proj(xo, un, uo, i)
                if not layer:
                    k_fft(56 + i)
            for s in range(NS):
                dft(0, s)

        @phase("conv")
        def _():
            done = []
            for rb in range(4):
                for i in range(16):
                    for s in range(NS):
                        if rb < 3 and s * (16 - SKEW) // NS == i:
                            last = dft(rb + 1, s)
                        if rb and s * (16 - SKEW) // NS + SKEW == i:
                            last = idft(rb - 1, s)
                    if layer and rb >= 2 and i < 8:
                        store_x(rb - 2, i)
                        if i == 7:
                            last = start_store(rb - 2, last)
                    done.append(last)
                    mark = conv(rb, i, done[-LAG] if len(done) >= LAG else None)
                    if rb < 3:
                        fence(spec[rb + 1], mark)

    with _scope("store_x"):
        for jj in range(8):
            store_x(2, jj)
        fence_io(3, start_store(2, jnp.zeros((8, R), F32)))
        for jj in range(8):
            idft(3, jj)
            idft(3, jj + 8)
            store_x(3, jj)
        stores[3].start()
    with _scope("tail"):
        for cp in stores:
            cp.wait()


@jax.jit
def pallas_interleave_layers__sliding_local_dilated__ssm_conv_s4__prompt_kernel(
    A_x: jax.Array,
    A_wqkv: jax.Array,
    A_wo: jax.Array,
    B_u: jax.Array,
    B_A_re: jax.Array,
    B_A_im: jax.Array,
    B_B_re: jax.Array,
    B_B_im: jax.Array,
    B_C_re: jax.Array,
    B_C_im: jax.Array,
    B_log_dt: jax.Array,
    B_Dskip: jax.Array,
):
    del B_u
    f = _dft_matrix()
    lane = (np.arange(R) - 7) % R
    order = 16 * (lane % 8) + lane // 8
    fk = (f[:, order].astype(np.float32) / L).astype(ml_dtypes.bfloat16)
    scratch = [
        pltpu.VMEM((D, L // 2), F32),
        pltpu.VMEM((D, L // 2), F32),
        pltpu.VMEM((D + 8, L // 2), U32),
        pltpu.VMEM((D + 8, L // 2), U32),
        pltpu.VMEM((4, 192, D), U32),
        pltpu.VMEM((D // 2, D), U32),
        pltpu.VMEM((D // 2, 128), U32),
        pltpu.VMEM((D, 128), F32),
        pltpu.VMEM((2, 12, 8, N), F32),
        pltpu.VMEM((2, 64, 2 * N), U32),
        *[pltpu.VMEM((n + 16, 2 * L), F32) for _, n in BLOCKS],
        pltpu.VMEM((D + 8, 2 * L), F32),
        pltpu.VMEM((D, 2 * L), F32),
        pltpu.VMEM((128, 8 * R), F32),
        pltpu.VMEM((128, 15 * R), F32),
        pltpu.VMEM((128, 15 * R), F32),
        pltpu.VMEM((128, 8 * R), F32),
        pltpu.VMEM((128, 15 * R), F32),
        pltpu.VMEM((128, 15 * R), F32),
        pltpu.VMEM((15, 8, R), F32),
        pltpu.VMEM((15, 8, R), F32),
        pltpu.VMEM((2, D, R), F32),
        *[pltpu.VMEM((L + 16, 128), BF16)] * 4,
        pltpu.VMEM((D, 3 * D), BF16),
        pltpu.VMEM((D, D), BF16),
        pltpu.VMEM((NS, R // 2, 2 * R), U32),
        pltpu.VMEM((NS, R // 2, 2 * R), U32),
        pltpu.VMEM((6, D, N), BF16),
        pltpu.SemaphoreType.DMA((10,)),
    ]
    hbm = pl.BlockSpec(memory_space=pl.ANY)
    vmem = pl.BlockSpec(memory_space=pltpu.VMEM)
    out = pl.pallas_call(
        _kernel,
        out_shape=jax.ShapeDtypeStruct((L, D), BF16),
        in_specs=[pl.BlockSpec(memory_space=pltpu.SMEM)] + [hbm] * 9 + [vmem] * 2 + [hbm] * 2,
        out_specs=hbm,
        scratch_shapes=scratch,
        compiler_params=pltpu.CompilerParams(vmem_limit_bytes=100 * 1024 * 1024),
    )(np.zeros((1,), np.int32), A_x.reshape(L, D), A_wqkv, A_wo, B_A_re, B_A_im, B_B_re, B_B_im, B_C_re, B_C_im,
      B_log_dt, B_Dskip, _pack_rows(f), _pack_rows(fk))
    return out.reshape(1, L, D)
```

```python
import contextlib

import jax
import jax.numpy as jnp
import jax.experimental.pallas as pl
import jax.experimental.pallas.tpu as pltpu
import ml_dtypes
import numpy as np

L = 2048
D = 512
N = 128
NS = 16
R = 128
W = 8
EPS = 1e-5
_H = float(np.sqrt(0.5))
LAG = 4
SKEW = 0
BLOCKS = ((0, 128), (128, 128), (256, 128), (384, 128))
F32 = jnp.float32
BF16 = jnp.bfloat16
U32 = jnp.uint32
NEG = float(ml_dtypes.bfloat16(-1e9))

_NT = (((1,), (1,)), ((), ()))


def _slab(j):
    return (j % 2) * 8 + j // 2


def _dft_matrix():
    r = np.arange(R)
    k = np.arange(R) + 0.5
    f = np.zeros((NS, R, 2 * R), np.float64)
    for j in range(NS):
        th = 2.0 * np.pi * np.outer(NS * r + j, k) / (2 * L)
        f[_slab(j), :, :R] = np.cos(th)
        f[_slab(j), :, R:] = -np.sin(th)
    return f.astype(np.float32).astype(ml_dtypes.bfloat16)


def _pack_rows(a):
    u = np.ascontiguousarray(a).view(np.uint16).astype(np.uint32)
    return u[:, 0::2] | (u[:, 1::2] << np.uint32(16))


def _lag_tables():
    rho = []
    for s in range(8):
        lag = (256 * s + np.arange(NS)).astype(np.float32)
        rho.append([int(v) - 256 * s for v in lag.astype(ml_dtypes.bfloat16).astype(np.float32)])
    return rho


_RHO = _lag_tables()


def _cmul(a, b):
    return (a[0] * b[0] - a[1] * b[1], a[0] * b[1] + a[1] * b[0])


def _csq(a):
    t = a[0] * a[1]
    return ((a[0] - a[1]) * (a[0] + a[1]), t + t)


def _cadd(a, b):
    return (a[0] + b[0], a[1] + b[1])


def _csub(a, b):
    return (a[0] - b[0], a[1] - b[1])


def _split(p, e):
    plus, minus = [], []
    for lo, hi in zip(p[:len(p) // 2], p[len(p) // 2:]):
        if e % 4:
            hi = ((hi[0] - hi[1]) * _H, (hi[0] + hi[1]) * _H)
        if e >= 4:
            plus.append((lo[0] - hi[1], lo[1] + hi[0]))
            minus.append((lo[0] + hi[1], lo[1] - hi[0]))
        else:
            plus.append(_cadd(lo, hi))
            minus.append(_csub(lo, hi))
    return plus, minus


def _merge(plus, minus, e):
    lo, hi = [], []
    for p, m in zip(plus, minus):
        lo.append(_cadd(p, m))
        d = (p[1] - m[1], m[0] - p[0]) if e >= 4 else _csub(p, m)
        hi.append(((d[0] + d[1]) * _H, (d[1] - d[0]) * _H) if e % 4 else d)
    return lo + hi


def _factor_coeffs(k, e):
    if e % 8 == 0:
        (p,), (m,) = _split(k, e // 2)
        return [(p[0] * 0.5, p[1] * 0.5), (m[0] * 0.5, m[1] * 0.5)]
    c, s = float(np.cos(np.pi * e / 8)), float(np.sin(np.pi * e / 8))
    wk = (k[1][0] * c - k[1][1] * s, k[1][0] * s + k[1][1] * c)
    return [k[0], _csub(wk, k[0]), _csub(k[1], k[0])]


def _factor_mul(a, coeffs, e):
    if e % 8 == 0:
        (p,), (m,) = _split(a, e // 2)
        return _merge([_cmul(p, coeffs[0])], [_cmul(m, coeffs[1])], e // 2)
    t = _cmul(_cadd(a[0], a[1]), coeffs[0])
    return [_cadd(t, _cmul(a[1], coeffs[1])), _cadd(t, _cmul(a[0], coeffs[2]))]


def _coeff_slots(e):
    if e % 8 == 0:
        return [e // 4, e // 4 + 1]
    n = 4 + 3 * [2, 4, 6, 10, 12, 14].index(e)
    return [n, n + 1, n + 2]


def _scope(name):
    return contextlib.nullcontext()


def _ds(i, n):
    if isinstance(i, int):
        return slice(i * n, (i + 1) * n)
    return pl.ds(pl.multiple_of(i * n, n), n)


def _pack(x):
    return pltpu.bitcast(x.astype(BF16), U32)


def _unpack(x):
    return pltpu.bitcast(x, BF16)


def _dot(a, b, dims=(((1,), (0,)), ((), ()))):
    return jax.lax.dot_general(a, b, dims, preferred_element_type=F32)


def _halves(u):
    return pltpu.bitcast(u << 16, F32), pltpu.bitcast(u & jnp.uint32(0xFFFF0000), F32)


def _kernel(zero_ref, x_hbm, wqkv_hbm, wo_hbm, are, aim, bre, bim, cre, cim,
            ldt_ref, dsk_ref, f_hbm, fk_hbm, o_hbm,
            xs, xo, un, uo, wt, wot, dtb, dskb, pw_ref, rhs_ref, s0, s1, s2, s3, kspec, khat, qa, ka, va, qb, kb, vb,
            ra, rb_, cen,
            io0, io1, io2, io3, wqkv_ref, wo_ref, f_ref, fk_ref, ssm, sems):
    def fetch_ssm(rows, sem):
        return [pltpu.make_async_copy(p.at[rows], ssm.at[n, rows], sem)
                for n, p in enumerate((are, aim, bre, bim, cre, cim))]

    first = fetch_ssm(pl.ds(0, 144), sems.at[8])
    for cp in first:
        cp.start()
    second = fetch_ssm(pl.ds(144, D - 144), sems.at[9])
    second += [pltpu.make_async_copy(fk_hbm, fk_ref, sems.at[4])]
    for cp in second:
        cp.start()
    xio = (io0, io1, io2, io3)
    loads = []
    loads += [pltpu.make_async_copy(x_hbm.at[:, c * 128:(c + 1) * 128], xio[c].at[0:L], sems.at[c])
              for c in range(4)]
    loads += [pltpu.make_async_copy(src, dst, sems.at[5 + n]) for n, (src, dst) in enumerate(
        [(wqkv_hbm, wqkv_ref), (wo_hbm, wo_ref), (f_hbm, f_ref)])]

    spec = (s0, s1, s2, s3)

    def fence(ref, val):
        row = ref.shape[0] - 8 + zero_ref[0]
        ref[pl.ds(pl.multiple_of(row, 8), 8), 0:128] = val

    dt_row = jnp.exp(ldt_ref[...].astype(F32)).reshape(1, D)
    dtb[...] = _pack(jnp.broadcast_to(dt_row, (128, D)).T)
    dskb[...] = jnp.broadcast_to(dsk_ref[...].astype(F32).reshape(1, D) * (2.0 / L), (128, D)).T

    lane8 = jax.lax.broadcasted_iota(jnp.int32, (8, R), 1)
    rev8 = 7 - jax.lax.broadcasted_iota(jnp.int32, (8, N), 0)
    steps = (1, 2, 4, 8, 256)

    def powers(i):
        dts = _halves(dtb[_ds(i, 8), :])
        are, aim, bre, bim, cre, cim = [
            _halves(pltpu.bitcast(ssm[n, _ds(i, 16), :], U32)) for n in range(6)]
        for h in range(2):
            dt = dts[h]
            li = dt * aim[h]
            mag = jnp.exp(dt * are[h])
            zp = {1: (mag * jnp.cos(li), mag * jnp.sin(li))}
            for e in (1, 2, 4, 8, 16, 32, 64, 128):
                zp[2 * e] = _csq(zp[e])
            w = _cmul((cre[h], cim[h]), (dt * bre[h], dt * bim[h]))
            for n, v in enumerate(zp[e] for e in steps):
                pw_ref[h, 2 * n] = v[0]
                pw_ref[h, 2 * n + 1] = v[1]
            w, step = [(jnp.take_along_axis(v[0], rev8, axis=0), -jnp.take_along_axis(v[1], rev8, axis=0))
                       for v in (w, zp[16])]
            pw = [w]
            for b in range(1, 16):
                pw.append(_cmul(pw[-1], step))
            rhs_ref[h] = _pack(jnp.concatenate([jnp.concatenate(v, axis=1) for v in pw], axis=0))

    keys = [(s, p) for s in range(8) for p in sorted(set(_RHO[s]) - {16})] + [(8, 0)]

    def taps(i):
        outs = []
        for h in range(2):
            zp = {e: (pw_ref[h, 2 * n], pw_ref[h, 2 * n + 1]) for n, e in enumerate(steps)}
            zp[0] = (jnp.ones((8, N), F32), jnp.zeros((8, N), F32))
            lhs = []
            for n, (s, p) in enumerate(keys):
                e = 256 * s + p
                if e not in zp:
                    if e % 2 == 0 and e // 2 in zp:
                        zp[e] = _csq(zp[e // 2])
                    else:
                        inc = p - keys[n - 1][1] if p else 256
                        zp[e] = _cmul(zp[e - inc], zp[inc])
                lhs.append(jnp.concatenate(zp[e], axis=1))
            outs.append(_dot(jnp.concatenate(lhs, axis=0), _unpack(rhs_ref[h]), _NT))
        both = pltpu.bitcast(pltpu.pack_elementwise(outs, packed_dtype=BF16), U32)
        piece = {}
        for n, (s, p) in enumerate(keys):
            piece[s, p] = pltpu.roll(both[8 * n:8 * n + 8], 126 - 7 if s == 8 else s, 1,
                                     stride=1, stride_axis=0)
        memo = {}
        for j in range(NS):
            key = ()
            acc = None
            for s in range(7, -1, -1):
                key = key + (_RHO[s][j],)
                if key not in memo:
                    pc = carry if _RHO[s][j] == 16 else piece[s, _RHO[s][j]]
                    same = acc is None or pc is acc
                    memo[key] = pc if same else jnp.where(((lane8 + 1) & 7) == s, pc, acc)
                acc = memo[key]
            (un, uo)[j % 2][_ds(i + D // 16, 8), _ds(j // 2, R)] = acc
            if j == 0:
                last_b = ((lane8 + 1) & 127) < 8
                carry = jnp.where(last_b, pltpu.roll(acc, 128 - 9, 1), pltpu.roll(acc, 128 - 8, 1))
                carry = jnp.where(lane8 == 6, pltpu.roll(piece[8, 0], 8, 1), carry)

    def gen_k(rb):
        for n in range(8):
            i = 8 * rb + n
            taps(i)
            powers(jnp.minimum(i + 1, D // 16 - 1))

    def dft_k(rb):
        for s in range(NS):
            u = (un, uo)[s // 8][_ds(rb + 4, 64), _ds(s % 8, R)]
            kspec[_ds(rb, 128), _ds(s, 2 * R)] = _dot(_unpack(u), _unpack(fk_ref[s]))

    def gen_step(rb, c):
        dft_k(rb - 1)
        gen_k(rb)
        return c

    with _scope("head"):
        for cp in first:
            cp.wait()
        for cp in loads:
            cp.start()

    with _scope("gen_k"):
        powers(0)
        gen_k(0)
        for cp in second:
            cp.wait()
        jax.lax.fori_loop(1, 4, gen_step, 0)

    for cp in loads:
        cp.wait()

    xu = [r.bitcast(U32) for r in xio]

    def load_x(b):
        for jj in range(8):
            ev, od = _halves(xu[b][pl.ds(jj, R, stride=8), :].T)
            xs[_ds(b, 128), _ds(jj, R)] = ev
            xo[_ds(b, 128), _ds(jj, R)] = od

    m_i = jax.lax.broadcasted_iota(jnp.int32, (128, 128), 0)
    c_i = jax.lax.broadcasted_iota(jnp.int32, (128, 128), 1)
    perm = jnp.where(c_i == (m_i & 7) * 16 + (m_i >> 3), 1.0, 0.0).astype(BF16)

    def prep_w(g):
        for t in range(3):
            wt[g, _ds(t, 64), :] = _pack(_dot(perm, wqkv_ref[:, _ds((t + 1) % 3 * 4 + g, 128)], _NT))
        wot[:, _ds(g, 128)] = _pack(_dot(perm, wo_ref[_ds(g, 128), :]).T)

    def dft(rb, s):
        at, n = BLOCKS[rb]
        u = (un, uo)[s // 8][at // 2:(at + n) // 2, _ds(s % 8, R)]
        y = _dot(_unpack(u), _unpack(f_ref[s]))
        spec[rb][0:n, _ds(s, 2 * R)] = y
        return y[-8:, R:]

    def idft(rb, s):
        at, n = BLOCKS[rb]
        y = _dot(spec[rb][0:n, _ds(s, 2 * R)], _unpack(f_ref[s]), _NT)
        (xs, xo)[s // 8][at:at + n, _ds(s % 8, R)] += y
        return y[-8:]

    def load_spec(ref, rows, order):
        return [(ref[rows, _ds(2 * s, R)], ref[rows, _ds(2 * s + 1, R)]) for s in order]

    def store_spec(ref, rows, order, vals):
        for s, v in zip(order, vals):
            ref[rows, _ds(2 * s, R)] = v[0]
            ref[rows, _ds(2 * s + 1, R)] = v[1]

    slabs = [_slab(j) for j in range(NS)]

    def half(buf, rows, e8, bias=None):
        out = []
        for j in range(8):
            lo, hi = load_spec(buf, rows, [slabs[j], slabs[j + 8]])
            if j == 0 and bias is not None:
                lo = (lo[0] + bias, lo[1])
            out.append(_csub(lo, hi) if e8 else _cadd(lo, hi))
        return out

    def k_fft_steps(i):
        rows = _ds(i, 8)
        for e8 in (8, 0):
            quartics = _split(half(kspec, rows, e8, dskb[rows, :]), e8 // 2)
            for e4, p4 in zip((e8 // 2, e8 // 2 + 8), quartics):
                for e2, p2 in zip((e4 // 2, e4 // 2 + 8), _split(p4, e4 // 2)):
                    store_spec(khat, rows, _coeff_slots(e2), _factor_coeffs(p2, e2))
                yield

    def k_fft(i):
        for _ in k_fft_steps(i):
            pass

    def conv(rb, i, after=None):
        at, size = BLOCKS[rb]
        buf, rows, park = spec[rb], _ds(i, 8), _ds(size // 8, 8)
        for e8 in (8, 0):
            quartics = []
            for e4, p4 in zip((e8 // 2, e8 // 2 + 8), _split(half(buf, rows, e8), e8 // 2)):
                prods = [_factor_mul(p2, load_spec(khat, _ds(at // 8 + i, 8), _coeff_slots(e2)), e2)
                         for e2, p2 in zip((e4 // 2, e4 // 2 + 8), _split(p4, e4 // 2))]
                quartics.append(_merge(*prods, e4 // 2))
                if e4 < 8:
                    fence(khat, prods[1][1][0])
            mark = prods[1][1][0]
            fence(buf, mark if e8 or after is None else after)
            for j, v in enumerate(_merge(*quartics, e8 // 2)):
                if e8:
                    store_spec(buf, park, [j], [v])
                else:
                    (o,) = load_spec(buf, park, [j])
                    store_spec(buf, rows, [slabs[j], slabs[j + 8]], [_cadd(v, o), _csub(v, o)])
        return mark

    lane = jax.lax.broadcasted_iota(jnp.int32, (128, R), 1)

    def qkv(g, u, qs, ks, vs, i):
        y = _dot(_unpack(wt[g]), _unpack(u[0:D // 2, _ds(i, R)]))
        k, v, q = y[0:128], y[128:256], y[256:384]
        qs[:, _ds(i, R)] = q
        ks[:, _ds(i + 7, R)] = k
        vs[:, _ds(i + 7, R)] = v
        if i:
            ks[:, _ds(i - 1, R)] = pltpu.roll(k, 1, 1)
            vs[:, _ds(i - 1, R)] = jnp.where(lane == 0, va[:, _ds(7, R)], pltpu.roll(v, 1, 1))

    never = lane8 < zero_ref[0]

    def attend(g, qs, ks, vs, rs, o, i, ways, side=None):
        logits = []
        for w in range(W):
            lg = None
            for c in range(16):
                term = qs[_ds(c, 8), _ds(i, R)] * ks[_ds(c, 8), _ds(7 + i - w, R)]
                if c:
                    lg = lg + term
                else:
                    lg = term if w < ways else jnp.where(never, logits[w - ways], term)
            logits.append(lg)
            if side and w in (1, 7):
                fence(kspec, lg)
                next(side)
        scale = rs[7 + i] * 0.25
        logits = [lg * scale * rs[7 + i - w] for w, lg in enumerate(logits)]
        logits = [jnp.where(lane8 == 0, NEG, lg) if w > i else lg for w, lg in enumerate(logits)]
        mx = logits[0]
        for lg in logits[1:]:
            mx = jnp.maximum(mx, lg)
        es = [jnp.exp(lg - mx) for lg in logits]
        den = es[0]
        for e in es[1:]:
            den = den + e
        inv = 1.0 / den
        probs = [e * rs[7 + i - w] * inv for w, e in enumerate(es)]
        outs = []
        for c in range(16):
            acc = None
            for w in range(W):
                term = vs[_ds(c, 8), _ds(7 + i - w, R)] * probs[w]
                if w:
                    acc = acc + term
                else:
                    acc = term if c < ways else jnp.where(never, outs[c - ways], term)
            outs.append(acc)
            if side and c in (3, 11):
                fence(kspec, acc)
                next(side)
        o[_ds(g + 4, 64), _ds(i, R)] = _pack(jnp.concatenate(outs, axis=0))

    def chain_sum(vals, ways):
        parts = vals[:ways]
        for n, v in enumerate(vals[ways:]):
            parts[n % ways] = parts[n % ways] + v
        return jnp.sum(sum(parts[1:], parts[0]), axis=0, keepdims=True)

    def center(x, i, total, ways, after=None):
        parts = [total[_ds(n, 8)] for n in range(D // 8)]
        if after is not None:
            parts[0] = jnp.where(never, after, parts[0])
        c = x[:, _ds(i, R)] - chain_sum(parts, 2) * (1.0 / D)
        sq = c * c
        v = chain_sum([sq[_ds(n, 8)] for n in range(D // 8)], ways) * (1.0 / D)
        return c, jnp.broadcast_to(jax.lax.rsqrt(v + EPS), (8, R))

    def norm(x, u, rs, i, ways, after=None):
        c, r = center(x, i, x[:, _ds(i, R)], ways, after)
        u[0:D // 2, _ds(i, R)] = _pack(c)
        rs[7 + i] = r
        if i:
            rs[i - 1] = jnp.where(lane8 == 0, ra[7], pltpu.roll(r, 1, 1))
        return r

    def proj(x, o, u, i):
        y = x[:, _ds(i, R)] + _dot(_unpack(wot[...]), _unpack(o[D // 2:D, _ds(i, R)]))
        x[:, _ds(i, R)] = y
        cen[i % 2], r = center(x, i, y, 1)
        u[0:D // 2, _ds(i, R)] = _pack(cen[i % 2] * r[0:1])

    stores = [pltpu.make_async_copy(xio[c].at[0:L], o_hbm.at[:, c * 128:(c + 1) * 128], sems.at[c])
              for c in range(4)]

    def store_x(b, jj):
        t = pltpu.pack_elementwise(
            [xs[_ds(b, 128), _ds(jj, R)], xo[_ds(b, 128), _ds(jj, R)]], packed_dtype=BF16)
        xu[b][pl.ds(jj, R, stride=8), :] = pltpu.bitcast(t, U32).T

    def fence_io(b, val):
        xio[b][pl.ds(pl.multiple_of(L + zero_ref[0], 16), 16), :] = pltpu.bitcast(val, BF16)

    def start_store(b, val):
        stores[b].start()
        fence_io(b, val)
        return pltpu.bitcast(xio[b][L:L + 16, :], F32)

    def phase(name):
        def run(fn):
            with _scope(name):
                pl.when(zero_ref[0] == 0)(fn)
        return run

    @phase("prep")
    def _():
        dft_k(3)
        for b in range(4):
            load_x(b)
            prep_w(b)
            for n in range(6):
                k_fft(6 * b + n)

    even, odd = (un, (qa, ka, va), ra), (uo, (qb, kb, vb), rb_)

    def overlap(g_next, nxt, g, cur, k0):
        for i in range(8):
            qkv(g_next, nxt[0], *nxt[1], i)
            attend(g, *cur[1], cur[2], nxt[0], i, 2, None if k0 is None else k_fft_steps(k0 + i))

    for layer in range(2):
        @phase("a_pro")
        def _():
            if layer:
                for s in range(8):
                    idft(3, s)
            r = norm(xs, un, ra, 0, 4)
            for i in range(8):
                if layer:
                    idft(3, i + 8)
                qkv(0, un, qa, ka, va, i)
                if i < 7:
                    r = norm(xs, un, ra, i + 1, 2 - layer, r)
                r = norm(xo, uo, rb_, i, 2 - layer, r)

        def group(g, c):
            overlap(g, odd, g, even, None if layer else 8 * g + 24)

            @pl.when(g < 3)
            def _():
                overlap(g + 1, even, g, odd, None)

            return c

        with _scope("a_grp"):
            jax.lax.fori_loop(0, 4, group, 0)

        @phase("a_proj")
        def _():
            for i in range(8):
                proj(xs, uo, un, i)
                attend(3, qb, kb, vb, rb_, un, i, 1)
            for i in range(8):
                proj(xo, un, uo, i)
                if not layer:
                    k_fft(56 + i)
            for s in range(NS):
                dft(0, s)

        @phase("conv")
        def _():
            done = []
            for rb in range(4):
                for i in range(16):
                    for s in range(NS):
                        if rb < 3 and s * (16 - SKEW) // NS == i:
                            last = dft(rb + 1, s)
                        if rb and s * (16 - SKEW) // NS + SKEW == i:
                            last = idft(rb - 1, s)
                    if layer and rb >= 2 and i < 8:
                        store_x(rb - 2, i)
                        if i == 7:
                            last = start_store(rb - 2, last)
                    done.append(last)
                    mark = conv(rb, i, done[-LAG] if len(done) >= LAG else None)
                    if rb < 3:
                        fence(spec[rb + 1], mark)

    with _scope("store_x"):
        for jj in range(8):
            store_x(2, jj)
        fence_io(3, start_store(2, jnp.zeros((8, R), F32)))
        for jj in range(8):
            idft(3, jj)
            idft(3, jj + 8)
            store_x(3, jj)
        stores[3].start()
    with _scope("tail"):
        for cp in stores:
            cp.wait()


@jax.jit
def pallas_interleave_layers__sliding_local_dilated__ssm_conv_s4__prompt_kernel(
    A_x: jax.Array,
    A_wqkv: jax.Array,
    A_wo: jax.Array,
    B_u: jax.Array,
    B_A_re: jax.Array,
    B_A_im: jax.Array,
    B_B_re: jax.Array,
    B_B_im: jax.Array,
    B_C_re: jax.Array,
    B_C_im: jax.Array,
    B_log_dt: jax.Array,
    B_Dskip: jax.Array,
):
    del B_u
    f = _dft_matrix()
    lane = (np.arange(R) - 7) % R
    order = 16 * (lane % 8) + lane // 8
    fk = (f[:, order].astype(np.float32) * (2.0 / L)).astype(ml_dtypes.bfloat16)
    scratch = [
        pltpu.VMEM((D, L // 2), F32),
        pltpu.VMEM((D, L // 2), F32),
        pltpu.VMEM((D + 8, L // 2), U32),
        pltpu.VMEM((D + 8, L // 2), U32),
        pltpu.VMEM((4, 192, D), U32),
        pltpu.VMEM((D // 2, D), U32),
        pltpu.VMEM((D // 2, 128), U32),
        pltpu.VMEM((D, 128), F32),
        pltpu.VMEM((2, 10, 8, N), F32),
        pltpu.VMEM((2, 64, 2 * N), U32),
        *[pltpu.VMEM((n + 16, 2 * L), F32) for _, n in BLOCKS],
        pltpu.VMEM((D + 8, 2 * L), F32),
        pltpu.VMEM((D + 8, 22 * 2 * R), F32),
        pltpu.VMEM((128, 8 * R), F32),
        pltpu.VMEM((128, 15 * R), F32),
        pltpu.VMEM((128, 15 * R), F32),
        pltpu.VMEM((128, 8 * R), F32),
        pltpu.VMEM((128, 15 * R), F32),
        pltpu.VMEM((128, 15 * R), F32),
        pltpu.VMEM((15, 8, R), F32),
        pltpu.VMEM((15, 8, R), F32),
        pltpu.VMEM((2, D, R), F32),
        *[pltpu.VMEM((L + 16, 128), BF16)] * 4,
        pltpu.VMEM((D, 3 * D), BF16),
        pltpu.VMEM((D, D), BF16),
        pltpu.VMEM((NS, R // 2, 2 * R), U32),
        pltpu.VMEM((NS, R // 2, 2 * R), U32),
        pltpu.VMEM((6, D, N), BF16),
        pltpu.SemaphoreType.DMA((10,)),
    ]
    hbm = pl.BlockSpec(memory_space=pl.ANY)
    vmem = pl.BlockSpec(memory_space=pltpu.VMEM)
    out = pl.pallas_call(
        _kernel,
        out_shape=jax.ShapeDtypeStruct((L, D), BF16),
        in_specs=[pl.BlockSpec(memory_space=pltpu.SMEM)] + [hbm] * 9 + [vmem] * 2 + [hbm] * 2,
        out_specs=hbm,
        scratch_shapes=scratch,
        compiler_params=pltpu.CompilerParams(vmem_limit_bytes=100 * 1024 * 1024),
    )(np.zeros((1,), np.int32), A_x.reshape(L, D), A_wqkv, A_wo, B_A_re, B_A_im, B_B_re, B_B_im, B_C_re, B_C_im,
      B_log_dt, B_Dskip, _pack_rows(f), _pack_rows(fk))
    return out.reshape(1, L, D)
```

```python
import contextlib

import jax
import jax.numpy as jnp
import jax.experimental.pallas as pl
import jax.experimental.pallas.tpu as pltpu
import ml_dtypes
import numpy as np

L = 2048
D = 512
N = 128
NS = 16
R = 128
W = 8
EPS = 1e-5
_H = float(np.sqrt(0.5))
LAG = 4
SKEW = 0
BLOCKS = ((0, 128), (128, 128), (256, 128), (384, 128))
F32 = jnp.float32
BF16 = jnp.bfloat16
U32 = jnp.uint32
NEG = float(ml_dtypes.bfloat16(-1e9))

_NT = (((1,), (1,)), ((), ()))


def _slab(j):
    return (j % 2) * 8 + j // 2


def _dft_matrix():
    r = np.arange(R)
    k = np.arange(R) + 0.5
    f = np.zeros((NS, R, 2 * R), np.float64)
    for j in range(NS):
        th = 2.0 * np.pi * np.outer(NS * r + j, k) / (2 * L)
        f[_slab(j), :, :R] = np.cos(th)
        f[_slab(j), :, R:] = -np.sin(th)
    return f.astype(np.float32).astype(ml_dtypes.bfloat16)


def _pack_rows(a):
    u = np.ascontiguousarray(a).view(np.uint16).astype(np.uint32)
    return u[:, 0::2] | (u[:, 1::2] << np.uint32(16))


def _lag_tables():
    rho = []
    for s in range(8):
        lag = (256 * s + np.arange(NS)).astype(np.float32)
        rho.append([int(v) - 256 * s for v in lag.astype(ml_dtypes.bfloat16).astype(np.float32)])
    return rho


_RHO = _lag_tables()


def _cmul(a, b):
    return (a[0] * b[0] - a[1] * b[1], a[0] * b[1] + a[1] * b[0])


def _csq(a):
    t = a[0] * a[1]
    return ((a[0] - a[1]) * (a[0] + a[1]), t + t)


def _cadd(a, b):
    return (a[0] + b[0], a[1] + b[1])


def _csub(a, b):
    return (a[0] - b[0], a[1] - b[1])


def _split(p, e):
    plus, minus = [], []
    for lo, hi in zip(p[:len(p) // 2], p[len(p) // 2:]):
        if e % 4:
            hi = ((hi[0] - hi[1]) * _H, (hi[0] + hi[1]) * _H)
        if e >= 4:
            plus.append((lo[0] - hi[1], lo[1] + hi[0]))
            minus.append((lo[0] + hi[1], lo[1] - hi[0]))
        else:
            plus.append(_cadd(lo, hi))
            minus.append(_csub(lo, hi))
    return plus, minus


def _merge(plus, minus, e):
    lo, hi = [], []
    for p, m in zip(plus, minus):
        lo.append(_cadd(p, m))
        d = (p[1] - m[1], m[0] - p[0]) if e >= 4 else _csub(p, m)
        hi.append(((d[0] + d[1]) * _H, (d[1] - d[0]) * _H) if e % 4 else d)
    return lo + hi


def _factor_coeffs(k, e):
    if e % 8 == 0:
        (p,), (m,) = _split(k, e // 2)
        return [(p[0] * 0.5, p[1] * 0.5), (m[0] * 0.5, m[1] * 0.5)]
    c, s = float(np.cos(np.pi * e / 8)), float(np.sin(np.pi * e / 8))
    wk = (k[1][0] * c - k[1][1] * s, k[1][0] * s + k[1][1] * c)
    return [k[0], _csub(wk, k[0]), _csub(k[1], k[0])]


def _factor_mul(a, coeffs, e):
    if e % 8 == 0:
        (p,), (m,) = _split(a, e // 2)
        return _merge([_cmul(p, coeffs[0])], [_cmul(m, coeffs[1])], e // 2)
    t = _cmul(_cadd(a[0], a[1]), coeffs[0])
    return [_cadd(t, _cmul(a[1], coeffs[1])), _cadd(t, _cmul(a[0], coeffs[2]))]


def _coeff_slots(e):
    if e % 8 == 0:
        return [e // 4, e // 4 + 1]
    n = 4 + 3 * [2, 4, 6, 10, 12, 14].index(e)
    return [n, n + 1, n + 2]


def _scope(name):
    return contextlib.nullcontext()


def _ds(i, n):
    if isinstance(i, int):
        return slice(i * n, (i + 1) * n)
    return pl.ds(pl.multiple_of(i * n, n), n)


def _pack(x):
    return pltpu.bitcast(x.astype(BF16), U32)


def _unpack(x):
    return pltpu.bitcast(x, BF16)


def _dot(a, b, dims=(((1,), (0,)), ((), ()))):
    return jax.lax.dot_general(a, b, dims, preferred_element_type=F32)


def _halves(u):
    return pltpu.bitcast(u << 16, F32), pltpu.bitcast(u & jnp.uint32(0xFFFF0000), F32)


def _kernel(zero_hbm, x_hbm, wqkv_hbm, wo_hbm, are, aim, bre, bim, cre, cim,
            ldt_hbm, dsk_hbm, f_hbm, fk_hbm, o_hbm,
            xs, xo, un, uo, wt, wot, dtb, dskb, pw_ref, rhs_ref, s0, s1, s2, s3, kspec, khat, qa, ka, va, qb, kb, vb,
            ra, rb_, cen,
            io0, io1, io2, io3, wqkv_ref, wo_ref, f_ref, fk_ref, ssm, zero_ref, ldt_ref, dsk_ref, sems):
    def fetch_ssm(rows, sem):
        return [pltpu.make_async_copy(p.at[rows], ssm.at[n, rows], sem)
                for n, p in enumerate((are, aim, bre, bim, cre, cim))]

    small = [pltpu.make_async_copy(src, dst, sems.at[10 + n]) for n, (src, dst) in enumerate(
        [(zero_hbm, zero_ref), (ldt_hbm, ldt_ref), (dsk_hbm, dsk_ref)])]
    for cp in small:
        cp.start()
    first = fetch_ssm(pl.ds(0, 144), sems.at[8])
    for cp in first:
        cp.start()
    second = fetch_ssm(pl.ds(144, D - 144), sems.at[9])
    second += [pltpu.make_async_copy(fk_hbm, fk_ref, sems.at[4])]
    for cp in second:
        cp.start()
    xio = (io0, io1, io2, io3)
    loads = []
    loads += [pltpu.make_async_copy(x_hbm.at[:, c * 128:(c + 1) * 128], xio[c].at[0:L], sems.at[c])
              for c in range(4)]
    loads += [pltpu.make_async_copy(src, dst, sems.at[5 + n]) for n, (src, dst) in enumerate(
        [(wqkv_hbm, wqkv_ref), (wo_hbm, wo_ref), (f_hbm, f_ref)])]

    spec = (s0, s1, s2, s3)

    def fence(ref, val):
        row = ref.shape[0] - 8 + zero_ref[0]
        ref[pl.ds(pl.multiple_of(row, 8), 8), 0:128] = val

    for cp in small:
        cp.wait()
    dt_row = jnp.exp(ldt_ref[...].astype(F32)).reshape(1, D)
    dtb[...] = _pack(jnp.broadcast_to(dt_row, (128, D)).T)
    dskb[...] = jnp.broadcast_to(dsk_ref[...].astype(F32).reshape(1, D) * (2.0 / L), (128, D)).T

    lane8 = jax.lax.broadcasted_iota(jnp.int32, (8, R), 1)
    rev8 = 7 - jax.lax.broadcasted_iota(jnp.int32, (8, N), 0)
    steps = (1, 2, 4, 8, 256)

    def powers(i):
        dts = _halves(dtb[_ds(i, 8), :])
        are, aim, bre, bim, cre, cim = [
            _halves(pltpu.bitcast(ssm[n, _ds(i, 16), :], U32)) for n in range(6)]
        for h in range(2):
            dt = dts[h]
            li = dt * aim[h]
            mag = jnp.exp(dt * are[h])
            zp = {1: (mag * jnp.cos(li), mag * jnp.sin(li))}
            for e in (1, 2, 4, 8, 16, 32, 64, 128):
                zp[2 * e] = _csq(zp[e])
            w = _cmul((cre[h], cim[h]), (dt * bre[h], dt * bim[h]))
            for n, v in enumerate(zp[e] for e in steps):
                pw_ref[h, 2 * n] = v[0]
                pw_ref[h, 2 * n + 1] = v[1]
            w, step = [(jnp.take_along_axis(v[0], rev8, axis=0), -jnp.take_along_axis(v[1], rev8, axis=0))
                       for v in (w, zp[16])]
            pw = [w]
            for b in range(1, 16):
                pw.append(_cmul(pw[-1], step))
            rhs_ref[h] = _pack(jnp.concatenate([jnp.concatenate(v, axis=1) for v in pw], axis=0))

    keys = [(s, p) for s in range(8) for p in sorted(set(_RHO[s]) - {16})] + [(8, 0)]

    def taps(i):
        outs = []
        for h in range(2):
            zp = {e: (pw_ref[h, 2 * n], pw_ref[h, 2 * n + 1]) for n, e in enumerate(steps)}
            zp[0] = (jnp.ones((8, N), F32), jnp.zeros((8, N), F32))
            lhs = []
            for n, (s, p) in enumerate(keys):
                e = 256 * s + p
                if e not in zp:
                    if e % 2 == 0 and e // 2 in zp:
                        zp[e] = _csq(zp[e // 2])
                    else:
                        inc = p - keys[n - 1][1] if p else 256
                        zp[e] = _cmul(zp[e - inc], zp[inc])
                lhs.append(jnp.concatenate(zp[e], axis=1))
            outs.append(_dot(jnp.concatenate(lhs, axis=0), _unpack(rhs_ref[h]), _NT))
        both = pltpu.bitcast(pltpu.pack_elementwise(outs, packed_dtype=BF16), U32)
        piece = {}
        for n, (s, p) in enumerate(keys):
            piece[s, p] = pltpu.roll(both[8 * n:8 * n + 8], 126 - 7 if s == 8 else s, 1,
                                     stride=1, stride_axis=0)
        memo = {}
        for j in range(NS):
            key = ()
            acc = None
            for s in range(7, -1, -1):
                key = key + (_RHO[s][j],)
                if key not in memo:
                    pc = carry if _RHO[s][j] == 16 else piece[s, _RHO[s][j]]
                    same = acc is None or pc is acc
                    memo[key] = pc if same else jnp.where(((lane8 + 1) & 7) == s, pc, acc)
                acc = memo[key]
            (un, uo)[j % 2][_ds(i + D // 16, 8), _ds(j // 2, R)] = acc
            if j == 0:
                last_b = ((lane8 + 1) & 127) < 8
                carry = jnp.where(last_b, pltpu.roll(acc, 128 - 9, 1), pltpu.roll(acc, 128 - 8, 1))
                carry = jnp.where(lane8 == 6, pltpu.roll(piece[8, 0], 8, 1), carry)

    def gen_k(rb):
        for n in range(8):
            i = 8 * rb + n
            taps(i)
            powers(jnp.minimum(i + 1, D // 16 - 1))

    def dft_k(rb):
        for s in range(NS):
            u = (un, uo)[s // 8][_ds(rb + 4, 64), _ds(s % 8, R)]
            kspec[_ds(rb, 128), _ds(s, 2 * R)] = _dot(_unpack(u), _unpack(fk_ref[s]))

    def gen_step(rb, c):
        dft_k(rb - 1)
        gen_k(rb)
        return c

    with _scope("head"):
        for cp in first:
            cp.wait()
        for cp in loads:
            cp.start()

    with _scope("gen_k"):
        powers(0)
        gen_k(0)
        for cp in second:
            cp.wait()
        jax.lax.fori_loop(1, 4, gen_step, 0)

    for cp in loads:
        cp.wait()

    xu = [r.bitcast(U32) for r in xio]

    def load_x(b):
        for jj in range(8):
            ev, od = _halves(xu[b][pl.ds(jj, R, stride=8), :].T)
            xs[_ds(b, 128), _ds(jj, R)] = ev
            xo[_ds(b, 128), _ds(jj, R)] = od

    m_i = jax.lax.broadcasted_iota(jnp.int32, (128, 128), 0)
    c_i = jax.lax.broadcasted_iota(jnp.int32, (128, 128), 1)
    perm = jnp.where(c_i == (m_i & 7) * 16 + (m_i >> 3), 1.0, 0.0).astype(BF16)

    def prep_w(g):
        for t in range(3):
            wt[g, _ds(t, 64), :] = _pack(_dot(perm, wqkv_ref[:, _ds((t + 1) % 3 * 4 + g, 128)], _NT))
        wot[:, _ds(g, 128)] = _pack(_dot(perm, wo_ref[_ds(g, 128), :]).T)

    def dft(rb, s):
        at, n = BLOCKS[rb]
        u = (un, uo)[s // 8][at // 2:(at + n) // 2, _ds(s % 8, R)]
        y = _dot(_unpack(u), _unpack(f_ref[s]))
        spec[rb][0:n, _ds(s, 2 * R)] = y
        return y[-8:, R:]

    def idft(rb, s):
        at, n = BLOCKS[rb]
        y = _dot(spec[rb][0:n, _ds(s, 2 * R)], _unpack(f_ref[s]), _NT)
        (xs, xo)[s // 8][at:at + n, _ds(s % 8, R)] += y
        return y[-8:]

    def load_spec(ref, rows, order):
        return [(ref[rows, _ds(2 * s, R)], ref[rows, _ds(2 * s + 1, R)]) for s in order]

    def store_spec(ref, rows, order, vals):
        for s, v in zip(order, vals):
            ref[rows, _ds(2 * s, R)] = v[0]
            ref[rows, _ds(2 * s + 1, R)] = v[1]

    slabs = [_slab(j) for j in range(NS)]

    def half(buf, rows, e8, bias=None):
        out = []
        for j in range(8):
            lo, hi = load_spec(buf, rows, [slabs[j], slabs[j + 8]])
            if j == 0 and bias is not None:
                lo = (lo[0] + bias, lo[1])
            out.append(_csub(lo, hi) if e8 else _cadd(lo, hi))
        return out

    def k_fft_steps(i):
        rows = _ds(i, 8)
        for e8 in (8, 0):
            quartics = _split(half(kspec, rows, e8, dskb[rows, :]), e8 // 2)
            for e4, p4 in zip((e8 // 2, e8 // 2 + 8), quartics):
                for e2, p2 in zip((e4 // 2, e4 // 2 + 8), _split(p4, e4 // 2)):
                    store_spec(khat, rows, _coeff_slots(e2), _factor_coeffs(p2, e2))
                yield

    def k_fft(i):
        for _ in k_fft_steps(i):
            pass

    def conv(rb, i, after=None):
        at, size = BLOCKS[rb]
        buf, rows, park = spec[rb], _ds(i, 8), _ds(size // 8, 8)
        for e8 in (8, 0):
            quartics = []
            for e4, p4 in zip((e8 // 2, e8 // 2 + 8), _split(half(buf, rows, e8), e8 // 2)):
                prods = [_factor_mul(p2, load_spec(khat, _ds(at // 8 + i, 8), _coeff_slots(e2)), e2)
                         for e2, p2 in zip((e4 // 2, e4 // 2 + 8), _split(p4, e4 // 2))]
                quartics.append(_merge(*prods, e4 // 2))
                if e4 < 8:
                    fence(khat, prods[1][1][0])
            mark = prods[1][1][0]
            fence(buf, mark if e8 or after is None else after)
            for j, v in enumerate(_merge(*quartics, e8 // 2)):
                if e8:
                    store_spec(buf, park, [j], [v])
                else:
                    (o,) = load_spec(buf, park, [j])
                    store_spec(buf, rows, [slabs[j], slabs[j + 8]], [_cadd(v, o), _csub(v, o)])
        return mark

    lane = jax.lax.broadcasted_iota(jnp.int32, (128, R), 1)

    def qkv(g, u, qs, ks, vs, i):
        y = _dot(_unpack(wt[g]), _unpack(u[0:D // 2, _ds(i, R)]))
        k, v, q = y[0:128], y[128:256], y[256:384]
        qs[:, _ds(i, R)] = q
        ks[:, _ds(i + 7, R)] = k
        vs[:, _ds(i + 7, R)] = v
        if i:
            ks[:, _ds(i - 1, R)] = pltpu.roll(k, 1, 1)
            vs[:, _ds(i - 1, R)] = jnp.where(lane == 0, va[:, _ds(7, R)], pltpu.roll(v, 1, 1))

    never = lane8 < zero_ref[0]

    def attend(g, qs, ks, vs, rs, o, i, ways, side=None):
        logits = []
        for w in range(W):
            lg = None
            for c in range(16):
                term = qs[_ds(c, 8), _ds(i, R)] * ks[_ds(c, 8), _ds(7 + i - w, R)]
                if c:
                    lg = lg + term
                else:
                    lg = term if w < ways else jnp.where(never, logits[w - ways], term)
            logits.append(lg)
            if side and w in (1, 7):
                fence(kspec, lg)
                next(side)
        scale = rs[7 + i] * 0.25
        logits = [lg * scale * rs[7 + i - w] for w, lg in enumerate(logits)]
        logits = [jnp.where(lane8 == 0, NEG, lg) if w > i else lg for w, lg in enumerate(logits)]
        mx = logits[0]
        for lg in logits[1:]:
            mx = jnp.maximum(mx, lg)
        es = [jnp.exp(lg - mx) for lg in logits]
        den = es[0]
        for e in es[1:]:
            den = den + e
        inv = 1.0 / den
        probs = [e * rs[7 + i - w] * inv for w, e in enumerate(es)]
        outs = []
        for c in range(16):
            acc = None
            for w in range(W):
                term = vs[_ds(c, 8), _ds(7 + i - w, R)] * probs[w]
                if w:
                    acc = acc + term
                else:
                    acc = term if c < ways else jnp.where(never, outs[c - ways], term)
            outs.append(acc)
            if side and c in (3, 11):
                fence(kspec, acc)
                next(side)
        o[_ds(g + 4, 64), _ds(i, R)] = _pack(jnp.concatenate(outs, axis=0))

    def chain_sum(vals, ways):
        parts = vals[:ways]
        for n, v in enumerate(vals[ways:]):
            parts[n % ways] = parts[n % ways] + v
        return jnp.sum(sum(parts[1:], parts[0]), axis=0, keepdims=True)

    def center(x, i, total, ways, after=None):
        parts = [total[_ds(n, 8)] for n in range(D // 8)]
        if after is not None:
            parts[0] = jnp.where(never, after, parts[0])
        c = x[:, _ds(i, R)] - chain_sum(parts, 2) * (1.0 / D)
        sq = c * c
        v = chain_sum([sq[_ds(n, 8)] for n in range(D // 8)], ways) * (1.0 / D)
        return c, jnp.broadcast_to(jax.lax.rsqrt(v + EPS), (8, R))

    def norm(x, u, rs, i, ways, after=None):
        c, r = center(x, i, x[:, _ds(i, R)], ways, after)
        u[0:D // 2, _ds(i, R)] = _pack(c)
        rs[7 + i] = r
        if i:
            rs[i - 1] = jnp.where(lane8 == 0, ra[7], pltpu.roll(r, 1, 1))
        return r

    def proj(x, o, u, i):
        y = x[:, _ds(i, R)] + _dot(_unpack(wot[...]), _unpack(o[D // 2:D, _ds(i, R)]))
        x[:, _ds(i, R)] = y
        cen[i % 2], r = center(x, i, y, 1)
        u[0:D // 2, _ds(i, R)] = _pack(cen[i % 2] * r[0:1])

    stores = [pltpu.make_async_copy(xio[c].at[0:L], o_hbm.at[:, c * 128:(c + 1) * 128], sems.at[c])
              for c in range(4)]

    def store_x(b, jj):
        t = pltpu.pack_elementwise(
            [xs[_ds(b, 128), _ds(jj, R)], xo[_ds(b, 128), _ds(jj, R)]], packed_dtype=BF16)
        xu[b][pl.ds(jj, R, stride=8), :] = pltpu.bitcast(t, U32).T

    def fence_io(b, val):
        xio[b][pl.ds(pl.multiple_of(L + zero_ref[0], 16), 16), :] = pltpu.bitcast(val, BF16)

    def start_store(b, val):
        stores[b].start()
        fence_io(b, val)
        return pltpu.bitcast(xio[b][L:L + 16, :], F32)

    def phase(name):
        def run(fn):
            with _scope(name):
                pl.when(zero_ref[0] == 0)(fn)
        return run

    @phase("prep")
    def _():
        dft_k(3)
        for b in range(4):
            load_x(b)
            prep_w(b)
            for n in range(6):
                k_fft(6 * b + n)

    even, odd = (un, (qa, ka, va), ra), (uo, (qb, kb, vb), rb_)

    def overlap(g_next, nxt, g, cur, k0):
        for i in range(8):
            qkv(g_next, nxt[0], *nxt[1], i)
            attend(g, *cur[1], cur[2], nxt[0], i, 2, None if k0 is None else k_fft_steps(k0 + i))

    for layer in range(2):
        @phase("a_pro")
        def _():
            if layer:
                for s in range(8):
                    idft(3, s)
            r = norm(xs, un, ra, 0, 4)
            for i in range(8):
                if layer:
                    idft(3, i + 8)
                qkv(0, un, qa, ka, va, i)
                if i < 7:
                    r = norm(xs, un, ra, i + 1, 2 - layer, r)
                r = norm(xo, uo, rb_, i, 2 - layer, r)

        def group(g, c):
            overlap(g, odd, g, even, None if layer else 8 * g + 24)

            @pl.when(g < 3)
            def _():
                overlap(g + 1, even, g, odd, None)

            return c

        with _scope("a_grp"):
            jax.lax.fori_loop(0, 4, group, 0)

        @phase("a_proj")
        def _():
            for i in range(8):
                proj(xs, uo, un, i)
                attend(3, qb, kb, vb, rb_, un, i, 1)
            for i in range(8):
                proj(xo, un, uo, i)
                if not layer:
                    k_fft(56 + i)
            for s in range(NS):
                dft(0, s)

        @phase("conv")
        def _():
            done = []
            for rb in range(4):
                for i in range(16):
                    for s in range(NS):
                        if rb < 3 and s * (16 - SKEW) // NS == i:
                            last = dft(rb + 1, s)
                        if rb and s * (16 - SKEW) // NS + SKEW == i:
                            last = idft(rb - 1, s)
                    if layer and rb >= 2 and i < 8:
                        store_x(rb - 2, i)
                        if i == 7:
                            last = start_store(rb - 2, last)
                    done.append(last)
                    mark = conv(rb, i, done[-LAG] if len(done) >= LAG else None)
                    if rb < 3:
                        fence(spec[rb + 1], mark)

    with _scope("store_x"):
        for jj in range(8):
            store_x(2, jj)
        fence_io(3, start_store(2, jnp.zeros((8, R), F32)))
        for jj in range(8):
            idft(3, jj)
            idft(3, jj + 8)
            store_x(3, jj)
        stores[3].start()
    with _scope("tail"):
        for cp in stores:
            cp.wait()


@jax.jit
def pallas_interleave_layers__sliding_local_dilated__ssm_conv_s4__prompt_kernel(
    A_x: jax.Array,
    A_wqkv: jax.Array,
    A_wo: jax.Array,
    B_u: jax.Array,
    B_A_re: jax.Array,
    B_A_im: jax.Array,
    B_B_re: jax.Array,
    B_B_im: jax.Array,
    B_C_re: jax.Array,
    B_C_im: jax.Array,
    B_log_dt: jax.Array,
    B_Dskip: jax.Array,
):
    del B_u
    f = _dft_matrix()
    lane = (np.arange(R) - 7) % R
    order = 16 * (lane % 8) + lane // 8
    fk = (f[:, order].astype(np.float32) * (2.0 / L)).astype(ml_dtypes.bfloat16)
    scratch = [
        pltpu.VMEM((D, L // 2), F32),
        pltpu.VMEM((D, L // 2), F32),
        pltpu.VMEM((D + 8, L // 2), U32),
        pltpu.VMEM((D + 8, L // 2), U32),
        pltpu.VMEM((4, 192, D), U32),
        pltpu.VMEM((D // 2, D), U32),
        pltpu.VMEM((D // 2, 128), U32),
        pltpu.VMEM((D, 128), F32),
        pltpu.VMEM((2, 10, 8, N), F32),
        pltpu.VMEM((2, 64, 2 * N), U32),
        *[pltpu.VMEM((n + 16, 2 * L), F32) for _, n in BLOCKS],
        pltpu.VMEM((D + 8, 2 * L), F32),
        pltpu.VMEM((D + 8, 22 * 2 * R), F32),
        pltpu.VMEM((128, 8 * R), F32),
        pltpu.VMEM((128, 15 * R), F32),
        pltpu.VMEM((128, 15 * R), F32),
        pltpu.VMEM((128, 8 * R), F32),
        pltpu.VMEM((128, 15 * R), F32),
        pltpu.VMEM((128, 15 * R), F32),
        pltpu.VMEM((15, 8, R), F32),
        pltpu.VMEM((15, 8, R), F32),
        pltpu.VMEM((2, D, R), F32),
        *[pltpu.VMEM((L + 16, 128), BF16)] * 4,
        pltpu.VMEM((D, 3 * D), BF16),
        pltpu.VMEM((D, D), BF16),
        pltpu.VMEM((NS, R // 2, 2 * R), U32),
        pltpu.VMEM((NS, R // 2, 2 * R), U32),
        pltpu.VMEM((6, D, N), BF16),
        pltpu.SMEM((1,), jnp.int32),
        pltpu.VMEM((D,), BF16),
        pltpu.VMEM((D,), BF16),
        pltpu.SemaphoreType.DMA((13,)),
    ]
    hbm = pl.BlockSpec(memory_space=pl.ANY)
    out = pl.pallas_call(
        _kernel,
        out_shape=jax.ShapeDtypeStruct((L, D), BF16),
        in_specs=[hbm] * 14,
        out_specs=hbm,
        scratch_shapes=scratch,
        compiler_params=pltpu.CompilerParams(vmem_limit_bytes=100 * 1024 * 1024),
    )(np.zeros((1,), np.int32), A_x.reshape(L, D), A_wqkv, A_wo, B_A_re, B_A_im, B_B_re, B_B_im, B_C_re, B_C_im,
      B_log_dt, B_Dskip, _pack_rows(f), _pack_rows(fk))
    return out.reshape(1, L, D)
```

```python
import contextlib

import jax
import jax.numpy as jnp
import jax.experimental.pallas as pl
import jax.experimental.pallas.tpu as pltpu
import ml_dtypes
import numpy as np

L = 2048
D = 512
N = 128
NS = 16
R = 128
W = 8
EPS = 1e-5
_H = float(np.sqrt(0.5))
LAG = 4
BLOCKS = ((0, 128), (128, 128), (256, 128), (384, 128))
F32 = jnp.float32
BF16 = jnp.bfloat16
U32 = jnp.uint32
NEG = float(ml_dtypes.bfloat16(-1e9))

_NT = (((1,), (1,)), ((), ()))


def _slab(j):
    return (j % 2) * 8 + j // 2


def _dft_matrix():
    r = np.arange(R)
    k = np.arange(R) + 0.5
    f = np.zeros((NS, R, 2 * R), np.float64)
    for j in range(NS):
        th = 2.0 * np.pi * np.outer(NS * r + j, k) / (2 * L)
        f[_slab(j), :, :R] = np.cos(th)
        f[_slab(j), :, R:] = -np.sin(th)
    return f.astype(np.float32).astype(ml_dtypes.bfloat16)


def _pack_rows(a):
    u = np.ascontiguousarray(a).view(np.uint16).astype(np.uint32)
    return u[:, 0::2] | (u[:, 1::2] << np.uint32(16))


def _lag_tables():
    rho = []
    for s in range(8):
        lag = (256 * s + np.arange(NS)).astype(np.float32)
        rho.append([int(v) - 256 * s for v in lag.astype(ml_dtypes.bfloat16).astype(np.float32)])
    return rho


_RHO = _lag_tables()


def _cmul(a, b):
    return (a[0] * b[0] - a[1] * b[1], a[0] * b[1] + a[1] * b[0])


def _csq(a):
    t = a[0] * a[1]
    return ((a[0] - a[1]) * (a[0] + a[1]), t + t)


def _cadd(a, b):
    return (a[0] + b[0], a[1] + b[1])


def _csub(a, b):
    return (a[0] - b[0], a[1] - b[1])


def _split(p, e):
    plus, minus = [], []
    for lo, hi in zip(p[:len(p) // 2], p[len(p) // 2:]):
        if e % 4:
            hi = ((hi[0] - hi[1]) * _H, (hi[0] + hi[1]) * _H)
        if e >= 4:
            plus.append((lo[0] - hi[1], lo[1] + hi[0]))
            minus.append((lo[0] + hi[1], lo[1] - hi[0]))
        else:
            plus.append(_cadd(lo, hi))
            minus.append(_csub(lo, hi))
    return plus, minus


def _merge(plus, minus, e):
    lo, hi = [], []
    for p, m in zip(plus, minus):
        lo.append(_cadd(p, m))
        d = (p[1] - m[1], m[0] - p[0]) if e >= 4 else _csub(p, m)
        hi.append(((d[0] + d[1]) * _H, (d[1] - d[0]) * _H) if e % 4 else d)
    return lo + hi


def _factor_coeffs(k, e):
    if e % 8 == 0:
        (p,), (m,) = _split(k, e // 2)
        return [(p[0] * 0.5, p[1] * 0.5), (m[0] * 0.5, m[1] * 0.5)]
    c, s = float(np.cos(np.pi * e / 8)), float(np.sin(np.pi * e / 8))
    wk = (k[1][0] * c - k[1][1] * s, k[1][0] * s + k[1][1] * c)
    return [k[0], _csub(wk, k[0]), _csub(k[1], k[0])]


def _factor_mul(a, coeffs, e):
    if e % 8 == 0:
        (p,), (m,) = _split(a, e // 2)
        return _merge([_cmul(p, coeffs[0])], [_cmul(m, coeffs[1])], e // 2)
    t = _cmul(_cadd(a[0], a[1]), coeffs[0])
    return [_cadd(t, _cmul(a[1], coeffs[1])), _cadd(t, _cmul(a[0], coeffs[2]))]


def _coeff_slots(e):
    if e % 8 == 0:
        return [e // 4, e // 4 + 1]
    n = 4 + 3 * [2, 4, 6, 10, 12, 14].index(e)
    return [n, n + 1, n + 2]


def _scope(name):
    return contextlib.nullcontext()


def _ds(i, n):
    if isinstance(i, int):
        return slice(i * n, (i + 1) * n)
    return pl.ds(pl.multiple_of(i * n, n), n)


def _pack(x):
    return pltpu.bitcast(x.astype(BF16), U32)


def _unpack(x):
    return pltpu.bitcast(x, BF16)


def _dot(a, b, dims=(((1,), (0,)), ((), ()))):
    return jax.lax.dot_general(a, b, dims, preferred_element_type=F32)


def _halves(u):
    return pltpu.bitcast(u << 16, F32), pltpu.bitcast(u & jnp.uint32(0xFFFF0000), F32)


def _kernel(zero_hbm, x_hbm, wqkv_hbm, wo_hbm, are, aim, bre, bim, cre, cim,
            ldt_hbm, dsk_hbm, f_hbm, fk_hbm, o_hbm,
            xs, xo, un, uo, wt, wot, dtb, dskb, pw_ref, rhs_ref, s0, s1, s2, s3, kspec, khat, qa, ka, va, qb, kb, vb,
            ra, rb_, cen,
            io0, io1, io2, io3, wqkv_ref, wo_ref, f_ref, fk_ref, ssm, zero_ref, ldt_ref, dsk_ref, sems):
    def fetch_ssm(rows, sem):
        return [pltpu.make_async_copy(p.at[rows], ssm.at[n, rows], sem)
                for n, p in enumerate((are, aim, bre, bim, cre, cim))]

    small = [pltpu.make_async_copy(src, dst, sems.at[10 + n]) for n, (src, dst) in enumerate(
        [(zero_hbm, zero_ref), (ldt_hbm, ldt_ref), (dsk_hbm, dsk_ref)])]
    for cp in small:
        cp.start()
    first = fetch_ssm(pl.ds(0, 144), sems.at[8])
    for cp in first:
        cp.start()
    second = fetch_ssm(pl.ds(144, D - 144), sems.at[9])
    second += [pltpu.make_async_copy(fk_hbm, fk_ref, sems.at[4])]
    for cp in second:
        cp.start()
    xio = (io0, io1, io2, io3)
    loads = []
    loads += [pltpu.make_async_copy(x_hbm.at[:, c * 128:(c + 1) * 128], xio[c].at[0:L], sems.at[c])
              for c in range(4)]
    loads += [pltpu.make_async_copy(src, dst, sems.at[5 + n]) for n, (src, dst) in enumerate(
        [(wqkv_hbm, wqkv_ref), (wo_hbm, wo_ref), (f_hbm, f_ref)])]

    spec = (s0, s1, s2, s3)

    def fence(ref, val):
        row = ref.shape[0] - 8 + zero_ref[0]
        ref[pl.ds(pl.multiple_of(row, 8), 8), 0:128] = val

    for cp in small:
        cp.wait()
    dt_row = jnp.exp(ldt_ref[...].astype(F32)).reshape(1, D)
    dtb[...] = _pack(jnp.broadcast_to(dt_row, (128, D)).T)
    dskb[...] = jnp.broadcast_to(dsk_ref[...].astype(F32).reshape(1, D) * (2.0 / L), (128, D)).T

    lane8 = jax.lax.broadcasted_iota(jnp.int32, (8, R), 1)
    rev8 = 7 - jax.lax.broadcasted_iota(jnp.int32, (8, N), 0)
    steps = (1, 2, 4, 8, 256)

    def powers(i):
        dts = _halves(dtb[_ds(i, 8), :])
        are, aim, bre, bim, cre, cim = [
            _halves(pltpu.bitcast(ssm[n, _ds(i, 16), :], U32)) for n in range(6)]
        for h in range(2):
            dt = dts[h]
            li = dt * aim[h]
            mag = jnp.exp(dt * are[h])
            zp = {1: (mag * jnp.cos(li), mag * jnp.sin(li))}
            for e in (1, 2, 4, 8, 16, 32, 64, 128):
                zp[2 * e] = _csq(zp[e])
            w = _cmul((cre[h], cim[h]), (dt * bre[h], dt * bim[h]))
            for n, v in enumerate(zp[e] for e in steps):
                pw_ref[h, 2 * n] = v[0]
                pw_ref[h, 2 * n + 1] = v[1]
            w, step = [(jnp.take_along_axis(v[0], rev8, axis=0), -jnp.take_along_axis(v[1], rev8, axis=0))
                       for v in (w, zp[16])]
            pw = [w]
            for b in range(1, 16):
                pw.append(_cmul(pw[-1], step))
            rhs_ref[h] = _pack(jnp.concatenate([jnp.concatenate(v, axis=1) for v in pw], axis=0))

    keys = [(s, p) for s in range(8) for p in sorted(set(_RHO[s]) - {16})] + [(8, 0)]

    def taps(i):
        outs = []
        for h in range(2):
            zp = {e: (pw_ref[h, 2 * n], pw_ref[h, 2 * n + 1]) for n, e in enumerate(steps)}
            zp[0] = (jnp.ones((8, N), F32), jnp.zeros((8, N), F32))
            lhs = []
            for n, (s, p) in enumerate(keys):
                e = 256 * s + p
                if e not in zp:
                    if e % 2 == 0 and e // 2 in zp:
                        zp[e] = _csq(zp[e // 2])
                    else:
                        inc = p - keys[n - 1][1] if p else 256
                        zp[e] = _cmul(zp[e - inc], zp[inc])
                lhs.append(jnp.concatenate(zp[e], axis=1))
            outs.append(_dot(jnp.concatenate(lhs, axis=0), _unpack(rhs_ref[h]), _NT))
        both = pltpu.bitcast(pltpu.pack_elementwise(outs, packed_dtype=BF16), U32)
        piece = {}
        for n, (s, p) in enumerate(keys):
            piece[s, p] = pltpu.roll(both[8 * n:8 * n + 8], 126 - 7 if s == 8 else s, 1,
                                     stride=1, stride_axis=0)
        memo = {}
        for j in range(NS):
            key = ()
            acc = None
            for s in range(7, -1, -1):
                key = key + (_RHO[s][j],)
                if key not in memo:
                    pc = carry if _RHO[s][j] == 16 else piece[s, _RHO[s][j]]
                    same = acc is None or pc is acc
                    memo[key] = pc if same else jnp.where(((lane8 + 1) & 7) == s, pc, acc)
                acc = memo[key]
            (un, uo)[j % 2][_ds(i + D // 16, 8), _ds(j // 2, R)] = acc
            if j == 0:
                last_b = ((lane8 + 1) & 127) < 8
                carry = jnp.where(last_b, pltpu.roll(acc, 128 - 9, 1), pltpu.roll(acc, 128 - 8, 1))
                carry = jnp.where(lane8 == 6, pltpu.roll(piece[8, 0], 8, 1), carry)

    def gen_k(rb):
        for n in range(8):
            i = 8 * rb + n
            taps(i)
            powers(jnp.minimum(i + 1, D // 16 - 1))

    def dft_k(rb):
        for s in range(NS):
            u = (un, uo)[s // 8][_ds(rb + 4, 64), _ds(s % 8, R)]
            kspec[_ds(rb, 128), _ds(s, 2 * R)] = _dot(_unpack(u), _unpack(fk_ref[s]))

    def gen_step(rb, c):
        dft_k(rb - 1)
        gen_k(rb)
        return c

    with _scope("head"):
        for cp in first:
            cp.wait()
        for cp in loads:
            cp.start()

    with _scope("gen_k"):
        powers(0)
        gen_k(0)
        for cp in second:
            cp.wait()
        jax.lax.fori_loop(1, 4, gen_step, 0)

    for cp in loads:
        cp.wait()

    xu = [r.bitcast(U32) for r in xio]

    def load_x(b):
        for jj in range(8):
            ev, od = _halves(xu[b][pl.ds(jj, R, stride=8), :].T)
            xs[_ds(b, 128), _ds(jj, R)] = ev
            xo[_ds(b, 128), _ds(jj, R)] = od

    m_i = jax.lax.broadcasted_iota(jnp.int32, (128, 128), 0)
    c_i = jax.lax.broadcasted_iota(jnp.int32, (128, 128), 1)
    perm = jnp.where(c_i == (m_i & 7) * 16 + (m_i >> 3), 1.0, 0.0).astype(BF16)

    def prep_w(g):
        for t in range(3):
            wt[g, _ds(t, 64), :] = _pack(_dot(perm, wqkv_ref[:, _ds((t + 1) % 3 * 4 + g, 128)], _NT))
        wot[:, _ds(g, 128)] = _pack(_dot(perm, wo_ref[_ds(g, 128), :]).T)

    def dft(rb, s):
        at, n = BLOCKS[rb]
        u = (un, uo)[s // 8][at // 2:(at + n) // 2, _ds(s % 8, R)]
        y = _dot(_unpack(u), _unpack(f_ref[s]))
        spec[rb][0:n, _ds(s, 2 * R)] = y
        return y[-8:, R:]

    def idft(rb, s):
        at, n = BLOCKS[rb]
        y = _dot(spec[rb][0:n, _ds(s, 2 * R)], _unpack(f_ref[s]), _NT)
        (xs, xo)[s // 8][at:at + n, _ds(s % 8, R)] += y
        return y[-8:]

    def load_spec(ref, rows, order):
        return [(ref[rows, _ds(2 * s, R)], ref[rows, _ds(2 * s + 1, R)]) for s in order]

    def store_spec(ref, rows, order, vals):
        for s, v in zip(order, vals):
            ref[rows, _ds(2 * s, R)] = v[0]
            ref[rows, _ds(2 * s + 1, R)] = v[1]

    slabs = [_slab(j) for j in range(NS)]

    def half(buf, rows, e8, bias=None):
        out = []
        for j in range(8):
            lo, hi = load_spec(buf, rows, [slabs[j], slabs[j + 8]])
            if j == 0 and bias is not None:
                lo = (lo[0] + bias, lo[1])
            out.append(_csub(lo, hi) if e8 else _cadd(lo, hi))
        return out

    def k_fft_steps(i):
        rows = _ds(i, 8)
        for e8 in (8, 0):
            quartics = _split(half(kspec, rows, e8, dskb[rows, :]), e8 // 2)
            for e4, p4 in zip((e8 // 2, e8 // 2 + 8), quartics):
                for e2, p2 in zip((e4 // 2, e4 // 2 + 8), _split(p4, e4 // 2)):
                    store_spec(khat, rows, _coeff_slots(e2), _factor_coeffs(p2, e2))
                yield

    def k_fft(i):
        for _ in k_fft_steps(i):
            pass

    def conv(rb, i, after=None):
        at, size = BLOCKS[rb]
        buf, rows, park = spec[rb], _ds(i, 8), _ds(size // 8, 8)
        for e8 in (8, 0):
            quartics = []
            for e4, p4 in zip((e8 // 2, e8 // 2 + 8), _split(half(buf, rows, e8), e8 // 2)):
                prods = [_factor_mul(p2, load_spec(khat, _ds(at // 8 + i, 8), _coeff_slots(e2)), e2)
                         for e2, p2 in zip((e4 // 2, e4 // 2 + 8), _split(p4, e4 // 2))]
                quartics.append(_merge(*prods, e4 // 2))
                if e4 < 8:
                    fence(khat, prods[1][1][0])
            mark = prods[1][1][0]
            fence(buf, mark if e8 or after is None else after)
            for j, v in enumerate(_merge(*quartics, e8 // 2)):
                if e8:
                    store_spec(buf, park, [j], [v])
                else:
                    (o,) = load_spec(buf, park, [j])
                    store_spec(buf, rows, [slabs[j], slabs[j + 8]], [_cadd(v, o), _csub(v, o)])
        return mark

    lane = jax.lax.broadcasted_iota(jnp.int32, (128, R), 1)

    def qkv(g, u, qs, ks, vs, i):
        y = _dot(_unpack(wt[g]), _unpack(u[0:D // 2, _ds(i, R)]))
        k, v, q = y[0:128], y[128:256], y[256:384]
        qs[:, _ds(i, R)] = q
        ks[:, _ds(i + 7, R)] = k
        vs[:, _ds(i + 7, R)] = v
        if i:
            ks[:, _ds(i - 1, R)] = pltpu.roll(k, 1, 1)
            vs[:, _ds(i - 1, R)] = jnp.where(lane == 0, va[:, _ds(7, R)], pltpu.roll(v, 1, 1))

    never = lane8 < zero_ref[0]

    def attend(g, qs, ks, vs, rs, o, i, ways, side=None):
        logits = []
        for w in range(W):
            lg = None
            for c in range(16):
                term = qs[_ds(c, 8), _ds(i, R)] * ks[_ds(c, 8), _ds(7 + i - w, R)]
                if c:
                    lg = lg + term
                else:
                    lg = term if w < ways else jnp.where(never, logits[w - ways], term)
            logits.append(lg)
            if side and w in (1, 7):
                fence(kspec, lg)
                next(side)
        scale = rs[7 + i] * 0.25
        logits = [lg * scale * rs[7 + i - w] for w, lg in enumerate(logits)]
        logits = [jnp.where(lane8 == 0, NEG, lg) if w > i else lg for w, lg in enumerate(logits)]
        mx = logits[0]
        for lg in logits[1:]:
            mx = jnp.maximum(mx, lg)
        es = [jnp.exp(lg - mx) for lg in logits]
        den = es[0]
        for e in es[1:]:
            den = den + e
        inv = 1.0 / den
        probs = [e * rs[7 + i - w] * inv for w, e in enumerate(es)]
        outs = []
        for c in range(16):
            acc = None
            for w in range(W):
                term = vs[_ds(c, 8), _ds(7 + i - w, R)] * probs[w]
                if w:
                    acc = acc + term
                else:
                    acc = term if c < ways else jnp.where(never, outs[c - ways], term)
            outs.append(acc)
            if side and c in (3, 11):
                fence(kspec, acc)
                next(side)
        o[_ds(g + 4, 64), _ds(i, R)] = _pack(jnp.concatenate(outs, axis=0))

    def chain_sum(vals, ways):
        parts = vals[:ways]
        for n, v in enumerate(vals[ways:]):
            parts[n % ways] = parts[n % ways] + v
        return jnp.sum(sum(parts[1:], parts[0]), axis=0, keepdims=True)

    def center(x, i, total, ways, after=None):
        parts = [total[_ds(n, 8)] for n in range(D // 8)]
        if after is not None:
            parts[0] = jnp.where(never, after, parts[0])
        c = x[:, _ds(i, R)] - chain_sum(parts, 2) * (1.0 / D)
        sq = c * c
        v = chain_sum([sq[_ds(n, 8)] for n in range(D // 8)], ways) * (1.0 / D)
        return c, jnp.broadcast_to(jax.lax.rsqrt(v + EPS), (8, R))

    def norm(x, u, rs, i, ways, after=None):
        c, r = center(x, i, x[:, _ds(i, R)], ways, after)
        u[0:D // 2, _ds(i, R)] = _pack(c)
        rs[7 + i] = r
        if i:
            rs[i - 1] = jnp.where(lane8 == 0, ra[7], pltpu.roll(r, 1, 1))
        return r

    def proj(x, o, u, i):
        y = x[:, _ds(i, R)] + _dot(_unpack(wot[...]), _unpack(o[D // 2:D, _ds(i, R)]))
        x[:, _ds(i, R)] = y
        cen[i % 2], r = center(x, i, y, 1)
        u[0:D // 2, _ds(i, R)] = _pack(cen[i % 2] * r[0:1])

    stores = [pltpu.make_async_copy(xio[c].at[0:L], o_hbm.at[:, c * 128:(c + 1) * 128], sems.at[c])
              for c in range(4)]

    def store_x(b, jj):
        t = pltpu.pack_elementwise(
            [xs[_ds(b, 128), _ds(jj, R)], xo[_ds(b, 128), _ds(jj, R)]], packed_dtype=BF16)
        xu[b][pl.ds(jj, R, stride=8), :] = pltpu.bitcast(t, U32).T

    def fence_io(b, val):
        xio[b][pl.ds(pl.multiple_of(L + zero_ref[0], 16), 16), :] = pltpu.bitcast(val, BF16)

    def start_store(b, val):
        stores[b].start()
        fence_io(b, val)
        return pltpu.bitcast(xio[b][L:L + 16, :], F32)

    def phase(name):
        def run(fn):
            with _scope(name):
                pl.when(zero_ref[0] == 0)(fn)
        return run

    @phase("prep")
    def _():
        dft_k(3)
        for b in range(4):
            load_x(b)
            prep_w(b)
            for n in range(6):
                k_fft(6 * b + n)

    even, odd = (un, (qa, ka, va), ra), (uo, (qb, kb, vb), rb_)

    def overlap(g_next, nxt, g, cur, k0):
        for i in range(8):
            qkv(g_next, nxt[0], *nxt[1], i)
            attend(g, *cur[1], cur[2], nxt[0], i, 2, None if k0 is None else k_fft_steps(k0 + i))

    for layer in range(2):
        @phase("a_pro")
        def _():
            if layer:
                for s in range(8):
                    idft(3, s)
            r = norm(xs, un, ra, 0, 4)
            for i in range(8):
                if layer:
                    idft(3, i + 8)
                qkv(0, un, qa, ka, va, i)
                if i < 7:
                    r = norm(xs, un, ra, i + 1, 2 - layer, r)
                r = norm(xo, uo, rb_, i, 2 - layer, r)

        def group(g, c):
            overlap(g, odd, g, even, None if layer else 8 * g + 24)

            @pl.when(g < 3)
            def _():
                overlap(g + 1, even, g, odd, None)

            return c

        with _scope("a_grp"):
            jax.lax.fori_loop(0, 4, group, 0)

        @phase("a_proj")
        def _():
            for i in range(8):
                proj(xs, uo, un, i)
                attend(3, qb, kb, vb, rb_, un, i, 1)
            for i in range(8):
                proj(xo, un, uo, i)
                if not layer:
                    k_fft(56 + i)
            for s in range(NS):
                dft(0, s)

        @phase("conv")
        def _():
            done = []
            for rb in range(4):
                for i in range(16):
                    if rb < 3:
                        last = dft(rb + 1, i)
                    if layer and rb == 3:
                        if i < 8:
                            idft(2, i)
                            last = idft(2, i + 8)
                        else:
                            store_x(2, i - 8)
                    elif rb:
                        last = idft(rb - 1, i)
                    if layer and rb >= 2 and i < 8:
                        store_x(rb - 2, i)
                        if i == 7:
                            last = start_store(rb - 2, last)
                    done.append(last)
                    mark = conv(rb, i, done[-LAG] if len(done) >= LAG else None)
                    if rb < 3:
                        fence(spec[rb + 1], mark)

    with _scope("store_x"):
        last = start_store(2, jnp.zeros((8, R), F32))
        fence(spec[3], last)
        for jj in range(8):
            idft(3, jj)
            idft(3, jj + 8)
            store_x(3, jj)
        stores[3].start()
    with _scope("tail"):
        for cp in stores:
            cp.wait()


@jax.jit
def pallas_interleave_layers__sliding_local_dilated__ssm_conv_s4__prompt_kernel(
    A_x: jax.Array,
    A_wqkv: jax.Array,
    A_wo: jax.Array,
    B_u: jax.Array,
    B_A_re: jax.Array,
    B_A_im: jax.Array,
    B_B_re: jax.Array,
    B_B_im: jax.Array,
    B_C_re: jax.Array,
    B_C_im: jax.Array,
    B_log_dt: jax.Array,
    B_Dskip: jax.Array,
):
    del B_u
    f = _dft_matrix()
    lane = (np.arange(R) - 7) % R
    order = 16 * (lane % 8) + lane // 8
    fk = (f[:, order].astype(np.float32) * (2.0 / L)).astype(ml_dtypes.bfloat16)
    scratch = [
        pltpu.VMEM((D, L // 2), F32),
        pltpu.VMEM((D, L // 2), F32),
        pltpu.VMEM((D + 8, L // 2), U32),
        pltpu.VMEM((D + 8, L // 2), U32),
        pltpu.VMEM((4, 192, D), U32),
        pltpu.VMEM((D // 2, D), U32),
        pltpu.VMEM((D // 2, 128), U32),
        pltpu.VMEM((D, 128), F32),
        pltpu.VMEM((2, 10, 8, N), F32),
        pltpu.VMEM((2, 64, 2 * N), U32),
        *[pltpu.VMEM((n + 16, 2 * L), F32) for _, n in BLOCKS],
        pltpu.VMEM((D + 8, 2 * L), F32),
        pltpu.VMEM((D + 8, 22 * 2 * R), F32),
        pltpu.VMEM((128, 8 * R), F32),
        pltpu.VMEM((128, 15 * R), F32),
        pltpu.VMEM((128, 15 * R), F32),
        pltpu.VMEM((128, 8 * R), F32),
        pltpu.VMEM((128, 15 * R), F32),
        pltpu.VMEM((128, 15 * R), F32),
        pltpu.VMEM((15, 8, R), F32),
        pltpu.VMEM((15, 8, R), F32),
        pltpu.VMEM((2, D, R), F32),
        *[pltpu.VMEM((L + 16, 128), BF16)] * 4,
        pltpu.VMEM((D, 3 * D), BF16),
        pltpu.VMEM((D, D), BF16),
        pltpu.VMEM((NS, R // 2, 2 * R), U32),
        pltpu.VMEM((NS, R // 2, 2 * R), U32),
        pltpu.VMEM((6, D, N), BF16),
        pltpu.SMEM((1,), jnp.int32),
        pltpu.VMEM((D,), BF16),
        pltpu.VMEM((D,), BF16),
        pltpu.SemaphoreType.DMA((13,)),
    ]
    hbm = pl.BlockSpec(memory_space=pl.ANY)
    out = pl.pallas_call(
        _kernel,
        out_shape=jax.ShapeDtypeStruct((L, D), BF16),
        in_specs=[hbm] * 14,
        out_specs=hbm,
        scratch_shapes=scratch,
        compiler_params=pltpu.CompilerParams(vmem_limit_bytes=100 * 1024 * 1024),
    )(np.zeros((1,), np.int32), A_x.reshape(L, D), A_wqkv, A_wo, B_A_re, B_A_im, B_B_re, B_B_im, B_C_re, B_C_im,
      B_log_dt, B_Dskip, _pack_rows(f), _pack_rows(fk))
    return out.reshape(1, L, D)
```

```python
import contextlib

import jax
import jax.numpy as jnp
import jax.experimental.pallas as pl
import jax.experimental.pallas.tpu as pltpu
import ml_dtypes
import numpy as np

L = 2048
D = 512
N = 128
NS = 16
R = 128
W = 8
EPS = 1e-5
_H = float(np.sqrt(0.5))
LAG = 4
BLOCKS = ((0, 128), (128, 128), (256, 128), (384, 128))
F32 = jnp.float32
BF16 = jnp.bfloat16
U32 = jnp.uint32
NEG = float(ml_dtypes.bfloat16(-1e9))

_NT = (((1,), (1,)), ((), ()))


def _slab(j):
    return (j % 2) * 8 + j // 2


def _dft_matrix():
    r = np.arange(R)
    k = np.arange(R) + 0.5
    f = np.zeros((NS, R, 2 * R), np.float64)
    for j in range(NS):
        th = 2.0 * np.pi * np.outer(NS * r + j, k) / (2 * L)
        f[_slab(j), :, :R] = np.cos(th)
        f[_slab(j), :, R:] = -np.sin(th)
    return f.astype(np.float32).astype(ml_dtypes.bfloat16)


def _pack_rows(a):
    u = np.ascontiguousarray(a).view(np.uint16).astype(np.uint32)
    return u[:, 0::2] | (u[:, 1::2] << np.uint32(16))


def _lag_tables():
    rho = []
    for s in range(8):
        lag = (256 * s + np.arange(NS)).astype(np.float32)
        rho.append([int(v) - 256 * s for v in lag.astype(ml_dtypes.bfloat16).astype(np.float32)])
    return rho


_RHO = _lag_tables()


def _cmul(a, b):
    return (a[0] * b[0] - a[1] * b[1], a[0] * b[1] + a[1] * b[0])


def _csq(a):
    t = a[0] * a[1]
    return ((a[0] - a[1]) * (a[0] + a[1]), t + t)


def _cadd(a, b):
    return (a[0] + b[0], a[1] + b[1])


def _csub(a, b):
    return (a[0] - b[0], a[1] - b[1])


def _split(p, e):
    plus, minus = [], []
    for lo, hi in zip(p[:len(p) // 2], p[len(p) // 2:]):
        if e % 4:
            hi = ((hi[0] - hi[1]) * _H, (hi[0] + hi[1]) * _H)
        if e >= 4:
            plus.append((lo[0] - hi[1], lo[1] + hi[0]))
            minus.append((lo[0] + hi[1], lo[1] - hi[0]))
        else:
            plus.append(_cadd(lo, hi))
            minus.append(_csub(lo, hi))
    return plus, minus


def _merge(plus, minus, e):
    lo, hi = [], []
    for p, m in zip(plus, minus):
        lo.append(_cadd(p, m))
        d = (p[1] - m[1], m[0] - p[0]) if e >= 4 else _csub(p, m)
        hi.append(((d[0] + d[1]) * _H, (d[1] - d[0]) * _H) if e % 4 else d)
    return lo + hi


def _factor_coeffs(k, e):
    if e % 8 == 0:
        (p,), (m,) = _split(k, e // 2)
        return [(p[0] * 0.5, p[1] * 0.5), (m[0] * 0.5, m[1] * 0.5)]
    c, s = float(np.cos(np.pi * e / 8)), float(np.sin(np.pi * e / 8))
    wk = (k[1][0] * c - k[1][1] * s, k[1][0] * s + k[1][1] * c)
    return [k[0], _csub(wk, k[0]), _csub(k[1], k[0])]


def _factor_mul(a, coeffs, e):
    if e % 8 == 0:
        (p,), (m,) = _split(a, e // 2)
        return _merge([_cmul(p, coeffs[0])], [_cmul(m, coeffs[1])], e // 2)
    t = _cmul(_cadd(a[0], a[1]), coeffs[0])
    return [_cadd(t, _cmul(a[1], coeffs[1])), _cadd(t, _cmul(a[0], coeffs[2]))]


def _coeff_slots(e):
    if e % 8 == 0:
        return [e // 4, e // 4 + 1]
    n = 4 + 3 * [2, 4, 6, 10, 12, 14].index(e)
    return [n, n + 1, n + 2]


def _scope(name):
    return contextlib.nullcontext()


def _ds(i, n):
    if isinstance(i, int):
        return slice(i * n, (i + 1) * n)
    return pl.ds(pl.multiple_of(i * n, n), n)


def _pack(x):
    return pltpu.bitcast(x.astype(BF16), U32)


def _unpack(x):
    return pltpu.bitcast(x, BF16)


def _dot(a, b, dims=(((1,), (0,)), ((), ()))):
    return jax.lax.dot_general(a, b, dims, preferred_element_type=F32)


def _halves(u):
    return pltpu.bitcast(u << 16, F32), pltpu.bitcast(u & jnp.uint32(0xFFFF0000), F32)


def _kernel(zero_hbm, x_hbm, wqkv_hbm, wo_hbm, are, aim, bre, bim, cre, cim,
            ldt_hbm, dsk_hbm, f_hbm, fk_hbm, o_hbm,
            xs, xo, un, uo, wt, wot, dtb, dskb, pw_ref, rhs_ref, s0, s1, s2, s3, kspec, khat, qa, ka, va, qb, kb, vb,
            ra, rb_, cen,
            io0, io1, io2, io3, wqkv_ref, wo_ref, f_ref, fk_ref, ssm, zero_ref, ldt_ref, dsk_ref, sems):
    def fetch_ssm(rows, sem):
        return [pltpu.make_async_copy(p.at[rows], ssm.at[n, rows], sem)
                for n, p in enumerate((are, aim, bre, bim, cre, cim))]

    small = [pltpu.make_async_copy(src, dst, sems.at[10 + n]) for n, (src, dst) in enumerate(
        [(zero_hbm, zero_ref), (ldt_hbm, ldt_ref), (dsk_hbm, dsk_ref)])]
    for cp in small:
        cp.start()
    first = fetch_ssm(pl.ds(0, 144), sems.at[8])
    for cp in first:
        cp.start()
    second = fetch_ssm(pl.ds(144, D - 144), sems.at[9])
    second += [pltpu.make_async_copy(fk_hbm, fk_ref, sems.at[4])]
    for cp in second:
        cp.start()
    xio = (io0, io1, io2, io3)
    loads = []
    loads += [pltpu.make_async_copy(x_hbm.at[:, c * 128:(c + 1) * 128], xio[c].at[0:L], sems.at[c])
              for c in range(4)]
    loads += [pltpu.make_async_copy(src, dst, sems.at[5 + n]) for n, (src, dst) in enumerate(
        [(wqkv_hbm, wqkv_ref), (wo_hbm, wo_ref), (f_hbm, f_ref)])]

    spec = (s0, s1, s2, s3)

    def fence(ref, val):
        row = ref.shape[0] - 8 + zero_ref[0]
        ref[pl.ds(pl.multiple_of(row, 8), 8), 0:128] = val

    for cp in small:
        cp.wait()
    dt_row = jnp.exp(ldt_ref[...].astype(F32)).reshape(1, D)
    dtb[...] = _pack(jnp.broadcast_to(dt_row, (128, D)).T)
    dskb[...] = jnp.broadcast_to(dsk_ref[...].astype(F32).reshape(1, D) * (2.0 / L), (128, D)).T

    lane8 = jax.lax.broadcasted_iota(jnp.int32, (8, R), 1)
    sub8 = jax.lax.broadcasted_iota(jnp.int32, (8, N), 0)
    low = sub8 < 4
    steps = (1, 2, 4, 256)

    def halves_of(a, b):
        return tuple(jnp.where(low, u, v) for u, v in zip(a, b))

    def powers(i):
        dts = _halves(dtb[_ds(i, 8), :])
        are, aim, bre, bim, cre, cim = [
            _halves(pltpu.bitcast(ssm[n, _ds(i, 16), :], U32)) for n in range(6)]
        for h in range(2):
            dt = dts[h]
            li = dt * aim[h]
            mag = jnp.exp(dt * are[h])
            zp = {1: (mag * jnp.cos(li), mag * jnp.sin(li))}
            for e in (1, 2, 4, 8, 16, 32, 64, 128):
                zp[2 * e] = _csq(zp[e])
            for n, e in enumerate(steps):
                pw_ref[h, 2 * n] = zp[e][0]
                pw_ref[h, 2 * n + 1] = zp[e][1]
            w = _cmul((cre[h], cim[h]), (dt * bre[h], dt * bim[h]))
            w, z8, z16 = [(v[0], -v[1]) for v in (w, zp[8], zp[16])]
            w8 = _cmul(w, z8)
            for t in range(2):
                def pick(v):
                    return tuple(jnp.take_along_axis(u, 4 * t + 3 - (sub8 & 3), axis=0) for u in v)

                step = pick(z16)
                rows = [halves_of(pick(w), pick(w8)) if t else halves_of(pick(w8), pick(_cmul(w, z16)))]
                for _ in range(15):
                    rows.append(_cmul(rows[-1], step))
                if not t:
                    rows = [halves_of(rows[-1], pick(w))] + rows[:-1]
                rhs_ref[2 * h + t] = jnp.concatenate([jnp.concatenate(v, axis=1) for v in rows], axis=0)

    offsets = sorted({256 * s + p % 8 for s in range(8) for p in _RHO[s]}) + [L]
    plain, turned = offsets[:11], offsets[11:]

    def turn(v):
        return pltpu.roll(v, 4, 0)

    def taps(i):
        outs = []
        for h in range(2):
            zp = {e: (pw_ref[h, 2 * n], pw_ref[h, 2 * n + 1]) for n, e in enumerate(steps)}
            zp[0] = (jnp.ones((8, N), F32), jnp.zeros((8, N), F32))
            zt = {e: (turn(zp[e][0]), turn(zp[e][1])) for e in (4, 256)}
            for table, exps in ((zp, plain + turned[:1]), (zt, turned[1:])):
                for e in exps:
                    if e in table:
                        continue
                    if e % 2 == 0 and e // 2 in table:
                        table[e] = _csq(table[e // 2])
                    else:
                        inc = next(v for v in steps if v in table and e - v in table)
                        table[e] = _cmul(table[e - inc], table[inc])
            zt[turned[0]] = tuple(turn(v) for v in zp[turned[0]])
            pairs = [(zp[a], zt[b]) for a, b in zip(plain, turned)] + [(zp[plain[-1]],) * 2]
            for t in range(2):
                lhs = [jnp.concatenate(halves_of(*v[::-1]) if t else halves_of(*v), axis=1) for v in pairs]
                outs.append(_dot(jnp.concatenate(lhs, axis=0), rhs_ref[2 * h + t], _NT))
        lo, hi = [pltpu.bitcast(pltpu.pack_elementwise([outs[t], outs[2 + t]], packed_dtype=BF16), U32)
                  for t in range(2)]
        merged = {a: jnp.where(low, lo[_ds(n, 8)], hi[_ds(n, 8)]) for n, a in enumerate(plain)}
        merged.update({a: turn(jnp.where(low, hi[_ds(n, 8)], lo[_ds(n, 8)])) for n, a in enumerate(turned)})

        def align(a, shift):
            return pltpu.roll(merged[a], shift, 1, stride=1, stride_axis=0)

        piece = {(s, p): align(256 * s + p % 8, s + 4 - 4 * (p // 8))
                 for s in range(8) for p in sorted(set(_RHO[s]) - {16})}
        pos = (lane8 - 11) & 127
        memo = {}
        for j in range(NS):
            key = ()
            acc = None
            for s in range(7, -1, -1):
                key = key + (_RHO[s][j],)
                if key not in memo:
                    pc = carry if _RHO[s][j] == 16 else piece[s, _RHO[s][j]]
                    same = acc is None or pc is acc
                    memo[key] = pc if same else jnp.where((pos & 7) == s, pc, acc)
                acc = memo[key]
            (un, uo)[j % 2][_ds(i + D // 16, 8), _ds(j // 2, R)] = acc
            if j == 0:
                carry = jnp.where(pos >= 120, pltpu.roll(acc, 128 - 9, 1), pltpu.roll(acc, 128 - 8, 1))
                carry = jnp.where(pos == 127, align(L, 3), carry)

    def gen_k(rb):
        for n in range(8):
            i = 8 * rb + n
            taps(i)
            if i + 1 < D // 16:
                powers(i + 1)
            if rb:
                dft_k(rb - 1, range(2 * n, 2 * n + 2))

    def dft_k(rb, which=range(NS)):
        for s in which:
            u = (un, uo)[s // 8][_ds(rb + 4, 64), _ds(s % 8, R)]
            kspec[_ds(rb, 128), _ds(s, 2 * R)] = _dot(_unpack(u), _unpack(fk_ref[s]))

    with _scope("head"):
        for cp in first:
            cp.wait()
        for cp in loads:
            cp.start()

    with _scope("gen_k"):
        powers(0)
        gen_k(0)
        for cp in second:
            cp.wait()
        for rb in range(1, 4):
            pl.when(zero_ref[0] < rb)(lambda: gen_k(rb))

    for cp in loads:
        cp.wait()

    xu = [r.bitcast(U32) for r in xio]

    def load_x(b):
        for jj in range(8):
            ev, od = _halves(xu[b][pl.ds(jj, R, stride=8), :].T)
            xs[_ds(b, 128), _ds(jj, R)] = ev
            xo[_ds(b, 128), _ds(jj, R)] = od

    m_i = jax.lax.broadcasted_iota(jnp.int32, (128, 128), 0)
    c_i = jax.lax.broadcasted_iota(jnp.int32, (128, 128), 1)
    perm = jnp.where(c_i == (m_i & 7) * 16 + (m_i >> 3), 1.0, 0.0).astype(BF16)

    def prep_w(g):
        for t in range(3):
            wt[g, _ds(t, 64), :] = _pack(_dot(perm, wqkv_ref[:, _ds((t + 1) % 3 * 4 + g, 128)], _NT))
        wot[:, _ds(g, 128)] = _pack(_dot(perm, wo_ref[_ds(g, 128), :]).T)

    def dft(rb, s):
        at, n = BLOCKS[rb]
        u = (un, uo)[s // 8][at // 2:(at + n) // 2, _ds(s % 8, R)]
        y = _dot(_unpack(u), _unpack(f_ref[s]))
        spec[rb][0:n, _ds(s, 2 * R)] = y
        return y[-8:, R:]

    def idft(rb, s):
        at, n = BLOCKS[rb]
        y = _dot(spec[rb][0:n, _ds(s, 2 * R)], _unpack(f_ref[s]), _NT)
        (xs, xo)[s // 8][at:at + n, _ds(s % 8, R)] += y
        return y[-8:]

    def load_spec(ref, rows, order):
        return [(ref[rows, _ds(2 * s, R)], ref[rows, _ds(2 * s + 1, R)]) for s in order]

    def store_spec(ref, rows, order, vals):
        for s, v in zip(order, vals):
            ref[rows, _ds(2 * s, R)] = v[0]
            ref[rows, _ds(2 * s + 1, R)] = v[1]

    slabs = [_slab(j) for j in range(NS)]

    def half(buf, rows, e8, bias=None):
        out = []
        for j in range(8):
            lo, hi = load_spec(buf, rows, [slabs[j], slabs[j + 8]])
            if j == 0 and bias is not None:
                lo = (lo[0] + bias, lo[1])
            out.append(_csub(lo, hi) if e8 else _cadd(lo, hi))
        return out

    def k_fft_steps(i):
        rows = _ds(i, 8)
        for e8 in (8, 0):
            quartics = _split(half(kspec, rows, e8, dskb[rows, :]), e8 // 2)
            for e4, p4 in zip((e8 // 2, e8 // 2 + 8), quartics):
                for e2, p2 in zip((e4 // 2, e4 // 2 + 8), _split(p4, e4 // 2)):
                    store_spec(khat, rows, _coeff_slots(e2), _factor_coeffs(p2, e2))
                yield

    def k_fft(i):
        for _ in k_fft_steps(i):
            pass

    def conv(rb, i, after=None):
        at, size = BLOCKS[rb]
        buf, rows, park = spec[rb], _ds(i, 8), _ds(size // 8, 8)
        for e8 in (8, 0):
            quartics = []
            for e4, p4 in zip((e8 // 2, e8 // 2 + 8), _split(half(buf, rows, e8), e8 // 2)):
                prods = [_factor_mul(p2, load_spec(khat, _ds(at // 8 + i, 8), _coeff_slots(e2)), e2)
                         for e2, p2 in zip((e4 // 2, e4 // 2 + 8), _split(p4, e4 // 2))]
                quartics.append(_merge(*prods, e4 // 2))
                if e4 < 8:
                    fence(khat, prods[1][1][0])
            mark = prods[1][1][0]
            fence(buf, mark if e8 or after is None else after)
            for j, v in enumerate(_merge(*quartics, e8 // 2)):
                if e8:
                    store_spec(buf, park, [j], [v])
                else:
                    (o,) = load_spec(buf, park, [j])
                    store_spec(buf, rows, [slabs[j], slabs[j + 8]], [_cadd(v, o), _csub(v, o)])
        return mark

    lane = jax.lax.broadcasted_iota(jnp.int32, (128, R), 1)

    def qkv(g, u, qs, ks, vs, i):
        y = _dot(_unpack(wt[g]), _unpack(u[0:D // 2, _ds(i, R)]))
        k, v, q = y[0:128], y[128:256], y[256:384]
        qs[:, _ds(i, R)] = q
        ks[:, _ds(i + 7, R)] = k
        vs[:, _ds(i + 7, R)] = v
        if i:
            ks[:, _ds(i - 1, R)] = pltpu.roll(k, 1, 1)
            vs[:, _ds(i - 1, R)] = jnp.where(lane == 0, va[:, _ds(7, R)], pltpu.roll(v, 1, 1))

    never = lane8 < zero_ref[0]

    def attend(g, qs, ks, vs, rs, o, i, ways, side=None):
        logits = []
        for w in range(W):
            lg = None
            for c in range(16):
                term = qs[_ds(c, 8), _ds(i, R)] * ks[_ds(c, 8), _ds(7 + i - w, R)]
                if c:
                    lg = lg + term
                else:
                    lg = term if w < ways else jnp.where(never, logits[w - ways], term)
            logits.append(lg)
            if side and w in (1, 7):
                fence(kspec, lg)
                next(side)
        scale = rs[7 + i] * 0.25
        logits = [lg * scale * rs[7 + i - w] for w, lg in enumerate(logits)]
        logits = [jnp.where(lane8 == 0, NEG, lg) if w > i else lg for w, lg in enumerate(logits)]
        mx = logits[0]
        for lg in logits[1:]:
            mx = jnp.maximum(mx, lg)
        es = [jnp.exp(lg - mx) for lg in logits]
        den = es[0]
        for e in es[1:]:
            den = den + e
        inv = 1.0 / den
        probs = [e * rs[7 + i - w] * inv for w, e in enumerate(es)]
        outs = []
        for c in range(16):
            acc = None
            for w in range(W):
                term = vs[_ds(c, 8), _ds(7 + i - w, R)] * probs[w]
                if w:
                    acc = acc + term
                else:
                    acc = term if c < ways else jnp.where(never, outs[c - ways], term)
            outs.append(acc)
            if side and c in (3, 11):
                fence(kspec, acc)
                next(side)
        o[_ds(g + 4, 64), _ds(i, R)] = _pack(jnp.concatenate(outs, axis=0))

    def chain_sum(vals, ways):
        parts = vals[:ways]
        for n, v in enumerate(vals[ways:]):
            parts[n % ways] = parts[n % ways] + v
        return jnp.sum(sum(parts[1:], parts[0]), axis=0, keepdims=True)

    def center(x, i, total, ways, after=None):
        parts = [total[_ds(n, 8)] for n in range(D // 8)]
        if after is not None:
            parts[0] = jnp.where(never, after, parts[0])
        c = x[:, _ds(i, R)] - chain_sum(parts, 2) * (1.0 / D)
        sq = c * c
        v = chain_sum([sq[_ds(n, 8)] for n in range(D // 8)], ways) * (1.0 / D)
        return c, jnp.broadcast_to(jax.lax.rsqrt(v + EPS), (8, R))

    def norm(x, u, rs, i, ways, after=None):
        c, r = center(x, i, x[:, _ds(i, R)], ways, after)
        u[0:D // 2, _ds(i, R)] = _pack(c)
        rs[7 + i] = r
        if i:
            rs[i - 1] = jnp.where(lane8 == 0, ra[7], pltpu.roll(r, 1, 1))
        return r

    def proj(x, o, u, i):
        y = x[:, _ds(i, R)] + _dot(_unpack(wot[...]), _unpack(o[D // 2:D, _ds(i, R)]))
        x[:, _ds(i, R)] = y
        cen[i % 2], r = center(x, i, y, 1)
        u[0:D // 2, _ds(i, R)] = _pack(cen[i % 2] * r[0:1])

    stores = [pltpu.make_async_copy(xio[c].at[0:L], o_hbm.at[:, c * 128:(c + 1) * 128], sems.at[c])
              for c in range(4)]

    def store_x(b, jj):
        t = pltpu.pack_elementwise(
            [xs[_ds(b, 128), _ds(jj, R)], xo[_ds(b, 128), _ds(jj, R)]], packed_dtype=BF16)
        xu[b][pl.ds(jj, R, stride=8), :] = pltpu.bitcast(t, U32).T

    def fence_io(b, val):
        xio[b][pl.ds(pl.multiple_of(L + zero_ref[0], 16), 16), :] = pltpu.bitcast(val, BF16)

    def start_store(b, val):
        stores[b].start()
        fence_io(b, val)
        return pltpu.bitcast(xio[b][L:L + 16, :], F32)

    def phase(name):
        def run(fn):
            with _scope(name):
                pl.when(zero_ref[0] == 0)(fn)
        return run

    @phase("prep")
    def _():
        dft_k(3)
        for b in range(4):
            load_x(b)
            prep_w(b)
            for n in range(6):
                k_fft(6 * b + n)

    even, odd = (un, (qa, ka, va), ra), (uo, (qb, kb, vb), rb_)

    def overlap(g_next, nxt, g, cur, k0):
        for i in range(8):
            qkv(g_next, nxt[0], *nxt[1], i)
            attend(g, *cur[1], cur[2], nxt[0], i, 2, None if k0 is None else k_fft_steps(k0 + i))

    for layer in range(2):
        @phase("a_pro")
        def _():
            if layer:
                for s in range(8):
                    idft(3, s)
            r = norm(xs, un, ra, 0, 4)
            for i in range(8):
                if layer:
                    idft(3, i + 8)
                qkv(0, un, qa, ka, va, i)
                if i < 7:
                    r = norm(xs, un, ra, i + 1, 2 - layer, r)
                r = norm(xo, uo, rb_, i, 2 - layer, r)

        def group(g, c):
            overlap(g, odd, g, even, None if layer else 8 * g + 24)

            @pl.when(g < 3)
            def _():
                overlap(g + 1, even, g, odd, None)

            return c

        with _scope("a_grp"):
            jax.lax.fori_loop(0, 4, group, 0)

        @phase("a_proj")
        def _():
            for i in range(8):
                proj(xs, uo, un, i)
                attend(3, qb, kb, vb, rb_, un, i, 1)
            for i in range(8):
                proj(xo, un, uo, i)
                if not layer:
                    k_fft(56 + i)
            for s in range(NS):
                dft(0, s)

        @phase("conv")
        def _():
            done = []
            for rb in range(4):
                for i in range(16):
                    if rb < 3:
                        last = dft(rb + 1, i)
                    if layer and rb == 3:
                        if i < 8:
                            idft(2, i)
                            last = idft(2, i + 8)
                        else:
                            store_x(2, i - 8)
                    elif rb:
                        last = idft(rb - 1, i)
                    if layer and rb >= 2 and i < 8:
                        store_x(rb - 2, i)
                        if i == 7:
                            last = start_store(rb - 2, last)
                    done.append(last)
                    mark = conv(rb, i, done[-LAG] if len(done) >= LAG else None)
                    if rb < 3:
                        fence(spec[rb + 1], mark)

    with _scope("store_x"):
        last = start_store(2, jnp.zeros((8, R), F32))
        fence(spec[3], last)
        for jj in range(8):
            idft(3, jj)
            idft(3, jj + 8)
            store_x(3, jj)
        stores[3].start()
    with _scope("tail"):
        for cp in stores:
            cp.wait()


@jax.jit
def pallas_interleave_layers__sliding_local_dilated__ssm_conv_s4__prompt_kernel(
    A_x: jax.Array,
    A_wqkv: jax.Array,
    A_wo: jax.Array,
    B_u: jax.Array,
    B_A_re: jax.Array,
    B_A_im: jax.Array,
    B_B_re: jax.Array,
    B_B_im: jax.Array,
    B_C_re: jax.Array,
    B_C_im: jax.Array,
    B_log_dt: jax.Array,
    B_Dskip: jax.Array,
):
    del B_u
    f = _dft_matrix()
    lane = (np.arange(R) - 11) % R
    order = 16 * (lane % 8) + lane // 8
    fk = (f[:, order].astype(np.float32) * (2.0 / L)).astype(ml_dtypes.bfloat16)
    scratch = [
        pltpu.VMEM((D, L // 2), F32),
        pltpu.VMEM((D, L // 2), F32),
        pltpu.VMEM((D + 8, L // 2), U32),
        pltpu.VMEM((D + 8, L // 2), U32),
        pltpu.VMEM((4, 192, D), U32),
        pltpu.VMEM((D // 2, D), U32),
        pltpu.VMEM((D // 2, 128), U32),
        pltpu.VMEM((D, 128), F32),
        pltpu.VMEM((2, 8, 8, N), F32),
        pltpu.VMEM((4, 128, 2 * N), F32),
        *[pltpu.VMEM((n + 16, 2 * L), F32) for _, n in BLOCKS],
        pltpu.VMEM((D + 8, 2 * L), F32),
        pltpu.VMEM((D + 8, 22 * 2 * R), F32),
        pltpu.VMEM((128, 8 * R), F32),
        pltpu.VMEM((128, 15 * R), F32),
        pltpu.VMEM((128, 15 * R), F32),
        pltpu.VMEM((128, 8 * R), F32),
        pltpu.VMEM((128, 15 * R), F32),
        pltpu.VMEM((128, 15 * R), F32),
        pltpu.VMEM((15, 8, R), F32),
        pltpu.VMEM((15, 8, R), F32),
        pltpu.VMEM((2, D, R), F32),
        *[pltpu.VMEM((L + 16, 128), BF16)] * 4,
        pltpu.VMEM((D, 3 * D), BF16),
        pltpu.VMEM((D, D), BF16),
        pltpu.VMEM((NS, R // 2, 2 * R), U32),
        pltpu.VMEM((NS, R // 2, 2 * R), U32),
        pltpu.VMEM((6, D, N), BF16),
        pltpu.SMEM((1,), jnp.int32),
        pltpu.VMEM((D,), BF16),
        pltpu.VMEM((D,), BF16),
        pltpu.SemaphoreType.DMA((13,)),
    ]
    hbm = pl.BlockSpec(memory_space=pl.ANY)
    out = pl.pallas_call(
        _kernel,
        out_shape=jax.ShapeDtypeStruct((L, D), BF16),
        in_specs=[hbm] * 14,
        out_specs=hbm,
        scratch_shapes=scratch,
        compiler_params=pltpu.CompilerParams(vmem_limit_bytes=100 * 1024 * 1024),
    )(np.zeros((1,), np.int32), A_x.reshape(L, D), A_wqkv, A_wo, B_A_re, B_A_im, B_B_re, B_B_im, B_C_re, B_C_im,
      B_log_dt, B_Dskip, _pack_rows(f), _pack_rows(fk))
    return out.reshape(1, L, D)
```

```python
import contextlib

import jax
import jax.numpy as jnp
import jax.experimental.pallas as pl
import jax.experimental.pallas.tpu as pltpu
import ml_dtypes
import numpy as np

L = 2048
D = 512
N = 128
NS = 16
R = 128
W = 8
EPS = 1e-5
_H = float(np.sqrt(0.5))
LAG = 4
BLOCKS = ((0, 128), (128, 128), (256, 128), (384, 128))
F32 = jnp.float32
BF16 = jnp.bfloat16
U32 = jnp.uint32
NEG = float(ml_dtypes.bfloat16(-1e9))

_NT = (((1,), (1,)), ((), ()))


def _slab(j):
    return (j % 2) * 8 + j // 2


def _dft_matrix():
    r = np.arange(R)
    k = np.arange(R) + 0.5
    f = np.zeros((NS, R, 2 * R), np.float64)
    for j in range(NS):
        th = 2.0 * np.pi * np.outer(NS * r + j, k) / (2 * L)
        f[_slab(j), :, :R] = np.cos(th)
        f[_slab(j), :, R:] = -np.sin(th)
    return f.astype(np.float32).astype(ml_dtypes.bfloat16)


def _pack_rows(a):
    u = np.ascontiguousarray(a).view(np.uint16).astype(np.uint32)
    return u[:, 0::2] | (u[:, 1::2] << np.uint32(16))


def _lag_tables():
    rho = []
    for s in range(8):
        lag = (256 * s + np.arange(NS)).astype(np.float32)
        rho.append([int(v) - 256 * s for v in lag.astype(ml_dtypes.bfloat16).astype(np.float32)])
    return rho


_RHO = _lag_tables()


def _cmul(a, b):
    return (a[0] * b[0] - a[1] * b[1], a[0] * b[1] + a[1] * b[0])


def _csq(a):
    t = a[0] * a[1]
    return ((a[0] - a[1]) * (a[0] + a[1]), t + t)


def _cadd(a, b):
    return (a[0] + b[0], a[1] + b[1])


def _csub(a, b):
    return (a[0] - b[0], a[1] - b[1])


def _split(p, e):
    plus, minus = [], []
    for lo, hi in zip(p[:len(p) // 2], p[len(p) // 2:]):
        if e % 4:
            hi = ((hi[0] - hi[1]) * _H, (hi[0] + hi[1]) * _H)
        if e >= 4:
            plus.append((lo[0] - hi[1], lo[1] + hi[0]))
            minus.append((lo[0] + hi[1], lo[1] - hi[0]))
        else:
            plus.append(_cadd(lo, hi))
            minus.append(_csub(lo, hi))
    return plus, minus


def _merge(plus, minus, e):
    lo, hi = [], []
    for p, m in zip(plus, minus):
        lo.append(_cadd(p, m))
        d = (p[1] - m[1], m[0] - p[0]) if e >= 4 else _csub(p, m)
        hi.append(((d[0] + d[1]) * _H, (d[1] - d[0]) * _H) if e % 4 else d)
    return lo + hi


def _factor_coeffs(k, e):
    if e % 8 == 0:
        (p,), (m,) = _split(k, e // 2)
        return [(p[0] * 0.5, p[1] * 0.5), (m[0] * 0.5, m[1] * 0.5)]
    c, s = float(np.cos(np.pi * e / 8)), float(np.sin(np.pi * e / 8))
    wk = (k[1][0] * c - k[1][1] * s, k[1][0] * s + k[1][1] * c)
    return [k[0], _csub(wk, k[0]), _csub(k[1], k[0])]


def _factor_mul(a, coeffs, e):
    if e % 8 == 0:
        (p,), (m,) = _split(a, e // 2)
        return _merge([_cmul(p, coeffs[0])], [_cmul(m, coeffs[1])], e // 2)
    t = _cmul(_cadd(a[0], a[1]), coeffs[0])
    return [_cadd(t, _cmul(a[1], coeffs[1])), _cadd(t, _cmul(a[0], coeffs[2]))]


def _coeff_slots(e):
    if e % 8 == 0:
        return [e // 4, e // 4 + 1]
    n = 4 + 3 * [2, 4, 6, 10, 12, 14].index(e)
    return [n, n + 1, n + 2]


def _scope(name):
    return contextlib.nullcontext()


def _ds(i, n):
    if isinstance(i, int):
        return slice(i * n, (i + 1) * n)
    return pl.ds(pl.multiple_of(i * n, n), n)


def _pack(x):
    return pltpu.bitcast(x.astype(BF16), U32)


def _unpack(x):
    return pltpu.bitcast(x, BF16)


def _dot(a, b, dims=(((1,), (0,)), ((), ()))):
    return jax.lax.dot_general(a, b, dims, preferred_element_type=F32)


def _halves(u):
    return pltpu.bitcast(u << 16, F32), pltpu.bitcast(u & jnp.uint32(0xFFFF0000), F32)


def _kernel(zero_hbm, x_hbm, wqkv_hbm, wo_hbm, are, aim, bre, bim, cre, cim,
            ldt_hbm, dsk_hbm, f_hbm, fk_hbm, o_hbm,
            xs, xo, un, uo, wt, wot, dtb, dskb, pw_ref, rhs_ref, s0, s1, s2, s3, kspec, khat, qa, ka, va, qb, kb, vb,
            ra, rb_, cen0, cen1,
            io0, io1, io2, io3, wqkv_ref, wo_ref, f_ref, fk_ref, ssm, zero_ref, ldt_ref, dsk_ref, sems):
    def fetch_ssm(rows, sem):
        return [pltpu.make_async_copy(p.at[rows], ssm.at[n, rows], sem)
                for n, p in enumerate((are, aim, bre, bim, cre, cim))]

    small = [pltpu.make_async_copy(src, dst, sems.at[10 + n]) for n, (src, dst) in enumerate(
        [(zero_hbm, zero_ref), (ldt_hbm, ldt_ref), (dsk_hbm, dsk_ref)])]
    for cp in small:
        cp.start()
    first = fetch_ssm(pl.ds(0, 144), sems.at[8])
    for cp in first:
        cp.start()
    second = fetch_ssm(pl.ds(144, D - 144), sems.at[9])
    second += [pltpu.make_async_copy(fk_hbm, fk_ref, sems.at[4])]
    for cp in second:
        cp.start()
    xio = (io0, io1, io2, io3)
    loads = []
    loads += [pltpu.make_async_copy(x_hbm.at[:, c * 128:(c + 1) * 128], xio[c].at[0:L], sems.at[c])
              for c in range(4)]
    loads += [pltpu.make_async_copy(src, dst, sems.at[5 + n]) for n, (src, dst) in enumerate(
        [(wqkv_hbm, wqkv_ref), (wo_hbm, wo_ref), (f_hbm, f_ref)])]

    spec = (s0, s1, s2, s3)
    cen = (cen0, cen1)

    def fence(ref, val):
        row = ref.shape[0] - 8 + zero_ref[0]
        ref[pl.ds(pl.multiple_of(row, 8), 8), 0:128] = val

    for cp in small:
        cp.wait()
    dt_row = jnp.exp(ldt_ref[...].astype(F32)).reshape(1, D)
    dtb[...] = _pack(jnp.broadcast_to(dt_row, (128, D)).T)
    dskb[...] = jnp.broadcast_to(dsk_ref[...].astype(F32).reshape(1, D) * (2.0 / L), (128, D)).T

    lane8 = jax.lax.broadcasted_iota(jnp.int32, (8, R), 1)
    sub8 = jax.lax.broadcasted_iota(jnp.int32, (8, N), 0)
    low = sub8 < 4
    steps = (1, 2, 4, 256)

    def halves_of(a, b):
        return tuple(jnp.where(low, u, v) for u, v in zip(a, b))

    def powers(i):
        dts = _halves(dtb[_ds(i, 8), :])
        are, aim, bre, bim, cre, cim = [
            _halves(pltpu.bitcast(ssm[n, _ds(i, 16), :], U32)) for n in range(6)]
        for h in range(2):
            dt = dts[h]
            li = dt * aim[h]
            mag = jnp.exp(dt * are[h])
            zp = {1: (mag * jnp.cos(li), mag * jnp.sin(li))}
            for e in (1, 2, 4, 8, 16, 32, 64, 128):
                zp[2 * e] = _csq(zp[e])
            for n, e in enumerate(steps):
                pw_ref[h, 2 * n] = zp[e][0]
                pw_ref[h, 2 * n + 1] = zp[e][1]
            w = _cmul((cre[h], cim[h]), (dt * bre[h], dt * bim[h]))
            w, z8, z16 = [(v[0], -v[1]) for v in (w, zp[8], zp[16])]
            w8 = _cmul(w, z8)
            for t in range(2):
                def pick(v):
                    return tuple(jnp.take_along_axis(u, 4 * t + 3 - (sub8 & 3), axis=0) for u in v)

                step = pick(z16)
                rows = [halves_of(pick(w), pick(w8)) if t else halves_of(pick(w8), pick(_cmul(w, z16)))]
                for _ in range(15):
                    rows.append(_cmul(rows[-1], step))
                if not t:
                    rows = [halves_of(rows[-1], pick(w))] + rows[:-1]
                rhs_ref[2 * h + t] = jnp.concatenate([jnp.concatenate(v, axis=1) for v in rows], axis=0)

    offsets = sorted({256 * s + p % 8 for s in range(8) for p in _RHO[s]}) + [L]
    plain, turned = offsets[:11], offsets[11:]

    def turn(v):
        return pltpu.roll(v, 4, 0)

    def taps(i):
        outs = []
        for h in range(2):
            zp = {e: (pw_ref[h, 2 * n], pw_ref[h, 2 * n + 1]) for n, e in enumerate(steps)}
            zp[0] = (jnp.ones((8, N), F32), jnp.zeros((8, N), F32))
            zt = {e: (turn(zp[e][0]), turn(zp[e][1])) for e in (4, 256)}
            for table, exps in ((zp, plain + turned[:1]), (zt, turned[1:])):
                for e in exps:
                    if e in table:
                        continue
                    if e % 2 == 0 and e // 2 in table:
                        table[e] = _csq(table[e // 2])
                    else:
                        inc = next(v for v in steps if v in table and e - v in table)
                        table[e] = _cmul(table[e - inc], table[inc])
            zt[turned[0]] = tuple(turn(v) for v in zp[turned[0]])
            pairs = [(zp[a], zt[b]) for a, b in zip(plain, turned)] + [(zp[plain[-1]],) * 2]
            for t in range(2):
                lhs = [jnp.concatenate(halves_of(*v[::-1]) if t else halves_of(*v), axis=1) for v in pairs]
                outs.append(_dot(jnp.concatenate(lhs, axis=0), rhs_ref[2 * h + t], _NT))
        lo, hi = [pltpu.bitcast(pltpu.pack_elementwise([outs[t], outs[2 + t]], packed_dtype=BF16), U32)
                  for t in range(2)]
        merged = {a: jnp.where(low, lo[_ds(n, 8)], hi[_ds(n, 8)]) for n, a in enumerate(plain)}
        merged.update({a: turn(jnp.where(low, hi[_ds(n, 8)], lo[_ds(n, 8)])) for n, a in enumerate(turned)})

        def align(a, shift):
            return pltpu.roll(merged[a], shift, 1, stride=1, stride_axis=0)

        piece = {(s, p): align(256 * s + p % 8, s + 4 - 4 * (p // 8))
                 for s in range(8) for p in sorted(set(_RHO[s]) - {16})}
        pos = (lane8 - 11) & 127
        memo = {}
        for j in range(NS):
            key = ()
            acc = None
            for s in range(7, -1, -1):
                key = key + (_RHO[s][j],)
                if key not in memo:
                    pc = carry if _RHO[s][j] == 16 else piece[s, _RHO[s][j]]
                    same = acc is None or pc is acc
                    memo[key] = pc if same else jnp.where((pos & 7) == s, pc, acc)
                acc = memo[key]
            (un, uo)[j % 2][_ds(i + D // 16, 8), _ds(j // 2, R)] = acc
            if j == 0:
                carry = jnp.where(pos >= 120, pltpu.roll(acc, 128 - 9, 1), pltpu.roll(acc, 128 - 8, 1))
                carry = jnp.where(pos == 127, align(L, 3), carry)

    def gen_k(rb):
        for n in range(8):
            i = 8 * rb + n
            taps(i)
            if i + 1 < D // 16:
                powers(i + 1)
            if rb:
                dft_k(rb - 1, range(2 * n, 2 * n + 2))

    def dft_k(rb, which=range(NS)):
        for s in which:
            u = (un, uo)[s // 8][_ds(rb + 4, 64), _ds(s % 8, R)]
            kspec[_ds(rb, 128), _ds(s, 2 * R)] = _dot(_unpack(u), _unpack(fk_ref[s]))

    with _scope("head"):
        for cp in first:
            cp.wait()
        for cp in loads:
            cp.start()

    with _scope("gen_k"):
        powers(0)
        gen_k(0)
        for cp in second:
            cp.wait()
        for rb in range(1, 4):
            pl.when(zero_ref[0] < rb)(lambda: gen_k(rb))

    for cp in loads:
        cp.wait()

    xu = [r.bitcast(U32) for r in xio]

    def load_x(b):
        for jj in range(8):
            ev, od = _halves(xu[b][pl.ds(jj, R, stride=8), :].T)
            xs[_ds(b, 128), _ds(jj, R)] = ev
            xo[_ds(b, 128), _ds(jj, R)] = od

    m_i = jax.lax.broadcasted_iota(jnp.int32, (128, 128), 0)
    c_i = jax.lax.broadcasted_iota(jnp.int32, (128, 128), 1)
    perm = jnp.where(c_i == (m_i & 7) * 16 + (m_i >> 3), 1.0, 0.0).astype(BF16)

    def prep_w(g):
        for t in range(3):
            wt[g, _ds(t, 64), :] = _pack(_dot(perm, wqkv_ref[:, _ds((t + 1) % 3 * 4 + g, 128)], _NT))
        wot[:, _ds(g, 128)] = _pack(_dot(perm, wo_ref[_ds(g, 128), :]).T)

    def dft(rb, s):
        at, n = BLOCKS[rb]
        u = (un, uo)[s // 8][at // 2:(at + n) // 2, _ds(s % 8, R)]
        y = _dot(_unpack(u), _unpack(f_ref[s]))
        spec[rb][0:n, _ds(s, 2 * R)] = y
        return y[-8:, R:]

    def idft(rb, s):
        at, n = BLOCKS[rb]
        y = _dot(spec[rb][0:n, _ds(s, 2 * R)], _unpack(f_ref[s]), _NT)
        (xs, xo)[s // 8][at:at + n, _ds(s % 8, R)] += y
        return y[-8:]

    def load_spec(ref, rows, order):
        return [(ref[rows, _ds(2 * s, R)], ref[rows, _ds(2 * s + 1, R)]) for s in order]

    def store_spec(ref, rows, order, vals):
        for s, v in zip(order, vals):
            ref[rows, _ds(2 * s, R)] = v[0]
            ref[rows, _ds(2 * s + 1, R)] = v[1]

    slabs = [_slab(j) for j in range(NS)]

    def half(buf, rows, e8, bias=None):
        out = []
        for j in range(8):
            lo, hi = load_spec(buf, rows, [slabs[j], slabs[j + 8]])
            if j == 0 and bias is not None:
                lo = (lo[0] + bias, lo[1])
            out.append(_csub(lo, hi) if e8 else _cadd(lo, hi))
        return out

    def k_fft_steps(i):
        rows = _ds(i, 8)
        for e8 in (8, 0):
            quartics = _split(half(kspec, rows, e8, dskb[rows, :]), e8 // 2)
            for e4, p4 in zip((e8 // 2, e8 // 2 + 8), quartics):
                for e2, p2 in zip((e4 // 2, e4 // 2 + 8), _split(p4, e4 // 2)):
                    store_spec(khat, rows, _coeff_slots(e2), _factor_coeffs(p2, e2))
                yield

    def k_fft(i):
        for _ in k_fft_steps(i):
            pass

    def conv(rb, i, after=None):
        at, size = BLOCKS[rb]
        buf, rows, park = spec[rb], _ds(i, 8), _ds(size // 8, 8)
        for e8 in (8, 0):
            quartics = []
            for e4, p4 in zip((e8 // 2, e8 // 2 + 8), _split(half(buf, rows, e8), e8 // 2)):
                prods = [_factor_mul(p2, load_spec(khat, _ds(at // 8 + i, 8), _coeff_slots(e2)), e2)
                         for e2, p2 in zip((e4 // 2, e4 // 2 + 8), _split(p4, e4 // 2))]
                quartics.append(_merge(*prods, e4 // 2))
                if e4 < 8:
                    fence(khat, prods[1][1][0])
            mark = prods[1][1][0]
            fence(buf, mark if e8 or after is None else after)
            for j, v in enumerate(_merge(*quartics, e8 // 2)):
                if e8:
                    store_spec(buf, park, [j], [v])
                else:
                    (o,) = load_spec(buf, park, [j])
                    store_spec(buf, rows, [slabs[j], slabs[j + 8]], [_cadd(v, o), _csub(v, o)])
        return mark

    lane = jax.lax.broadcasted_iota(jnp.int32, (128, R), 1)

    def qkv(g, u, qs, ks, vs, i):
        y = _dot(_unpack(wt[g]), _unpack(u[0:D // 2, _ds(i, R)]))
        k, v, q = y[0:128], y[128:256], y[256:384]
        qs[:, _ds(i, R)] = q
        ks[:, _ds(i + 7, R)] = k
        vs[:, _ds(i + 7, R)] = v
        if i:
            ks[:, _ds(i - 1, R)] = pltpu.roll(k, 1, 1)
            vs[:, _ds(i - 1, R)] = jnp.where(lane == 0, va[:, _ds(7, R)], pltpu.roll(v, 1, 1))

    never = lane8 < zero_ref[0]

    def attend(g, qs, ks, vs, rs, o, i, ways, side=None):
        logits = []
        for w in range(W):
            lg = None
            for c in range(16):
                term = qs[_ds(c, 8), _ds(i, R)] * ks[_ds(c, 8), _ds(7 + i - w, R)]
                if c:
                    lg = lg + term
                else:
                    lg = term if w < ways else jnp.where(never, logits[w - ways], term)
            logits.append(lg)
            if side and w in (1, 7):
                fence(kspec, lg)
                next(side)
        scale = rs[7 + i] * 0.25
        logits = [lg * scale * rs[7 + i - w] for w, lg in enumerate(logits)]
        logits = [jnp.where(lane8 == 0, NEG, lg) if w > i else lg for w, lg in enumerate(logits)]
        mx = logits[0]
        for lg in logits[1:]:
            mx = jnp.maximum(mx, lg)
        es = [jnp.exp(lg - mx) for lg in logits]
        den = es[0]
        for e in es[1:]:
            den = den + e
        inv = 1.0 / den
        probs = [e * rs[7 + i - w] * inv for w, e in enumerate(es)]
        outs = []
        for c in range(16):
            acc = None
            for w in range(W):
                term = vs[_ds(c, 8), _ds(7 + i - w, R)] * probs[w]
                if w:
                    acc = acc + term
                else:
                    acc = term if c < ways else jnp.where(never, outs[c - ways], term)
            outs.append(acc)
            if side and c in (3, 11):
                fence(kspec, acc)
                next(side)
        o[_ds(g + 4, 64), _ds(i, R)] = _pack(jnp.concatenate(outs, axis=0))

    def chain_sum(vals, ways):
        parts = vals[:ways]
        for n, v in enumerate(vals[ways:]):
            parts[n % ways] = parts[n % ways] + v
        return jnp.sum(sum(parts[1:], parts[0]), axis=0, keepdims=True)

    def row_mean(x, ways, after=None):
        parts = [x[_ds(n, 8)] for n in range(D // 8)]
        if after is not None:
            parts[0] = jnp.where(never, after, parts[0])
        return chain_sum(parts, ways) * (1.0 / D)

    def norm(x, u, rs, i, ways, after=None):
        c = x[:, _ds(i, R)] - row_mean(x[:, _ds(i, R)], 2, after)
        r = jnp.broadcast_to(jax.lax.rsqrt(row_mean(c * c, ways) + EPS), (8, R))
        u[0:D // 2, _ds(i, R)] = _pack(c)
        rs[7 + i] = r
        if i:
            rs[i - 1] = jnp.where(lane8 == 0, ra[7], pltpu.roll(r, 1, 1))
        return r

    def proj(x, o, u, i):
        y = x[:, _ds(i, R)] + _dot(_unpack(wot[...]), _unpack(o[D // 2:D, _ds(i, R)]))
        x[:, _ds(i, R)] = y
        cen_ = cen[i % 2]
        cen_[...] = x[:, _ds(i, R)] - row_mean(y, 2)
        c = cen_[pl.ds(pl.multiple_of(zero_ref[0], 8), D)]
        u[0:D // 2, _ds(i, R)] = _pack(cen_[...] * jax.lax.rsqrt(row_mean(c * c, 1) + EPS))

    stores = [pltpu.make_async_copy(xio[c].at[0:L], o_hbm.at[:, c * 128:(c + 1) * 128], sems.at[c])
              for c in range(4)]

    def store_x(b, jj):
        t = pltpu.pack_elementwise(
            [xs[_ds(b, 128), _ds(jj, R)], xo[_ds(b, 128), _ds(jj, R)]], packed_dtype=BF16)
        xu[b][pl.ds(jj, R, stride=8), :] = pltpu.bitcast(t, U32).T

    def fence_io(b, val):
        xio[b][pl.ds(pl.multiple_of(L + zero_ref[0], 16), 16), :] = pltpu.bitcast(val, BF16)

    def start_store(b, val):
        stores[b].start()
        fence_io(b, val)
        return pltpu.bitcast(xio[b][L:L + 16, :], F32)

    def phase(name):
        def run(fn):
            with _scope(name):
                pl.when(zero_ref[0] == 0)(fn)
        return run

    @phase("prep")
    def _():
        dft_k(3)
        for b in range(4):
            load_x(b)
            prep_w(b)
            for n in range(6):
                k_fft(6 * b + n)

    even, odd = (un, (qa, ka, va), ra), (uo, (qb, kb, vb), rb_)

    def overlap(g_next, nxt, g, cur, k0):
        for i in range(8):
            qkv(g_next, nxt[0], *nxt[1], i)
            attend(g, *cur[1], cur[2], nxt[0], i, 2, None if k0 is None else k_fft_steps(k0 + i))

    for layer in range(2):
        @phase("a_pro")
        def _():
            if layer:
                for s in range(8):
                    idft(3, s)
            r = norm(xs, un, ra, 0, 4)
            for i in range(8):
                if layer:
                    idft(3, i + 8)
                qkv(0, un, qa, ka, va, i)
                if i < 7:
                    r = norm(xs, un, ra, i + 1, 2 - layer, r)
                r = norm(xo, uo, rb_, i, 2 - layer, r)

        def group(g, c):
            overlap(g, odd, g, even, None if layer else 8 * g + 24)

            @pl.when(g < 3)
            def _():
                overlap(g + 1, even, g, odd, None)

            return c

        with _scope("a_grp"):
            jax.lax.fori_loop(0, 4, group, 0)

        @phase("a_proj")
        def _():
            for i in range(8):
                proj(xs, uo, un, i)
                attend(3, qb, kb, vb, rb_, un, i, 1)
            for i in range(8):
                proj(xo, un, uo, i)
                if not layer:
                    k_fft(56 + i)
            for s in range(NS):
                dft(0, s)

        @phase("conv")
        def _():
            done = []
            for rb in range(4):
                for i in range(16):
                    if rb < 3:
                        last = dft(rb + 1, i)
                    if layer and rb == 3:
                        if i < 8:
                            idft(2, i)
                            last = idft(2, i + 8)
                        else:
                            store_x(2, i - 8)
                    elif rb:
                        last = idft(rb - 1, i)
                    if layer and rb >= 2 and i < 8:
                        store_x(rb - 2, i)
                        if i == 7:
                            last = start_store(rb - 2, last)
                    done.append(last)
                    mark = conv(rb, i, done[-LAG] if len(done) >= LAG else None)
                    if rb < 3:
                        fence(spec[rb + 1], mark)

    with _scope("store_x"):
        last = start_store(2, jnp.zeros((8, R), F32))
        fence(spec[3], last)
        for jj in range(8):
            idft(3, jj)
            idft(3, jj + 8)
            store_x(3, jj)
        stores[3].start()
    with _scope("tail"):
        for cp in stores:
            cp.wait()


@jax.jit
def pallas_interleave_layers__sliding_local_dilated__ssm_conv_s4__prompt_kernel(
    A_x: jax.Array,
    A_wqkv: jax.Array,
    A_wo: jax.Array,
    B_u: jax.Array,
    B_A_re: jax.Array,
    B_A_im: jax.Array,
    B_B_re: jax.Array,
    B_B_im: jax.Array,
    B_C_re: jax.Array,
    B_C_im: jax.Array,
    B_log_dt: jax.Array,
    B_Dskip: jax.Array,
):
    del B_u
    f = _dft_matrix()
    lane = (np.arange(R) - 11) % R
    order = 16 * (lane % 8) + lane // 8
    fk = (f[:, order].astype(np.float32) * (2.0 / L)).astype(ml_dtypes.bfloat16)
    scratch = [
        pltpu.VMEM((D, L // 2), F32),
        pltpu.VMEM((D, L // 2), F32),
        pltpu.VMEM((D + 8, L // 2), U32),
        pltpu.VMEM((D + 8, L // 2), U32),
        pltpu.VMEM((4, 192, D), U32),
        pltpu.VMEM((D // 2, D), U32),
        pltpu.VMEM((D // 2, 128), U32),
        pltpu.VMEM((D, 128), F32),
        pltpu.VMEM((2, 8, 8, N), F32),
        pltpu.VMEM((4, 128, 2 * N), F32),
        *[pltpu.VMEM((n + 16, 2 * L), F32) for _, n in BLOCKS],
        pltpu.VMEM((D + 8, 2 * L), F32),
        pltpu.VMEM((D + 8, 22 * 2 * R), F32),
        pltpu.VMEM((128, 8 * R), F32),
        pltpu.VMEM((128, 15 * R), F32),
        pltpu.VMEM((128, 15 * R), F32),
        pltpu.VMEM((128, 8 * R), F32),
        pltpu.VMEM((128, 15 * R), F32),
        pltpu.VMEM((128, 15 * R), F32),
        pltpu.VMEM((15, 8, R), F32),
        pltpu.VMEM((15, 8, R), F32),
        *[pltpu.VMEM((D, R), F32)] * 2,
        *[pltpu.VMEM((L + 16, 128), BF16)] * 4,
        pltpu.VMEM((D, 3 * D), BF16),
        pltpu.VMEM((D, D), BF16),
        pltpu.VMEM((NS, R // 2, 2 * R), U32),
        pltpu.VMEM((NS, R // 2, 2 * R), U32),
        pltpu.VMEM((6, D, N), BF16),
        pltpu.SMEM((1,), jnp.int32),
        pltpu.VMEM((D,), BF16),
        pltpu.VMEM((D,), BF16),
        pltpu.SemaphoreType.DMA((13,)),
    ]
    hbm = pl.BlockSpec(memory_space=pl.ANY)
    out = pl.pallas_call(
        _kernel,
        out_shape=jax.ShapeDtypeStruct((L, D), BF16),
        in_specs=[hbm] * 14,
        out_specs=hbm,
        scratch_shapes=scratch,
        compiler_params=pltpu.CompilerParams(vmem_limit_bytes=100 * 1024 * 1024),
    )(np.zeros((1,), np.int32), A_x.reshape(L, D), A_wqkv, A_wo, B_A_re, B_A_im, B_B_re, B_B_im, B_C_re, B_C_im,
      B_log_dt, B_Dskip, _pack_rows(f), _pack_rows(fk))
    return out.reshape(1, L, D)
```

```python
import contextlib

import jax
import jax.numpy as jnp
import jax.experimental.pallas as pl
import jax.experimental.pallas.tpu as pltpu
import ml_dtypes
import numpy as np

L = 2048
D = 512
N = 128
NS = 16
R = 128
W = 8
EPS = 1e-5
_H = float(np.sqrt(0.5))
LAG = 4
BLOCKS = ((0, 128), (128, 128), (256, 128), (384, 128))
F32 = jnp.float32
BF16 = jnp.bfloat16
U32 = jnp.uint32
NEG = float(ml_dtypes.bfloat16(-1e9))

_NT = (((1,), (1,)), ((), ()))


def _slab(j):
    return (j % 2) * 8 + j // 2


def _dft_matrix():
    r = np.arange(R)
    k = np.arange(R) + 0.5
    f = np.zeros((NS, R, 2 * R), np.float64)
    for j in range(NS):
        th = 2.0 * np.pi * np.outer(NS * r + j, k) / (2 * L)
        f[_slab(j), :, :R] = np.cos(th)
        f[_slab(j), :, R:] = -np.sin(th)
    return f.astype(np.float32).astype(ml_dtypes.bfloat16)


def _pack_rows(a):
    u = np.ascontiguousarray(a).view(np.uint16).astype(np.uint32)
    return u[:, 0::2] | (u[:, 1::2] << np.uint32(16))


def _lag_tables():
    rho = []
    for s in range(8):
        lag = (256 * s + np.arange(NS)).astype(np.float32)
        rho.append([int(v) - 256 * s for v in lag.astype(ml_dtypes.bfloat16).astype(np.float32)])
    return rho


_RHO = _lag_tables()


def _cmul(a, b):
    return (a[0] * b[0] - a[1] * b[1], a[0] * b[1] + a[1] * b[0])


def _csq(a):
    t = a[0] * a[1]
    return ((a[0] - a[1]) * (a[0] + a[1]), t + t)


def _cadd(a, b):
    return (a[0] + b[0], a[1] + b[1])


def _csub(a, b):
    return (a[0] - b[0], a[1] - b[1])


def _split(p, e):
    plus, minus = [], []
    for lo, hi in zip(p[:len(p) // 2], p[len(p) // 2:]):
        if e % 4:
            hi = ((hi[0] - hi[1]) * _H, (hi[0] + hi[1]) * _H)
        if e >= 4:
            plus.append((lo[0] - hi[1], lo[1] + hi[0]))
            minus.append((lo[0] + hi[1], lo[1] - hi[0]))
        else:
            plus.append(_cadd(lo, hi))
            minus.append(_csub(lo, hi))
    return plus, minus


def _merge(plus, minus, e):
    lo, hi = [], []
    for p, m in zip(plus, minus):
        lo.append(_cadd(p, m))
        d = (p[1] - m[1], m[0] - p[0]) if e >= 4 else _csub(p, m)
        hi.append(((d[0] + d[1]) * _H, (d[1] - d[0]) * _H) if e % 4 else d)
    return lo + hi


def _factor_coeffs(k, e):
    if e % 8 == 0:
        (p,), (m,) = _split(k, e // 2)
        return [(p[0] * 0.5, p[1] * 0.5), (m[0] * 0.5, m[1] * 0.5)]
    c, s = float(np.cos(np.pi * e / 8)), float(np.sin(np.pi * e / 8))
    wk = (k[1][0] * c - k[1][1] * s, k[1][0] * s + k[1][1] * c)
    return [k[0], _csub(wk, k[0]), _csub(k[1], k[0])]


def _factor_mul(a, coeffs, e):
    if e % 8 == 0:
        (p,), (m,) = _split(a, e // 2)
        return _merge([_cmul(p, coeffs[0])], [_cmul(m, coeffs[1])], e // 2)
    t = _cmul(_cadd(a[0], a[1]), coeffs[0])
    return [_cadd(t, _cmul(a[1], coeffs[1])), _cadd(t, _cmul(a[0], coeffs[2]))]


def _coeff_slots(e):
    if e % 8 == 0:
        return [e // 4, e // 4 + 1]
    n = 4 + 3 * [2, 4, 6, 10, 12, 14].index(e)
    return [n, n + 1, n + 2]


def _scope(name):
    return contextlib.nullcontext()


def _ds(i, n):
    if isinstance(i, int):
        return slice(i * n, (i + 1) * n)
    return pl.ds(pl.multiple_of(i * n, n), n)


def _pack(x):
    return pltpu.bitcast(x.astype(BF16), U32)


def _unpack(x):
    return pltpu.bitcast(x, BF16)


def _dot(a, b, dims=(((1,), (0,)), ((), ()))):
    return jax.lax.dot_general(a, b, dims, preferred_element_type=F32)


def _halves(u):
    return pltpu.bitcast(u << 16, F32), pltpu.bitcast(u & jnp.uint32(0xFFFF0000), F32)


def _kernel(zero_hbm, x_hbm, wqkv_hbm, wo_hbm, are, aim, bre, bim, cre, cim,
            ldt_hbm, dsk_hbm, f_hbm, fk_hbm, o_hbm,
            xs, xo, un, uo, wt, wot, dtb, dskb, pw_ref, rhs_ref, s0, s1, s2, s3, kspec, khat, qa, ka, va, qb, kb, vb,
            ra, rb_, cen0, cen1,
            io0, io1, io2, io3, wqkv_ref, wo_ref, f_ref, fk_ref, ssm, zero_ref, ldt_ref, dsk_ref, sems):
    def fetch_ssm(rows, sem):
        return [pltpu.make_async_copy(p.at[rows], ssm.at[n, rows], sem)
                for n, p in enumerate((are, aim, bre, bim, cre, cim))]

    small = [pltpu.make_async_copy(src, dst, sems.at[10 + n]) for n, (src, dst) in enumerate(
        [(zero_hbm, zero_ref), (ldt_hbm, ldt_ref), (dsk_hbm, dsk_ref)])]
    for cp in small:
        cp.start()
    first = fetch_ssm(pl.ds(0, 144), sems.at[8])
    for cp in first:
        cp.start()
    second = fetch_ssm(pl.ds(144, D - 144), sems.at[9])
    second += [pltpu.make_async_copy(fk_hbm, fk_ref, sems.at[4])]
    for cp in second:
        cp.start()
    xio = (io0, io1, io2, io3)
    loads = []
    loads += [pltpu.make_async_copy(x_hbm.at[:, c * 128:(c + 1) * 128], xio[c].at[0:L], sems.at[c])
              for c in range(4)]
    loads += [pltpu.make_async_copy(src, dst, sems.at[5 + n]) for n, (src, dst) in enumerate(
        [(wqkv_hbm, wqkv_ref), (wo_hbm, wo_ref), (f_hbm, f_ref)])]

    spec = (s0, s1, s2, s3)
    cen = (cen0, cen1)

    def fence(ref, val):
        row = ref.shape[0] - 8 + zero_ref[0]
        ref[pl.ds(pl.multiple_of(row, 8), 8), 0:128] = val

    for cp in small:
        cp.wait()
    dt_row = jnp.exp(ldt_ref[...].astype(F32)).reshape(1, D)
    dtb[...] = _pack(jnp.broadcast_to(dt_row, (128, D)).T)
    dskb[...] = jnp.broadcast_to(dsk_ref[...].astype(F32).reshape(1, D) * (2.0 / L), (128, D)).T

    lane8 = jax.lax.broadcasted_iota(jnp.int32, (8, R), 1)
    sub8 = jax.lax.broadcasted_iota(jnp.int32, (8, N), 0)
    low = sub8 < 4
    steps = (1, 2, 4, 256)

    def halves_of(a, b):
        return tuple(jnp.where(low, u, v) for u, v in zip(a, b))

    def powers(i):
        dts = _halves(dtb[_ds(i, 8), :])
        are, aim, bre, bim, cre, cim = [
            _halves(pltpu.bitcast(ssm[n, _ds(i, 16), :], U32)) for n in range(6)]
        for h in range(2):
            dt = dts[h]
            li = dt * aim[h]
            mag = jnp.exp(dt * are[h])
            zp = {1: (mag * jnp.cos(li), mag * jnp.sin(li))}
            for e in (1, 2, 4, 8, 16, 32, 64, 128):
                zp[2 * e] = _csq(zp[e])
            for n, e in enumerate(steps):
                pw_ref[h, 2 * n] = zp[e][0]
                pw_ref[h, 2 * n + 1] = zp[e][1]
            w = _cmul((cre[h], cim[h]), (dt * bre[h], dt * bim[h]))
            w, z8, z16 = [(v[0], -v[1]) for v in (w, zp[8], zp[16])]
            w8 = _cmul(w, z8)
            for t in range(2):
                def pick(v):
                    return tuple(jnp.take_along_axis(u, 4 * t + 3 - (sub8 & 3), axis=0) for u in v)

                step = pick(z16)
                rows = [halves_of(pick(w), pick(w8)) if t else halves_of(pick(w8), pick(_cmul(w, z16)))]
                for _ in range(15):
                    rows.append(_cmul(rows[-1], step))
                if not t:
                    rows = [halves_of(rows[-1], pick(w))] + rows[:-1]
                rhs_ref[2 * h + t] = jnp.concatenate([jnp.concatenate(v, axis=1) for v in rows], axis=0)

    offsets = sorted({256 * s + p % 8 for s in range(8) for p in _RHO[s]}) + [L]
    plain, turned = offsets[:11], offsets[11:]

    def turn(v):
        return pltpu.roll(v, 4, 0)

    def taps(i):
        outs = []
        for h in range(2):
            zp = {e: (pw_ref[h, 2 * n], pw_ref[h, 2 * n + 1]) for n, e in enumerate(steps)}
            zp[0] = (jnp.ones((8, N), F32), jnp.zeros((8, N), F32))
            zt = {e: (turn(zp[e][0]), turn(zp[e][1])) for e in (4, 256)}
            for table, exps in ((zp, plain + turned[:1]), (zt, turned[1:])):
                for e in exps:
                    if e in table:
                        continue
                    if e % 2 == 0 and e // 2 in table:
                        table[e] = _csq(table[e // 2])
                    else:
                        inc = next(v for v in steps if v in table and e - v in table)
                        table[e] = _cmul(table[e - inc], table[inc])
            zt[turned[0]] = tuple(turn(v) for v in zp[turned[0]])
            pairs = [(zp[a], zt[b]) for a, b in zip(plain, turned)] + [(zp[plain[-1]],) * 2]
            for t in range(2):
                lhs = [jnp.concatenate(halves_of(*v[::-1]) if t else halves_of(*v), axis=1) for v in pairs]
                outs.append(_dot(jnp.concatenate(lhs, axis=0), rhs_ref[2 * h + t], _NT))
        lo, hi = [pltpu.bitcast(pltpu.pack_elementwise([outs[t], outs[2 + t]], packed_dtype=BF16), U32)
                  for t in range(2)]
        merged = {a: jnp.where(low, lo[_ds(n, 8)], hi[_ds(n, 8)]) for n, a in enumerate(plain)}
        merged.update({a: turn(jnp.where(low, hi[_ds(n, 8)], lo[_ds(n, 8)])) for n, a in enumerate(turned)})

        def align(a, shift):
            return pltpu.roll(merged[a], shift, 1, stride=1, stride_axis=0)

        piece = {(s, p): align(256 * s + p % 8, s + 4 - 4 * (p // 8))
                 for s in range(8) for p in sorted(set(_RHO[s]) - {16})}
        pos = (lane8 - 11) & 127
        memo = {}
        for j in range(NS):
            key = ()
            acc = None
            for s in range(7, -1, -1):
                key = key + (_RHO[s][j],)
                if key not in memo:
                    pc = carry if _RHO[s][j] == 16 else piece[s, _RHO[s][j]]
                    same = acc is None or pc is acc
                    memo[key] = pc if same else jnp.where((pos & 7) == s, pc, acc)
                acc = memo[key]
            (un, uo)[j % 2][_ds(i + D // 16, 8), _ds(j // 2, R)] = acc
            if j == 0:
                carry = jnp.where(pos >= 120, pltpu.roll(acc, 128 - 9, 1), pltpu.roll(acc, 128 - 8, 1))
                carry = jnp.where(pos == 127, align(L, 3), carry)

    def gen_k(rb):
        for n in range(8):
            i = 8 * rb + n
            taps(i)
            if i + 1 < D // 16:
                powers(i + 1)
            if rb:
                dft_k(rb - 1, range(2 * n, 2 * n + 2))

    def dft_k(rb, which=range(NS)):
        for s in which:
            u = (un, uo)[s // 8][_ds(rb + 4, 64), _ds(s % 8, R)]
            kspec[_ds(rb, 128), _ds(s, 2 * R)] = _dot(_unpack(u), _unpack(fk_ref[s]))

    with _scope("head"):
        for cp in first:
            cp.wait()
        for cp in loads:
            cp.start()

    with _scope("gen_k"):
        powers(0)
        gen_k(0)
        for cp in second:
            cp.wait()
        for rb in range(1, 4):
            pl.when(zero_ref[0] < rb)(lambda: gen_k(rb))

    for cp in loads:
        cp.wait()

    xu = [r.bitcast(U32) for r in xio]

    def load_x(b):
        for jj in range(8):
            ev, od = _halves(xu[b][pl.ds(jj, R, stride=8), :].T)
            xs[_ds(b, 128), _ds(jj, R)] = ev
            xo[_ds(b, 128), _ds(jj, R)] = od

    m_i = jax.lax.broadcasted_iota(jnp.int32, (128, 128), 0)
    c_i = jax.lax.broadcasted_iota(jnp.int32, (128, 128), 1)
    perm = jnp.where(c_i == (m_i & 7) * 16 + (m_i >> 3), 1.0, 0.0).astype(BF16)

    def prep_w(g):
        for t in range(3):
            wt[g, _ds(t, 64), :] = _pack(_dot(perm, wqkv_ref[:, _ds((t + 1) % 3 * 4 + g, 128)], _NT))
        wot[:, _ds(g, 128)] = _pack(_dot(perm, wo_ref[_ds(g, 128), :]).T)

    def dft(rb, s):
        at, n = BLOCKS[rb]
        u = (un, uo)[s // 8][at // 2:(at + n) // 2, _ds(s % 8, R)]
        y = _dot(_unpack(u), _unpack(f_ref[s]))
        spec[rb][0:n, _ds(s, 2 * R)] = y
        return y[-8:, R:]

    def idft(rb, s):
        at, n = BLOCKS[rb]
        y = _dot(spec[rb][0:n, _ds(s, 2 * R)], _unpack(f_ref[s]), _NT)
        (xs, xo)[s // 8][at:at + n, _ds(s % 8, R)] += y
        return y[-8:]

    def load_spec(ref, rows, order):
        return [(ref[rows, _ds(2 * s, R)], ref[rows, _ds(2 * s + 1, R)]) for s in order]

    def store_spec(ref, rows, order, vals):
        for s, v in zip(order, vals):
            ref[rows, _ds(2 * s, R)] = v[0]
            ref[rows, _ds(2 * s + 1, R)] = v[1]

    slabs = [_slab(j) for j in range(NS)]

    def half(buf, rows, e8, bias=None):
        out = []
        for j in range(8):
            lo, hi = load_spec(buf, rows, [slabs[j], slabs[j + 8]])
            if j == 0 and bias is not None:
                lo = (lo[0] + bias, lo[1])
            out.append(_csub(lo, hi) if e8 else _cadd(lo, hi))
        return out

    def k_fft_steps(i):
        rows = _ds(i, 8)
        for e8 in (8, 0):
            quartics = _split(half(kspec, rows, e8, dskb[rows, :]), e8 // 2)
            for e4, p4 in zip((e8 // 2, e8 // 2 + 8), quartics):
                for e2, p2 in zip((e4 // 2, e4 // 2 + 8), _split(p4, e4 // 2)):
                    store_spec(khat, rows, _coeff_slots(e2), _factor_coeffs(p2, e2))
                yield

    def k_fft(i):
        for _ in k_fft_steps(i):
            pass

    def conv(rb, i, after=None):
        at, size = BLOCKS[rb]
        buf, rows, park = spec[rb], _ds(i, 8), _ds(size // 8, 8)
        for e8 in (8, 0):
            quartics = []
            for e4, p4 in zip((e8 // 2, e8 // 2 + 8), _split(half(buf, rows, e8), e8 // 2)):
                prods = [_factor_mul(p2, load_spec(khat, _ds(at // 8 + i, 8), _coeff_slots(e2)), e2)
                         for e2, p2 in zip((e4 // 2, e4 // 2 + 8), _split(p4, e4 // 2))]
                quartics.append(_merge(*prods, e4 // 2))
                if e4 < 8:
                    fence(khat, prods[1][1][0])
            mark = prods[1][1][0]
            fence(buf, mark if e8 or after is None else after)
            for j, v in enumerate(_merge(*quartics, e8 // 2)):
                if e8:
                    store_spec(buf, park, [j], [v])
                else:
                    (o,) = load_spec(buf, park, [j])
                    store_spec(buf, rows, [slabs[j], slabs[j + 8]], [_cadd(v, o), _csub(v, o)])
        return mark

    lane = jax.lax.broadcasted_iota(jnp.int32, (128, R), 1)

    def qkv(g, u, qs, ks, vs, i):
        y = _dot(_unpack(wt[g]), _unpack(u[0:D // 2, _ds(i, R)]))
        k, v, q = y[0:128], y[128:256], y[256:384]
        qs[:, _ds(i, R)] = q
        ks[:, _ds(i + 7, R)] = k
        vs[:, _ds(i + 7, R)] = v
        if i:
            ks[:, _ds(i - 1, R)] = pltpu.roll(k, 1, 1)
            vs[:, _ds(i - 1, R)] = jnp.where(lane == 0, va[:, _ds(7, R)], pltpu.roll(v, 1, 1))

    never = lane8 < zero_ref[0]

    def attend(g, qs, ks, vs, rs, o, i, ways, side=None):
        logits = []
        for w in range(W):
            lg = None
            for c in range(16):
                term = qs[_ds(c, 8), _ds(i, R)] * ks[_ds(c, 8), _ds(7 + i - w, R)]
                if c:
                    lg = lg + term
                else:
                    lg = term if w < ways else jnp.where(never, logits[w - ways], term)
            logits.append(lg)
            if side and w in (1, 7):
                fence(kspec, lg)
                next(side)
        scale = rs[7 + i] * 0.25
        logits = [lg * scale * rs[7 + i - w] for w, lg in enumerate(logits)]
        logits = [jnp.where(lane8 == 0, NEG, lg) if w > i else lg for w, lg in enumerate(logits)]
        mx = logits[0]
        for lg in logits[1:]:
            mx = jnp.maximum(mx, lg)
        es = [jnp.exp(lg - mx) for lg in logits]
        den = es[0]
        for e in es[1:]:
            den = den + e
        inv = 1.0 / den
        probs = [e * rs[7 + i - w] * inv for w, e in enumerate(es)]
        outs = []
        for c in range(16):
            acc = None
            for w in range(W):
                term = vs[_ds(c, 8), _ds(7 + i - w, R)] * probs[w]
                if w:
                    acc = acc + term
                else:
                    acc = term if c < ways else jnp.where(never, outs[c - ways], term)
            outs.append(acc)
            if side and c in (3, 11):
                fence(kspec, acc)
                next(side)
        o[_ds(g + 4, 64), _ds(i, R)] = _pack(jnp.concatenate(outs, axis=0))

    def chain_sum(vals, ways):
        parts = vals[:ways]
        for n, v in enumerate(vals[ways:]):
            parts[n % ways] = parts[n % ways] + v
        return jnp.sum(sum(parts[1:], parts[0]), axis=0, keepdims=True)

    def row_mean(x, ways, after=None):
        parts = [x[_ds(n, 8)] for n in range(D // 8)]
        if after is not None:
            parts[0] = jnp.where(never, after, parts[0])
        return chain_sum(parts, ways) * (1.0 / D)

    def norm(x, u, rs, i, ways, after=None):
        c = x[:, _ds(i, R)] - row_mean(x[:, _ds(i, R)], 2, after)
        r = jnp.broadcast_to(jax.lax.rsqrt(row_mean(c * c, ways) + EPS), (8, R))
        u[0:D // 2, _ds(i, R)] = _pack(c)
        rs[7 + i] = r
        if i:
            rs[i - 1] = jnp.where(lane8 == 0, ra[7], pltpu.roll(r, 1, 1))
        return r

    def proj(x, o, u, i):
        y = x[:, _ds(i, R)] + _dot(_unpack(wot[...]), _unpack(o[D // 2:D, _ds(i, R)]))
        x[:, _ds(i, R)] = y
        cen_ = cen[i % 2]
        cen_[...] = x[:, _ds(i, R)] - row_mean(y, 2)
        c = cen_[pl.ds(pl.multiple_of(zero_ref[0], 8), D)]
        u[0:D // 2, _ds(i, R)] = _pack(cen_[...] * jax.lax.rsqrt(row_mean(c * c, 1) + EPS))

    stores = [pltpu.make_async_copy(xio[c].at[0:L], o_hbm.at[:, c * 128:(c + 1) * 128], sems.at[c])
              for c in range(4)]

    def store_x(b, jj):
        t = pltpu.pack_elementwise(
            [xs[_ds(b, 128), _ds(jj, R)], xo[_ds(b, 128), _ds(jj, R)]], packed_dtype=BF16)
        xu[b][pl.ds(jj, R, stride=8), :] = pltpu.bitcast(t, U32).T

    def fence_io(b, val):
        xio[b][pl.ds(pl.multiple_of(L + zero_ref[0], 16), 16), :] = pltpu.bitcast(val, BF16)

    def start_store(b, val):
        stores[b].start()
        fence_io(b, val)
        return pltpu.bitcast(xio[b][L:L + 16, :], F32)

    def phase(name):
        def run(fn):
            with _scope(name):
                pl.when(zero_ref[0] == 0)(fn)
        return run

    @phase("prep")
    def _():
        dft_k(3)
        for b in range(4):
            load_x(b)
            prep_w(b)
            for n in range(2):
                k_fft(2 * b + n)

    even, odd = (un, (qa, ka, va), ra), (uo, (qb, kb, vb), rb_)

    def overlap(g_next, nxt, g, cur, k0):
        for i in range(8):
            qkv(g_next, nxt[0], *nxt[1], i)
            attend(g, *cur[1], cur[2], nxt[0], i, 2, None if k0 is None else k_fft_steps(k0 + i))

    for layer in range(2):
        @phase("a_pro")
        def _():
            if layer:
                for s in range(8):
                    idft(3, s)
            r = norm(xs, un, ra, 0, 4)
            for i in range(8):
                if layer:
                    idft(3, i + 8)
                qkv(0, un, qa, ka, va, i)
                if i < 7:
                    r = norm(xs, un, ra, i + 1, 2 - layer, r)
                r = norm(xo, uo, rb_, i, 2 - layer, r)

        def group(g, c):
            overlap(g, odd, g, even, None if layer else 8 * g + 8)

            @pl.when(g < 3)
            def _():
                overlap(g + 1, even, g, odd, None if layer else 8 * g + 40)

            return c

        with _scope("a_grp"):
            jax.lax.fori_loop(0, 4, group, 0)

        @phase("a_proj")
        def _():
            for i in range(8):
                proj(xs, uo, un, i)
                attend(3, qb, kb, vb, rb_, un, i, 1)
            for i in range(8):
                proj(xo, un, uo, i)
            for s in range(NS):
                dft(0, s)

        @phase("conv")
        def _():
            done = []
            for rb in range(4):
                for i in range(16):
                    if rb < 3:
                        last = dft(rb + 1, i)
                    if layer and rb == 3:
                        if i < 8:
                            idft(2, i)
                            last = idft(2, i + 8)
                        else:
                            store_x(2, i - 8)
                    elif rb:
                        last = idft(rb - 1, i)
                    if layer and rb >= 2 and i < 8:
                        store_x(rb - 2, i)
                        if i == 7:
                            last = start_store(rb - 2, last)
                    done.append(last)
                    mark = conv(rb, i, done[-LAG] if len(done) >= LAG else None)
                    if rb < 3:
                        fence(spec[rb + 1], mark)

    with _scope("store_x"):
        last = start_store(2, jnp.zeros((8, R), F32))
        fence(spec[3], last)
        for jj in range(8):
            idft(3, jj)
            idft(3, jj + 8)
            store_x(3, jj)
        stores[3].start()
    with _scope("tail"):
        for cp in stores:
            cp.wait()


@jax.jit
def pallas_interleave_layers__sliding_local_dilated__ssm_conv_s4__prompt_kernel(
    A_x: jax.Array,
    A_wqkv: jax.Array,
    A_wo: jax.Array,
    B_u: jax.Array,
    B_A_re: jax.Array,
    B_A_im: jax.Array,
    B_B_re: jax.Array,
    B_B_im: jax.Array,
    B_C_re: jax.Array,
    B_C_im: jax.Array,
    B_log_dt: jax.Array,
    B_Dskip: jax.Array,
):
    del B_u
    f = _dft_matrix()
    lane = (np.arange(R) - 11) % R
    order = 16 * (lane % 8) + lane // 8
    fk = (f[:, order].astype(np.float32) * (2.0 / L)).astype(ml_dtypes.bfloat16)
    scratch = [
        pltpu.VMEM((D, L // 2), F32),
        pltpu.VMEM((D, L // 2), F32),
        pltpu.VMEM((D + 8, L // 2), U32),
        pltpu.VMEM((D + 8, L // 2), U32),
        pltpu.VMEM((4, 192, D), U32),
        pltpu.VMEM((D // 2, D), U32),
        pltpu.VMEM((D // 2, 128), U32),
        pltpu.VMEM((D, 128), F32),
        pltpu.VMEM((2, 8, 8, N), F32),
        pltpu.VMEM((4, 128, 2 * N), F32),
        *[pltpu.VMEM((n + 16, 2 * L), F32) for _, n in BLOCKS],
        pltpu.VMEM((D + 8, 2 * L), F32),
        pltpu.VMEM((D + 8, 22 * 2 * R), F32),
        pltpu.VMEM((128, 8 * R), F32),
        pltpu.VMEM((128, 15 * R), F32),
        pltpu.VMEM((128, 15 * R), F32),
        pltpu.VMEM((128, 8 * R), F32),
        pltpu.VMEM((128, 15 * R), F32),
        pltpu.VMEM((128, 15 * R), F32),
        pltpu.VMEM((15, 8, R), F32),
        pltpu.VMEM((15, 8, R), F32),
        *[pltpu.VMEM((D, R), F32)] * 2,
        *[pltpu.VMEM((L + 16, 128), BF16)] * 4,
        pltpu.VMEM((D, 3 * D), BF16),
        pltpu.VMEM((D, D), BF16),
        pltpu.VMEM((NS, R // 2, 2 * R), U32),
        pltpu.VMEM((NS, R // 2, 2 * R), U32),
        pltpu.VMEM((6, D, N), BF16),
        pltpu.SMEM((1,), jnp.int32),
        pltpu.VMEM((D,), BF16),
        pltpu.VMEM((D,), BF16),
        pltpu.SemaphoreType.DMA((13,)),
    ]
    hbm = pl.BlockSpec(memory_space=pl.ANY)
    out = pl.pallas_call(
        _kernel,
        out_shape=jax.ShapeDtypeStruct((L, D), BF16),
        in_specs=[hbm] * 14,
        out_specs=hbm,
        scratch_shapes=scratch,
        compiler_params=pltpu.CompilerParams(vmem_limit_bytes=100 * 1024 * 1024),
    )(np.zeros((1,), np.int32), A_x.reshape(L, D), A_wqkv, A_wo, B_A_re, B_A_im, B_B_re, B_B_im, B_C_re, B_C_im,
      B_log_dt, B_Dskip, _pack_rows(f), _pack_rows(fk))
    return out.reshape(1, L, D)
```

```python
import jax
import jax.numpy as jnp
import jax.experimental.pallas as pl
import jax.experimental.pallas.tpu as pltpu
import ml_dtypes
import numpy as np

L = 2048
D = 512
N = 128
NS = 16
R = 128
W = 8
EPS = 1e-5
_H = float(np.sqrt(0.5))
LAG = 4
F32 = jnp.float32
BF16 = jnp.bfloat16
U32 = jnp.uint32
NEG = float(ml_dtypes.bfloat16(-1e9))

_NT = (((1,), (1,)), ((), ()))


def _slab(j):
    return (j % 2) * 8 + j // 2


def _dft_matrix():
    r = np.arange(R)
    k = np.arange(R) + 0.5
    f = np.zeros((NS, R, 2 * R), np.float64)
    for j in range(NS):
        th = 2.0 * np.pi * np.outer(NS * r + j, k) / (2 * L)
        f[_slab(j), :, :R] = np.cos(th)
        f[_slab(j), :, R:] = -np.sin(th)
    return f.astype(np.float32).astype(ml_dtypes.bfloat16)


def _pack_rows(a):
    u = np.ascontiguousarray(a).view(np.uint16).astype(np.uint32)
    return u[:, 0::2] | (u[:, 1::2] << np.uint32(16))


def _lag_tables():
    rho = []
    for s in range(8):
        lag = (256 * s + np.arange(NS)).astype(np.float32)
        rho.append([int(v) - 256 * s for v in lag.astype(ml_dtypes.bfloat16).astype(np.float32)])
    return rho


_RHO = _lag_tables()


def _cmul(a, b):
    return (a[0] * b[0] - a[1] * b[1], a[0] * b[1] + a[1] * b[0])


def _csq(a):
    t = a[0] * a[1]
    return ((a[0] - a[1]) * (a[0] + a[1]), t + t)


def _cadd(a, b):
    return (a[0] + b[0], a[1] + b[1])


def _csub(a, b):
    return (a[0] - b[0], a[1] - b[1])


def _split(p, e):
    plus, minus = [], []
    for lo, hi in zip(p[:len(p) // 2], p[len(p) // 2:]):
        if e % 4:
            hi = ((hi[0] - hi[1]) * _H, (hi[0] + hi[1]) * _H)
        if e >= 4:
            plus.append((lo[0] - hi[1], lo[1] + hi[0]))
            minus.append((lo[0] + hi[1], lo[1] - hi[0]))
        else:
            plus.append(_cadd(lo, hi))
            minus.append(_csub(lo, hi))
    return plus, minus


def _merge(plus, minus, e):
    lo, hi = [], []
    for p, m in zip(plus, minus):
        lo.append(_cadd(p, m))
        d = (p[1] - m[1], m[0] - p[0]) if e >= 4 else _csub(p, m)
        hi.append(((d[0] + d[1]) * _H, (d[1] - d[0]) * _H) if e % 4 else d)
    return lo + hi


def _factor_coeffs(k, e):
    if e % 8 == 0:
        (p,), (m,) = _split(k, e // 2)
        return [(p[0] * 0.5, p[1] * 0.5), (m[0] * 0.5, m[1] * 0.5)]
    c, s = float(np.cos(np.pi * e / 8)), float(np.sin(np.pi * e / 8))
    wk = (k[1][0] * c - k[1][1] * s, k[1][0] * s + k[1][1] * c)
    return [k[0], _csub(wk, k[0]), _csub(k[1], k[0])]


def _factor_mul(a, coeffs, e):
    if e % 8 == 0:
        (p,), (m,) = _split(a, e // 2)
        return _merge([_cmul(p, coeffs[0])], [_cmul(m, coeffs[1])], e // 2)
    t = _cmul(_cadd(a[0], a[1]), coeffs[0])
    return [_cadd(t, _cmul(a[1], coeffs[1])), _cadd(t, _cmul(a[0], coeffs[2]))]


def _coeff_slots(e):
    if e % 8 == 0:
        return [e // 4, e // 4 + 1]
    n = 4 + 3 * [2, 4, 6, 10, 12, 14].index(e)
    return [n, n + 1, n + 2]


def _ds(i, n):
    if isinstance(i, int):
        return slice(i * n, (i + 1) * n)
    return pl.ds(pl.multiple_of(i * n, n), n)


def _pack(x):
    return pltpu.bitcast(x.astype(BF16), U32)


def _unpack(x):
    return pltpu.bitcast(x, BF16)


def _dot(a, b, dims=(((1,), (0,)), ((), ()))):
    return jax.lax.dot_general(a, b, dims, preferred_element_type=F32)


def _halves(u):
    return pltpu.bitcast(u << 16, F32), pltpu.bitcast(u & jnp.uint32(0xFFFF0000), F32)


def _kernel(zero_hbm, x_hbm, wqkv_hbm, wo_hbm, are, aim, bre, bim, cre, cim,
            ldt_hbm, dsk_hbm, f_hbm, fk_hbm, o_hbm,
            xs, xo, un, uo, wt, wot, dtb, dskb, pw_ref, rhs_ref, s0, s1, s2, s3, kspec, khat,
            qa, ka, va, qb, kb, vb, ra, rb_, cen0, cen1,
            io0, io1, io2, io3, wqkv_ref, wo_ref, f_ref, fk_ref, ssm, zero_ref, ldt_ref, dsk_ref, sems):
    def fetch_ssm(rows, sem):
        return [pltpu.make_async_copy(p.at[rows], ssm.at[n, rows], sem)
                for n, p in enumerate((are, aim, bre, bim, cre, cim))]

    small = [pltpu.make_async_copy(src, dst, sems.at[10 + n]) for n, (src, dst) in enumerate(
        [(zero_hbm, zero_ref), (ldt_hbm, ldt_ref), (dsk_hbm, dsk_ref)])]
    for cp in small:
        cp.start()
    first = fetch_ssm(pl.ds(0, 144), sems.at[8])
    for cp in first:
        cp.start()
    second = fetch_ssm(pl.ds(144, D - 144), sems.at[9])
    second += [pltpu.make_async_copy(fk_hbm, fk_ref, sems.at[4])]
    for cp in second:
        cp.start()
    xio = (io0, io1, io2, io3)
    loads = [pltpu.make_async_copy(x_hbm.at[:, c * 128:(c + 1) * 128], xio[c].at[0:L], sems.at[c])
             for c in range(4)]
    loads += [pltpu.make_async_copy(src, dst, sems.at[5 + n]) for n, (src, dst) in enumerate(
        [(wqkv_hbm, wqkv_ref), (wo_hbm, wo_ref), (f_hbm, f_ref)])]

    spec = (s0, s1, s2, s3)
    cen = (cen0, cen1)

    def fence(ref, val):
        row = ref.shape[0] - 8 + zero_ref[0]
        ref[pl.ds(pl.multiple_of(row, 8), 8), 0:128] = val

    for cp in small:
        cp.wait()
    dt_row = jnp.exp(ldt_ref[...].astype(F32)).reshape(1, D)
    dtb[...] = _pack(jnp.broadcast_to(dt_row, (128, D)).T)
    dskb[...] = jnp.broadcast_to(dsk_ref[...].astype(F32).reshape(1, D) * (2.0 / L), (128, D)).T

    lane8 = jax.lax.broadcasted_iota(jnp.int32, (8, R), 1)
    sub8 = jax.lax.broadcasted_iota(jnp.int32, (8, N), 0)
    low = sub8 < 4
    steps = (1, 2, 4, 256)

    def halves_of(a, b):
        return tuple(jnp.where(low, u, v) for u, v in zip(a, b))

    def powers(i):
        dts = _halves(dtb[_ds(i, 8), :])
        are, aim, bre, bim, cre, cim = [
            _halves(pltpu.bitcast(ssm[n, _ds(i, 16), :], U32)) for n in range(6)]
        for h in range(2):
            dt = dts[h]
            li = dt * aim[h]
            mag = jnp.exp(dt * are[h])
            zp = {1: (mag * jnp.cos(li), mag * jnp.sin(li))}
            for e in (1, 2, 4, 8, 16, 32, 64, 128):
                zp[2 * e] = _csq(zp[e])
            for n, e in enumerate(steps):
                pw_ref[h, 2 * n] = zp[e][0]
                pw_ref[h, 2 * n + 1] = zp[e][1]
            w = _cmul((cre[h], cim[h]), (dt * bre[h], dt * bim[h]))
            w, z8, z16 = [(v[0], -v[1]) for v in (w, zp[8], zp[16])]
            w8 = _cmul(w, z8)
            for t in range(2):
                def pick(v):
                    return tuple(jnp.take_along_axis(u, 4 * t + 3 - (sub8 & 3), axis=0) for u in v)

                step = pick(z16)
                rows = [halves_of(pick(w), pick(w8)) if t else halves_of(pick(w8), pick(_cmul(w, z16)))]
                for _ in range(15):
                    rows.append(_cmul(rows[-1], step))
                if not t:
                    rows = [halves_of(rows[-1], pick(w))] + rows[:-1]
                rhs_ref[2 * h + t] = jnp.concatenate([jnp.concatenate(v, axis=1) for v in rows], axis=0)

    offsets = sorted({256 * s + p % 8 for s in range(8) for p in _RHO[s]}) + [L]
    plain, turned = offsets[:11], offsets[11:]

    def turn(v):
        return pltpu.roll(v, 4, 0)

    def taps(i):
        outs = []
        for h in range(2):
            zp = {e: (pw_ref[h, 2 * n], pw_ref[h, 2 * n + 1]) for n, e in enumerate(steps)}
            zp[0] = (jnp.ones((8, N), F32), jnp.zeros((8, N), F32))
            zt = {e: (turn(zp[e][0]), turn(zp[e][1])) for e in (4, 256)}
            for table, exps in ((zp, plain + turned[:1]), (zt, turned[1:])):
                for e in exps:
                    if e in table:
                        continue
                    if e % 2 == 0 and e // 2 in table:
                        table[e] = _csq(table[e // 2])
                    else:
                        inc = next(v for v in steps if v in table and e - v in table)
                        table[e] = _cmul(table[e - inc], table[inc])
            zt[turned[0]] = tuple(turn(v) for v in zp[turned[0]])
            pairs = [(zp[a], zt[b]) for a, b in zip(plain, turned)] + [(zp[plain[-1]],) * 2]
            for t in range(2):
                lhs = [jnp.concatenate(halves_of(*v[::-1]) if t else halves_of(*v), axis=1) for v in pairs]
                outs.append(_dot(jnp.concatenate(lhs, axis=0), rhs_ref[2 * h + t], _NT))
        lo, hi = [pltpu.bitcast(pltpu.pack_elementwise([outs[t], outs[2 + t]], packed_dtype=BF16), U32)
                  for t in range(2)]
        merged = {a: jnp.where(low, lo[_ds(n, 8)], hi[_ds(n, 8)]) for n, a in enumerate(plain)}
        merged.update({a: turn(jnp.where(low, hi[_ds(n, 8)], lo[_ds(n, 8)])) for n, a in enumerate(turned)})

        def align(a, shift):
            return pltpu.roll(merged[a], shift, 1, stride=1, stride_axis=0)

        piece = {(s, p): align(256 * s + p % 8, s + 4 - 4 * (p // 8))
                 for s in range(8) for p in sorted(set(_RHO[s]) - {16})}
        pos = (lane8 - 11) & 127
        memo = {}
        for j in range(NS):
            key = ()
            acc = None
            for s in range(7, -1, -1):
                key = key + (_RHO[s][j],)
                if key not in memo:
                    pc = carry if _RHO[s][j] == 16 else piece[s, _RHO[s][j]]
                    same = acc is None or pc is acc
                    memo[key] = pc if same else jnp.where((pos & 7) == s, pc, acc)
                acc = memo[key]
            (un, uo)[j % 2][_ds(i + D // 16, 8), _ds(j // 2, R)] = acc
            if j == 0:
                carry = jnp.where(pos >= 120, pltpu.roll(acc, 128 - 9, 1), pltpu.roll(acc, 128 - 8, 1))
                carry = jnp.where(pos == 127, align(L, 3), carry)

    def gen_k(rb):
        for n in range(8):
            i = 8 * rb + n
            taps(i)
            if i + 1 < D // 16:
                powers(i + 1)
            if rb:
                dft_k(rb - 1, range(2 * n, 2 * n + 2))

    def dft_k(rb, which=range(NS)):
        for s in which:
            u = (un, uo)[s // 8][_ds(rb + 4, 64), _ds(s % 8, R)]
            kspec[_ds(rb, 128), _ds(s, 2 * R)] = _dot(_unpack(u), _unpack(fk_ref[s]))

    for cp in first:
        cp.wait()
    for cp in loads:
        cp.start()

    powers(0)
    gen_k(0)
    for cp in second:
        cp.wait()
    for rb in range(1, 4):
        pl.when(zero_ref[0] < rb)(lambda: gen_k(rb))

    for cp in loads:
        cp.wait()

    xu = [r.bitcast(U32) for r in xio]

    def load_x(b):
        for jj in range(8):
            ev, od = _halves(xu[b][pl.ds(jj, R, stride=8), :].T)
            xs[_ds(b, 128), _ds(jj, R)] = ev
            xo[_ds(b, 128), _ds(jj, R)] = od

    m_i = jax.lax.broadcasted_iota(jnp.int32, (128, 128), 0)
    c_i = jax.lax.broadcasted_iota(jnp.int32, (128, 128), 1)
    perm = jnp.where(c_i == (m_i & 7) * 16 + (m_i >> 3), 1.0, 0.0).astype(BF16)

    def prep_w(g):
        for t in range(3):
            wt[g, _ds(t, 64), :] = _pack(_dot(perm, wqkv_ref[:, _ds((t + 1) % 3 * 4 + g, 128)], _NT))
        wot[:, _ds(g, 128)] = _pack(_dot(perm, wo_ref[_ds(g, 128), :]).T)

    def dft(rb, s):
        u = (un, uo)[s // 8][_ds(rb, 64), _ds(s % 8, R)]
        y = _dot(_unpack(u), _unpack(f_ref[s]))
        spec[rb][0:128, _ds(s, 2 * R)] = y
        return y[-8:, R:]

    def idft(rb, s):
        y = _dot(spec[rb][0:128, _ds(s, 2 * R)], _unpack(f_ref[s]), _NT)
        (xs, xo)[s // 8][_ds(rb, 128), _ds(s % 8, R)] += y
        return y[-8:]

    def load_spec(ref, rows, order):
        return [(ref[rows, _ds(2 * s, R)], ref[rows, _ds(2 * s + 1, R)]) for s in order]

    def store_spec(ref, rows, order, vals):
        for s, v in zip(order, vals):
            ref[rows, _ds(2 * s, R)] = v[0]
            ref[rows, _ds(2 * s + 1, R)] = v[1]

    slabs = [_slab(j) for j in range(NS)]

    def half(buf, rows, e8, bias=None):
        out = []
        for j in range(8):
            lo, hi = load_spec(buf, rows, [slabs[j], slabs[j + 8]])
            if j == 0 and bias is not None:
                lo = (lo[0] + bias, lo[1])
            out.append(_csub(lo, hi) if e8 else _cadd(lo, hi))
        return out

    def k_fft_steps(i):
        rows = _ds(i, 8)
        for e8 in (8, 0):
            quartics = _split(half(kspec, rows, e8, dskb[rows, :]), e8 // 2)
            for e4, p4 in zip((e8 // 2, e8 // 2 + 8), quartics):
                for e2, p2 in zip((e4 // 2, e4 // 2 + 8), _split(p4, e4 // 2)):
                    store_spec(khat, rows, _coeff_slots(e2), _factor_coeffs(p2, e2))
                yield

    def k_fft(i):
        for _ in k_fft_steps(i):
            pass

    def conv(rb, i, after=None):
        buf, rows, park = spec[rb], _ds(i, 8), _ds(16, 8)
        for e8 in (8, 0):
            quartics = []
            for e4, p4 in zip((e8 // 2, e8 // 2 + 8), _split(half(buf, rows, e8), e8 // 2)):
                prods = [_factor_mul(p2, load_spec(khat, _ds(16 * rb + i, 8), _coeff_slots(e2)), e2)
                         for e2, p2 in zip((e4 // 2, e4 // 2 + 8), _split(p4, e4 // 2))]
                quartics.append(_merge(*prods, e4 // 2))
                if e4 < 8:
                    fence(khat, prods[1][1][0])
            mark = prods[1][1][0]
            fence(buf, mark if e8 or after is None else after)
            for j, v in enumerate(_merge(*quartics, e8 // 2)):
                if e8:
                    store_spec(buf, park, [j], [v])
                else:
                    (o,) = load_spec(buf, park, [j])
                    store_spec(buf, rows, [slabs[j], slabs[j + 8]], [_cadd(v, o), _csub(v, o)])
        return mark

    lane = jax.lax.broadcasted_iota(jnp.int32, (128, R), 1)

    def qkv(g, u, qs, ks, vs, i):
        y = _dot(_unpack(wt[g]), _unpack(u[0:D // 2, _ds(i, R)]))
        k, v, q = y[0:128], y[128:256], y[256:384]
        qs[:, _ds(i, R)] = q
        ks[:, _ds(i + 7, R)] = k
        vs[:, _ds(i + 7, R)] = v
        if i:
            ks[:, _ds(i - 1, R)] = pltpu.roll(k, 1, 1)
            vs[:, _ds(i - 1, R)] = jnp.where(lane == 0, va[:, _ds(7, R)], pltpu.roll(v, 1, 1))

    never = lane8 < zero_ref[0]

    def attend(g, qs, ks, vs, rs, o, i, ways, side=None):
        logits = []
        for w in range(W):
            lg = None
            for c in range(16):
                term = qs[_ds(c, 8), _ds(i, R)] * ks[_ds(c, 8), _ds(7 + i - w, R)]
                if c:
                    lg = lg + term
                else:
                    lg = term if w < ways else jnp.where(never, logits[w - ways], term)
            logits.append(lg)
            if side and w in (1, 7):
                fence(kspec, lg)
                next(side)
        scale = rs[7 + i] * 0.25
        logits = [lg * scale * rs[7 + i - w] for w, lg in enumerate(logits)]
        logits = [jnp.where(lane8 == 0, NEG, lg) if w > i else lg for w, lg in enumerate(logits)]
        mx = logits[0]
        for lg in logits[1:]:
            mx = jnp.maximum(mx, lg)
        es = [jnp.exp(lg - mx) for lg in logits]
        den = es[0]
        for e in es[1:]:
            den = den + e
        inv = 1.0 / den
        probs = [e * rs[7 + i - w] * inv for w, e in enumerate(es)]
        outs = []
        for c in range(16):
            acc = None
            for w in range(W):
                term = vs[_ds(c, 8), _ds(7 + i - w, R)] * probs[w]
                if w:
                    acc = acc + term
                else:
                    acc = term if c < ways else jnp.where(never, outs[c - ways], term)
            outs.append(acc)
            if side and c in (3, 11):
                fence(kspec, acc)
                next(side)
        o[_ds(g + 4, 64), _ds(i, R)] = _pack(jnp.concatenate(outs, axis=0))

    def chain_sum(vals, ways):
        parts = vals[:ways]
        for n, v in enumerate(vals[ways:]):
            parts[n % ways] = parts[n % ways] + v
        return jnp.sum(sum(parts[1:], parts[0]), axis=0, keepdims=True)

    def row_mean(x, ways, after=None):
        parts = [x[_ds(n, 8)] for n in range(D // 8)]
        if after is not None:
            parts[0] = jnp.where(never, after, parts[0])
        return chain_sum(parts, ways) * (1.0 / D)

    def norm(x, u, rs, i, ways, after=None):
        c = x[:, _ds(i, R)] - row_mean(x[:, _ds(i, R)], 2, after)
        r = jnp.broadcast_to(jax.lax.rsqrt(row_mean(c * c, ways) + EPS), (8, R))
        u[0:D // 2, _ds(i, R)] = _pack(c)
        rs[7 + i] = r
        if i:
            rs[i - 1] = jnp.where(lane8 == 0, ra[7], pltpu.roll(r, 1, 1))
        return r

    def proj(x, o, u, i):
        y = x[:, _ds(i, R)] + _dot(_unpack(wot[...]), _unpack(o[D // 2:D, _ds(i, R)]))
        x[:, _ds(i, R)] = y
        cen_ = cen[i % 2]
        cen_[...] = x[:, _ds(i, R)] - row_mean(y, 2)
        c = cen_[pl.ds(pl.multiple_of(zero_ref[0], 8), D)]
        u[0:D // 2, _ds(i, R)] = _pack(cen_[...] * jax.lax.rsqrt(row_mean(c * c, 1) + EPS))

    stores = [pltpu.make_async_copy(xio[c].at[0:L], o_hbm.at[:, c * 128:(c + 1) * 128], sems.at[c])
              for c in range(4)]

    def store_x(b, jj):
        t = pltpu.pack_elementwise(
            [xs[_ds(b, 128), _ds(jj, R)], xo[_ds(b, 128), _ds(jj, R)]], packed_dtype=BF16)
        xu[b][pl.ds(jj, R, stride=8), :] = pltpu.bitcast(t, U32).T

    def fence_io(b, val):
        xio[b][pl.ds(pl.multiple_of(L + zero_ref[0], 16), 16), :] = pltpu.bitcast(val, BF16)

    def start_store(b, val):
        stores[b].start()
        fence_io(b, val)
        return pltpu.bitcast(xio[b][L:L + 16, :], F32)

    def phase(fn):
        pl.when(zero_ref[0] == 0)(fn)

    @phase
    def _prepare():
        dft_k(3)
        for b in range(4):
            load_x(b)
            prep_w(b)
            for n in range(2):
                k_fft(2 * b + n)

    even, odd = (un, (qa, ka, va), ra), (uo, (qb, kb, vb), rb_)

    def overlap(g_next, nxt, g, cur, k0):
        for i in range(8):
            qkv(g_next, nxt[0], *nxt[1], i)
            attend(g, *cur[1], cur[2], nxt[0], i, 2, None if k0 is None else k_fft_steps(k0 + i))

    for layer in range(2):
        @phase
        def _first_projection():
            if layer:
                for s in range(8):
                    idft(3, s)
            r = norm(xs, un, ra, 0, 4)
            for i in range(8):
                if layer:
                    idft(3, i + 8)
                qkv(0, un, qa, ka, va, i)
                if i < 7:
                    r = norm(xs, un, ra, i + 1, 2 - layer, r)
                r = norm(xo, uo, rb_, i, 2 - layer, r)

        def group(g, c):
            overlap(g, odd, g, even, None if layer else 8 * g + 8)

            @pl.when(g < 3)
            def _():
                overlap(g + 1, even, g, odd, None if layer else 8 * g + 40)

            return c

        jax.lax.fori_loop(0, 4, group, 0)

        @phase
        def _output_projection():
            for i in range(8):
                proj(xs, uo, un, i)
                attend(3, qb, kb, vb, rb_, un, i, 1)
            for i in range(8):
                proj(xo, un, uo, i)
            for s in range(NS):
                dft(0, s)

        @phase
        def _long_conv():
            done = []
            for rb in range(4):
                for i in range(16):
                    if rb < 3:
                        last = dft(rb + 1, i)
                    if layer and rb == 3:
                        if i < 8:
                            idft(2, i)
                            last = idft(2, i + 8)
                        else:
                            store_x(2, i - 8)
                    elif rb:
                        last = idft(rb - 1, i)
                    if layer and rb >= 2 and i < 8:
                        store_x(rb - 2, i)
                        if i == 7:
                            last = start_store(rb - 2, last)
                    done.append(last)
                    mark = conv(rb, i, done[-LAG] if len(done) >= LAG else None)
                    if rb < 3:
                        fence(spec[rb + 1], mark)

    last = start_store(2, jnp.zeros((8, R), F32))
    fence(spec[3], last)
    for jj in range(8):
        idft(3, jj)
        idft(3, jj + 8)
        store_x(3, jj)
    stores[3].start()
    for cp in stores:
        cp.wait()


@jax.jit
def pallas_interleave_layers__sliding_local_dilated__ssm_conv_s4__prompt_kernel(
    A_x: jax.Array,
    A_wqkv: jax.Array,
    A_wo: jax.Array,
    B_u: jax.Array,
    B_A_re: jax.Array,
    B_A_im: jax.Array,
    B_B_re: jax.Array,
    B_B_im: jax.Array,
    B_C_re: jax.Array,
    B_C_im: jax.Array,
    B_log_dt: jax.Array,
    B_Dskip: jax.Array,
):
    del B_u
    f = _dft_matrix()
    lane = (np.arange(R) - 11) % R
    order = 16 * (lane % 8) + lane // 8
    fk = (f[:, order].astype(np.float32) * (2.0 / L)).astype(ml_dtypes.bfloat16)
    scratch = [
        pltpu.VMEM((D, L // 2), F32),
        pltpu.VMEM((D, L // 2), F32),
        pltpu.VMEM((D + 8, L // 2), U32),
        pltpu.VMEM((D + 8, L // 2), U32),
        pltpu.VMEM((4, 192, D), U32),
        pltpu.VMEM((D // 2, D), U32),
        pltpu.VMEM((D // 2, 128), U32),
        pltpu.VMEM((D, 128), F32),
        pltpu.VMEM((2, 8, 8, N), F32),
        pltpu.VMEM((4, 128, 2 * N), F32),
        *[pltpu.VMEM((128 + 16, 2 * L), F32)] * 4,
        pltpu.VMEM((D + 8, 2 * L), F32),
        pltpu.VMEM((D + 8, 22 * 2 * R), F32),
        pltpu.VMEM((128, 8 * R), F32),
        pltpu.VMEM((128, 15 * R), F32),
        pltpu.VMEM((128, 15 * R), F32),
        pltpu.VMEM((128, 8 * R), F32),
        pltpu.VMEM((128, 15 * R), F32),
        pltpu.VMEM((128, 15 * R), F32),
        pltpu.VMEM((15, 8, R), F32),
        pltpu.VMEM((15, 8, R), F32),
        *[pltpu.VMEM((D, R), F32)] * 2,
        *[pltpu.VMEM((L + 16, 128), BF16)] * 4,
        pltpu.VMEM((D, 3 * D), BF16),
        pltpu.VMEM((D, D), BF16),
        pltpu.VMEM((NS, R // 2, 2 * R), U32),
        pltpu.VMEM((NS, R // 2, 2 * R), U32),
        pltpu.VMEM((6, D, N), BF16),
        pltpu.SMEM((1,), jnp.int32),
        pltpu.VMEM((D,), BF16),
        pltpu.VMEM((D,), BF16),
        pltpu.SemaphoreType.DMA((13,)),
    ]
    hbm = pl.BlockSpec(memory_space=pl.ANY)
    out = pl.pallas_call(
        _kernel,
        out_shape=jax.ShapeDtypeStruct((L, D), BF16),
        in_specs=[hbm] * 14,
        out_specs=hbm,
        scratch_shapes=scratch,
        compiler_params=pltpu.CompilerParams(vmem_limit_bytes=100 * 1024 * 1024),
    )(np.zeros((1,), np.int32), A_x.reshape(L, D), A_wqkv, A_wo, B_A_re, B_A_im, B_B_re, B_B_im, B_C_re, B_C_im,
      B_log_dt, B_Dskip, _pack_rows(f), _pack_rows(fk))
    return out.reshape(1, L, D)
```

```python
import jax
import jax.numpy as jnp
import jax.experimental.pallas as pl
import jax.experimental.pallas.tpu as pltpu
import ml_dtypes
import numpy as np

L = 2048
D = 512
N = 128
NS = 16
R = 128
W = 8
EPS = 1e-5
_H = float(np.sqrt(0.5))
LAG = 4
F32 = jnp.float32
BF16 = jnp.bfloat16
U32 = jnp.uint32
NEG = float(ml_dtypes.bfloat16(-1e9))

_NT = (((1,), (1,)), ((), ()))


def _slab(j):
    return (j % 2) * 8 + j // 2


def _dft_matrix():
    r = np.arange(R)
    k = np.arange(R) + 0.5
    f = np.zeros((NS, R, 2 * R), np.float64)
    for j in range(NS):
        th = 2.0 * np.pi * np.outer(NS * r + j, k) / (2 * L)
        f[_slab(j), :, :R] = np.cos(th)
        f[_slab(j), :, R:] = -np.sin(th)
    return f.astype(np.float32).astype(ml_dtypes.bfloat16)


def _pack_rows(a):
    u = np.ascontiguousarray(a).view(np.uint16).astype(np.uint32)
    return u[:, 0::2] | (u[:, 1::2] << np.uint32(16))


def _lag_tables():
    rho = []
    for s in range(8):
        lag = (256 * s + np.arange(NS)).astype(np.float32)
        rho.append([int(v) - 256 * s for v in lag.astype(ml_dtypes.bfloat16).astype(np.float32)])
    return rho


_RHO = _lag_tables()


def _cmul(a, b):
    return (a[0] * b[0] - a[1] * b[1], a[0] * b[1] + a[1] * b[0])


def _csq(a):
    t = a[0] * a[1]
    return ((a[0] - a[1]) * (a[0] + a[1]), t + t)


def _cadd(a, b):
    return (a[0] + b[0], a[1] + b[1])


def _csub(a, b):
    return (a[0] - b[0], a[1] - b[1])


def _split(p, e):
    plus, minus = [], []
    for lo, hi in zip(p[:len(p) // 2], p[len(p) // 2:]):
        if e % 4:
            hi = ((hi[0] - hi[1]) * _H, (hi[0] + hi[1]) * _H)
        if e >= 4:
            plus.append((lo[0] - hi[1], lo[1] + hi[0]))
            minus.append((lo[0] + hi[1], lo[1] - hi[0]))
        else:
            plus.append(_cadd(lo, hi))
            minus.append(_csub(lo, hi))
    return plus, minus


def _merge(plus, minus, e):
    lo, hi = [], []
    for p, m in zip(plus, minus):
        lo.append(_cadd(p, m))
        d = (p[1] - m[1], m[0] - p[0]) if e >= 4 else _csub(p, m)
        hi.append(((d[0] + d[1]) * _H, (d[1] - d[0]) * _H) if e % 4 else d)
    return lo + hi


def _factor_coeffs(k, e):
    if e % 8 == 0:
        (p,), (m,) = _split(k, e // 2)
        return [(p[0] * 0.5, p[1] * 0.5), (m[0] * 0.5, m[1] * 0.5)]
    c, s = float(np.cos(np.pi * e / 8)), float(np.sin(np.pi * e / 8))
    wk = (k[1][0] * c - k[1][1] * s, k[1][0] * s + k[1][1] * c)
    return [k[0], _csub(wk, k[0]), _csub(k[1], k[0])]


def _factor_mul(a, coeffs, e):
    if e % 8 == 0:
        (p,), (m,) = _split(a, e // 2)
        return _merge([_cmul(p, coeffs[0])], [_cmul(m, coeffs[1])], e // 2)
    t = _cmul(_cadd(a[0], a[1]), coeffs[0])
    return [_cadd(t, _cmul(a[1], coeffs[1])), _cadd(t, _cmul(a[0], coeffs[2]))]


def _coeff_slots(e):
    if e % 8 == 0:
        return [e // 4, e // 4 + 1]
    n = 4 + 3 * [2, 4, 6, 10, 12, 14].index(e)
    return [n, n + 1, n + 2]


def _ds(i, n):
    if isinstance(i, int):
        return slice(i * n, (i + 1) * n)
    return pl.ds(pl.multiple_of(i * n, n), n)


def _pack(x):
    return pltpu.bitcast(x.astype(BF16), U32)


def _unpack(x):
    return pltpu.bitcast(x, BF16)


def _dot(a, b, dims=(((1,), (0,)), ((), ()))):
    return jax.lax.dot_general(a, b, dims, preferred_element_type=F32)


def _halves(u):
    return pltpu.bitcast(u << 16, F32), pltpu.bitcast(u & jnp.uint32(0xFFFF0000), F32)


def _kernel(zero_hbm, x_hbm, wqkv_hbm, wo_hbm, are, aim, bre, bim, cre, cim,
            ldt_hbm, dsk_hbm, f_hbm, fk_hbm, o_hbm,
            xs, xo, un, uo, wt, wot, dtb, dskb, pw_ref, rhs_ref, s0, s1, s2, s3, kspec, khat,
            qa, ka, va, qb, kb, vb, ra, rb_, cen0, cen1,
            io0, io1, io2, io3, wqkv_ref, wo_ref, f_ref, fk_ref, ssm, zero_ref, ldt_ref, dsk_ref, sems):
    def fetch_ssm(rows, sem):
        return [pltpu.make_async_copy(p.at[rows], ssm.at[n, rows], sem)
                for n, p in enumerate((are, aim, bre, bim, cre, cim))]

    small = [pltpu.make_async_copy(src, dst, sems.at[10 + n]) for n, (src, dst) in enumerate(
        [(zero_hbm, zero_ref), (ldt_hbm, ldt_ref), (dsk_hbm, dsk_ref)])]
    for cp in small:
        cp.start()
    first = fetch_ssm(pl.ds(0, 144), sems.at[8])
    for cp in first:
        cp.start()
    second = fetch_ssm(pl.ds(144, D - 144), sems.at[9])
    second += [pltpu.make_async_copy(fk_hbm, fk_ref, sems.at[4])]
    for cp in second:
        cp.start()
    xio = (io0, io1, io2, io3)
    loads = [pltpu.make_async_copy(x_hbm.at[:, c * 128:(c + 1) * 128], xio[c].at[0:L], sems.at[c])
             for c in range(4)]
    loads += [pltpu.make_async_copy(src, dst, sems.at[5 + n]) for n, (src, dst) in enumerate(
        [(wqkv_hbm, wqkv_ref), (wo_hbm, wo_ref), (f_hbm, f_ref)])]

    spec = (s0, s1, s2, s3)
    cen = (cen0, cen1)

    def fence(ref, val):
        row = ref.shape[0] - 8 + zero_ref[0]
        ref[pl.ds(pl.multiple_of(row, 8), 8), 0:128] = val

    for cp in small:
        cp.wait()
    dt_row = jnp.exp(ldt_ref[...].astype(F32)).reshape(1, D)
    dtb[...] = _pack(jnp.broadcast_to(dt_row, (128, D)).T)
    dskb[...] = jnp.broadcast_to(dsk_ref[...].astype(F32).reshape(1, D) * (2.0 / L), (128, D)).T

    lane8 = jax.lax.broadcasted_iota(jnp.int32, (8, R), 1)
    sub8 = jax.lax.broadcasted_iota(jnp.int32, (8, N), 0)
    low = sub8 < 4
    steps = (1, 2, 4, 256)

    def halves_of(a, b):
        return tuple(jnp.where(low, u, v) for u, v in zip(a, b))

    def powers(i):
        dts = _halves(dtb[_ds(i, 8), :])
        are, aim, bre, bim, cre, cim = [
            _halves(pltpu.bitcast(ssm[n, _ds(i, 16), :], U32)) for n in range(6)]
        for h in range(2):
            dt = dts[h]
            li = dt * aim[h]
            mag = jnp.exp(dt * are[h])
            zp = {1: (mag * jnp.cos(li), mag * jnp.sin(li))}
            for e in (1, 2, 4, 8, 16, 32, 64, 128):
                zp[2 * e] = _csq(zp[e])
            for n, e in enumerate(steps):
                pw_ref[h, 2 * n] = zp[e][0]
                pw_ref[h, 2 * n + 1] = zp[e][1]
            w = _cmul((cre[h], cim[h]), (dt * bre[h], dt * bim[h]))
            w, z8, z16 = [(v[0], -v[1]) for v in (w, zp[8], zp[16])]
            w8 = _cmul(w, z8)
            for t in range(2):
                def pick(v):
                    return tuple(jnp.take_along_axis(u, 4 * t + 3 - (sub8 & 3), axis=0) for u in v)

                step = pick(z16)
                rows = [halves_of(pick(w), pick(w8)) if t else halves_of(pick(w8), pick(_cmul(w, z16)))]
                for _ in range(15):
                    rows.append(_cmul(rows[-1], step))
                if not t:
                    rows = [halves_of(rows[-1], pick(w))] + rows[:-1]
                rhs_ref[2 * h + t] = jnp.concatenate([jnp.concatenate(v, axis=1) for v in rows], axis=0)

    offsets = sorted({256 * s + p % 8 for s in range(8) for p in _RHO[s]}) + [L]
    plain, turned = offsets[:11], offsets[11:]

    def turn(v):
        return pltpu.roll(v, 4, 0)

    def taps(i):
        outs = []
        for h in range(2):
            zp = {e: (pw_ref[h, 2 * n], pw_ref[h, 2 * n + 1]) for n, e in enumerate(steps)}
            zp[0] = (jnp.ones((8, N), F32), jnp.zeros((8, N), F32))
            zt = {e: (turn(zp[e][0]), turn(zp[e][1])) for e in (4, 256)}
            for table, exps in ((zp, plain + turned[:1]), (zt, turned[1:])):
                for e in exps:
                    if e in table:
                        continue
                    if e % 2 == 0 and e // 2 in table:
                        table[e] = _csq(table[e // 2])
                    else:
                        inc = next(v for v in steps if v in table and e - v in table)
                        table[e] = _cmul(table[e - inc], table[inc])
            zt[turned[0]] = tuple(turn(v) for v in zp[turned[0]])
            pairs = [(zp[a], zt[b]) for a, b in zip(plain, turned)] + [(zp[plain[-1]],) * 2]
            for t in range(2):
                lhs = [jnp.concatenate(halves_of(*v[::-1]) if t else halves_of(*v), axis=1) for v in pairs]
                outs.append(_dot(jnp.concatenate(lhs, axis=0), rhs_ref[2 * h + t], _NT))
        lo, hi = [pltpu.bitcast(pltpu.pack_elementwise([outs[t], outs[2 + t]], packed_dtype=BF16), U32)
                  for t in range(2)]
        merged = {a: jnp.where(low, lo[_ds(n, 8)], hi[_ds(n, 8)]) for n, a in enumerate(plain)}
        merged.update({a: turn(jnp.where(low, hi[_ds(n, 8)], lo[_ds(n, 8)])) for n, a in enumerate(turned)})

        def align(a, shift):
            return pltpu.roll(merged[a], shift, 1, stride=1, stride_axis=0)

        piece = {(s, p): align(256 * s + p % 8, s + 4 - 4 * (p // 8))
                 for s in range(8) for p in sorted(set(_RHO[s]) - {16})}
        pos = (lane8 - 11) & 127
        memo = {}
        for j in range(NS):
            key = ()
            acc = None
            for s in range(7, -1, -1):
                key = key + (_RHO[s][j],)
                if key not in memo:
                    pc = carry if _RHO[s][j] == 16 else piece[s, _RHO[s][j]]
                    same = acc is None or pc is acc
                    memo[key] = pc if same else jnp.where((pos & 7) == s, pc, acc)
                acc = memo[key]
            (un, uo)[j % 2][_ds(i + D // 16, 8), _ds(j // 2, R)] = acc
            if j == 0:
                carry = jnp.where(pos >= 120, pltpu.roll(acc, 128 - 9, 1), pltpu.roll(acc, 128 - 8, 1))
                carry = jnp.where(pos == 127, align(L, 3), carry)

    def gen_k(rb):
        for n in range(8):
            i = 8 * rb + n
            taps(i)
            if i + 1 < D // 16:
                powers(i + 1)
            if rb:
                dft_k(rb - 1, range(2 * n, 2 * n + 2))

    def dft_k(rb, which=range(NS)):
        for s in which:
            u = (un, uo)[s // 8][_ds(rb + 4, 64), _ds(s % 8, R)]
            kspec[_ds(rb, 128), _ds(s, 2 * R)] = _dot(_unpack(u), _unpack(fk_ref[s]))

    for cp in first:
        cp.wait()
    for cp in loads:
        cp.start()

    powers(0)
    gen_k(0)
    for cp in second:
        cp.wait()
    for rb in range(1, 4):
        pl.when(zero_ref[0] < rb)(lambda: gen_k(rb))

    for cp in loads:
        cp.wait()

    xu = [r.bitcast(U32) for r in xio]

    def load_x(b):
        for jj in range(8):
            ev, od = _halves(xu[b][pl.ds(jj, R, stride=8), :].T)
            xs[_ds(b, 128), _ds(jj, R)] = ev
            xo[_ds(b, 128), _ds(jj, R)] = od

    m_i = jax.lax.broadcasted_iota(jnp.int32, (128, 128), 0)
    c_i = jax.lax.broadcasted_iota(jnp.int32, (128, 128), 1)
    perm = jnp.where(c_i == (m_i & 7) * 16 + (m_i >> 3), 1.0, 0.0).astype(BF16)

    def prep_w(g):
        for t in range(3):
            wt[g, _ds(t, 64), :] = _pack(_dot(perm, wqkv_ref[:, _ds((t + 1) % 3 * 4 + g, 128)], _NT))
        wot[:, _ds(g, 128)] = _pack(_dot(perm, wo_ref[_ds(g, 128), :]).T)

    def dft(rb, s):
        u = (un, uo)[s // 8][_ds(rb, 64), _ds(s % 8, R)]
        y = _dot(_unpack(u), _unpack(f_ref[s]))
        spec[rb][0:128, _ds(s, 2 * R)] = y
        return y[-8:, R:]

    def idft(rb, s):
        y = _dot(spec[rb][0:128, _ds(s, 2 * R)], _unpack(f_ref[s]), _NT)
        (xs, xo)[s // 8][_ds(rb, 128), _ds(s % 8, R)] += y
        return y[-8:]

    def load_spec(ref, rows, order):
        return [(ref[rows, _ds(2 * s, R)], ref[rows, _ds(2 * s + 1, R)]) for s in order]

    def store_spec(ref, rows, order, vals):
        for s, v in zip(order, vals):
            ref[rows, _ds(2 * s, R)] = v[0]
            ref[rows, _ds(2 * s + 1, R)] = v[1]

    slabs = [_slab(j) for j in range(NS)]

    def half(buf, rows, e8):
        pairs = [load_spec(buf, rows, [slabs[j], slabs[j + 8]]) for j in range(8)]
        return [_csub(lo, hi) if e8 else _cadd(lo, hi) for lo, hi in pairs]

    def k_fft(i, last):
        rows = _ds(i, 8)

        def paced(v):
            return v if last[0] is None else tuple(jnp.where(never, a, b) for a, b in zip(last[0], v))

        def split(p, e):
            plus, minus = [], []
            for lo, hi in zip(p[:len(p) // 2], p[len(p) // 2:]):
                (u,), (last[0],) = _split([lo, paced(hi)], e)
                plus.append(u)
                minus.append(last[0])
            return plus, minus

        for e8 in (8, 0):
            poly = []
            for j in range(8):
                lo, hi = load_spec(kspec, rows, [slabs[j], slabs[j + 8]])
                if j == 0:
                    lo = (lo[0] + dskb[rows, :], lo[1])
                last[0] = _csub(paced(lo), hi) if e8 else _cadd(paced(lo), hi)
                poly.append(last[0])
            for e4, p4 in zip((e8 // 2, e8 // 2 + 8), split(poly, e8 // 2)):
                for e2, p2 in zip((e4 // 2, e4 // 2 + 8), split(p4, e4 // 2)):
                    coeffs = _factor_coeffs([p2[0], paced(p2[1])], e2)
                    last[0] = coeffs[1]
                    store_spec(khat, rows, _coeff_slots(e2), coeffs)

    def conv(rb, i, after=None):
        buf, rows, park = spec[rb], _ds(i, 8), _ds(16, 8)
        for e8 in (8, 0):
            quartics = []
            for e4, p4 in zip((e8 // 2, e8 // 2 + 8), _split(half(buf, rows, e8), e8 // 2)):
                prods = [_factor_mul(p2, load_spec(khat, _ds(16 * rb + i, 8), _coeff_slots(e2)), e2)
                         for e2, p2 in zip((e4 // 2, e4 // 2 + 8), _split(p4, e4 // 2))]
                quartics.append(_merge(*prods, e4 // 2))
                if e4 < 8:
                    fence(khat, prods[1][1][0])
            mark = prods[1][1][0]
            fence(buf, mark if e8 or after is None else after)
            for j, v in enumerate(_merge(*quartics, e8 // 2)):
                if e8:
                    store_spec(buf, park, [j], [v])
                else:
                    (o,) = load_spec(buf, park, [j])
                    store_spec(buf, rows, [slabs[j], slabs[j + 8]], [_cadd(v, o), _csub(v, o)])
        return mark

    lane = jax.lax.broadcasted_iota(jnp.int32, (128, R), 1)

    def qkv(g, u, qs, ks, vs, i):
        y = _dot(_unpack(wt[g]), _unpack(u[0:D // 2, _ds(i, R)]))
        k, v, q = y[0:128], y[128:256], y[256:384]
        qs[:, _ds(i, R)] = q
        ks[:, _ds(i + 7, R)] = k
        vs[:, _ds(i + 7, R)] = v
        if i:
            ks[:, _ds(i - 1, R)] = pltpu.roll(k, 1, 1)
            vs[:, _ds(i - 1, R)] = jnp.where(lane == 0, va[:, _ds(7, R)], pltpu.roll(v, 1, 1))

    never = lane8 < zero_ref[0]

    def attend(g, qs, ks, vs, rs, o, i, ways):
        logits = []
        for w in range(W):
            lg = None
            for c in range(16):
                term = qs[_ds(c, 8), _ds(i, R)] * ks[_ds(c, 8), _ds(7 + i - w, R)]
                if c:
                    lg = lg + term
                else:
                    lg = term if w < ways else jnp.where(never, logits[w - ways], term)
            logits.append(lg)
        scale = rs[7 + i] * 0.25
        logits = [lg * scale * rs[7 + i - w] for w, lg in enumerate(logits)]
        logits = [jnp.where(lane8 == 0, NEG, lg) if w > i else lg for w, lg in enumerate(logits)]
        mx = logits[0]
        for lg in logits[1:]:
            mx = jnp.maximum(mx, lg)
        es = [jnp.exp(lg - mx) for lg in logits]
        den = es[0]
        for e in es[1:]:
            den = den + e
        inv = 1.0 / den
        probs = [e * rs[7 + i - w] * inv for w, e in enumerate(es)]
        outs = []
        for c in range(16):
            acc = None
            for w in range(W):
                term = vs[_ds(c, 8), _ds(7 + i - w, R)] * probs[w]
                if w:
                    acc = acc + term
                else:
                    acc = term if c < ways else jnp.where(never, outs[c - ways], term)
            outs.append(acc)
        o[_ds(g + 4, 64), _ds(i, R)] = _pack(jnp.concatenate(outs, axis=0))

    def chain_sum(vals, ways):
        parts = vals[:ways]
        for n, v in enumerate(vals[ways:]):
            parts[n % ways] = parts[n % ways] + v
        return jnp.sum(sum(parts[1:], parts[0]), axis=0, keepdims=True)

    def row_mean(x, ways, after=None):
        parts = [x[_ds(n, 8)] for n in range(D // 8)]
        if after is not None:
            parts[0] = jnp.where(never, after, parts[0])
        return chain_sum(parts, ways) * (1.0 / D)

    def norm(x, u, rs, i, ways, after=None):
        c = x[:, _ds(i, R)] - row_mean(x[:, _ds(i, R)], 2, after)
        r = jnp.broadcast_to(jax.lax.rsqrt(row_mean(c * c, ways) + EPS), (8, R))
        u[0:D // 2, _ds(i, R)] = _pack(c)
        rs[7 + i] = r
        if i:
            rs[i - 1] = jnp.where(lane8 == 0, ra[7], pltpu.roll(r, 1, 1))
        return r

    def proj(x, o, u, i):
        y = x[:, _ds(i, R)] + _dot(_unpack(wot[...]), _unpack(o[D // 2:D, _ds(i, R)]))
        x[:, _ds(i, R)] = y
        cen_ = cen[i % 2]
        cen_[...] = x[:, _ds(i, R)] - row_mean(y, 2)
        c = cen_[pl.ds(pl.multiple_of(zero_ref[0], 8), D)]
        u[0:D // 2, _ds(i, R)] = _pack(cen_[...] * jax.lax.rsqrt(row_mean(c * c, 1) + EPS))

    stores = [pltpu.make_async_copy(xio[c].at[0:L], o_hbm.at[:, c * 128:(c + 1) * 128], sems.at[c])
              for c in range(4)]

    def store_x(b, jj):
        t = pltpu.pack_elementwise(
            [xs[_ds(b, 128), _ds(jj, R)], xo[_ds(b, 128), _ds(jj, R)]], packed_dtype=BF16)
        xu[b][pl.ds(jj, R, stride=8), :] = pltpu.bitcast(t, U32).T

    def fence_io(b, val):
        xio[b][pl.ds(pl.multiple_of(L + zero_ref[0], 16), 16), :] = pltpu.bitcast(val, BF16)

    def start_store(b, val):
        stores[b].start()
        fence_io(b, val)
        return pltpu.bitcast(xio[b][L:L + 16, :], F32)

    def phase(fn):
        pl.when(zero_ref[0] == 0)(fn)

    @phase
    def _prepare():
        dft_k(3)
        for b in range(4):
            load_x(b)
            prep_w(b)

    even, odd = (un, (qa, ka, va), ra), (uo, (qb, kb, vb), rb_)

    def overlap(g_next, nxt, g, cur, side):
        last = [None]
        for i in range(8):
            qkv(g_next, nxt[0], *nxt[1], i)
            attend(g, *cur[1], cur[2], nxt[0], i, 2)
            for k in side[i * len(side) // 8:(i + 1) * len(side) // 8]:
                k_fft(k, last)

    for layer in range(2):
        @phase
        def _first_projection():
            if layer:
                for s in range(8):
                    idft(3, s)
            r = norm(xs, un, ra, 0, 4)
            for i in range(8):
                if layer:
                    idft(3, i + 8)
                qkv(0, un, qa, ka, va, i)
                if i < 7:
                    r = norm(xs, un, ra, i + 1, 2 - layer, r)
                r = norm(xo, uo, rb_, i, 2 - layer, r)

        def group(g, c):
            overlap(g, odd, g, even, [] if layer else [10 * g + n for n in range(10)])

            @pl.when(g < 3)
            def _():
                overlap(g + 1, even, g, odd, [] if layer else [8 * g + 40 + n for n in range(8)])

            return c

        jax.lax.fori_loop(0, 4, group, 0)

        @phase
        def _output_projection():
            for i in range(8):
                proj(xs, uo, un, i)
                attend(3, qb, kb, vb, rb_, un, i, 1)
            for i in range(8):
                proj(xo, un, uo, i)
            for s in range(NS):
                dft(0, s)

        @phase
        def _long_conv():
            done = []
            for rb in range(4):
                for i in range(16):
                    if rb < 3:
                        last = dft(rb + 1, i)
                    if layer and rb == 3:
                        if i < 8:
                            idft(2, i)
                            last = idft(2, i + 8)
                        else:
                            store_x(2, i - 8)
                    elif rb:
                        last = idft(rb - 1, i)
                    if layer and rb >= 2 and i < 8:
                        store_x(rb - 2, i)
                        if i == 7:
                            last = start_store(rb - 2, last)
                    done.append(last)
                    mark = conv(rb, i, done[-LAG] if len(done) >= LAG else None)
                    if rb < 3:
                        fence(spec[rb + 1], mark)

    last = start_store(2, jnp.zeros((8, R), F32))
    fence(spec[3], last)
    for jj in range(8):
        idft(3, jj)
        idft(3, jj + 8)
        store_x(3, jj)
    stores[3].start()
    for cp in stores:
        cp.wait()


@jax.jit
def pallas_interleave_layers__sliding_local_dilated__ssm_conv_s4__prompt_kernel(
    A_x: jax.Array,
    A_wqkv: jax.Array,
    A_wo: jax.Array,
    B_u: jax.Array,
    B_A_re: jax.Array,
    B_A_im: jax.Array,
    B_B_re: jax.Array,
    B_B_im: jax.Array,
    B_C_re: jax.Array,
    B_C_im: jax.Array,
    B_log_dt: jax.Array,
    B_Dskip: jax.Array,
):
    del B_u
    f = _dft_matrix()
    lane = (np.arange(R) - 11) % R
    order = 16 * (lane % 8) + lane // 8
    fk = (f[:, order].astype(np.float32) * (2.0 / L)).astype(ml_dtypes.bfloat16)
    scratch = [
        pltpu.VMEM((D, L // 2), F32),
        pltpu.VMEM((D, L // 2), F32),
        pltpu.VMEM((D + 8, L // 2), U32),
        pltpu.VMEM((D + 8, L // 2), U32),
        pltpu.VMEM((4, 192, D), U32),
        pltpu.VMEM((D // 2, D), U32),
        pltpu.VMEM((D // 2, 128), U32),
        pltpu.VMEM((D, 128), F32),
        pltpu.VMEM((2, 8, 8, N), F32),
        pltpu.VMEM((4, 128, 2 * N), F32),
        *[pltpu.VMEM((128 + 16, 2 * L), F32)] * 4,
        pltpu.VMEM((D, 2 * L), F32),
        pltpu.VMEM((D + 8, 22 * 2 * R), F32),
        pltpu.VMEM((128, 8 * R), F32),
        pltpu.VMEM((128, 15 * R), F32),
        pltpu.VMEM((128, 15 * R), F32),
        pltpu.VMEM((128, 8 * R), F32),
        pltpu.VMEM((128, 15 * R), F32),
        pltpu.VMEM((128, 15 * R), F32),
        pltpu.VMEM((15, 8, R), F32),
        pltpu.VMEM((15, 8, R), F32),
        *[pltpu.VMEM((D, R), F32)] * 2,
        *[pltpu.VMEM((L + 16, 128), BF16)] * 4,
        pltpu.VMEM((D, 3 * D), BF16),
        pltpu.VMEM((D, D), BF16),
        pltpu.VMEM((NS, R // 2, 2 * R), U32),
        pltpu.VMEM((NS, R // 2, 2 * R), U32),
        pltpu.VMEM((6, D, N), BF16),
        pltpu.SMEM((1,), jnp.int32),
        pltpu.VMEM((D,), BF16),
        pltpu.VMEM((D,), BF16),
        pltpu.SemaphoreType.DMA((13,)),
    ]
    hbm = pl.BlockSpec(memory_space=pl.ANY)
    out = pl.pallas_call(
        _kernel,
        out_shape=jax.ShapeDtypeStruct((L, D), BF16),
        in_specs=[hbm] * 14,
        out_specs=hbm,
        scratch_shapes=scratch,
        compiler_params=pltpu.CompilerParams(vmem_limit_bytes=100 * 1024 * 1024),
    )(np.zeros((1,), np.int32), A_x.reshape(L, D), A_wqkv, A_wo, B_A_re, B_A_im, B_B_re, B_B_im, B_C_re, B_C_im,
      B_log_dt, B_Dskip, _pack_rows(f), _pack_rows(fk))
    return out.reshape(1, L, D)
```

```python
import jax
import jax.numpy as jnp
import jax.experimental.pallas as pl
import jax.experimental.pallas.tpu as pltpu
import ml_dtypes
import numpy as np

L = 2048
D = 512
N = 128
NS = 16
R = 128
W = 8
EPS = 1e-5
_H = float(np.sqrt(0.5))
LAG = 4
F32 = jnp.float32
BF16 = jnp.bfloat16
U32 = jnp.uint32
NEG = float(ml_dtypes.bfloat16(-1e9))

_NT = (((1,), (1,)), ((), ()))


def _slab(j):
    return (j % 2) * 8 + j // 2


def _dft_matrix():
    r = np.arange(R)
    k = np.arange(R) + 0.5
    f = np.zeros((NS, R, 2 * R), np.float64)
    for j in range(NS):
        th = 2.0 * np.pi * np.outer(NS * r + j, k) / (2 * L)
        f[_slab(j), :, :R] = np.cos(th)
        f[_slab(j), :, R:] = -np.sin(th)
    return f.astype(np.float32).astype(ml_dtypes.bfloat16)


def _pack_rows(a):
    u = np.ascontiguousarray(a).view(np.uint16).astype(np.uint32)
    return u[:, 0::2] | (u[:, 1::2] << np.uint32(16))


def _lag_tables():
    rho = []
    for s in range(8):
        lag = (256 * s + np.arange(NS)).astype(np.float32)
        rho.append([int(v) - 256 * s for v in lag.astype(ml_dtypes.bfloat16).astype(np.float32)])
    return rho


_RHO = _lag_tables()


def _cmul(a, b):
    return (a[0] * b[0] - a[1] * b[1], a[0] * b[1] + a[1] * b[0])


def _csq(a):
    t = a[0] * a[1]
    return ((a[0] - a[1]) * (a[0] + a[1]), t + t)


def _cadd(a, b):
    return (a[0] + b[0], a[1] + b[1])


def _csub(a, b):
    return (a[0] - b[0], a[1] - b[1])


def _split(p, e):
    plus, minus = [], []
    for lo, hi in zip(p[:len(p) // 2], p[len(p) // 2:]):
        if e % 4:
            hi = ((hi[0] - hi[1]) * _H, (hi[0] + hi[1]) * _H)
        if e >= 4:
            plus.append((lo[0] - hi[1], lo[1] + hi[0]))
            minus.append((lo[0] + hi[1], lo[1] - hi[0]))
        else:
            plus.append(_cadd(lo, hi))
            minus.append(_csub(lo, hi))
    return plus, minus


def _merge(plus, minus, e):
    lo, hi = [], []
    for p, m in zip(plus, minus):
        lo.append(_cadd(p, m))
        d = (p[1] - m[1], m[0] - p[0]) if e >= 4 else _csub(p, m)
        hi.append(((d[0] + d[1]) * _H, (d[1] - d[0]) * _H) if e % 4 else d)
    return lo + hi


def _factor_coeffs(k, e):
    if e % 8 == 0:
        (p,), (m,) = _split(k, e // 2)
        return [(p[0] * 0.5, p[1] * 0.5), (m[0] * 0.5, m[1] * 0.5)]
    c, s = float(np.cos(np.pi * e / 8)), float(np.sin(np.pi * e / 8))
    wk = (k[1][0] * c - k[1][1] * s, k[1][0] * s + k[1][1] * c)
    return [k[0], _csub(wk, k[0]), _csub(k[1], k[0])]


def _factor_mul(a, coeffs, e):
    if e % 8 == 0:
        (p,), (m,) = _split(a, e // 2)
        return _merge([_cmul(p, coeffs[0])], [_cmul(m, coeffs[1])], e // 2)
    t = _cmul(_cadd(a[0], a[1]), coeffs[0])
    return [_cadd(t, _cmul(a[1], coeffs[1])), _cadd(t, _cmul(a[0], coeffs[2]))]


def _coeff_slots(e):
    if e % 8 == 0:
        return [e // 4, e // 4 + 1]
    n = 4 + 3 * [2, 4, 6, 10, 12, 14].index(e)
    return [n, n + 1, n + 2]


def _ds(i, n):
    if isinstance(i, int):
        return slice(i * n, (i + 1) * n)
    return pl.ds(pl.multiple_of(i * n, n), n)


def _pack(x):
    return pltpu.bitcast(x.astype(BF16), U32)


def _unpack(x):
    return pltpu.bitcast(x, BF16)


def _dot(a, b, dims=(((1,), (0,)), ((), ()))):
    return jax.lax.dot_general(a, b, dims, preferred_element_type=F32)


def _halves(u):
    return pltpu.bitcast(u << 16, F32), pltpu.bitcast(u & jnp.uint32(0xFFFF0000), F32)


def _kernel(zero_hbm, x_hbm, wqkv_hbm, wo_hbm, are, aim, bre, bim, cre, cim,
            ldt_hbm, dsk_hbm, f_hbm, fk_hbm, o_hbm,
            xs, xo, un, uo, wt, wot, dtb, dskb, pw_ref, rhs_ref, s0, s1, s2, s3, kspec, khat,
            qa, ka, va, qb, kb, vb, ra, rb_, cen0, cen1,
            io0, io1, io2, io3, wqkv_ref, wo_ref, f_ref, fk_ref, ssm, zero_ref, ldt_ref, dsk_ref, sems):
    def fetch_ssm(rows, sem):
        return [pltpu.make_async_copy(p.at[rows], ssm.at[n, rows], sem)
                for n, p in enumerate((are, aim, bre, bim, cre, cim))]

    small = [pltpu.make_async_copy(src, dst, sems.at[10 + n]) for n, (src, dst) in enumerate(
        [(zero_hbm, zero_ref), (ldt_hbm, ldt_ref), (dsk_hbm, dsk_ref)])]
    for cp in small:
        cp.start()
    first = fetch_ssm(pl.ds(0, 144), sems.at[8])
    for cp in first:
        cp.start()
    second = fetch_ssm(pl.ds(144, D - 144), sems.at[9])
    second += [pltpu.make_async_copy(fk_hbm, fk_ref, sems.at[4])]
    for cp in second:
        cp.start()
    xio = (io0, io1, io2, io3)
    loads = [pltpu.make_async_copy(x_hbm.at[:, c * 128:(c + 1) * 128], xio[c].at[0:L], sems.at[c])
             for c in range(4)]
    loads += [pltpu.make_async_copy(src, dst, sems.at[5 + n]) for n, (src, dst) in enumerate(
        [(wqkv_hbm, wqkv_ref), (wo_hbm, wo_ref), (f_hbm, f_ref)])]

    spec = (s0, s1, s2, s3)
    cen = (cen0, cen1)

    def fence(ref, val):
        row = ref.shape[0] - 8 + zero_ref[0]
        ref[pl.ds(pl.multiple_of(row, 8), 8), 0:128] = val

    for cp in small:
        cp.wait()
    dt_row = jnp.exp(ldt_ref[...].astype(F32)).reshape(1, D)
    dtb[...] = _pack(jnp.broadcast_to(dt_row, (128, D)).T)
    dskb[...] = jnp.broadcast_to(dsk_ref[...].astype(F32).reshape(1, D) * (2.0 / L), (128, D)).T

    lane8 = jax.lax.broadcasted_iota(jnp.int32, (8, R), 1)
    sub8 = jax.lax.broadcasted_iota(jnp.int32, (8, N), 0)
    low = sub8 < 4
    steps = (1, 2, 4, 256)

    def halves_of(a, b):
        return tuple(jnp.where(low, u, v) for u, v in zip(a, b))

    def powers(i):
        dts = _halves(dtb[_ds(i, 8), :])
        are, aim, bre, bim, cre, cim = [
            _halves(pltpu.bitcast(ssm[n, _ds(i, 16), :], U32)) for n in range(6)]
        for h in range(2):
            dt = dts[h]
            li = dt * aim[h]
            mag = jnp.exp(dt * are[h])
            zp = {1: (mag * jnp.cos(li), mag * jnp.sin(li))}
            for e in (1, 2, 4, 8, 16, 32, 64, 128):
                zp[2 * e] = _csq(zp[e])
            for n, e in enumerate(steps):
                pw_ref[h, 2 * n] = zp[e][0]
                pw_ref[h, 2 * n + 1] = zp[e][1]
            w = _cmul((cre[h], cim[h]), (dt * bre[h], dt * bim[h]))
            w, z8, z16 = [(v[0], -v[1]) for v in (w, zp[8], zp[16])]
            w8 = _cmul(w, z8)
            for t in range(2):
                def pick(v):
                    return tuple(jnp.take_along_axis(u, 4 * t + 3 - (sub8 & 3), axis=0) for u in v)

                step = pick(z16)
                rows = [halves_of(pick(w), pick(w8)) if t else halves_of(pick(w8), pick(_cmul(w, z16)))]
                for _ in range(15):
                    rows.append(_cmul(rows[-1], step))
                if not t:
                    rows = [halves_of(rows[-1], pick(w))] + rows[:-1]
                rhs_ref[2 * h + t] = jnp.concatenate([jnp.concatenate(v, axis=1) for v in rows], axis=0)

    offsets = sorted({256 * s + p % 8 for s in range(8) for p in _RHO[s]}) + [L]
    plain, turned = offsets[:11], offsets[11:]

    def turn(v):
        return pltpu.roll(v, 4, 0)

    def taps(i):
        outs = []
        for h in range(2):
            zp = {e: (pw_ref[h, 2 * n], pw_ref[h, 2 * n + 1]) for n, e in enumerate(steps)}
            zp[0] = (jnp.ones((8, N), F32), jnp.zeros((8, N), F32))
            zt = {e: (turn(zp[e][0]), turn(zp[e][1])) for e in (4, 256)}
            for table, exps in ((zp, plain + turned[:1]), (zt, turned[1:])):
                for e in exps:
                    if e in table:
                        continue
                    if e % 2 == 0 and e // 2 in table:
                        table[e] = _csq(table[e // 2])
                    else:
                        inc = next(v for v in steps if v in table and e - v in table)
                        table[e] = _cmul(table[e - inc], table[inc])
            zt[turned[0]] = tuple(turn(v) for v in zp[turned[0]])
            pairs = [(zp[a], zt[b]) for a, b in zip(plain, turned)] + [(zp[plain[-1]],) * 2]
            for t in range(2):
                lhs = [jnp.concatenate(halves_of(*v[::-1]) if t else halves_of(*v), axis=1) for v in pairs]
                outs.append(_dot(jnp.concatenate(lhs, axis=0), rhs_ref[2 * h + t], _NT))
        lo, hi = [pltpu.bitcast(pltpu.pack_elementwise([outs[t], outs[2 + t]], packed_dtype=BF16), U32)
                  for t in range(2)]
        merged = {a: jnp.where(low, lo[_ds(n, 8)], hi[_ds(n, 8)]) for n, a in enumerate(plain)}
        merged.update({a: turn(jnp.where(low, hi[_ds(n, 8)], lo[_ds(n, 8)])) for n, a in enumerate(turned)})

        def align(a, shift):
            return pltpu.roll(merged[a], shift, 1, stride=1, stride_axis=0)

        piece = {(s, p): align(256 * s + p % 8, s + 4 - 4 * (p // 8))
                 for s in range(8) for p in sorted(set(_RHO[s]) - {16})}
        pos = (lane8 - 11) & 127
        memo = {}
        for j in range(NS):
            key = ()
            acc = None
            for s in range(7, -1, -1):
                key = key + (_RHO[s][j],)
                if key not in memo:
                    pc = carry if _RHO[s][j] == 16 else piece[s, _RHO[s][j]]
                    same = acc is None or pc is acc
                    memo[key] = pc if same else jnp.where((pos & 7) == s, pc, acc)
                acc = memo[key]
            (un, uo)[j % 2][_ds(i + D // 16, 8), _ds(j // 2, R)] = acc
            if j == 0:
                carry = jnp.where(pos >= 120, pltpu.roll(acc, 128 - 9, 1), pltpu.roll(acc, 128 - 8, 1))
                carry = jnp.where(pos == 127, align(L, 3), carry)

    def gen_k(rb):
        for n in range(8):
            i = 8 * rb + n
            taps(i)
            if i + 1 < D // 16:
                powers(i + 1)
            if rb:
                dft_k(rb - 1, range(2 * n, 2 * n + 2))

    def dft_k(rb, which=range(NS)):
        for s in which:
            u = (un, uo)[s // 8][_ds(rb + 4, 64), _ds(s % 8, R)]
            kspec[_ds(rb, 128), _ds(s, 2 * R)] = _dot(_unpack(u), _unpack(fk_ref[s]))

    for cp in first:
        cp.wait()
    for cp in loads:
        cp.start()

    powers(0)
    gen_k(0)
    for cp in second:
        cp.wait()
    for rb in range(1, 4):
        pl.when(zero_ref[0] < rb)(lambda: gen_k(rb))

    for cp in loads:
        cp.wait()

    xu = [r.bitcast(U32) for r in xio]

    def load_x(b):
        for jj in range(8):
            ev, od = _halves(xu[b][pl.ds(jj, R, stride=8), :].T)
            xs[_ds(b, 128), _ds(jj, R)] = ev
            xo[_ds(b, 128), _ds(jj, R)] = od

    m_i = jax.lax.broadcasted_iota(jnp.int32, (128, 128), 0)
    c_i = jax.lax.broadcasted_iota(jnp.int32, (128, 128), 1)
    perm = jnp.where(c_i == (m_i & 7) * 16 + (m_i >> 3), 1.0, 0.0).astype(BF16)

    def prep_w(g):
        for t in range(3):
            wt[g, _ds(t, 64), :] = _pack(_dot(perm, wqkv_ref[:, _ds((t + 1) % 3 * 4 + g, 128)], _NT))
        wot[:, _ds(g, 128)] = _pack(_dot(perm, wo_ref[_ds(g, 128), :]).T)

    def dft(rb, s):
        u = (un, uo)[s // 8][_ds(rb, 64), _ds(s % 8, R)]
        y = _dot(_unpack(u), _unpack(f_ref[s]))
        spec[rb][0:128, _ds(s, 2 * R)] = y
        return y[-8:, R:]

    def idft(rb, s):
        y = _dot(spec[rb][0:128, _ds(s, 2 * R)], _unpack(f_ref[s]), _NT)
        (xs, xo)[s // 8][_ds(rb, 128), _ds(s % 8, R)] += y
        return y[-8:]

    def load_spec(ref, rows, order):
        return [(ref[rows, _ds(2 * s, R)], ref[rows, _ds(2 * s + 1, R)]) for s in order]

    def store_spec(ref, rows, order, vals):
        for s, v in zip(order, vals):
            ref[rows, _ds(2 * s, R)] = v[0]
            ref[rows, _ds(2 * s + 1, R)] = v[1]

    slabs = [_slab(j) for j in range(NS)]

    def half(buf, rows, e8):
        pairs = [load_spec(buf, rows, [slabs[j], slabs[j + 8]]) for j in range(8)]
        return [_csub(lo, hi) if e8 else _cadd(lo, hi) for lo, hi in pairs]

    def k_fft(i, last):
        rows = _ds(i, 8)

        def paced(v):
            return v if last[0] is None else tuple(jnp.where(never, a, b) for a, b in zip(last[0], v))

        def split(p, e):
            plus, minus = [], []
            for lo, hi in zip(p[:len(p) // 2], p[len(p) // 2:]):
                (u,), (last[0],) = _split([lo, paced(hi)], e)
                plus.append(u)
                minus.append(last[0])
            return plus, minus

        for e8 in (8, 0):
            poly = []
            for j in range(8):
                lo, hi = load_spec(kspec, rows, [slabs[j], slabs[j + 8]])
                if j == 0:
                    lo = (lo[0] + dskb[rows, :], lo[1])
                last[0] = _csub(paced(lo), hi) if e8 else _cadd(paced(lo), hi)
                poly.append(last[0])
            for e4, p4 in zip((e8 // 2, e8 // 2 + 8), split(poly, e8 // 2)):
                for e2, p2 in zip((e4 // 2, e4 // 2 + 8), split(p4, e4 // 2)):
                    coeffs = _factor_coeffs([p2[0], paced(p2[1])], e2)
                    last[0] = coeffs[1]
                    store_spec(khat, rows, _coeff_slots(e2), coeffs)

    def conv(rb, i, after=None):
        buf, rows, park = spec[rb], _ds(i, 8), _ds(16, 8)
        for e8 in (8, 0):
            quartics = []
            for e4, p4 in zip((e8 // 2, e8 // 2 + 8), _split(half(buf, rows, e8), e8 // 2)):
                prods = [_factor_mul(p2, load_spec(khat, _ds(16 * rb + i, 8), _coeff_slots(e2)), e2)
                         for e2, p2 in zip((e4 // 2, e4 // 2 + 8), _split(p4, e4 // 2))]
                quartics.append(_merge(*prods, e4 // 2))
                if e4 < 8:
                    fence(khat, prods[1][1][0])
            mark = prods[1][1][0]
            fence(buf, mark if e8 or after is None else after)
            for j, v in enumerate(_merge(*quartics, e8 // 2)):
                if e8:
                    store_spec(buf, park, [j], [v])
                else:
                    (o,) = load_spec(buf, park, [j])
                    store_spec(buf, rows, [slabs[j], slabs[j + 8]], [_cadd(v, o), _csub(v, o)])
        return mark

    lane = jax.lax.broadcasted_iota(jnp.int32, (128, R), 1)

    def qkv(g, u, qs, ks, vs, i):
        y = _dot(_unpack(wt[g]), _unpack(u[0:D // 2, _ds(i, R)]))
        k, v, q = y[0:128], y[128:256], y[256:384]
        qs[:, _ds(i, R)] = q
        ks[:, _ds(i + 7, R)] = k
        vs[:, _ds(i + 7, R)] = v
        if i:
            ks[:, _ds(i - 1, R)] = pltpu.roll(k, 1, 1)
            vs[:, _ds(i - 1, R)] = jnp.where(lane == 0, va[:, _ds(7, R)], pltpu.roll(v, 1, 1))

    never = lane8 < zero_ref[0]

    def attend(g, qs, ks, vs, rs, o, i, ways):
        logits = []
        for w in range(W):
            lg = None
            for c in range(16):
                term = qs[_ds(c, 8), _ds(i, R)] * ks[_ds(c, 8), _ds(7 + i - w, R)]
                if c:
                    lg = lg + term
                else:
                    lg = term if w < ways else jnp.where(never, logits[w - ways], term)
            logits.append(lg)
        scale = rs[7 + i] * 0.25
        logits = [lg * scale * rs[7 + i - w] for w, lg in enumerate(logits)]
        logits = [jnp.where(lane8 == 0, NEG, lg) if w > i else lg for w, lg in enumerate(logits)]
        mx = logits[0]
        for lg in logits[1:]:
            mx = jnp.maximum(mx, lg)
        es = [jnp.exp(lg - mx) for lg in logits]
        den = es[0]
        for e in es[1:]:
            den = den + e
        inv = 1.0 / den
        probs = [e * rs[7 + i - w] * inv for w, e in enumerate(es)]
        outs = []
        for c in range(16):
            acc = None
            for w in range(W):
                term = vs[_ds(c, 8), _ds(7 + i - w, R)] * probs[w]
                if w:
                    acc = acc + term
                else:
                    acc = term if c < ways else jnp.where(never, outs[c - ways], term)
            outs.append(acc)
        o[_ds(g + 4, 64), _ds(i, R)] = _pack(jnp.concatenate(outs, axis=0))

    def chain_sum(vals, ways):
        parts = vals[:ways]
        for n, v in enumerate(vals[ways:]):
            parts[n % ways] = parts[n % ways] + v
        return jnp.sum(sum(parts[1:], parts[0]), axis=0, keepdims=True)

    def row_mean(x, ways, after=None):
        parts = [x[_ds(n, 8)] for n in range(D // 8)]
        if after is not None:
            parts[0] = jnp.where(never, after, parts[0])
        return chain_sum(parts, ways) * (1.0 / D)

    def norm(x, u, rs, i, ways, after=None):
        c = x[:, _ds(i, R)] - row_mean(x[:, _ds(i, R)], 2, after)
        r = jnp.broadcast_to(jax.lax.rsqrt(row_mean(c * c, ways) + EPS), (8, R))
        u[0:D // 2, _ds(i, R)] = _pack(c)
        rs[7 + i] = r
        if i:
            rs[i - 1] = jnp.where(lane8 == 0, ra[7], pltpu.roll(r, 1, 1))
        return r

    def proj(x, o, u, i):
        y = x[:, _ds(i, R)] + _dot(_unpack(wot[...]), _unpack(o[D // 2:D, _ds(i, R)]))
        x[:, _ds(i, R)] = y
        cen_ = cen[i % 2]
        cen_[...] = x[:, _ds(i, R)] - row_mean(y, 2)
        c = cen_[pl.ds(pl.multiple_of(zero_ref[0], 8), D)]
        u[0:D // 2, _ds(i, R)] = _pack(cen_[...] * jax.lax.rsqrt(row_mean(c * c, 1) + EPS))

    stores = [pltpu.make_async_copy(xio[c].at[0:L], o_hbm.at[:, c * 128:(c + 1) * 128], sems.at[c])
              for c in range(4)]

    def store_x(b, jj):
        t = pltpu.pack_elementwise(
            [xs[_ds(b, 128), _ds(jj, R)], xo[_ds(b, 128), _ds(jj, R)]], packed_dtype=BF16)
        xu[b][pl.ds(jj, R, stride=8), :] = pltpu.bitcast(t, U32).T

    def fence_io(b, val):
        xio[b][pl.ds(pl.multiple_of(L + zero_ref[0], 16), 16), :] = pltpu.bitcast(val, BF16)

    def start_store(b, val):
        stores[b].start()
        fence_io(b, val)
        return pltpu.bitcast(xio[b][L:L + 16, :], F32)

    def phase(fn):
        pl.when(zero_ref[0] == 0)(fn)

    @phase
    def _prepare():
        dft_k(3)
        for b in range(4):
            load_x(b)
            prep_w(b)

    even, odd = (un, (qa, ka, va), ra), (uo, (qb, kb, vb), rb_)

    def overlap(g_next, nxt, g, cur, side):
        last = [None]
        for i in range(8):
            qkv(g_next, nxt[0], *nxt[1], i)
            attend(g, *cur[1], cur[2], nxt[0], i, 2)
            for k in side[i * len(side) // 8:(i + 1) * len(side) // 8]:
                k_fft(k, last)

    for layer in range(2):
        @phase
        def _first_projection():
            if layer:
                for s in range(8):
                    idft(3, s)
            r = norm(xs, un, ra, 0, 4)
            for i in range(8):
                if layer:
                    idft(3, i + 8)
                qkv(0, un, qa, ka, va, i)
                if i < 7:
                    r = norm(xs, un, ra, i + 1, 2 - layer, r)
                r = norm(xo, uo, rb_, i, 2 - layer, r)

        def group(g, c):
            overlap(g, odd, g, even, [] if layer else [10 * g + n for n in range(10)])

            @pl.when(g < 3)
            def _():
                overlap(g + 1, even, g, odd, [] if layer else [8 * g + 40 + n for n in range(8)])

            return c

        jax.lax.fori_loop(0, 4, group, 0)

        @phase
        def _output_projection():
            for i in range(8):
                proj(xs, uo, un, i)
                attend(3, qb, kb, vb, rb_, un, i, 1)
            for i in range(8):
                proj(xo, un, uo, i)
            for s in range(NS):
                dft(0, s)

        @phase
        def _long_conv():
            done = []
            for rb in range(4):
                for i in range(16):
                    if rb < 3:
                        last = dft(rb + 1, i)
                    if layer and rb == 3:
                        if i < 8:
                            idft(2, i)
                            last = idft(2, i + 8)
                        else:
                            store_x(2, i - 8)
                    elif rb:
                        last = idft(rb - 1, i)
                    if layer and rb == 2 and i % 2:
                        store_x(0, i // 2)
                        if i == 15:
                            last = start_store(0, last)
                    if layer and rb == 3 and i < 8:
                        store_x(1, i)
                        if i == 7:
                            last = start_store(1, last)
                    done.append(last)
                    mark = conv(rb, i, done[-LAG] if len(done) >= LAG else None)
                    if rb < 3:
                        fence(spec[rb + 1], mark)

    last = start_store(2, jnp.zeros((8, R), F32))
    fence(spec[3], last)
    for jj in range(8):
        idft(3, jj)
        idft(3, jj + 8)
        store_x(3, jj)
    stores[3].start()
    for cp in stores:
        cp.wait()


@jax.jit
def pallas_interleave_layers__sliding_local_dilated__ssm_conv_s4__prompt_kernel(
    A_x: jax.Array,
    A_wqkv: jax.Array,
    A_wo: jax.Array,
    B_u: jax.Array,
    B_A_re: jax.Array,
    B_A_im: jax.Array,
    B_B_re: jax.Array,
    B_B_im: jax.Array,
    B_C_re: jax.Array,
    B_C_im: jax.Array,
    B_log_dt: jax.Array,
    B_Dskip: jax.Array,
):
    del B_u
    f = _dft_matrix()
    lane = (np.arange(R) - 11) % R
    order = 16 * (lane % 8) + lane // 8
    fk = (f[:, order].astype(np.float32) * (2.0 / L)).astype(ml_dtypes.bfloat16)
    scratch = [
        pltpu.VMEM((D, L // 2), F32),
        pltpu.VMEM((D, L // 2), F32),
        pltpu.VMEM((D + 8, L // 2), U32),
        pltpu.VMEM((D + 8, L // 2), U32),
        pltpu.VMEM((4, 192, D), U32),
        pltpu.VMEM((D // 2, D), U32),
        pltpu.VMEM((D // 2, 128), U32),
        pltpu.VMEM((D, 128), F32),
        pltpu.VMEM((2, 8, 8, N), F32),
        pltpu.VMEM((4, 128, 2 * N), F32),
        *[pltpu.VMEM((128 + 16, 2 * L), F32)] * 4,
        pltpu.VMEM((D, 2 * L), F32),
        pltpu.VMEM((D + 8, 22 * 2 * R), F32),
        pltpu.VMEM((128, 8 * R), F32),
        pltpu.VMEM((128, 15 * R), F32),
        pltpu.VMEM((128, 15 * R), F32),
        pltpu.VMEM((128, 8 * R), F32),
        pltpu.VMEM((128, 15 * R), F32),
        pltpu.VMEM((128, 15 * R), F32),
        pltpu.VMEM((15, 8, R), F32),
        pltpu.VMEM((15, 8, R), F32),
        *[pltpu.VMEM((D, R), F32)] * 2,
        *[pltpu.VMEM((L + 16, 128), BF16)] * 4,
        pltpu.VMEM((D, 3 * D), BF16),
        pltpu.VMEM((D, D), BF16),
        pltpu.VMEM((NS, R // 2, 2 * R), U32),
        pltpu.VMEM((NS, R // 2, 2 * R), U32),
        pltpu.VMEM((6, D, N), BF16),
        pltpu.SMEM((1,), jnp.int32),
        pltpu.VMEM((D,), BF16),
        pltpu.VMEM((D,), BF16),
        pltpu.SemaphoreType.DMA((13,)),
    ]
    hbm = pl.BlockSpec(memory_space=pl.ANY)
    out = pl.pallas_call(
        _kernel,
        out_shape=jax.ShapeDtypeStruct((L, D), BF16),
        in_specs=[hbm] * 14,
        out_specs=hbm,
        scratch_shapes=scratch,
        compiler_params=pltpu.CompilerParams(vmem_limit_bytes=100 * 1024 * 1024),
    )(np.zeros((1,), np.int32), A_x.reshape(L, D), A_wqkv, A_wo, B_A_re, B_A_im, B_B_re, B_B_im, B_C_re, B_C_im,
      B_log_dt, B_Dskip, _pack_rows(f), _pack_rows(fk))
    return out.reshape(1, L, D)
```
